```python
import jax
import jax.numpy as jnp

def _softmax(x, axis=-1):
    return jax.nn.softmax(x, axis=axis)
def _gelu(x):
    return jax.nn.gelu(x, approximate=True)
def _silu(x):
    return jax.nn.silu(x)
def _sigmoid(x):
    return jax.nn.sigmoid(x)
def _layernorm(x, axis=-1, eps=1e-5):
    m = jnp.mean(x, axis=axis, keepdims=True)
    v = jnp.var(x, axis=axis, keepdims=True)
    return (x - m) / jnp.sqrt(v + eps)
def _scatter_add(tgt, idx, src, axis=0):
    return tgt.at[idx].add(src)
def _segment_sum(src, seg, n):
    return jax.ops.segment_sum(src, seg, n)
class _Rng:
    def __init__(self, key):
        self._k = key
    def _next(self):
        self._k, sub = jax.random.split(self._k)
        return sub
    def normal(self, shape):
        return jax.random.normal(self._next(), shape, dtype=jnp.bfloat16)
    def randint(self, lo, hi, shape):
        return jax.random.randint(self._next(), shape, lo, hi, dtype=jnp.int32)
    def uniform(self, shape, lo=0.0, hi=1.0):
        return jax.random.uniform(self._next(), shape, jnp.bfloat16, lo, hi)
    def permutation(self, n):
        return jax.random.permutation(self._next(), n)


kernel_name = 'recurrent_scan__linear_kernel_hedgehog__moe_arch_mod__prompt'

def setup_inputs():
    _rng = _Rng(jax.random.key(int.from_bytes(__import__("os").urandom(4), "little")))
    _w = (lambda a: (lambda t: t.astype(jnp.bfloat16) if jnp.issubdtype(t.dtype, jnp.floating) else t)(jnp.asarray(a)))
    def _A_setup():
        B, S, D, H = 1, 2048, 1024, 32
        Dh = D // H
        return {
            "x": _w((lambda *s: _rng.normal(s) * 0.05)(B, S, D)),
            "wqkv": _w((lambda *s: _rng.normal(s) * 0.05)(D, 3 * D)),
            "w_phi": _w((lambda *s: _rng.normal(s) * 0.05)(H, Dh, Dh) * (Dh ** -0.5)),
            "wo": _w((lambda *s: _rng.normal(s) * 0.05)(D, D)),
        }
    _A_in = _A_setup()

    def _B_setup():
        B, S, D, F, C = 1, 2048, 1024, 3584, 1
        return {
            "x": _w((lambda *s: _rng.normal(s) * 0.05)(B, S, D)),
            "w_r": _w((lambda *s: _rng.normal(s) * 0.05)(D)),
            "w_gate": _w((lambda *s: _rng.normal(s) * 0.05)(D, F)),
            "w_up": _w((lambda *s: _rng.normal(s) * 0.05)(D, F)),
            "w_down": _w((lambda *s: _rng.normal(s) * 0.05)(F, D)),
        }
    _B_in = _B_setup()

    return {
        "A_x": _A_in["x"],
        "A_wqkv": _A_in["wqkv"],
        "A_w_phi": _A_in["w_phi"],
        "A_wo": _A_in["wo"],
        "B_x": _B_in["x"],
        "B_w_r": _B_in["w_r"],
        "B_w_gate": _B_in["w_gate"],
        "B_w_up": _B_in["w_up"],
        "B_w_down": _B_in["w_down"],
    }

def reference(A_x, A_wqkv, A_w_phi, A_wo, B_x, B_w_r, B_w_gate, B_w_up, B_w_down):
    def _A_ref(x, wqkv, w_phi, wo):
        B, S, D = x.shape
        H = 32; Dh = D // H
        qkv = (lambda x, *d: x.transpose(*d))((x @ wqkv).reshape(B, S, 3, H, Dh), 2, 0, 3, 1, 4)
        q, k, v = qkv[0], qkv[1], qkv[2]
        pq = jnp.einsum("bhsd,hdf->bhsf", q, w_phi)
        pk = jnp.einsum("bhsd,hdf->bhsf", k, w_phi)
        phi_q = jnp.concatenate([_softmax(pq, axis=-1), _softmax(-pq, axis=-1)], axis=-1)
        phi_k = jnp.concatenate([_softmax(pk, axis=-1), _softmax(-pk, axis=-1)], axis=-1)
        kv = jnp.einsum("bhsf,bhsd->bhfd", phi_k, v)
        z  = jnp.einsum("bhsf->bhf", phi_k)
        num = jnp.einsum("bhqf,bhfd->bhqd", phi_q, kv)
        den = jnp.einsum("bhqf,bhf->bhq", phi_q, z)[..., None] + 1e-6
        o = num / den
        return (lambda x, *d: x.transpose(*d))(o, 0, 2, 1, 3).reshape(B, S, D) @ wo

    def _B_ref(x, w_r, w_gate, w_up, w_down):
        B, S, D = x.shape
        C = 1
        r = x @ w_r
        idx = jnp.argsort(-r, axis=-1)[:, :C]
        idx_e = jnp.repeat(idx.reshape(B, C, 1), D, axis=2)
        x_sel = jnp.take_along_axis(x, idx_e, axis=1)
        g = _silu(x_sel @ w_gate)
        u = x_sel @ w_up
        y = (g * u) @ w_down
        r_sel = _sigmoid(jnp.take_along_axis(r, idx, axis=1))
        y = y * r_sel.reshape(B, C, 1)
        b_off = (jnp.arange(B) * S).reshape(B, 1)
        flat_idx = (idx + b_off).reshape(B * C)
        zero = (x * 0.0).reshape(B * S, D)
        upd = _scatter_add(zero, flat_idx, y.reshape(B * C, D), axis=0)
        return x + upd.reshape(B, S, D)

    x = A_x
    xn = _layernorm(x, axis=-1)
    s = _A_ref(xn, A_wqkv, A_w_phi, A_wo)
    g = _silu(_B_ref(xn, B_w_r, B_w_gate, B_w_up, B_w_down))
    return x + s * g
```

```python
import functools
import math

import jax
import jax.numpy as jnp
from jax import lax
import jax.experimental.pallas as pl
import jax.experimental.pallas.tpu as pltpu

S, D, H, DH, F = 2048, 1024, 32, 32, 3584
T = 512
NT_ = S // T
FC = F // NT_
LOG2E = math.log2(math.e)
_NT = (((1,), (1,)), ((), ()))
_NN = (((1,), (0,)), ((), ()))
f32, bf16 = jnp.float32, jnp.bfloat16


def _dot(a, b, dn):
    return lax.dot_general(a, b, dn, preferred_element_type=f32)


def _rb(v):
    return v.astype(bf16).astype(f32)


def _allreduce(v, op):
    r = v[0]
    for i in range(1, 8):
        r = op(r, v[i])
    r = op(r, pltpu.roll(r, 4, 0))
    return op(r, pltpu.roll(r, 2, 0))


def _dual_softmax(p):
    n = p.shape[1]
    p3 = p.reshape(8, 8, n)
    mx = _allreduce(p3, jnp.maximum)
    mn = _allreduce(p3, jnp.minimum)
    ep = jnp.exp2(p3 - mx[None])
    en = jnp.exp2(mn[None] - p3)
    ip = 1.0 / _allreduce(ep, jnp.add)
    im = 1.0 / _allreduce(en, jnp.add)
    return ep * ip[None], en * im[None]


def _kernel(x_hbm, wqkv_hbm, wphi_hbm, wo_hbm, wr_hbm, wg_hbm, wu_hbm, wd_hbm, out_hbm,
            x_v, xn_v, wraw_v, wkv_v, wq_v, wo_v, wg_v, wu_v, wd_v, out_v,
            wphi_v, wr_v, bd_v, kv_acc, z_acc, kvt_v, zb_v, best_v, bidx_v, y_v,
            sem_x, sem_w, sem_misc, sem_ffn, sem_out):
    def x_cp(t):
        return pltpu.make_async_copy(x_hbm.at[pl.ds(t * T, T)], x_v.at[t], sem_x.at[t])

    def w_cp(j):
        return pltpu.make_async_copy(wqkv_hbm.at[:, pl.ds(j * 128, 128)], wraw_v.at[j], sem_w.at[j])

    cp_phi = pltpu.make_async_copy(wphi_hbm, wphi_v, sem_misc.at[0])
    cp_r = pltpu.make_async_copy(wr_hbm, wr_v, sem_misc.at[1])
    cp_o = pltpu.make_async_copy(wo_hbm, wo_v, sem_misc.at[2])

    def ffn_cp(i):
        return (
            pltpu.make_async_copy(wg_hbm.at[:, pl.ds(i * FC, FC)], wg_v.at[i], sem_ffn.at[0, i]),
            pltpu.make_async_copy(wu_hbm.at[:, pl.ds(i * FC, FC)], wu_v.at[i], sem_ffn.at[1, i]),
            pltpu.make_async_copy(wd_hbm.at[pl.ds(i * FC, FC)], wd_v.at[i], sem_ffn.at[2, i]),
        )

    cp_phi.start()
    cp_r.start()
    x_cp(0).start()
    for j in range(8, 24):
        w_cp(j).start()
    for t in range(1, NT_):
        x_cp(t).start()
    for j in range(8):
        w_cp(j).start()
    cp_o.start()
    for i in range(NT_):
        for c in ffn_cp(i):
            c.start()

    def layernorm(t):
        wr = wr_v[...].astype(f32)
        for s in range(T // 128):
            x = x_v[t, pl.ds(s * 128, 128), :].astype(f32)
            m = jnp.mean(x, axis=-1, keepdims=True)
            xc = x - m
            v = jnp.mean(xc * xc, axis=-1, keepdims=True)
            inv = 1.0 / _rb(jnp.sqrt(_rb(_rb(v) + _rb(jnp.full_like(v, 1e-5)))))
            xn = (x - _rb(m)) * inv
            xn_v[t, pl.ds(s * 128, 128), :] = xn.astype(bf16)
            r = _rb(jnp.sum(xn * wr, axis=-1, keepdims=True))
            r8 = jnp.broadcast_to(r, (128, 128)).reshape(16, 8, 128)
            best, bidx = best_v[...], bidx_v[...]
            row = lax.broadcasted_iota(jnp.int32, (8, 128), 0) + (t * T + s * 128)
            for i in range(16):
                better = r8[i] > best
                best = jnp.where(better, r8[i], best)
                bidx = jnp.where(better, row + 8 * i, bidx)
            best_v[...] = best
            bidx_v[...] = bidx

    best_v[...] = jnp.full((8, 128), -jnp.inf, f32)
    bidx_v[...] = lax.broadcasted_iota(jnp.int32, (8, 128), 0)
    kv_acc[...] = jnp.zeros_like(kv_acc)
    z_acc[...] = jnp.zeros_like(z_acc)
    y_v[...] = jnp.zeros_like(y_v)

    cp_phi.wait()
    row = lax.broadcasted_iota(jnp.int32, (128, DH), 0)
    col = lax.broadcasted_iota(jnp.int32, (128, DH), 1)
    expand = jnp.where(((row & 63) >> 1) == col, 1.0, 0.0).astype(bf16)
    l0 = _dot(expand, wphi_v[...], _NT)
    row = lax.broadcasted_iota(jnp.int32, (128, D), 0)
    col = lax.broadcasted_iota(jnp.int32, (128, D), 1)
    same = (((row >> 6) << 1) | (row & 1)) == ((col >> 5) & 3)
    bd_v[...] = jnp.where(same, l0, 0.0).astype(bf16)

    cp_r.wait()
    x_cp(0).wait()
    layernorm(0)

    def fold(c, j):
        return (_dot(bd_v[:, pl.ds(c * 128, 128)], wraw_v[j], _NT) * LOG2E).astype(bf16)

    for c in range(8):
        w_cp(8 + c).wait()
        wkv_v[c, pl.ds(0, 128), :] = fold(c, 8 + c)
    for c in range(8):
        w_cp(16 + c).wait()
        wkv_v[c, pl.ds(128, 128), :] = wraw_v[16 + c].T

    def phase1(t, carry):
        nxt = lax.rem(t + 1, NT_)

        @pl.when(t + 1 < NT_)
        def _():
            x_cp(t + 1).wait()

        def proj(c):
            return _dot(wkv_v[c], xn_v[t], _NT)

        cur = proj(0)
        for c in range(8):
            new = proj(c + 1) if c + 1 < 8 else None
            vt = cur[128:].astype(bf16)
            for p in range(2):
                pos, neg = _dual_softmax(cur[64 * p:64 * p + 64])
                phi = jnp.concatenate([pos.reshape(64, T), neg.reshape(64, T)], axis=0)
                zs = phi[:, :128]
                for n in range(1, T // 128):
                    zs = zs + phi[:, n * 128:(n + 1) * 128]
                z_acc[2 * c + p] += zs
                kv_acc[2 * c + p] += _dot(vt[64 * p:64 * p + 64], phi.astype(bf16), _NT)
            cur = new
        layernorm(nxt)
        return carry

    lax.fori_loop(0, NT_, phase1, 0)

    best, bidx = best_v[...], bidx_v[...]
    r_max = jnp.max(best)
    idx = jnp.min(jnp.where(best == r_max, bidx, S))
    idx = jnp.clip(idx, 0, S - 1)
    t_sel = idx // T
    grp = pl.multiple_of((idx % T) // 16 * 16, 16)
    gate = jax.nn.sigmoid(jnp.full((16, D), r_max, f32))
    rows = lax.broadcasted_iota(jnp.int32, (16, D), 0)
    x_sel = jnp.where(rows == idx % 16, xn_v[t_sel, pl.ds(grp, 16), :].astype(f32), 0.0).astype(bf16)

    row = lax.broadcasted_iota(jnp.int32, (64, 128), 0)
    col = lax.broadcasted_iota(jnp.int32, (64, 128), 1)
    own = (row >> 5) == (col & 1)
    for j in range(16):
        kvt_v[j] = jnp.where(own, kv_acc[j], 0.0).astype(bf16)
        zb_v[j] = jnp.broadcast_to(jnp.sum(z_acc[j], axis=-1, keepdims=True), (128, 128))
    for c in range(8):
        w_cp(c).wait()
        wq_v[c // 2, pl.ds((c % 2) * 128, 128), :] = fold(c, c)
    cp_o.wait()

    def out_cp(t):
        return pltpu.make_async_copy(out_v.at[t], out_hbm.at[pl.ds(t * T, T)], sem_out.at[t])

    def phase2(i, carry):
        t = lax.rem(t_sel + 1 + i, NT_)
        for c in ffn_cp(i):
            c.wait()
        g = _dot(x_sel, wg_v[i], _NN)
        u = _dot(x_sel, wu_v[i], _NN)
        h = (g * jax.nn.sigmoid(g) * u).astype(bf16)
        y = y_v[...] + _dot(h, wd_v[i], _NN)
        y_v[...] = y

        def proj(c):
            return _dot(wq_v[c], xn_v[t], _NT)

        even = (lax.broadcasted_iota(jnp.int32, (8, T), 0) & 1) == 0
        ot = []
        cur = proj(0)
        for c in range(4):
            new = proj(c + 1) if c + 1 < 4 else None
            for p in range(4):
                j = 4 * c + p
                pos, neg = _dual_softmax(cur[64 * p:64 * p + 64])
                zb = zb_v[j]
                zb = jnp.concatenate([zb] * (T // 128), axis=1).reshape(16, 8, T)
                den = _allreduce(pos * zb[:8] + neg * zb[8:], jnp.add) + 1e-6
                inv = 1.0 / den
                sh = pltpu.roll(inv, 1, 0)
                phi = jnp.concatenate([pos.reshape(64, T), neg.reshape(64, T)], axis=0)
                num = _dot(kvt_v[j], phi.astype(bf16), _NN).reshape(2, 4, 8, T)
                ot.append((num[0] * jnp.where(even, inv, sh)[None]).reshape(32, T).astype(bf16))
                ot.append((num[1] * jnp.where(even, sh, inv)[None]).reshape(32, T).astype(bf16))
            cur = new
        o = jnp.concatenate(ot, axis=0).T
        s = _dot(o, wo_v[...], _NN)
        upd = jnp.where(i == NT_ - 1, _rb(y * gate), 0.0)
        xn_v[t, pl.ds(grp, 16), :] = (xn_v[t, pl.ds(grp, 16), :].astype(f32) + upd).astype(bf16)
        a = xn_v[t].astype(f32)
        out_v[t] = (x_v[t].astype(f32) + s * (a * jax.nn.sigmoid(a))).astype(bf16)
        out_cp(t).start()
        return carry

    lax.fori_loop(0, NT_, phase2, 0)
    for t in range(NT_):
        out_cp(t).wait()


@jax.jit
def pallas_recurrent_scan__linear_kernel_hedgehog__moe_arch_mod__prompt_kernel(
    A_x: jax.Array,
    A_wqkv: jax.Array,
    A_w_phi: jax.Array,
    A_wo: jax.Array,
    B_x: jax.Array,
    B_w_r: jax.Array,
    B_w_gate: jax.Array,
    B_w_up: jax.Array,
    B_w_down: jax.Array,
):
    del B_x
    hbm = pl.BlockSpec(memory_space=pl.ANY)
    out = pl.pallas_call(
        _kernel,
        out_shape=jax.ShapeDtypeStruct((S, D), bf16),
        in_specs=[hbm] * 8,
        out_specs=hbm,
        scratch_shapes=[
            pltpu.VMEM((NT_, T, D), bf16),
            pltpu.VMEM((NT_, T, D), bf16),
            pltpu.VMEM((24, D, 128), bf16),
            pltpu.VMEM((8, 256, D), bf16),
            pltpu.VMEM((4, 256, D), bf16),
            pltpu.VMEM((D, D), bf16),
            pltpu.VMEM((NT_, D, FC), bf16),
            pltpu.VMEM((NT_, D, FC), bf16),
            pltpu.VMEM((NT_, FC, D), bf16),
            pltpu.VMEM((NT_, T, D), bf16),
            pltpu.VMEM((D, DH), bf16),
            pltpu.VMEM((1, D), bf16),
            pltpu.VMEM((128, D), bf16),
            pltpu.VMEM((16, 64, 128), f32),
            pltpu.VMEM((16, 128, 128), f32),
            pltpu.VMEM((16, 64, 128), bf16),
            pltpu.VMEM((16, 128, 128), f32),
            pltpu.VMEM((8, 128), f32),
            pltpu.VMEM((8, 128), jnp.int32),
            pltpu.VMEM((16, D), f32),
            pltpu.SemaphoreType.DMA((NT_,)),
            pltpu.SemaphoreType.DMA((24,)),
            pltpu.SemaphoreType.DMA((3,)),
            pltpu.SemaphoreType.DMA((3, NT_)),
            pltpu.SemaphoreType.DMA((NT_,)),
        ],
        compiler_params=pltpu.CompilerParams(vmem_limit_bytes=100 * 1024 * 1024),
        name="hedgehog_mod",
    )(
        A_x.reshape(S, D), A_wqkv, A_w_phi.reshape(H * DH, DH), A_wo,
        B_w_r.reshape(1, D), B_w_gate, B_w_up, B_w_down,
    )
    return out.reshape(1, S, D)
```

```python
import functools
import math

import jax
import jax.numpy as jnp
from jax import lax
import jax.experimental.pallas as pl
import jax.experimental.pallas.tpu as pltpu

S, D, H, DH, F = 2048, 1024, 32, 32, 3584
T = 512
NT_ = S // T
FC = F // NT_
LOG2E = math.log2(math.e)
_NT = (((1,), (1,)), ((), ()))
_NN = (((1,), (0,)), ((), ()))
f32, bf16 = jnp.float32, jnp.bfloat16


def _dot(a, b, dn):
    return lax.dot_general(a, b, dn, preferred_element_type=f32)


def _rb(v):
    return v.astype(bf16).astype(f32)


def _allreduce(v, op):
    r = v[0]
    for i in range(1, 8):
        r = op(r, v[i])
    r = op(r, pltpu.roll(r, 4, 0))
    return op(r, pltpu.roll(r, 2, 0))


def _dual_softmax(p):
    n = p.shape[1]
    p3 = p.reshape(8, 8, n)
    mx = _allreduce(p3, jnp.maximum)
    mn = _allreduce(p3, jnp.minimum)
    ep = jnp.exp2(p3 - mx[None])
    en = jnp.exp2(mn[None] - p3)
    ip = 1.0 / _allreduce(ep, jnp.add)
    im = 1.0 / _allreduce(en, jnp.add)
    return ep * ip[None], en * im[None]


def _kernel(x_hbm, wqkv_hbm, wphi_hbm, wo_hbm, wr_hbm, wg_hbm, wu_hbm, wd_hbm, out_hbm,
            x_v, xn_v, wraw_v, wkv_v, wq_v, wo_v, wg_v, wu_v, wd_v, out_v,
            wphi_v, wr_v, bd_v, kv_acc, z_acc, kvt_v, zb_v, best_v, bidx_v, y_v,
            sems):
    def x_cp(t):
        return pltpu.make_async_copy(x_hbm.at[pl.ds(t * T, T)], x_v.at[t], sems.at[t])

    def w_cp(j):
        return pltpu.make_async_copy(wqkv_hbm.at[:, pl.ds(j * 128, 128)], wraw_v.at[j], sems.at[4 + j])

    cp_phi = pltpu.make_async_copy(wphi_hbm, wphi_v, sems.at[28])
    cp_r = pltpu.make_async_copy(wr_hbm, wr_v, sems.at[29])
    cp_o = pltpu.make_async_copy(wo_hbm, wo_v, sems.at[30])

    def ffn_cp(i):
        return (
            pltpu.make_async_copy(wg_hbm.at[:, pl.ds(i * FC, FC)], wg_v.at[i], sems.at[32 + i]),
            pltpu.make_async_copy(wu_hbm.at[:, pl.ds(i * FC, FC)], wu_v.at[i], sems.at[36 + i]),
            pltpu.make_async_copy(wd_hbm.at[pl.ds(i * FC, FC)], wd_v.at[i], sems.at[40 + i]),
        )

    cp_phi.start()
    cp_r.start()
    x_cp(0).start()
    for j in range(8, 24):
        w_cp(j).start()
    for t in range(1, NT_):
        x_cp(t).start()
    for j in range(8):
        w_cp(j).start()
    cp_o.start()
    for i in range(NT_):
        for c in ffn_cp(i):
            c.start()

    def layernorm(t):
        wr = wr_v[...].astype(f32).reshape(1, D)
        for s in range(T // 128):
            x = x_v[t, pl.ds(s * 128, 128), :].astype(f32)
            m = jnp.mean(x, axis=-1, keepdims=True)
            xc = x - m
            v = jnp.mean(xc * xc, axis=-1, keepdims=True)
            inv = 1.0 / _rb(jnp.sqrt(_rb(_rb(v) + _rb(jnp.full_like(v, 1e-5)))))
            xn = (x - _rb(m)) * inv
            xn_v[t, pl.ds(s * 128, 128), :] = xn.astype(bf16)
            r = _rb(jnp.sum(xn * wr, axis=-1, keepdims=True))
            r8 = jnp.broadcast_to(r, (128, 128)).reshape(16, 8, 128)
            best, bidx = best_v[...], bidx_v[...]
            row = lax.broadcasted_iota(jnp.int32, (8, 128), 0) + (t * T + s * 128)
            for i in range(16):
                better = r8[i] > best
                best = jnp.where(better, r8[i], best)
                bidx = jnp.where(better, row + 8 * i, bidx)
            best_v[...] = best
            bidx_v[...] = bidx

    best_v[...] = jnp.full((8, 128), -jnp.inf, f32)
    bidx_v[...] = lax.broadcasted_iota(jnp.int32, (8, 128), 0)
    kv_acc[...] = jnp.zeros_like(kv_acc)
    z_acc[...] = jnp.zeros_like(z_acc)
    y_v[...] = jnp.zeros_like(y_v)

    cp_phi.wait()
    row = lax.broadcasted_iota(jnp.int32, (128, DH), 0)
    col = lax.broadcasted_iota(jnp.int32, (128, DH), 1)
    expand = jnp.where(((row & 63) >> 1) == col, 1.0, 0.0).astype(bf16)
    l0 = _dot(expand, wphi_v[...], _NT)
    row = lax.broadcasted_iota(jnp.int32, (128, D), 0)
    col = lax.broadcasted_iota(jnp.int32, (128, D), 1)
    same = (((row >> 6) << 1) | (row & 1)) == ((col >> 5) & 3)
    bd_v[...] = jnp.where(same, l0, 0.0).astype(bf16)

    cp_r.wait()
    x_cp(0).wait()
    layernorm(0)

    def fold(c, j):
        return (_dot(bd_v[:, pl.ds(c * 128, 128)], wraw_v[j], _NT) * LOG2E).astype(bf16)

    for c in range(8):
        w_cp(8 + c).wait()
        wkv_v[c, pl.ds(0, 128), :] = fold(c, 8 + c)
    for c in range(8):
        w_cp(16 + c).wait()
        wkv_v[c, pl.ds(128, 128), :] = wraw_v[16 + c].T

    def phase1(t, carry):
        nxt = lax.rem(t + 1, NT_)

        @pl.when(t + 1 < NT_)
        def _():
            x_cp(t + 1).wait()

        def proj(c):
            return _dot(wkv_v[c], xn_v[t], _NT)

        cur = proj(0)
        for c in range(8):
            new = proj(c + 1) if c + 1 < 8 else None
            vt = cur[128:].astype(bf16)
            for p in range(2):
                pos, neg = _dual_softmax(cur[64 * p:64 * p + 64])
                phi = jnp.concatenate([pos.reshape(64, T), neg.reshape(64, T)], axis=0)
                zs = phi[:, :128]
                for n in range(1, T // 128):
                    zs = zs + phi[:, n * 128:(n + 1) * 128]
                z_acc[2 * c + p] += zs
                kv_acc[2 * c + p] += _dot(vt[64 * p:64 * p + 64], phi.astype(bf16), _NT)
            cur = new
        layernorm(nxt)
        return carry

    lax.fori_loop(0, NT_, phase1, 0)

    best, bidx = best_v[...], bidx_v[...]
    r_max = jnp.max(best)
    idx = jnp.min(jnp.where(best == r_max, bidx, S))
    idx = jnp.clip(idx, 0, S - 1)
    t_sel = idx // T
    grp = pl.multiple_of((idx % T) // 16 * 16, 16)
    gate = jax.nn.sigmoid(jnp.full((16, D), r_max, f32))
    rows = lax.broadcasted_iota(jnp.int32, (16, D), 0)
    x_sel = jnp.where(rows == idx % 16, xn_v[t_sel, pl.ds(grp, 16), :].astype(f32), 0.0).astype(bf16)

    row = lax.broadcasted_iota(jnp.int32, (64, 128), 0)
    col = lax.broadcasted_iota(jnp.int32, (64, 128), 1)
    own = (row >> 5) == (col & 1)
    for j in range(16):
        kvt_v[j] = jnp.where(own, kv_acc[j], 0.0).astype(bf16)
        zb_v[j] = jnp.broadcast_to(jnp.sum(z_acc[j], axis=-1, keepdims=True), (128, 128))
    for c in range(8):
        w_cp(c).wait()
        wq_v[c // 2, pl.ds((c % 2) * 128, 128), :] = fold(c, c)
    cp_o.wait()

    def out_cp(t):
        return pltpu.make_async_copy(out_v.at[t], out_hbm.at[pl.ds(t * T, T)], sems.at[44 + t])

    def phase2(i, carry):
        t = lax.rem(t_sel + 1 + i, NT_)
        for c in ffn_cp(i):
            c.wait()
        g = _dot(x_sel, wg_v[i], _NN)
        u = _dot(x_sel, wu_v[i], _NN)
        h = (g * jax.nn.sigmoid(g) * u).astype(bf16)
        y = y_v[...] + _dot(h, wd_v[i], _NN)
        y_v[...] = y

        def proj(c):
            return _dot(wq_v[c], xn_v[t], _NT)

        even = (lax.broadcasted_iota(jnp.int32, (8, T), 0) & 1) == 0
        ot = []
        cur = proj(0)
        for c in range(4):
            new = proj(c + 1) if c + 1 < 4 else None
            for p in range(4):
                j = 4 * c + p
                pos, neg = _dual_softmax(cur[64 * p:64 * p + 64])
                zb = zb_v[j]
                zb = jnp.concatenate([zb] * (T // 128), axis=1).reshape(16, 8, T)
                den = _allreduce(pos * zb[:8] + neg * zb[8:], jnp.add) + 1e-6
                inv = 1.0 / den
                sh = pltpu.roll(inv, 1, 0)
                phi = jnp.concatenate([pos.reshape(64, T), neg.reshape(64, T)], axis=0)
                num = _dot(kvt_v[j], phi.astype(bf16), _NN).reshape(2, 4, 8, T)
                ot.append((num[0] * jnp.where(even, inv, sh)[None]).reshape(32, T).astype(bf16))
                ot.append((num[1] * jnp.where(even, sh, inv)[None]).reshape(32, T).astype(bf16))
            cur = new
        o = jnp.concatenate(ot, axis=0).T
        s = _dot(o, wo_v[...], _NN)
        upd = jnp.where(i == NT_ - 1, _rb(y * gate), 0.0)
        xn_v[t, pl.ds(grp, 16), :] = (xn_v[t, pl.ds(grp, 16), :].astype(f32) + upd).astype(bf16)
        a = xn_v[t].astype(f32)
        out_v[t] = (x_v[t].astype(f32) + s * (a * jax.nn.sigmoid(a))).astype(bf16)
        out_cp(t).start()
        return carry

    lax.fori_loop(0, NT_, phase2, 0)
    for t in range(NT_):
        out_cp(t).wait()


@jax.jit
def pallas_recurrent_scan__linear_kernel_hedgehog__moe_arch_mod__prompt_kernel(
    A_x: jax.Array,
    A_wqkv: jax.Array,
    A_w_phi: jax.Array,
    A_wo: jax.Array,
    B_x: jax.Array,
    B_w_r: jax.Array,
    B_w_gate: jax.Array,
    B_w_up: jax.Array,
    B_w_down: jax.Array,
):
    del B_x
    hbm = pl.BlockSpec(memory_space=pl.ANY)
    out = pl.pallas_call(
        _kernel,
        out_shape=jax.ShapeDtypeStruct((S, D), bf16),
        in_specs=[hbm] * 8,
        out_specs=hbm,
        scratch_shapes=[
            pltpu.VMEM((NT_, T, D), bf16),
            pltpu.VMEM((NT_, T, D), bf16),
            pltpu.VMEM((24, D, 128), bf16),
            pltpu.VMEM((8, 256, D), bf16),
            pltpu.VMEM((4, 256, D), bf16),
            pltpu.VMEM((D, D), bf16),
            pltpu.VMEM((NT_, D, FC), bf16),
            pltpu.VMEM((NT_, D, FC), bf16),
            pltpu.VMEM((NT_, FC, D), bf16),
            pltpu.VMEM((NT_, T, D), bf16),
            pltpu.VMEM((D, DH), bf16),
            pltpu.VMEM((D,), bf16),
            pltpu.VMEM((128, D), bf16),
            pltpu.VMEM((16, 64, 128), f32),
            pltpu.VMEM((16, 128, 128), f32),
            pltpu.VMEM((16, 64, 128), bf16),
            pltpu.VMEM((16, 128, 128), f32),
            pltpu.VMEM((8, 128), f32),
            pltpu.VMEM((8, 128), jnp.int32),
            pltpu.VMEM((16, D), f32),
            pltpu.SemaphoreType.DMA((48,)),
        ],
        compiler_params=pltpu.CompilerParams(vmem_limit_bytes=100 * 1024 * 1024),
        name="hedgehog_mod",
    )(
        A_x.reshape(S, D), A_wqkv, A_w_phi.reshape(H * DH, DH), A_wo,
        B_w_r, B_w_gate, B_w_up, B_w_down,
    )
    return out.reshape(1, S, D)
```

```python
import math

import jax
import jax.numpy as jnp
from jax import lax
import jax.experimental.pallas as pl
import jax.experimental.pallas.tpu as pltpu

S, D, H, DH, F = 2048, 1024, 32, 32, 3584
T = 512
NT_ = S // T
NF = F // 128
LN_ROWS = 16
LOG2E = math.log2(math.e)
_NT = (((1,), (1,)), ((), ()))
_NN = (((1,), (0,)), ((), ()))
f32, bf16 = jnp.float32, jnp.bfloat16


def _dot(a, b, dn):
    return lax.dot_general(a, b, dn, preferred_element_type=f32)


def _rb(v):
    return v.astype(bf16).astype(f32)


def _rcp(v):
    r = pl.reciprocal(v, approx=True)
    return r * (2.0 - v * r)


def _silu(a):
    return a * pl.reciprocal(1.0 + jnp.exp2(a * -LOG2E), approx=True)


def _allreduce(v, op):
    r = v[0]
    for i in range(1, 8):
        r = op(r, v[i])
    r = op(r, pltpu.roll(r, 4, 0))
    return op(r, pltpu.roll(r, 2, 0))


def _dual_softmax(p):
    n = p.shape[1]
    p3 = p.reshape(8, 8, n)
    mx = _allreduce(p3, jnp.maximum)
    mn = _allreduce(p3, jnp.minimum)
    ep = jnp.exp2(p3 - mx[None])
    en = jnp.exp2(mn[None] - p3)
    ip = _rcp(_allreduce(ep, jnp.add))
    im = _rcp(_allreduce(en, jnp.add))
    return ep * ip[None], en * im[None]


def _kernel(x_hbm, wqkv_hbm, wphi_hbm, wo_hbm, wr_hbm, wg_hbm, wu_hbm, wd_hbm, out_hbm,
            x_v, xn_v, wraw_v, wt_v, wo_v, wg_v, wu_v, wd_v, out_v, wphi_v, wr_v, sems):
    n_sem = [0]

    def copy(src, dst):
        n_sem[0] += 1
        return pltpu.make_async_copy(src, dst, sems.at[n_sem[0] - 1])

    cp_x0 = [copy(x_hbm.at[pl.ds(s * 128, 128)], x_v.at[0, pl.ds(s * 128, 128)]) for s in range(T // 128)]
    cp_x = [None] + [copy(x_hbm.at[pl.ds(t * T, T)], x_v.at[t]) for t in range(1, NT_)]
    cp_w = [copy(wqkv_hbm.at[:, pl.ds(j * 128, 128)], wraw_v.at[j]) for j in range(24)]
    cp_phi, cp_r, cp_o = copy(wphi_hbm, wphi_v), copy(wr_hbm, wr_v), copy(wo_hbm, wo_v)
    cp_ffn = [copy(wg_hbm, wg_v), copy(wu_hbm, wu_v), copy(wd_hbm, wd_v)]
    for c in ([cp_phi, cp_w[8], cp_r] + cp_x0 + cp_w[9:24] + cp_x[1:] + cp_w[:8] + [cp_o] + cp_ffn):
        c.start()

    route = {"best": jnp.full((8, 128), -jnp.inf, f32),
             "idx": lax.broadcasted_iota(jnp.int32, (8, 128), 0)}

    def layernorm(t, r0, nrows):
        wr = wr_v[...].astype(f32).reshape(1, D)
        row = lax.broadcasted_iota(jnp.int32, (8, 128), 0)
        for r in range(r0, r0 + nrows, LN_ROWS):
            x = x_v[t, pl.ds(r, LN_ROWS), :].astype(f32)
            xc = x - jnp.mean(x, axis=-1, keepdims=True)
            v = jnp.mean(xc * xc, axis=-1, keepdims=True)
            xn = xc * _rcp(_rb(jnp.sqrt(_rb(_rb(v) + _rb(jnp.full_like(v, 1e-5))))))
            xn_v[t, pl.ds(r, LN_ROWS), :] = xn.astype(bf16)
            sc = _rb(jnp.sum(xn * wr, axis=-1, keepdims=True))
            sc = jnp.broadcast_to(sc, (LN_ROWS, 128))
            for i in range(LN_ROWS // 8):
                sc8 = sc[8 * i:8 * i + 8]
                better = sc8 > route["best"]
                route["best"] = jnp.where(better, sc8, route["best"])
                route["idx"] = jnp.where(better, row + (t * T + r + 8 * i), route["idx"])

    cp_phi.wait()
    row = lax.broadcasted_iota(jnp.int32, (128, DH), 0)
    col = lax.broadcasted_iota(jnp.int32, (128, DH), 1)
    expand = jnp.where(((row & 63) >> 1) == col, 1.0, 0.0).astype(bf16)
    l0 = _dot(expand, wphi_v[...], _NT)
    row = lax.broadcasted_iota(jnp.int32, (128, D), 0)
    col = lax.broadcasted_iota(jnp.int32, (128, D), 1)
    same = (((row >> 6) << 1) | (row & 1)) == ((col >> 5) & 3)
    bd = jnp.where(same, l0, 0.0).astype(bf16)

    def fold(j):
        c = j % 8
        w = _dot(bd[:, c * 128:(c + 1) * 128], wraw_v[j], _NT) * LOG2E
        wt_v[pl.ds(j * 128, 128), :] = w.astype(bf16)

    kv = [None] * 16
    zs = [None] * 16

    def key_features(p, j0):
        out = []
        for q in range(p.shape[0] // 64):
            pos, neg = _dual_softmax(p[64 * q:64 * q + 64])
            phi = jnp.concatenate([pos.reshape(64, T), neg.reshape(64, T)], axis=0)
            z = zs[j0 + q]
            for n in range(T // 128):
                piece = phi[:, n * 128:(n + 1) * 128]
                z = piece if z is None else z + piece
            zs[j0 + q] = z
            out.append(phi.astype(bf16))
        return out

    def kv_update(vt, j0, phis):
        vt = vt.astype(bf16)
        for q in range(vt.shape[0] // 64):
            upd = _dot(vt[64 * q:64 * q + 64], phis[j0 + q], _NT)
            kv[j0 + q] = upd if kv[j0 + q] is None else kv[j0 + q] + upd

    def proj(r0, nrows, t):
        return _dot(wt_v[pl.ds(r0, nrows), :], xn_v[t], _NT)

    cp_w[8].wait()
    fold(8)
    cp_r.wait()
    for s in range(T // 128):
        cp_x0[s].wait()
        layernorm(0, s * 128, 128)
    phis, prev = [], None
    for r0, nrows, blocks in ((0, 128, ()), (128, 256, (9, 10)), (384, 128, (11, 12, 13, 14, 15)),
                              (512, 256, ()), (768, 256, ())):
        for j in blocks:
            cp_w[j].wait()
        for j in blocks:
            fold(j)
        cur = (proj(D + r0, nrows, 0), r0 // 64)
        if prev is not None:
            phis += key_features(*prev)
        prev = cur
    for c in cp_w[16:24] + [cp_x[1]]:
        c.wait()
    for j in range(16, 24):
        wt_v[pl.ds(j * 128, 128), :] = wraw_v[j].T
    pend_v = None
    for c in range(4):
        cur = (proj(2 * D + 256 * c, 256, 0), 4 * c)
        if c == 0:
            phis += key_features(*prev)
        if pend_v is not None:
            kv_update(*pend_v, phis)
        pend_v = cur
    layernorm(1, 0, T)

    barrier = {1: [cp_x[2]] + cp_w[:8], 2: [cp_x[3]], 3: [cp_o]}
    for t in range(1, NT_):
        for c in barrier[t]:
            c.wait()
        old_phis, phis = phis, []
        for c in range(4):
            cur_k = (proj(D + 256 * c, 256, t), 4 * c)
            kv_update(*pend_v, old_phis if c == 0 else phis)
            pend_v = (proj(2 * D + 256 * c, 256, t), 4 * c)
            phis += key_features(*cur_k)
            if t == 1:
                fold(2 * c)
                fold(2 * c + 1)
        if t + 1 < NT_:
            layernorm(t + 1, 0, T)

    for c in cp_ffn:
        c.wait()
    best, bidx = route["best"], route["idx"]
    r_max = jnp.max(best)
    idx = jnp.min(jnp.where(best == r_max, bidx, S))
    idx = jnp.clip(idx, 0, S - 1)
    t_sel = idx // T
    grp = pl.multiple_of((idx % T) // 16 * 16, 16)
    gate = jax.nn.sigmoid(jnp.full((8, D), r_max, f32))
    rows = lax.broadcasted_iota(jnp.int32, (16, D), 0)
    x_sel = jnp.where(rows == idx % 16, xn_v[t_sel, pl.ds(grp, 16), :].astype(f32), 0.0)
    x_sel = jnp.broadcast_to(jnp.sum(x_sel, axis=0, keepdims=True), (16, D)).astype(bf16)

    ffn = {"y": [None, None]}

    def ffn_program():
        def down(h, n):
            for hf in range(2):
                part = _dot(h, wd_v[pl.ds(n * 128, 128), pl.ds(hf * 512, 512)], _NN)[:8]
                ffn["y"][hf] = part if ffn["y"][hf] is None else ffn["y"][hf] + part
                yield
        h = None
        for n in range(NF):
            acc = []
            for w in (wg_v, wu_v):
                a = _dot(x_sel[:, :512], w[pl.ds(0, 512), pl.ds(n * 128, 128)], _NN)
                yield
                acc.append(a + _dot(x_sel[:, 512:], w[pl.ds(512, 512), pl.ds(n * 128, 128)], _NN))
                yield
            if h is not None:
                yield from down(h, n - 1)
            h = (_silu(acc[0]) * acc[1]).astype(bf16)
        yield
        yield from down(h, NF - 1)

    ffn_steps = ffn_program()

    def q_proj(c, t):
        cols = []
        for n in range(T // 128):
            acc = None
            for kh in range(2):
                part = _dot(wt_v[pl.ds(256 * c, 256), pl.ds(kh * 512, 512)],
                            xn_v[t, pl.ds(n * 128, 128), pl.ds(kh * 512, 512)], _NT)
                acc = part if acc is None else acc + part
                if (n, kh) != (T // 128 - 1, 1):
                    next(ffn_steps, None)
            cols.append(acc)
        return jnp.concatenate(cols, axis=1)

    even = (lax.broadcasted_iota(jnp.int32, (8, T), 0) & 1) == 0
    state = {}

    def attend(p, j0):
        out = []
        for q in range(4):
            pos, neg = _dual_softmax(p[64 * q:64 * q + 64])
            zb = jnp.concatenate([state["z"][j0 + q]] * (T // 128), axis=1).reshape(16, 8, T)
            inv = _rcp(_allreduce(pos * zb[:8] + neg * zb[8:], jnp.add) + 1e-6)
            sh = pltpu.roll(inv, 1, 0)
            phi = jnp.concatenate([pos.reshape(64, T), neg.reshape(64, T)], axis=0)
            num = _dot(state["kv"][j0 + q], phi.astype(bf16), _NN).reshape(2, 4, 8, T)
            out.append((num[0] * jnp.where(even, inv, sh)[None]).reshape(32, T))
            out.append((num[1] * jnp.where(even, sh, inv)[None]).reshape(32, T))
        return jnp.concatenate(out, axis=0).T.astype(bf16)

    cp_out = []

    def out_proj(i, t, o, n):
        last = i == NT_ - 1
        cols = pl.ds(n * 256, 256)
        halves = []
        for nn in range(2):
            rows_out = []
            for mh in range(2):
                acc = None
                for kh in range(2):
                    lhs = jnp.concatenate([o[2 * kh][mh * 256:(mh + 1) * 256],
                                           o[2 * kh + 1][mh * 256:(mh + 1) * 256]], axis=1)
                    part = _dot(lhs, wo_v[pl.ds(kh * 512, 512), pl.ds(n * 256 + nn * 128, 128)], _NN)
                    acc = part if acc is None else acc + part
                    next(ffn_steps, None)
                rows_out.append(acc)
            halves.append(jnp.concatenate(rows_out, axis=0))
        s = jnp.concatenate(halves, axis=1)
        a = xn_v[t, :, cols].astype(f32)
        if last:
            hit = lax.broadcasted_iota(jnp.int32, (T // 8, 8, 256), 0) * 8 + \
                lax.broadcasted_iota(jnp.int32, (T // 8, 8, 256), 1) == idx % T
            a3 = a.reshape(T // 8, 8, 256)
            a = jnp.where(hit, a3 + state["y"][:, n * 256:(n + 1) * 256][None], a3).reshape(T, 256)
        out_v[i, :, cols] = (x_v[t, :, cols].astype(f32) + s * _silu(a)).astype(bf16)
        if last:
            cp_out.append(copy(out_v.at[i, :, cols], out_hbm.at[pl.ds(t * T, T), cols]))
            cp_out[-1].start()
        elif n == D // 256 - 1:
            cp_out.append(copy(out_v.at[i], out_hbm.at[pl.ds(t * T, T)]))
            cp_out[-1].start()

    tiles = [lax.rem(t_sel + 1 + i, NT_) for i in range(NT_)]
    o_prev, o_cur, prev = None, [], None
    for i in range(NT_):
        for c in range(4):
            cur = (q_proj(c, tiles[i]), 4 * c)
            if i == 0 and c == 0:
                kv_update(*pend_v, phis)
                row = lax.broadcasted_iota(jnp.int32, (64, 128), 0)
                col = lax.broadcasted_iota(jnp.int32, (64, 128), 1)
                own = (row >> 5) == (col & 1)
                state["kv"] = [jnp.where(own, a, 0.0).astype(bf16) for a in kv]
                state["z"] = [jnp.broadcast_to(jnp.sum(z, axis=-1, keepdims=True), (128, 128)) for z in zs]
            if prev is not None:
                o_cur.append(attend(*prev))
                if len(o_cur) == 4:
                    o_prev, o_cur = o_cur, []
            prev = cur
            if i > 0 and c > 0:
                out_proj(i - 1, tiles[i - 1], o_prev, c - 1)
            elif i > 1:
                out_proj(i - 2, tiles[i - 2], o_old, 3)
            if c == 3:
                o_old = o_prev
    out_proj(NT_ - 2, tiles[NT_ - 2], o_old, 3)
    o_cur.append(attend(*prev))
    for _ in ffn_steps:
        pass
    state["y"] = _rb(jnp.concatenate(ffn["y"], axis=1) * gate)
    for n in range(4):
        out_proj(NT_ - 1, tiles[NT_ - 1], o_cur, n)
    for c in cp_out:
        c.wait()


@jax.jit
def pallas_recurrent_scan__linear_kernel_hedgehog__moe_arch_mod__prompt_kernel(
    A_x: jax.Array,
    A_wqkv: jax.Array,
    A_w_phi: jax.Array,
    A_wo: jax.Array,
    B_x: jax.Array,
    B_w_r: jax.Array,
    B_w_gate: jax.Array,
    B_w_up: jax.Array,
    B_w_down: jax.Array,
):
    del B_x
    hbm = pl.BlockSpec(memory_space=pl.ANY)
    out = pl.pallas_call(
        _kernel,
        out_shape=jax.ShapeDtypeStruct((S, D), bf16),
        in_specs=[hbm] * 8,
        out_specs=hbm,
        scratch_shapes=[
            pltpu.VMEM((NT_, T, D), bf16),
            pltpu.VMEM((NT_, T, D), bf16),
            pltpu.VMEM((24, D, 128), bf16),
            pltpu.VMEM((3 * D, D), bf16),
            pltpu.VMEM((D, D), bf16),
            pltpu.VMEM((D, F), bf16),
            pltpu.VMEM((D, F), bf16),
            pltpu.VMEM((F, D), bf16),
            pltpu.VMEM((NT_, T, D), bf16),
            pltpu.VMEM((H * DH, DH), bf16),
            pltpu.VMEM((D,), bf16),
            pltpu.SemaphoreType.DMA((48,)),
        ],
        compiler_params=pltpu.CompilerParams(vmem_limit_bytes=110 * 1024 * 1024),
        name="hedgehog_mod",
    )(
        A_x.reshape(S, D), A_wqkv, A_w_phi.reshape(H * DH, DH), A_wo,
        B_w_r, B_w_gate, B_w_up, B_w_down,
    )
    return out.reshape(1, S, D)
```

```python
import math

import jax
import jax.numpy as jnp
from jax import lax
import jax.experimental.pallas as pl
import jax.experimental.pallas.tpu as pltpu

S, D, H, DH, F = 2048, 1024, 32, 32, 3584
T = 512
NT_ = S // T
NF = F // 128
LN_ROWS = 16
LOG2E = math.log2(math.e)
_NT = (((1,), (1,)), ((), ()))
_NN = (((1,), (0,)), ((), ()))
f32, bf16 = jnp.float32, jnp.bfloat16


def _dot(a, b, dn):
    return lax.dot_general(a, b, dn, preferred_element_type=f32)


def _rb(v):
    return v.astype(bf16).astype(f32)


def _rcp(v):
    r = pl.reciprocal(v, approx=True)
    return r * (2.0 - v * r)


def _silu(a):
    return a * pl.reciprocal(1.0 + jnp.exp2(a * -LOG2E), approx=True)


def _lhs_terms(a11, a12, a21, a22):
    return [a11 + a22, a21 + a22, a11, a22, a11 + a12, a21 - a11, a12 - a22]


def _rhs_terms(b11, b12, b21, b22):
    return [b11 + b22, b11, b12 - b22, b21 - b11, b22, b11 + b12, b21 + b22]


def _strassen(product):
    m = product(0)
    c11, c22 = m, m
    c21 = product(3)
    c11 = c11 + c21
    c12 = product(4)
    c11 = c11 - c12
    c11 = c11 + product(6)
    m = product(2)
    c12, c22 = c12 + m, c22 + m
    m = product(1)
    c21, c22 = c21 + m, c22 - m
    c22 = c22 + product(5)
    return c11, c12, c21, c22


def _allreduce(v, op):
    r = v[0]
    for i in range(1, 8):
        r = op(r, v[i])
    r = op(r, pltpu.roll(r, 4, 0))
    return op(r, pltpu.roll(r, 2, 0))


def _dual_softmax(p):
    n = p.shape[1]
    p3 = p.reshape(8, 8, n)
    mx = _allreduce(p3, jnp.maximum)
    mn = _allreduce(p3, jnp.minimum)
    ep = jnp.exp2(p3 - mx[None])
    en = jnp.exp2(mn[None] - p3)
    ip = _rcp(_allreduce(ep, jnp.add))
    im = _rcp(_allreduce(en, jnp.add))
    return ep * ip[None], en * im[None]


def _kernel(x_hbm, wqkv_hbm, wphi_hbm, wo_hbm, wr_hbm, wg_hbm, wu_hbm, wd_hbm, out_hbm,
            x_v, xs_v, wraw_v, ws_v, wo_v, wos_v, wg_v, wu_v, wd_v, out_v, wphi_v, wr_v, sems):
    n_sem = [0]

    def copy(src, dst):
        n_sem[0] += 1
        return pltpu.make_async_copy(src, dst, sems.at[n_sem[0] - 1])

    cp_x0 = [copy(x_hbm.at[pl.ds(s * 256, 256)], x_v.at[0, pl.ds(s * 256, 256)]) for s in range(2)]
    cp_x = [None] + [copy(x_hbm.at[pl.ds(t * T, T)], x_v.at[t]) for t in range(1, NT_)]
    cp_w = [copy(wqkv_hbm.at[:, pl.ds(j * 256, 256)], wraw_v.at[j]) for j in range(12)]
    cp_phi, cp_r, cp_o = copy(wphi_hbm, wphi_v), copy(wr_hbm, wr_v), copy(wo_hbm, wo_v)
    cp_ffn = [copy(wg_hbm, wg_v), copy(wu_hbm, wu_v), copy(wd_hbm, wd_v)]
    for c in ([cp_phi, cp_w[4], cp_r] + cp_x0 + cp_w[5:12] + cp_x[1:] + cp_w[:4] + [cp_o] + cp_ffn):
        c.start()

    route = {"best": jnp.full((8, 128), -jnp.inf, f32),
             "idx": lax.broadcasted_iota(jnp.int32, (8, 128), 0)}

    def layernorm(t, g):
        wr = wr_v[...].astype(f32).reshape(1, D)
        row = lax.broadcasted_iota(jnp.int32, (8, 128), 0)

        def rows(r):
            x = x_v[t, pl.ds(r, LN_ROWS), :].astype(f32)
            xc = x - jnp.mean(x, axis=-1, keepdims=True)
            v = jnp.mean(xc * xc, axis=-1, keepdims=True)
            xn = xc * _rcp(_rb(jnp.sqrt(_rb(_rb(v) + _rb(jnp.full_like(v, 1e-5))))))
            sc = _rb(jnp.sum(xn * wr, axis=-1, keepdims=True))
            sc = jnp.broadcast_to(sc, (LN_ROWS, 128))
            for i in range(LN_ROWS // 8):
                sc8, tok = sc[8 * i:8 * i + 8], row + (t * T + r + 8 * i)
                better = (sc8 > route["best"]) | ((sc8 == route["best"]) & (tok < route["idx"]))
                route["best"] = jnp.where(better, sc8, route["best"])
                route["idx"] = jnp.where(better, tok, route["idx"])
            return xn

        for r in range(0, 128, LN_ROWS):
            a, b = rows(256 * g + r), rows(256 * g + 128 + r)
            b11, b21, b12, b22 = a[:, :512], a[:, 512:], b[:, :512], b[:, 512:]
            for i, term in enumerate(_rhs_terms(b11, b12, b21, b22) + [b21, b12]):
                xs_v[t, g, i, pl.ds(r, LN_ROWS), :] = term.astype(bf16)

    def xn_block(t, g, hf, kh, cols):
        return xs_v[t, g, ((1, 7), (8, 4))[hf][kh], :, cols]

    cp_phi.wait()
    row = lax.broadcasted_iota(jnp.int32, (128, DH), 0)
    col = lax.broadcasted_iota(jnp.int32, (128, DH), 1)
    expand = jnp.where(((row & 63) >> 1) == col, 1.0, 0.0).astype(bf16)
    l0 = _dot(expand, wphi_v[...], _NT)
    row = lax.broadcasted_iota(jnp.int32, (128, D), 0)
    col = lax.broadcasted_iota(jnp.int32, (128, D), 1)
    same = (((row >> 6) << 1) | (row & 1)) == ((col >> 5) & 3)
    bd = jnp.where(same, l0, 0.0).astype(bf16)

    def prepare_w(j):
        blocks = []
        for b in range(2):
            w = wraw_v[j, :, pl.ds(128 * b, 128)]
            if j < 8:
                c = (2 * j + b) % 8
                blocks.append(_dot(bd[:, c * 128:(c + 1) * 128], w, _NT) * LOG2E)
            else:
                blocks.append(w.astype(f32).T)
        a, b = blocks
        for i, term in enumerate(_lhs_terms(a[:, :512], a[:, 512:], b[:, :512], b[:, 512:])):
            ws_v[j // 2, i, pl.ds(128 * (j % 2), 128), :] = term.astype(bf16)

    def prepare_wo(n):
        for c in range(4):
            w = wo_v[pl.ds(256 * c, 256), pl.ds(256 * n, 256)].astype(f32)
            terms = _rhs_terms(w[:128, :128], w[:128, 128:], w[128:, :128], w[128:, 128:])
            for i, term in enumerate(terms):
                wos_v[n, i, pl.ds(128 * c, 128), :] = term.astype(bf16)

    def no_op():
        pass

    def proj(j0, nj, t, between=no_op):
        rows = pl.ds(128 * (j0 % 2), 128 * nj)
        groups = []
        for g in range(T // 256):
            def product(i):
                m = _dot(ws_v[j0 // 2, i, rows, :], xs_v[t, g, i], _NT)
                between()
                return m
            groups.append(_strassen(product))
        out = []
        for j in range(nj):
            for b in range(2):
                out.append(jnp.concatenate(
                    [c[2 * b + hf][128 * j:128 * (j + 1)] for c in groups for hf in range(2)], axis=1))
        return out

    kv = [None] * 16
    zs = [None] * 16

    def key_features(blocks, j0):
        out = []
        for q in range(2 * len(blocks)):
            pos, neg = _dual_softmax(blocks[q // 2][64 * (q % 2):64 * (q % 2) + 64])
            phi = jnp.concatenate([pos.reshape(64, T), neg.reshape(64, T)], axis=0)
            z = zs[j0 + q]
            for n in range(T // 128):
                piece = phi[:, n * 128:(n + 1) * 128]
                z = piece if z is None else z + piece
            zs[j0 + q] = z
            out.append(phi.astype(bf16))
        return out

    def kv_update(blocks, j0, phis):
        for q in range(2 * len(blocks)):
            vt = blocks[q // 2][64 * (q % 2):64 * (q % 2) + 64].astype(bf16)
            upd = _dot(vt, phis[j0 + q], _NT)
            kv[j0 + q] = upd if kv[j0 + q] is None else kv[j0 + q] + upd

    cp_w[4].wait()
    prepare_w(4)
    cp_r.wait()
    for g in range(2):
        cp_x0[g].wait()
        layernorm(0, g)
    phis, prev = [], None
    for j0, nj, blocks in ((4, 1, ()), (5, 1, (5,)), (6, 2, (6, 7))):
        for j in blocks:
            cp_w[j].wait()
        for j in blocks:
            prepare_w(j)
        cur = (proj(j0, nj, 0), 4 * (j0 - 4))
        if prev is not None:
            phis += key_features(*prev)
        prev = cur
    for c in cp_w[8:12] + [cp_x[1]]:
        c.wait()
    for j in range(8, 12):
        prepare_w(j)
    pend_v = (proj(8, 2, 0), 0)
    phis += key_features(*prev)
    cur = (proj(10, 2, 0), 8)
    kv_update(*pend_v, phis)
    pend_v = cur
    for g in range(2):
        layernorm(1, g)

    barrier = {1: [cp_x[2]] + cp_w[:4], 2: [cp_x[3], cp_o], 3: [cp_ffn[0]]}
    for t in range(1, NT_):
        for c in barrier[t]:
            c.wait()
        old_phis, phis = phis, []
        for c in range(2):
            cur_k = (proj(4 + 2 * c, 2, t), 8 * c)
            kv_update(*pend_v, old_phis if c == 0 else phis)
            pend_v = (proj(8 + 2 * c, 2, t), 8 * c)
            phis += key_features(*cur_k)
            if t == 1:
                prepare_w(2 * c)
                prepare_w(2 * c + 1)
            if t == 3:
                prepare_wo(2 * c)
                prepare_wo(2 * c + 1)
        if t + 1 < NT_:
            for g in range(2):
                layernorm(t + 1, g)

    for c in cp_ffn[1:]:
        c.wait()
    best, bidx = route["best"], route["idx"]
    r_max = jnp.max(best)
    idx = jnp.min(jnp.where(best == r_max, bidx, S))
    idx = jnp.clip(idx, 0, S - 1)
    t_sel = idx // T
    g_sel, r_sel = (idx % T) // 256, idx % 128
    hf_sel = (idx // 128) % 2
    grp = pl.ds(pl.multiple_of(r_sel // 16 * 16, 16), 16)
    x_sel = jnp.concatenate([xs_v[t_sel, g_sel, 1 + 7 * hf_sel, grp, :],
                             xs_v[t_sel, g_sel, 7 - 3 * hf_sel, grp, :]], axis=1).astype(f32)
    rows = lax.broadcasted_iota(jnp.int32, (16, D), 0)
    x_sel = jnp.where(rows == idx % 16, x_sel, 0.0)
    x_sel = jnp.broadcast_to(jnp.sum(x_sel, axis=0, keepdims=True), (16, D)).astype(bf16)
    gate = jax.nn.sigmoid(jnp.full((8, D), r_max, f32))

    ffn = {"y": [None, None]}

    def ffn_program():
        def down(h, n):
            for hf in range(2):
                part = _dot(h, wd_v[pl.ds(n * 128, 128), pl.ds(hf * 512, 512)], _NN)[:8]
                ffn["y"][hf] = part if ffn["y"][hf] is None else ffn["y"][hf] + part
                yield
        h = None
        for n in range(NF):
            acc = []
            for w in (wg_v, wu_v):
                a = _dot(x_sel[:, :512], w[pl.ds(0, 512), pl.ds(n * 128, 128)], _NN)
                yield
                acc.append(a + _dot(x_sel[:, 512:], w[pl.ds(512, 512), pl.ds(n * 128, 128)], _NN))
                yield
            if h is not None:
                yield from down(h, n - 1)
            h = (_silu(acc[0]) * acc[1]).astype(bf16)
        yield
        yield from down(h, NF - 1)

    ffn_steps = ffn_program()

    def ffn_step():
        next(ffn_steps, None)

    even = (lax.broadcasted_iota(jnp.int32, (8, T), 0) & 1) == 0
    state = {}

    def attend(blocks, j0):
        out, terms = [], []
        for q in range(2 * len(blocks)):
            pos, neg = _dual_softmax(blocks[q // 2][64 * (q % 2):64 * (q % 2) + 64])
            zb = jnp.concatenate([state["z"][j0 + q]] * (T // 128), axis=1).reshape(16, 8, T)
            inv = _rcp(_allreduce(pos * zb[:8] + neg * zb[8:], jnp.add) + 1e-6)
            sh = pltpu.roll(inv, 1, 0)
            phi = jnp.concatenate([pos.reshape(64, T), neg.reshape(64, T)], axis=0)
            num = _dot(state["kv"][j0 + q], phi.astype(bf16), _NN).reshape(2, 4, 8, T)
            out.append((num[0] * jnp.where(even, inv, sh)[None]).reshape(32, T))
            out.append((num[1] * jnp.where(even, sh, inv)[None]).reshape(32, T))
            if q % 4 == 3:
                ot = jnp.concatenate(out, axis=0)
                out = []
                terms.append([a.T.astype(bf16) for a in _lhs_terms(
                    ot[:128, :256], ot[128:, :256], ot[:128, 256:], ot[128:, 256:])])
        return terms

    cp_out = []

    def out_proj(i, t, o_terms, n):
        last = i == NT_ - 1

        def product(k):
            m = _dot(jnp.concatenate([a[k] for a in o_terms], axis=1), wos_v[n, k], _NN)
            ffn_step()
            return m

        c = _strassen(product)
        for g in range(2):
            for nn in range(2):
                col0 = 256 * n + 128 * nn
                cols = pl.ds(col0, 128)
                a = jnp.concatenate(
                    [xn_block(t, g, hf, col0 // 512, pl.ds(col0 % 512, 128)) for hf in range(2)],
                    axis=0).astype(f32)
                if last:
                    hit = lax.broadcasted_iota(jnp.int32, (32, 8, 128), 0) * 8 + \
                        lax.broadcasted_iota(jnp.int32, (32, 8, 128), 1) == idx % T - 256 * g
                    a3 = a.reshape(32, 8, 128)
                    a = jnp.where(hit, a3 + state["y"][:, col0:col0 + 128][None], a3).reshape(256, 128)
                tok = pl.ds(256 * g, 256)
                out_v[i, tok, cols] = (x_v[t, tok, cols].astype(f32) + c[2 * g + nn] * _silu(a)).astype(bf16)
        cols = pl.ds(256 * n, 256)
        if last:
            cp_out.append(copy(out_v.at[i, :, cols], out_hbm.at[pl.ds(t * T, T), cols]))
            cp_out[-1].start()
        elif n == D // 256 - 1:
            cp_out.append(copy(out_v.at[i], out_hbm.at[pl.ds(t * T, T)]))
            cp_out[-1].start()

    tiles = [lax.rem(t_sel + 1 + i, NT_) for i in range(NT_)]
    o_prev, o_cur, prev = None, [], None
    for i in range(NT_):
        for c in range(2):
            cur = (proj(2 * c, 2, tiles[i], ffn_step), 8 * c)
            if i == 0 and c == 0:
                kv_update(*pend_v, phis)
                row = lax.broadcasted_iota(jnp.int32, (64, 128), 0)
                col = lax.broadcasted_iota(jnp.int32, (64, 128), 1)
                own = (row >> 5) == (col & 1)
                state["kv"] = [jnp.where(own, a, 0.0).astype(bf16) for a in kv]
                state["z"] = [jnp.broadcast_to(jnp.sum(z, axis=-1, keepdims=True), (128, 128)) for z in zs]
            if prev is not None:
                o_cur += attend(*prev)
                if len(o_cur) == 4:
                    o_old, o_prev, o_cur = o_prev, o_cur, []
            prev = cur
            if i > 0 and c == 1:
                out_proj(i - 1, tiles[i - 1], o_prev, 0)
                out_proj(i - 1, tiles[i - 1], o_prev, 1)
            elif i > 1:
                out_proj(i - 2, tiles[i - 2], o_old, 2)
                out_proj(i - 2, tiles[i - 2], o_old, 3)
    o_cur += attend(*prev)
    out_proj(NT_ - 2, tiles[NT_ - 2], o_prev, 2)
    out_proj(NT_ - 2, tiles[NT_ - 2], o_prev, 3)
    for _ in ffn_steps:
        pass
    state["y"] = _rb(jnp.concatenate(ffn["y"], axis=1) * gate)
    for n in range(4):
        out_proj(NT_ - 1, tiles[NT_ - 1], o_cur, n)
    for c in cp_out:
        c.wait()


@jax.jit
def pallas_recurrent_scan__linear_kernel_hedgehog__moe_arch_mod__prompt_kernel(
    A_x: jax.Array,
    A_wqkv: jax.Array,
    A_w_phi: jax.Array,
    A_wo: jax.Array,
    B_x: jax.Array,
    B_w_r: jax.Array,
    B_w_gate: jax.Array,
    B_w_up: jax.Array,
    B_w_down: jax.Array,
):
    del B_x
    hbm = pl.BlockSpec(memory_space=pl.ANY)
    out = pl.pallas_call(
        _kernel,
        out_shape=jax.ShapeDtypeStruct((S, D), bf16),
        in_specs=[hbm] * 8,
        out_specs=hbm,
        scratch_shapes=[
            pltpu.VMEM((NT_, T, D), bf16),
            pltpu.VMEM((NT_, 2, 9, 128, 512), bf16),
            pltpu.VMEM((12, D, 256), bf16),
            pltpu.VMEM((6, 7, 256, 512), bf16),
            pltpu.VMEM((D, D), bf16),
            pltpu.VMEM((4, 7, 512, 128), bf16),
            pltpu.VMEM((D, F), bf16),
            pltpu.VMEM((D, F), bf16),
            pltpu.VMEM((F, D), bf16),
            pltpu.VMEM((NT_, T, D), bf16),
            pltpu.VMEM((H * DH, DH), bf16),
            pltpu.VMEM((D,), bf16),
            pltpu.SemaphoreType.DMA((48,)),
        ],
        compiler_params=pltpu.CompilerParams(vmem_limit_bytes=110 * 1024 * 1024),
        name="hedgehog_mod",
    )(
        A_x.reshape(S, D), A_wqkv, A_w_phi.reshape(H * DH, DH), A_wo,
        B_w_r, B_w_gate, B_w_up, B_w_down,
    )
    return out.reshape(1, S, D)
```

```python
import math

import jax
import jax.numpy as jnp
from jax import lax
import jax.experimental.pallas as pl
import jax.experimental.pallas.tpu as pltpu

S, D, H, DH, F = 2048, 1024, 32, 32, 3584
T = 512
NT_ = S // T
NF = F // 128
LN_ROWS = 16
LOG2E = math.log2(math.e)
_NT = (((1,), (1,)), ((), ()))
_NN = (((1,), (0,)), ((), ()))
f32, bf16 = jnp.float32, jnp.bfloat16


def _dot(a, b, dn):
    return lax.dot_general(a, b, dn, preferred_element_type=f32)


def _rb(v):
    return v.astype(bf16).astype(f32)


def _rcp(v):
    r = pl.reciprocal(v, approx=True)
    return r * (2.0 - v * r)


def _silu(a):
    return a * pl.reciprocal(1.0 + jnp.exp2(a * -LOG2E), approx=True)


def _lhs_terms(a11, a12, a21, a22):
    return [a11 + a22, a21 + a22, a11, a22, a11 + a12, a21 - a11, a12 - a22]


def _rhs_terms(b11, b12, b21, b22):
    return [b11 + b22, b11, b12 - b22, b21 - b11, b22, b11 + b12, b21 + b22]


def _strassen(product):
    m = product(0)
    c11, c22 = m, m
    c21 = product(3)
    c11 = c11 + c21
    c12 = product(4)
    c11 = c11 - c12
    c11 = c11 + product(6)
    m = product(2)
    c12, c22 = c12 + m, c22 + m
    m = product(1)
    c21, c22 = c21 + m, c22 - m
    c22 = c22 + product(5)
    return c11, c12, c21, c22


def _allreduce(v, op):
    r = v[0]
    for i in range(1, 8):
        r = op(r, v[i])
    r = op(r, pltpu.roll(r, 4, 0))
    return op(r, pltpu.roll(r, 2, 0))


def _dual_softmax(p):
    n = p.shape[1]
    p3 = p.reshape(8, 8, n)
    mx = _allreduce(p3, jnp.maximum)
    mn = _allreduce(p3, jnp.minimum)
    ep = jnp.exp2(p3 - mx[None])
    en = jnp.exp2(mn[None] - p3)
    ip = _rcp(_allreduce(ep, jnp.add))
    im = _rcp(_allreduce(en, jnp.add))
    return ep * ip[None], en * im[None]


def _kernel(x_hbm, wqkv_hbm, wphi_hbm, wo_hbm, wr_hbm, wg_hbm, wu_hbm, wd_hbm, out_hbm,
            x_v, xs_v, wraw_v, ws_v, wo_v, wos_v, wg_v, wu_v, wd_v, out_v, wphi_v, wr_v, sems):
    n_sem = [0]

    def copy(src, dst):
        n_sem[0] += 1
        return pltpu.make_async_copy(src, dst, sems.at[n_sem[0] - 1])

    cp_x0 = [copy(x_hbm.at[pl.ds(s * 256, 256)], x_v.at[0, pl.ds(s * 256, 256)]) for s in range(2)]
    cp_x = [None] + [copy(x_hbm.at[pl.ds(t * T, T)], x_v.at[t]) for t in range(1, NT_)]
    cp_w = [copy(wqkv_hbm.at[:, pl.ds(j * 256, 256)], wraw_v.at[j]) for j in range(12)]
    cp_phi, cp_r, cp_o = copy(wphi_hbm, wphi_v), copy(wr_hbm, wr_v), copy(wo_hbm, wo_v)
    cp_ffn = [copy(wg_hbm, wg_v), copy(wu_hbm, wu_v), copy(wd_hbm, wd_v)]
    for c in ([cp_phi, cp_w[4], cp_r] + cp_x0 + cp_w[5:12] + [cp_x[1]] + cp_w[:4] + cp_x[2:] + [cp_o]
              + cp_ffn):
        c.start()

    top = [(jnp.full((8, 128), -jnp.inf, f32), lax.broadcasted_iota(jnp.int32, (8, 128), 0))] * 2

    def layernorm(t, g, chains):
        wr = wr_v[...].astype(f32).reshape(1, D)
        row = lax.broadcasted_iota(jnp.int32, (8, 128), 0)

        def rows(r, hf):
            x = x_v[t, pl.ds(r, LN_ROWS), :].astype(f32)
            total = x[:, :128]
            for i in range(1, D // 128):
                total = total + x[:, 128 * i:128 * (i + 1)]
            if chains:
                prev = top[hf if chains == 2 else 1 - hf][1]
                total = jnp.where(jnp.concatenate([prev] * (LN_ROWS // 8), axis=0) >= 0, total, 0.0)
            xc = x - jnp.sum(total, axis=-1, keepdims=True) * (1.0 / D)
            v = jnp.mean(xc * xc, axis=-1, keepdims=True)
            xn = xc * _rcp(_rb(jnp.sqrt(_rb(_rb(v) + _rb(jnp.full_like(v, 1e-5))))))
            sc = _rb(jnp.sum(xn * wr, axis=-1, keepdims=True))
            sc = jnp.broadcast_to(sc, (LN_ROWS, 128))
            best, idx = top[hf]
            for i in range(LN_ROWS // 8):
                better = sc[8 * i:8 * i + 8] > best
                best = jnp.where(better, sc[8 * i:8 * i + 8], best)
                idx = jnp.where(better, row + (t * T + r + 8 * i), idx)
            top[hf] = (best, idx)
            return xn

        for r in range(0, 128, LN_ROWS):
            a, b = rows(256 * g + r, 0), rows(256 * g + 128 + r, 1)
            b11, b21, b12, b22 = a[:, :512], a[:, 512:], b[:, :512], b[:, 512:]
            for i, term in enumerate(_rhs_terms(b11, b12, b21, b22) + [b21, b12]):
                xs_v[t, g, i, pl.ds(r, LN_ROWS), :] = term.astype(bf16)

    def xn_block(t, g, hf, kh, cols):
        return xs_v[t, g, ((1, 7), (8, 4))[hf][kh], :, cols]

    cp_phi.wait()
    row = lax.broadcasted_iota(jnp.int32, (128, DH), 0)
    col = lax.broadcasted_iota(jnp.int32, (128, DH), 1)
    expand = jnp.where(((row & 63) >> 1) == col, 1.0, 0.0).astype(bf16)
    l0 = _dot(expand, wphi_v[...], _NT)
    row = lax.broadcasted_iota(jnp.int32, (128, D), 0)
    col = lax.broadcasted_iota(jnp.int32, (128, D), 1)
    same = (((row >> 6) << 1) | (row & 1)) == ((col >> 5) & 3)
    bd = jnp.where(same, l0, 0.0).astype(bf16)

    def prepare_w(j):
        blocks = []
        for b in range(2):
            w = wraw_v[j, :, pl.ds(128 * b, 128)]
            if j < 8:
                c = (2 * j + b) % 8
                blocks.append(_dot(bd[:, c * 128:(c + 1) * 128], w, _NT) * LOG2E)
            else:
                blocks.append(w.astype(f32).T)
        a, b = blocks
        for i, term in enumerate(_lhs_terms(a[:, :512], a[:, 512:], b[:, :512], b[:, 512:])):
            ws_v[j // 2, i, pl.ds(128 * (j % 2), 128), :] = term.astype(bf16)

    def prepare_wo(n):
        for c in range(4):
            w = wo_v[pl.ds(256 * c, 256), pl.ds(256 * n, 256)].astype(f32)
            terms = _rhs_terms(w[:128, :128], w[:128, 128:], w[128:, :128], w[128:, 128:])
            for i, term in enumerate(terms):
                wos_v[n, i, pl.ds(128 * c, 128), :] = term.astype(bf16)

    def plain(lhs, rhs, dn):
        return _dot(lhs, rhs, dn)

    def proj(j0, nj, t, matmul=plain):
        rows = pl.ds(128 * (j0 % 2), 128 * nj)
        groups = []
        for g in range(T // 256):
            def product(i):
                return matmul(ws_v[j0 // 2, i + g * opaque[0], rows, :], xs_v[t, g, i], _NT)
            groups.append(_strassen(product))
        out = []
        for j in range(nj):
            for b in range(2):
                out.append(jnp.concatenate(
                    [c[2 * b + hf][128 * j:128 * (j + 1)] for c in groups for hf in range(2)], axis=1))
        return out

    kv = [None] * 16
    zs = [None] * 16

    def kv_update(k_blocks, v_blocks, j0):
        for q in range(2 * len(k_blocks)):
            rows = slice(64 * (q % 2), 64 * (q % 2) + 64)
            pos, neg = _dual_softmax(k_blocks[q // 2][rows])
            phi = jnp.concatenate([pos.reshape(64, T), neg.reshape(64, T)], axis=0)
            z = zs[j0 + q]
            for n in range(T // 128):
                piece = phi[:, n * 128:(n + 1) * 128]
                z = piece if z is None else z + piece
            zs[j0 + q] = z
            upd = _dot(v_blocks[q // 2][rows].astype(bf16), phi.astype(bf16), _NT)
            kv[j0 + q] = upd if kv[j0 + q] is None else kv[j0 + q] + upd

    cp_w[4].wait()
    cp_r.wait()
    prepare_w(4)
    for g in range(2):
        cp_x0[g].wait()
        layernorm(0, g, 0)
    opaque = [jnp.min(top[0][1]) >> 31]
    k0 = proj(4, 1, 0)
    for c in cp_w[5:7]:
        c.wait()
    for j in (5, 6):
        prepare_w(j)
        k0 += proj(j, 1, 0)
    for c in cp_w[7:10]:
        c.wait()
    for j in (7, 8, 9):
        prepare_w(j)
    k0 += proj(7, 1, 0)
    for c in cp_w[10:12] + [cp_x[1]]:
        c.wait()
    for j in (10, 11):
        prepare_w(j)
    pending = [(k0[:4], proj(8, 2, 0), 0), (k0[4:], proj(10, 2, 0), 8)]
    for g in range(2):
        layernorm(1, g, 2)

    for c in cp_w[:4] + cp_x[2:]:
        c.wait()
    for t in range(1, NT_):
        for c in range(2):
            cur_k = proj(4 + 2 * c, 2, t)
            kv_update(*pending.pop(0))
            cur_v = proj(8 + 2 * c, 2, t)
            if pending:
                kv_update(*pending.pop(0))
            pending.append((cur_k, cur_v, 8 * c))
            if t == 1:
                prepare_w(2 * c)
                prepare_w(2 * c + 1)
        if t + 1 < NT_:
            for g in range(2):
                layernorm(t + 1, g, 1)

    for c in [cp_o] + cp_ffn:
        c.wait()
    for n in range(4):
        prepare_wo(n)
    best, bidx = (jnp.concatenate([top[0][i], top[1][i]], axis=0) for i in range(2))
    r_max = jnp.max(best)
    idx = jnp.min(jnp.where(best == r_max, bidx, S))
    idx = jnp.clip(idx, 0, S - 1)
    t_sel = idx // T
    g_sel, r_sel = (idx % T) // 256, idx % 128
    hf_sel = (idx // 128) % 2
    grp = pl.ds(pl.multiple_of(r_sel // 16 * 16, 16), 16)
    x_sel = jnp.concatenate([xs_v[t_sel, g_sel, 1 + 7 * hf_sel, grp, :],
                             xs_v[t_sel, g_sel, 7 - 3 * hf_sel, grp, :]], axis=1).astype(f32)
    rows = lax.broadcasted_iota(jnp.int32, (16, D), 0)
    x_sel = jnp.where(rows == idx % 16, x_sel, 0.0)
    x_sel = jnp.broadcast_to(jnp.sum(x_sel, axis=0, keepdims=True), (16, D)).astype(bf16)
    gate = jax.nn.sigmoid(jnp.full((8, D), r_max, f32))

    ffn = {"y": [None, None]}

    zero = top[0][1] >> 31

    def after(lhs, dep):
        ok = (pltpu.bitcast(dep, jnp.int32) & zero) == 0
        ok = jnp.concatenate([jnp.concatenate([ok] * 2, axis=0)] * (lhs.shape[1] // 128), axis=1)
        head = jnp.where(ok, lhs[:16], jnp.zeros_like(lhs[:16]))
        return head if lhs.shape[0] == 16 else jnp.concatenate([head, lhs[16:]], axis=0)

    def ffn_program():
        def down(h, n):
            for hf in range(2):
                dep = yield
                part = _dot(after(h, dep), wd_v[pl.ds(n * 128, 128), pl.ds(hf * 512, 512)], _NN)[:8]
                ffn["y"][hf] = part if ffn["y"][hf] is None else ffn["y"][hf] + part
                ffn["done"].append(part[:, 384:])
        h = None
        for n in range(NF):
            acc = []
            for w in (wg_v, wu_v):
                parts = []
                for kh in range(2):
                    dep = yield
                    parts.append(_dot(after(x_sel[:, 512 * kh:512 * (kh + 1)], dep),
                                      w[pl.ds(512 * kh, 512), pl.ds(n * 128, 128)], _NN))
                    ffn["done"].append(parts[-1][:8])
                acc.append(parts[0] + parts[1])
            if h is not None:
                yield from down(h, n - 1)
            h = (_silu(acc[0]) * acc[1]).astype(bf16)
        yield
        ffn["done"].append(None)
        yield from down(h, NF - 1)

    ffn_steps = ffn_program()
    next(ffn_steps)
    ffn["done"], ffn["main"], ffn["live"] = [None, None], best[:8], True

    def ffn_step():
        try:
            ffn_steps.send(ffn["main"])
        except StopIteration:
            ffn["live"] = False

    def with_ffn(lhs, rhs, dn):
        dep = ffn["done"].pop(0) if ffn["done"] else None
        m = _dot(lhs if dep is None else after(lhs, dep), rhs, dn)
        if ffn["live"]:
            ffn_step()
        ffn["main"] = m[-8:]
        return m

    even = (lax.broadcasted_iota(jnp.int32, (8, T), 0) & 1) == 0
    state = {}

    def attend(blocks, j0):
        out, terms = [], []
        for q in range(2 * len(blocks)):
            pos, neg = _dual_softmax(blocks[q // 2][64 * (q % 2):64 * (q % 2) + 64])
            zb = jnp.concatenate([state["z"][j0 + q]] * (T // 128), axis=1).reshape(16, 8, T)
            inv = _rcp(_allreduce(pos * zb[:8] + neg * zb[8:], jnp.add) + 1e-6)
            sh = pltpu.roll(inv, 1, 0)
            phi = jnp.concatenate([pos.reshape(64, T), neg.reshape(64, T)], axis=0)
            num = _dot(state["kv"][j0 + q], phi.astype(bf16), _NN).reshape(2, 4, 8, T)
            out.append((num[0] * jnp.where(even, inv, sh)[None]).reshape(32, T))
            out.append((num[1] * jnp.where(even, sh, inv)[None]).reshape(32, T))
            if q % 4 == 3:
                ot = jnp.concatenate(out, axis=0)
                out = []
                terms.append([a.T for a in _lhs_terms(
                    ot[:128, :256], ot[128:, :256], ot[:128, 256:], ot[128:, 256:])])
        return terms

    cp_out = []

    def out_proj(i, t, o_terms, n):
        last = i == NT_ - 1

        def product(k):
            return with_ffn(jnp.concatenate([a[k] for a in o_terms], axis=1).astype(bf16), wos_v[n, k], _NN)

        c = _strassen(product)
        for g in range(2):
            for nn in range(2):
                col0 = 256 * n + 128 * nn
                cols = pl.ds(col0, 128)
                a = jnp.concatenate(
                    [xn_block(t, g, hf, col0 // 512, pl.ds(col0 % 512, 128)) for hf in range(2)],
                    axis=0).astype(f32)
                if last:
                    hit = lax.broadcasted_iota(jnp.int32, (32, 8, 128), 0) * 8 + \
                        lax.broadcasted_iota(jnp.int32, (32, 8, 128), 1) == idx % T - 256 * g
                    a3 = a.reshape(32, 8, 128)
                    a = jnp.where(hit, a3 + state["y"][:, col0:col0 + 128][None], a3).reshape(256, 128)
                tok = pl.ds(256 * g, 256)
                out_v[i, tok, cols] = (x_v[t, tok, cols].astype(f32) + c[2 * g + nn] * _silu(a)).astype(bf16)
        cols = pl.ds(256 * n, 256)
        if last:
            cp_out.append(copy(out_v.at[i, :, cols], out_hbm.at[pl.ds(t * T, T), cols]))
            cp_out[-1].start()
        elif n == D // 256 - 1:
            cp_out.append(copy(out_v.at[i], out_hbm.at[pl.ds(t * T, T)]))
            cp_out[-1].start()

    tiles = [lax.rem(t_sel + 1 + i, NT_) for i in range(NT_)]
    o_prev, o_cur, prev = None, [], None
    for i in range(NT_):
        for c in range(2):
            cur = (proj(2 * c, 2, tiles[i], with_ffn), 8 * c)
            if i == 0 and c == 0:
                kv_update(*pending.pop(0))
                row = lax.broadcasted_iota(jnp.int32, (64, 128), 0)
                col = lax.broadcasted_iota(jnp.int32, (64, 128), 1)
                own = (row >> 5) == (col & 1)
                state["kv"] = [jnp.where(own, a, 0.0).astype(bf16) for a in kv]
                state["z"] = [jnp.broadcast_to(jnp.sum(z, axis=-1, keepdims=True), (128, 128)) for z in zs]
            if prev is not None:
                o_cur += attend(*prev)
                if len(o_cur) == 4:
                    o_old, o_prev, o_cur = o_prev, o_cur, []
            prev = cur
            if i > 0 and c == 1:
                out_proj(i - 1, tiles[i - 1], o_prev, 0)
                out_proj(i - 1, tiles[i - 1], o_prev, 1)
            elif i > 1:
                out_proj(i - 2, tiles[i - 2], o_old, 2)
                out_proj(i - 2, tiles[i - 2], o_old, 3)
    o_cur += attend(*prev)
    out_proj(NT_ - 2, tiles[NT_ - 2], o_prev, 2)
    out_proj(NT_ - 2, tiles[NT_ - 2], o_prev, 3)
    while ffn["live"]:
        ffn_step()
    state["y"] = _rb(jnp.concatenate(ffn["y"], axis=1) * gate)
    for n in range(4):
        out_proj(NT_ - 1, tiles[NT_ - 1], o_cur, n)
    for c in cp_out:
        c.wait()


@jax.jit
def pallas_recurrent_scan__linear_kernel_hedgehog__moe_arch_mod__prompt_kernel(
    A_x: jax.Array,
    A_wqkv: jax.Array,
    A_w_phi: jax.Array,
    A_wo: jax.Array,
    B_x: jax.Array,
    B_w_r: jax.Array,
    B_w_gate: jax.Array,
    B_w_up: jax.Array,
    B_w_down: jax.Array,
):
    del B_x
    hbm = pl.BlockSpec(memory_space=pl.ANY)
    out = pl.pallas_call(
        _kernel,
        out_shape=jax.ShapeDtypeStruct((S, D), bf16),
        in_specs=[hbm] * 8,
        out_specs=hbm,
        scratch_shapes=[
            pltpu.VMEM((NT_, T, D), bf16),
            pltpu.VMEM((NT_, 2, 9, 128, 512), bf16),
            pltpu.VMEM((12, D, 256), bf16),
            pltpu.VMEM((6, 7, 256, 512), bf16),
            pltpu.VMEM((D, D), bf16),
            pltpu.VMEM((4, 7, 512, 128), bf16),
            pltpu.VMEM((D, F), bf16),
            pltpu.VMEM((D, F), bf16),
            pltpu.VMEM((F, D), bf16),
            pltpu.VMEM((NT_, T, D), bf16),
            pltpu.VMEM((H * DH, DH), bf16),
            pltpu.VMEM((D,), bf16),
            pltpu.SemaphoreType.DMA((48,)),
        ],
        compiler_params=pltpu.CompilerParams(vmem_limit_bytes=110 * 1024 * 1024),
        name="hedgehog_mod",
    )(
        A_x.reshape(S, D), A_wqkv, A_w_phi.reshape(H * DH, DH), A_wo,
        B_w_r, B_w_gate, B_w_up, B_w_down,
    )
    return out.reshape(1, S, D)
```

```python
import functools
import math

import jax
import jax.numpy as jnp
from jax import lax
import jax.experimental.pallas as pl
import jax.experimental.pallas.tpu as pltpu

S, D, H, DH, F = 2048, 1024, 32, 32, 3584
T = 512
NT_ = S // T
LOG2E = math.log2(math.e)
_NT = (((1,), (1,)), ((), ()))
_NN = (((1,), (0,)), ((), ()))
f32, bf16 = jnp.float32, jnp.bfloat16


def _dot(a, b, dn):
    return lax.dot_general(a, b, dn, preferred_element_type=f32)


def _rb(v):
    return v.astype(bf16).astype(f32)


def _rcp(v):
    r = pl.reciprocal(v, approx=True)
    return r * (2.0 - v * r)


def _silu(a):
    return a * pl.reciprocal(1.0 + jnp.exp2(a * -LOG2E), approx=True)


def _bits(v):
    return pltpu.bitcast(v, jnp.int32)


def _lhs_terms(a11, a12, a21, a22):
    return [a11 + a22, a21 + a22, a11, a22, a11 + a12, a21 - a11, a12 - a22]


def _rhs_terms(b11, b12, b21, b22):
    return [b11 + b22, b11, b12 - b22, b21 - b11, b22, b11 + b12, b21 + b22]


def _strassen(product):
    m = product(0)
    c11, c22 = m, m
    c21 = product(3)
    c11 = c11 + c21
    c12 = product(4)
    c11 = c11 - c12
    c11 = c11 + product(6)
    m = product(2)
    c12, c22 = c12 + m, c22 + m
    m = product(1)
    c21, c22 = c21 + m, c22 - m
    c22 = c22 + product(5)
    return c11, c12, c21, c22


def _allreduce(v, op):
    r = v[0]
    for i in range(1, 8):
        r = op(r, v[i])
    r = op(r, pltpu.roll(r, 4, 0))
    return op(r, pltpu.roll(r, 2, 0))


def _features(p):
    p3 = p.reshape(8, 8, p.shape[1])
    mx = _allreduce(p3, jnp.maximum)
    mn = _allreduce(p3, jnp.minimum)
    ep = jnp.exp2(p3 - mx[None])
    en = jnp.exp2(mn[None] - p3)
    ip = _rcp(_allreduce(ep, jnp.add))
    im = _rcp(_allreduce(en, jnp.add))
    return jnp.concatenate([ep * ip[None], en * im[None]], axis=0)


def _kernel(x_hbm, wqkv_hbm, wphi_hbm, wo_hbm, wr_hbm, wg_hbm, wu_hbm, wd_hbm, out_hbm,
            x_v, xs_v, wqkv_v, ws_v, wo_v, wos_v, wg_v, wu_v, wd_v, out_v, wphi_v, wr_v, sems):
    def group(k, *pairs):
        return [pltpu.make_async_copy(src, dst, sems.at[k]) for src, dst in pairs]

    def x_rows(r0, n):
        return x_hbm.at[pl.ds(r0, n)], x_v.at[pl.ds(r0, n)]

    def w_cols(j0, nj):
        cols = pl.ds(256 * j0, 256 * nj)
        return wqkv_hbm.at[:, cols], wqkv_v.at[:, cols]

    loads = [
        group(0, x_rows(0, 256), (wr_hbm, wr_v)),
        group(1, w_cols(8, 1)),
        group(2, x_rows(256, 256)),
        group(3, w_cols(9, 2)),
        group(4, w_cols(11, 1), (wphi_hbm, wphi_v), w_cols(4, 2)),
        group(5, w_cols(6, 2), x_rows(T, T)),
        group(6, w_cols(0, 4), x_rows(2 * T, S - 2 * T)),
        group(7, (wo_hbm, wo_v), (wg_hbm, wg_v), (wu_hbm, wu_v), (wd_hbm, wd_v)),
    ]
    for copies in loads:
        for c in copies:
            c.start()

    def wait_loads():
        for c in loads.pop(0):
            c.wait()

    tasks = []
    pace = {}

    def after(lhs, dep):
        ok = (dep & pace["zero"]) == 0
        first = jnp.where(jnp.concatenate([ok, ok], axis=0), lhs[:16, :128], jnp.zeros((16, 128), bf16))
        if lhs.shape[1] > 128:
            first = jnp.concatenate([first, lhs[:16, 128:]], axis=1)
        return first if lhs.shape[0] == 16 else jnp.concatenate([first, lhs[16:]], axis=0)

    ffn = {"steps": None, "done": [], "y": [None, None]}

    def ffn_step():
        try:
            ffn["steps"].send(ffn["main"])
        except StopIteration:
            ffn["steps"] = None

    def matmul(lhs, rhs, dn):
        task = tasks.pop(0) if tasks else None
        dep = task() if task is not None else None
        if ffn["done"]:
            dep = ffn["done"].pop(0)
        m = _dot(lhs if dep is None else after(lhs, dep), rhs, dn)
        if ffn["steps"] is not None:
            ffn_step()
        ffn["main"] = _bits(m[-8:, -128:])
        return m

    top = [jnp.full((8, 128), -jnp.inf, f32), lax.broadcasted_iota(jnp.int32, (8, 128), 0)]
    chain = []

    def layernorm(t, g, lag):
        wr = wr_v[...].astype(f32).reshape(1, D)
        row = lax.broadcasted_iota(jnp.int32, (8, 128), 0)
        for r in range(0, 128, 16):
            halves = []
            for r0 in (T * t + 256 * g + r, T * t + 256 * g + 128 + r):
                x = x_v[pl.ds(r0, 16), :].astype(f32)
                total = x[:, :128]
                for i in range(1, D // 128):
                    total = total + x[:, 128 * i:128 * (i + 1)]
                if lag:
                    total = jnp.where(jnp.concatenate([chain[-lag]] * 2, axis=0) >= 0, total, 0.0)
                xc = x - jnp.sum(total, axis=-1, keepdims=True) * (1.0 / D)
                v = jnp.mean(xc * xc, axis=-1, keepdims=True)
                xn = xc * _rcp(_rb(jnp.sqrt(_rb(_rb(v) + _rb(jnp.full_like(v, 1e-5))))))
                halves.append(xn)
                score = jnp.broadcast_to(_rb(jnp.sum(xn * wr, axis=-1, keepdims=True)), (16, 128))
                for i in range(2):
                    sc, tok = score[8 * i:8 * i + 8], row + (r0 + 8 * i)
                    better = (sc > top[0]) | ((sc == top[0]) & (tok < top[1]))
                    top[:] = jnp.where(better, sc, top[0]), jnp.where(better, tok, top[1])
                chain.append(top[1])
            a, b = halves
            b11, b21, b12, b22 = a[:, :512], a[:, 512:], b[:, :512], b[:, 512:]
            for i, term in enumerate(_rhs_terms(b11, b12, b21, b22) + [b21, b12]):
                xs_v[t, g, i, pl.ds(r, 16), :] = term.astype(bf16)

    def xn_block(t, g, hf, kh, rows, cols):
        return xs_v[t, g, 7 - 3 * hf if kh else 1 + 7 * hf, rows, cols]

    def feature_map():
        row = lax.broadcasted_iota(jnp.int32, (128, DH), 0)
        col = lax.broadcasted_iota(jnp.int32, (128, DH), 1)
        expand = jnp.where(((row & 63) >> 1) == col, 1.0, 0.0).astype(bf16)
        full = _dot(expand, wphi_v[...], _NT)
        row = lax.broadcasted_iota(jnp.int32, (128, D), 0)
        col = lax.broadcasted_iota(jnp.int32, (128, D), 1)
        same = (((row >> 6) << 1) | (row & 1)) == ((col >> 5) & 3)
        return jnp.where(same, full, 0.0).astype(bf16)

    def prepare_w(j):
        blocks = []
        for c in (2 * j, 2 * j + 1):
            w = wqkv_v[:, pl.ds(128 * c, 128)]
            if j < 8:
                blocks.append(_dot(bd[:, 128 * (c % 8):128 * (c % 8 + 1)], w, _NT) * LOG2E)
            else:
                blocks.append(w.astype(f32).T)
        a, b = blocks
        for i, term in enumerate(_lhs_terms(a[:, :512], a[:, 512:], b[:, :512], b[:, 512:])):
            ws_v[j // 2, i, pl.ds(128 * (j % 2), 128), :] = term.astype(bf16)

    def prepare_wo(n):
        for c in range(4):
            w = wo_v[pl.ds(256 * c, 256), pl.ds(256 * n, 256)].astype(f32)
            terms = _rhs_terms(w[:128, :128], w[:128, 128:], w[128:, :128], w[128:, 128:])
            for i, term in enumerate(terms):
                wos_v[n, i, pl.ds(128 * c, 128), :] = term.astype(bf16)

    def proj(j0, nj, t):
        rows = pl.ds(128 * (j0 % 2), 128 * nj)
        groups = [_strassen(lambda i: matmul(ws_v[j0 // 2, i, rows, :], xs_v[t, g, i], _NT))
                  for g in range(T // 256)]
        return [jnp.concatenate([c[2 * b + hf][128 * j + 64 * q:128 * j + 64 * q + 64]
                                 for c in groups for hf in range(2)], axis=1)
                for j in range(nj) for b in range(2) for q in range(2)]

    kv = [None] * 16
    phi_k = [None] * 16

    def key_features(j, p):
        phi = _features(p)
        phi_k[j] = phi.reshape(128, T).astype(bf16)
        return functools.reduce(jnp.bitwise_or, [_bits(phi[i][:, n:n + 128]) for i in (7, 15)
                                                 for n in range(0, T, 128)])

    def key_tasks(blocks, j0):
        return [None] * 5 + [functools.partial(key_features, j0 + q, p) for q, p in enumerate(blocks)]

    def kv_update(v_blocks, j0):
        for j, v in enumerate(v_blocks, j0):
            v1 = jnp.concatenate([v, jnp.ones((16, T), f32)], axis=0).astype(bf16)
            upd = _dot(v1, phi_k[j], _NT)
            kv[j] = upd if kv[j] is None else kv[j] + upd

    wait_loads()
    layernorm(0, 0, 0)
    pace["zero"] = top[1] >> 31
    wait_loads()
    prepare_w(8)
    wait_loads()
    layernorm(0, 1, 0)
    v0 = proj(8, 1, 0)
    wait_loads()
    for j in (9, 10):
        prepare_w(j)
        v0 += proj(j, 1, 0)
    wait_loads()
    prepare_w(11)
    v0 += proj(11, 1, 0)
    bd = feature_map()
    for j in (4, 5):
        prepare_w(j)
    wait_loads()
    k = proj(4, 2, 0)
    for j in (6, 7):
        prepare_w(j)
    tasks += key_tasks(k, 0)
    k = proj(6, 2, 0)
    for g in range(2):
        layernorm(1, g, 2)
    wait_loads()
    pending = [(v0[:8], 0), (v0[8:], 8)]
    j0 = 8
    for t in range(1, NT_):
        for c in range(2):
            tasks += key_tasks(k, j0)
            v = proj(8 + 2 * c, 2, t)
            if len(pending) > 1:
                kv_update(*pending.pop(0))
            k, j0 = proj(4 + 2 * c, 2, t), 8 * c
            kv_update(*pending.pop(0))
            pending.append((v, j0))
            if t == NT_ - 1:
                prepare_w(2 * c)
                prepare_w(2 * c + 1)
        for g in range(2 if t + 1 < NT_ else 0):
            layernorm(t + 1, g, 1)
    tasks += key_tasks(k, j0)

    r_max = jnp.max(top[0])
    idx = jnp.clip(jnp.min(jnp.where(top[0] == r_max, top[1], S)), 0, S - 1)
    t_sel = idx // T
    grp = pl.ds(pl.multiple_of(idx % 128 // 16 * 16, 16), 16)
    x_sel = jnp.concatenate(
        [xn_block(t_sel, idx % T // 256, idx // 128 % 2, kh, grp, slice(None)) for kh in range(2)],
        axis=1).astype(f32)
    x_sel = jnp.where(lax.broadcasted_iota(jnp.int32, (16, D), 0) == idx % 16, x_sel, 0.0)
    x_sel = jnp.broadcast_to(jnp.sum(x_sel, axis=0, keepdims=True), (16, D)).astype(bf16)
    gate = jax.nn.sigmoid(jnp.full((8, D), r_max, f32))

    def ffn_program():
        def down(h, n):
            for hf in range(2):
                dep = yield
                part = _dot(after(h, dep), wd_v[pl.ds(n * 128, 128), pl.ds(hf * 512, 512)], _NN)[:8]
                ffn["y"][hf] = part if ffn["y"][hf] is None else ffn["y"][hf] + part
                ffn["done"].append(_bits(part[:, 384:]))
        h = None
        for n in range(F // 128):
            acc = []
            for w in (wg_v, wu_v):
                parts = []
                for kh in range(2):
                    dep = yield
                    parts.append(_dot(after(x_sel[:, 512 * kh:512 * (kh + 1)], dep),
                                      w[pl.ds(512 * kh, 512), pl.ds(n * 128, 128)], _NN))
                    ffn["done"].append(_bits(parts[-1][:8]))
                acc.append(parts[0] + parts[1])
            if h is not None:
                yield from down(h, n - 1)
            h = (_silu(acc[0]) * acc[1]).astype(bf16)
        yield
        ffn["done"].append(None)
        yield from down(h, F // 128 - 1)

    def attend(blocks, j0):
        terms, out = [], []
        for j, p in enumerate(blocks, j0):
            num = _dot(kv[j], _features(p).reshape(128, T).astype(bf16), _NN)
            for hd in range(2):
                inv = _rcp(num[64 + 8 * hd:72 + 8 * hd] + 1e-6)
                out.append((num[32 * hd:32 * hd + 32].reshape(4, 8, T) * inv[None]).reshape(32, T))
            if j % 4 == 3:
                ot, out = jnp.concatenate(out, axis=0), []
                terms.append([a.T for a in _lhs_terms(
                    ot[:128, :256], ot[128:, :256], ot[:128, 256:], ot[128:, 256:])])
        return terms

    stores = []

    def out_proj(i, t, o_terms, n):
        last = i == NT_ - 1
        c = _strassen(lambda k: matmul(
            jnp.concatenate([a[k] for a in o_terms], axis=1).astype(bf16), wos_v[n, k], _NN))
        for g in range(2):
            for nn in range(2):
                col0 = 256 * n + 128 * nn
                cols, tok = pl.ds(col0, 128), pl.ds(pl.multiple_of(T * t + 256 * g, 256), 256)
                a = jnp.concatenate(
                    [xn_block(t, g, hf, col0 // 512, slice(None), pl.ds(col0 % 512, 128))
                     for hf in range(2)], axis=0).astype(f32)
                if last:
                    hit = (lax.broadcasted_iota(jnp.int32, (32, 8, 128), 0) * 8
                           + lax.broadcasted_iota(jnp.int32, (32, 8, 128), 1)) == idx % T - 256 * g
                    a3 = a.reshape(32, 8, 128)
                    a = jnp.where(hit, a3 + ffn["y"][:, col0:col0 + 128][None], a3).reshape(256, 128)
                rows = pl.ds(T * i + 256 * g, 256)
                out_v[rows, cols] = (x_v[tok, cols].astype(f32) + c[2 * g + nn] * _silu(a)).astype(bf16)
                if last and n == 3:
                    stores.extend(group(9, (out_v.at[rows, cols], out_hbm.at[tok, cols])))
                    stores[-1].start()
        if last != (n == 3):
            cols = pl.ds(256 * n, 256) if last else slice(None)
            stores.extend(group(9, (out_v.at[pl.ds(T * i, T), cols],
                                    out_hbm.at[pl.ds(pl.multiple_of(T * t, T), T), cols])))
            stores[-1].start()

    tiles = [lax.rem(t_sel + 1 + i, NT_) for i in range(NT_)]
    o_terms = [[] for _ in range(NT_)]
    halves = [(i, c) for i in range(NT_) for c in range(2)]

    def out_half(h):
        i, c = halves[h]
        for n in (2 * c, 2 * c + 1):
            out_proj(i, tiles[i], o_terms[i], n)

    for h, (i, c) in enumerate(halves):
        q = proj(2 * c, 2, tiles[i])
        if h == 0:
            kv_update(*pending.pop(0))
            row = lax.broadcasted_iota(jnp.int32, (80, 128), 0)
            col = lax.broadcasted_iota(jnp.int32, (80, 128), 1)
            own = jnp.where(row < 64, row >> 5, (row >> 3) & 1) == (col & 1)
            kv[:] = [jnp.where(own, a, 0.0).astype(bf16) for a in kv]
            wait_loads()
            for n in range(4):
                prepare_wo(n)
            ffn["steps"], ffn["done"] = ffn_program(), [None, None]
            next(ffn["steps"])
        else:
            o_terms[halves[h - 1][0]] += attend(prev_q, 8 * halves[h - 1][1])
        prev_q = q
        if h >= 3:
            out_half(h - 3)
    o_terms[-1] += attend(prev_q, 8)
    out_half(len(halves) - 3)
    while ffn["steps"] is not None:
        ffn_step()
    ffn["y"] = _rb(jnp.concatenate(ffn["y"], axis=1) * gate)
    out_half(len(halves) - 2)
    out_half(len(halves) - 1)
    for c in stores:
        c.wait()


@jax.jit
def pallas_recurrent_scan__linear_kernel_hedgehog__moe_arch_mod__prompt_kernel(
    A_x: jax.Array,
    A_wqkv: jax.Array,
    A_w_phi: jax.Array,
    A_wo: jax.Array,
    B_x: jax.Array,
    B_w_r: jax.Array,
    B_w_gate: jax.Array,
    B_w_up: jax.Array,
    B_w_down: jax.Array,
):
    del B_x
    hbm = pl.BlockSpec(memory_space=pl.ANY)
    out = pl.pallas_call(
        _kernel,
        out_shape=jax.ShapeDtypeStruct((S, D), bf16),
        in_specs=[hbm] * 8,
        out_specs=hbm,
        scratch_shapes=[
            pltpu.VMEM((S, D), bf16),
            pltpu.VMEM((NT_, 2, 9, 128, 512), bf16),
            pltpu.VMEM((D, 3 * D), bf16),
            pltpu.VMEM((6, 7, 256, 512), bf16),
            pltpu.VMEM((D, D), bf16),
            pltpu.VMEM((4, 7, 512, 128), bf16),
            pltpu.VMEM((D, F), bf16),
            pltpu.VMEM((D, F), bf16),
            pltpu.VMEM((F, D), bf16),
            pltpu.VMEM((S, D), bf16),
            pltpu.VMEM((H * DH, DH), bf16),
            pltpu.VMEM((D,), bf16),
            pltpu.SemaphoreType.DMA((10,)),
        ],
        compiler_params=pltpu.CompilerParams(vmem_limit_bytes=110 * 1024 * 1024),
        name="hedgehog_mod",
    )(
        A_x.reshape(S, D), A_wqkv, A_w_phi.reshape(H * DH, DH), A_wo,
        B_w_r, B_w_gate, B_w_up, B_w_down,
    )
    return out.reshape(1, S, D)
```

```python
import functools
import math

import jax
import jax.numpy as jnp
from jax import lax
import jax.experimental.pallas as pl
import jax.experimental.pallas.tpu as pltpu

S, D, H, DH, F = 2048, 1024, 32, 32, 3584
T = 512
NT_ = S // T
LOG2E = math.log2(math.e)
_NT = (((1,), (1,)), ((), ()))
_NN = (((1,), (0,)), ((), ()))
f32, bf16 = jnp.float32, jnp.bfloat16


def _dot(a, b, dn):
    return lax.dot_general(a, b, dn, preferred_element_type=f32)


def _rb(v):
    return v.astype(bf16).astype(f32)


def _rcp(v):
    r = pl.reciprocal(v, approx=True)
    return r * (2.0 - v * r)


def _silu(a):
    return a * pl.reciprocal(1.0 + jnp.exp2(a * -LOG2E), approx=True)


def _bits(v):
    return pltpu.bitcast(v, jnp.int32)


def _lhs_terms(a11, a12, a21, a22):
    return [a11 + a22, a21 + a22, a11, a22, a11 + a12, a21 - a11, a12 - a22]


def _rhs_terms(b11, b12, b21, b22):
    return [b11 + b22, b11, b12 - b22, b21 - b11, b22, b11 + b12, b21 + b22]


def _strassen(product):
    m = product(0)
    c11, c22 = m, m
    c21 = product(3)
    c11 = c11 + c21
    c12 = product(4)
    c11 = c11 - c12
    c11 = c11 + product(6)
    m = product(2)
    c12, c22 = c12 + m, c22 + m
    m = product(1)
    c21, c22 = c21 + m, c22 - m
    c22 = c22 + product(5)
    return c11, c12, c21, c22


def _allreduce(v, op):
    r = v[0]
    for i in range(1, 8):
        r = op(r, v[i])
    r = op(r, pltpu.roll(r, 4, 0))
    return op(r, pltpu.roll(r, 2, 0))


def _features(p):
    p3 = p.reshape(8, 8, p.shape[1])
    mx = _allreduce(p3, jnp.maximum)
    mn = _allreduce(p3, jnp.minimum)
    ep = jnp.exp2(p3 - mx[None])
    en = jnp.exp2(mn[None] - p3)
    ip = _rcp(_allreduce(ep, jnp.add))
    im = _rcp(_allreduce(en, jnp.add))
    return jnp.concatenate([ep * ip[None], en * im[None]], axis=0)


def _kernel(x_hbm, wqkv_hbm, wphi_hbm, wo_hbm, wr_hbm, wg_hbm, wu_hbm, wd_hbm, out_hbm,
            x_v, xs_v, wqkv_v, ws_v, wo_v, wos_v, wg_v, wu_v, wd_v, out_v, wphi_v, wr_v, sems):
    def group(k, *pairs):
        return [pltpu.make_async_copy(src, dst, sems.at[k]) for src, dst in pairs]

    def x_rows(r0, n):
        return x_hbm.at[pl.ds(r0, n)], x_v.at[pl.ds(r0, n)]

    def w_cols(j0, nj):
        cols = pl.ds(256 * j0, 256 * nj)
        return wqkv_hbm.at[:, cols], wqkv_v.at[:, cols]

    loads = [
        group(0, x_rows(0, 256), (wr_hbm, wr_v)),
        group(1, w_cols(8, 1)),
        group(2, x_rows(256, 256)),
        group(3, w_cols(9, 1)),
        group(4, w_cols(10, 2)),
        group(5, (wphi_hbm, wphi_v), w_cols(4, 2)),
        group(6, w_cols(6, 2), x_rows(T, T)),
        group(7, x_rows(2 * T, S - 2 * T)),
        group(8, w_cols(0, 4)),
        group(9, (wo_hbm, wo_v), (wg_hbm, wg_v), (wu_hbm, wu_v), (wd_hbm, wd_v)),
    ]
    for copies in loads:
        for c in copies:
            c.start()

    def wait_loads():
        for c in loads.pop(0):
            c.wait()

    tasks = []
    pace = {}

    def after(lhs, dep):
        ok = (dep & pace["zero"]) == 0
        first = jnp.where(jnp.concatenate([ok, ok], axis=0), lhs[:16, :128], jnp.zeros((16, 128), bf16))
        if lhs.shape[1] > 128:
            first = jnp.concatenate([first, lhs[:16, 128:]], axis=1)
        return first if lhs.shape[0] == 16 else jnp.concatenate([first, lhs[16:]], axis=0)

    ffn = {"steps": None, "done": [], "y": [None, None]}

    def ffn_step():
        try:
            ffn["steps"].send(ffn["main"])
        except StopIteration:
            ffn["steps"] = None

    def matmul(lhs, rhs, dn):
        task = tasks.pop(0) if tasks else None
        dep = task() if task is not None else None
        if ffn["done"]:
            dep = ffn["done"].pop(0)
        m = _dot(lhs if dep is None else after(lhs, dep), rhs, dn)
        if ffn["steps"] is not None:
            ffn_step()
        ffn["main"] = _bits(m[-8:, -128:])
        return m

    top = [jnp.full((8, 128), -jnp.inf, f32), lax.broadcasted_iota(jnp.int32, (8, 128), 0)]
    chain = []

    def layernorm(t, g, lag):
        wr = wr_v[...].astype(f32).reshape(1, D)
        row = lax.broadcasted_iota(jnp.int32, (8, 128), 0)
        for r in range(0, 128, 16):
            halves = []
            for r0 in (T * t + 256 * g + r, T * t + 256 * g + 128 + r):
                x = x_v[pl.ds(r0, 16), :].astype(f32)
                total = x[:, :128]
                for i in range(1, D // 128):
                    total = total + x[:, 128 * i:128 * (i + 1)]
                if lag:
                    total = jnp.where(jnp.concatenate([chain[-lag]] * 2, axis=0) >= 0, total, 0.0)
                xc = x - jnp.sum(total, axis=-1, keepdims=True) * (1.0 / D)
                v = jnp.mean(xc * xc, axis=-1, keepdims=True)
                xn = xc * _rcp(_rb(jnp.sqrt(_rb(_rb(v) + _rb(jnp.full_like(v, 1e-5))))))
                halves.append(xn)
                score = jnp.broadcast_to(_rb(jnp.sum(xn * wr, axis=-1, keepdims=True)), (16, 128))
                for i in range(2):
                    sc, tok = score[8 * i:8 * i + 8], row + (r0 + 8 * i)
                    better = (sc > top[0]) | ((sc == top[0]) & (tok < top[1]))
                    top[:] = jnp.where(better, sc, top[0]), jnp.where(better, tok, top[1])
                chain.append(top[1])
            a, b = halves
            b11, b21, b12, b22 = a[:, :512], a[:, 512:], b[:, :512], b[:, 512:]
            for i, term in enumerate(_rhs_terms(b11, b12, b21, b22) + [b21, b12]):
                xs_v[t, g, i, pl.ds(r, 16), :] = term.astype(bf16)

    def xn_block(t, g, hf, kh, rows, cols):
        return xs_v[t, g, 7 - 3 * hf if kh else 1 + 7 * hf, rows, cols]

    def feature_map():
        row = lax.broadcasted_iota(jnp.int32, (128, DH), 0)
        col = lax.broadcasted_iota(jnp.int32, (128, DH), 1)
        expand = jnp.where(((row & 63) >> 1) == col, 1.0, 0.0).astype(bf16)
        full = _dot(expand, wphi_v[...], _NT)
        row = lax.broadcasted_iota(jnp.int32, (128, D), 0)
        col = lax.broadcasted_iota(jnp.int32, (128, D), 1)
        same = (((row >> 6) << 1) | (row & 1)) == ((col >> 5) & 3)
        return jnp.where(same, full, 0.0).astype(bf16)

    def prepare_w(j):
        blocks = []
        for c in (2 * j, 2 * j + 1):
            w = wqkv_v[:, pl.ds(128 * c, 128)]
            if j < 8:
                blocks.append(_dot(bd[:, 128 * (c % 8):128 * (c % 8 + 1)], w, _NT) * LOG2E)
            else:
                blocks.append(w.astype(f32).T)
        a, b = blocks
        for i, term in enumerate(_lhs_terms(a[:, :512], a[:, 512:], b[:, :512], b[:, 512:])):
            ws_v[j // 2, i, pl.ds(128 * (j % 2), 128), :] = term.astype(bf16)

    def prepare_wo(n):
        for c in range(4):
            w = wo_v[pl.ds(256 * c, 256), pl.ds(256 * n, 256)].astype(f32)
            terms = _rhs_terms(w[:128, :128], w[:128, 128:], w[128:, :128], w[128:, 128:])
            for i, term in enumerate(terms):
                wos_v[n, i, pl.ds(128 * c, 128), :] = term.astype(bf16)

    def proj_group(j0, nj, t, g):
        rows = pl.ds(128 * (j0 % 2), 128 * nj)
        return _strassen(lambda i: matmul(ws_v[j0 // 2, i, rows, :], xs_v[t, g, i], _NT))

    def pairs(groups):
        return [jnp.concatenate([c[2 * b + hf][r:r + 64] for c in groups for hf in range(2)], axis=1)
                for j in range(groups[0][0].shape[0] // 128) for b in range(2)
                for r in (128 * j, 128 * j + 64)]

    def proj(j0, t):
        return pairs([proj_group(j0, 2, t, g) for g in range(2)])

    kv = [None] * 16
    phi_k = [None] * 16

    def key_features(j, p):
        phi = _features(p)
        phi_k[j] = phi.reshape(128, T).astype(bf16)
        return functools.reduce(jnp.bitwise_or, [_bits(phi[i][:, n:n + 128]) for i in (7, 15)
                                                 for n in range(0, T, 128)])

    def key_tasks(blocks, j0):
        return [None] * 5 + [functools.partial(key_features, j0 + q, p) for q, p in enumerate(blocks)]

    def kv_update(v_blocks, j0):
        for j, v in enumerate(v_blocks, j0):
            v1 = jnp.concatenate([v, jnp.ones((16, T), f32)], axis=0).astype(bf16)
            upd = _dot(v1, phi_k[j], _NT)
            kv[j] = upd if kv[j] is None else kv[j] + upd

    wait_loads()
    layernorm(0, 0, 0)
    pace["zero"] = top[1] >> 31
    wait_loads()
    prepare_w(8)
    wait_loads()
    layernorm(0, 1, 0)
    first = proj_group(8, 1, 0, 0)
    wait_loads()
    v0 = pairs([first, proj_group(8, 1, 0, 1)])
    prepare_w(9)
    first = proj_group(9, 1, 0, 0)
    wait_loads()
    v0 += pairs([first, proj_group(9, 1, 0, 1)])
    for j in (10, 11):
        prepare_w(j)
    if "0" == "0":
        v0 += pairs([proj_group(10, 1, 0, g) for g in range(2)])
        first = proj_group(11, 1, 0, 0)
        wait_loads()
        v0 += pairs([first, proj_group(11, 1, 0, 1)])
    else:
        first = proj_group(10, 2, 0, 0)
        wait_loads()
        v0 += pairs([first, proj_group(10, 2, 0, 1)])
    bd = feature_map()
    for j in (4, 5):
        prepare_w(j)
    first = proj_group(4, 2, 0, 0)
    wait_loads()
    k = pairs([first, proj_group(4, 2, 0, 1)])
    for j in (6, 7):
        prepare_w(j)
    tasks += key_tasks(k, 0)
    k = proj(6, 0)
    for g in range(2):
        layernorm(1, g, 3)
    wait_loads()
    pending = [(v0[:8], 0), (v0[8:], 8)]
    j0 = 8
    for t in range(1, NT_):
        if t == NT_ - 1:
            wait_loads()
        for c in range(2):
            tasks += key_tasks(k, j0)
            v = proj(8 + 2 * c, t)
            if len(pending) > 1:
                kv_update(*pending.pop(0))
            k, j0 = proj(4 + 2 * c, t), 8 * c
            kv_update(*pending.pop(0))
            pending.append((v, j0))
            if t == NT_ - 1:
                prepare_w(2 * c)
                prepare_w(2 * c + 1)
        for g in range(2 if t + 1 < NT_ else 0):
            layernorm(t + 1, g, 1)
    tasks += key_tasks(k, j0)

    r_max = jnp.max(top[0])
    idx = jnp.clip(jnp.min(jnp.where(top[0] == r_max, top[1], S)), 0, S - 1)
    t_sel = idx // T
    grp = pl.ds(pl.multiple_of(idx % 128 // 16 * 16, 16), 16)
    x_sel = jnp.concatenate(
        [xn_block(t_sel, idx % T // 256, idx // 128 % 2, kh, grp, slice(None)) for kh in range(2)],
        axis=1).astype(f32)
    x_sel = jnp.where(lax.broadcasted_iota(jnp.int32, (16, D), 0) == idx % 16, x_sel, 0.0)
    x_sel = jnp.broadcast_to(jnp.sum(x_sel, axis=0, keepdims=True), (16, D)).astype(bf16)
    gate = jax.nn.sigmoid(jnp.full((8, D), r_max, f32))

    def ffn_program():
        def down(h, n):
            for hf in range(2):
                dep = yield
                part = _dot(after(h, dep), wd_v[pl.ds(n * 128, 128), pl.ds(hf * 512, 512)], _NN)[:8]
                ffn["y"][hf] = part if ffn["y"][hf] is None else ffn["y"][hf] + part
                ffn["done"].append(_bits(part[:, 384:]))
        h = None
        for n in range(F // 128):
            acc = []
            for w in (wg_v, wu_v):
                parts = []
                for kh in range(2):
                    dep = yield
                    parts.append(_dot(after(x_sel[:, 512 * kh:512 * (kh + 1)], dep),
                                      w[pl.ds(512 * kh, 512), pl.ds(n * 128, 128)], _NN))
                    ffn["done"].append(_bits(parts[-1][:8]))
                acc.append(parts[0] + parts[1])
            if h is not None:
                yield from down(h, n - 1)
            h = (_silu(acc[0]) * acc[1]).astype(bf16)
        yield
        ffn["done"].append(None)
        yield from down(h, F // 128 - 1)

    def attend(blocks, j0):
        terms, out = [], []
        for j, p in enumerate(blocks, j0):
            num = _dot(kv[j], _features(p).reshape(128, T).astype(bf16), _NN)
            for hd in range(2):
                inv = _rcp(num[64 + 8 * hd:72 + 8 * hd] + 1e-6)
                out.append((num[32 * hd:32 * hd + 32].reshape(4, 8, T) * inv[None]).reshape(32, T))
            if j % 4 == 3:
                ot, out = jnp.concatenate(out, axis=0), []
                terms.append([a.T for a in _lhs_terms(
                    ot[:128, :256], ot[128:, :256], ot[:128, 256:], ot[128:, 256:])])
        return terms

    stores = []

    def out_proj(i, t, o_terms, n):
        last = i == NT_ - 1
        c = _strassen(lambda k: matmul(
            jnp.concatenate([a[k] for a in o_terms], axis=1).astype(bf16), wos_v[n, k], _NN))
        for g in range(2):
            for nn in range(2):
                col0 = 256 * n + 128 * nn
                cols, tok = pl.ds(col0, 128), pl.ds(pl.multiple_of(T * t + 256 * g, 256), 256)
                a = jnp.concatenate(
                    [xn_block(t, g, hf, col0 // 512, slice(None), pl.ds(col0 % 512, 128))
                     for hf in range(2)], axis=0).astype(f32)
                if last:
                    hit = (lax.broadcasted_iota(jnp.int32, (32, 8, 128), 0) * 8
                           + lax.broadcasted_iota(jnp.int32, (32, 8, 128), 1)) == idx % T - 256 * g
                    a3 = a.reshape(32, 8, 128)
                    a = jnp.where(hit, a3 + ffn["y"][:, col0:col0 + 128][None], a3).reshape(256, 128)
                rows = pl.ds(T * i + 256 * g, 256)
                out_v[rows, cols] = (x_v[tok, cols].astype(f32) + c[2 * g + nn] * _silu(a)).astype(bf16)
                if last and n == 3:
                    stores.extend(group(10, (out_v.at[rows, cols], out_hbm.at[tok, cols])))
                    stores[-1].start()
        if last != (n == 3):
            cols = pl.ds(256 * n, 256) if last else slice(None)
            stores.extend(group(10, (out_v.at[pl.ds(T * i, T), cols],
                                    out_hbm.at[pl.ds(pl.multiple_of(T * t, T), T), cols])))
            stores[-1].start()

    tiles = [lax.rem(t_sel + 1 + i, NT_) for i in range(NT_)]
    o_terms = [[] for _ in range(NT_)]
    halves = [(i, c) for i in range(NT_) for c in range(2)]

    def out_half(h):
        i, c = halves[h]
        for n in (2 * c, 2 * c + 1):
            out_proj(i, tiles[i], o_terms[i], n)

    for h, (i, c) in enumerate(halves):
        q = proj(2 * c, tiles[i])
        if h == 0:
            kv_update(*pending.pop(0))
            row = lax.broadcasted_iota(jnp.int32, (80, 128), 0)
            col = lax.broadcasted_iota(jnp.int32, (80, 128), 1)
            own = jnp.where(row < 64, row >> 5, (row >> 3) & 1) == (col & 1)
            kv[:] = [jnp.where(own, a, 0.0).astype(bf16) for a in kv]
            wait_loads()
            for n in range(4):
                prepare_wo(n)
            ffn["steps"], ffn["done"] = ffn_program(), [None, None]
            next(ffn["steps"])
        else:
            o_terms[halves[h - 1][0]] += attend(prev_q, 8 * halves[h - 1][1])
        prev_q = q
        if h >= 3:
            out_half(h - 3)
    o_terms[-1] += attend(prev_q, 8)
    out_half(len(halves) - 3)
    while ffn["steps"] is not None:
        ffn_step()
    ffn["y"] = _rb(jnp.concatenate(ffn["y"], axis=1) * gate)
    out_half(len(halves) - 2)
    out_half(len(halves) - 1)
    for c in stores:
        c.wait()


@jax.jit
def pallas_recurrent_scan__linear_kernel_hedgehog__moe_arch_mod__prompt_kernel(
    A_x: jax.Array,
    A_wqkv: jax.Array,
    A_w_phi: jax.Array,
    A_wo: jax.Array,
    B_x: jax.Array,
    B_w_r: jax.Array,
    B_w_gate: jax.Array,
    B_w_up: jax.Array,
    B_w_down: jax.Array,
):
    del B_x
    hbm = pl.BlockSpec(memory_space=pl.ANY)
    out = pl.pallas_call(
        _kernel,
        out_shape=jax.ShapeDtypeStruct((S, D), bf16),
        in_specs=[hbm] * 8,
        out_specs=hbm,
        scratch_shapes=[
            pltpu.VMEM((S, D), bf16),
            pltpu.VMEM((NT_, 2, 9, 128, 512), bf16),
            pltpu.VMEM((D, 3 * D), bf16),
            pltpu.VMEM((6, 7, 256, 512), bf16),
            pltpu.VMEM((D, D), bf16),
            pltpu.VMEM((4, 7, 512, 128), bf16),
            pltpu.VMEM((D, F), bf16),
            pltpu.VMEM((D, F), bf16),
            pltpu.VMEM((F, D), bf16),
            pltpu.VMEM((S, D), bf16),
            pltpu.VMEM((H * DH, DH), bf16),
            pltpu.VMEM((D,), bf16),
            pltpu.SemaphoreType.DMA((11,)),
        ],
        compiler_params=pltpu.CompilerParams(vmem_limit_bytes=110 * 1024 * 1024),
        name="hedgehog_mod",
    )(
        A_x.reshape(S, D), A_wqkv, A_w_phi.reshape(H * DH, DH), A_wo,
        B_w_r, B_w_gate, B_w_up, B_w_down,
    )
    return out.reshape(1, S, D)
```

```python
import functools
import math

import jax
import jax.numpy as jnp
from jax import lax
import jax.experimental.pallas as pl
import jax.experimental.pallas.tpu as pltpu

S, D, H, DH, F = 2048, 1024, 32, 32, 3584
T = 512
NT_ = S // T
LOG2E = math.log2(math.e)
_NT = (((1,), (1,)), ((), ()))
_NN = (((1,), (0,)), ((), ()))
f32, bf16 = jnp.float32, jnp.bfloat16


def _dot(a, b, dn):
    return lax.dot_general(a, b, dn, preferred_element_type=f32)


def _rb(v):
    return v.astype(bf16).astype(f32)


def _rcp(v):
    r = pl.reciprocal(v, approx=True)
    return r * (2.0 - v * r)


def _silu(a):
    return a * pl.reciprocal(1.0 + jnp.exp2(a * -LOG2E), approx=True)


def _bits(v):
    return pltpu.bitcast(v, jnp.int32)


def _pack(v):
    m, n = v.shape
    v = v.reshape(m // 16, 2, 8, n)
    return pltpu.pack_elementwise([v[:, 0], v[:, 1]], packed_dtype=bf16).reshape(m // 2, n)


def _unpack(words):
    return pltpu.bitcast(words, bf16)


def _lhs_terms(a11, a12, a21, a22):
    return [a11 + a22, a21 + a22, a11, a22, a11 + a12, a21 - a11, a12 - a22]


def _rhs_terms(b11, b12, b21, b22):
    return [b11 + b22, b11, b12 - b22, b21 - b11, b22, b11 + b12, b21 + b22]


def _strassen(product):
    m = product(0)
    c11, c22 = m, m
    c21 = product(3)
    c11 = c11 + c21
    c12 = product(4)
    c11 = c11 - c12
    c11 = c11 + product(6)
    m = product(2)
    c12, c22 = c12 + m, c22 + m
    m = product(1)
    c21, c22 = c21 + m, c22 - m
    c22 = c22 + product(5)
    return c11, c12, c21, c22


def _allreduce(v, op):
    r = v[0]
    for i in range(1, 8):
        r = op(r, v[i])
    r = op(r, pltpu.roll(r, 4, 0))
    return op(r, pltpu.roll(r, 2, 0))


def _features(p):
    p3 = p.reshape(8, 8, p.shape[1])
    mx = _allreduce(p3, jnp.maximum)
    mn = _allreduce(p3, jnp.minimum)
    ep = jnp.exp2(p3 - mx[None])
    en = jnp.exp2(mn[None] - p3)
    ip = _rcp(_allreduce(ep, jnp.add))
    im = _rcp(_allreduce(en, jnp.add))
    return jnp.concatenate([ep * ip[None], en * im[None]], axis=0)


def _kernel(x_hbm, wqkv_hbm, wphi_hbm, wo_hbm, wr_hbm, wg_hbm, wu_hbm, wd_hbm, out_hbm,
            x_v, xs_v, wqkv_v, ws_v, wo_v, wos_v, wg_v, wu_v, wd_v, out_v, wphi_v, wr_v, sems):
    def group(k, *pairs):
        return [pltpu.make_async_copy(src, dst, sems.at[k]) for src, dst in pairs]

    def x_rows(r0, n):
        return x_hbm.at[pl.ds(r0, n)], x_v.at[pl.ds(r0, n)]

    def w_cols(j0, nj):
        cols = pl.ds(256 * j0, 256 * nj)
        return wqkv_hbm.at[:, cols], wqkv_v.at[:, cols]

    loads = [
        group(0, x_rows(0, 256), (wr_hbm, wr_v)),
        group(1, w_cols(8, 1)),
        group(2, x_rows(256, 256)),
        group(3, w_cols(9, 1)),
        group(4, w_cols(10, 2)),
        group(5, (wphi_hbm, wphi_v), w_cols(4, 2)),
        group(6, w_cols(6, 2), x_rows(T, T)),
        group(7, x_rows(2 * T, S - 2 * T)),
        group(8, w_cols(0, 4)),
        group(9, (wo_hbm, wo_v), (wg_hbm, wg_v), (wu_hbm, wu_v), (wd_hbm, wd_v)),
    ]
    for copies in loads:
        for c in copies:
            c.start()

    def wait_loads():
        for c in loads.pop(0):
            c.wait()

    tasks = []
    pace = {}

    def after(lhs, dep):
        ok = (dep & pace["zero"]) == 0
        first = jnp.where(jnp.concatenate([ok, ok], axis=0), lhs[:16, :128], jnp.zeros((16, 128), bf16))
        if lhs.shape[1] > 128:
            first = jnp.concatenate([first, lhs[:16, 128:]], axis=1)
        return first if lhs.shape[0] == 16 else jnp.concatenate([first, lhs[16:]], axis=0)

    ffn = {"steps": None, "done": [], "y": [None, None]}

    def ffn_step():
        try:
            ffn["steps"].send(ffn["main"])
        except StopIteration:
            ffn["steps"] = None

    def matmul(lhs, rhs, dn):
        task = tasks.pop(0) if tasks else None
        dep = task() if task is not None else None
        if ffn["done"]:
            dep = ffn["done"].pop(0)
        m = _dot(lhs if dep is None else after(lhs, dep), rhs, dn)
        if ffn["steps"] is not None:
            ffn_step()
        ffn["main"] = _bits(m[-8:, -128:])
        return m

    top = [jnp.full((8, 128), -jnp.inf, f32), lax.broadcasted_iota(jnp.int32, (8, 128), 0)]
    chain = []

    def layernorm(t, g, lag):
        wr = wr_v[...].astype(f32).reshape(1, D)
        row = lax.broadcasted_iota(jnp.int32, (8, 128), 0)
        for r in range(0, 128, 16):
            halves = []
            for r0 in (T * t + 256 * g + r, T * t + 256 * g + 128 + r):
                x = x_v[pl.ds(r0, 16), :].astype(f32)
                total = x[:, :128]
                for i in range(1, D // 128):
                    total = total + x[:, 128 * i:128 * (i + 1)]
                if lag:
                    total = jnp.where(jnp.concatenate([chain[-lag]] * 2, axis=0) >= 0, total, 0.0)
                xc = x - jnp.sum(total, axis=-1, keepdims=True) * (1.0 / D)
                v = jnp.mean(xc * xc, axis=-1, keepdims=True)
                xn = xc * _rcp(_rb(jnp.sqrt(_rb(_rb(v) + _rb(jnp.full_like(v, 1e-5))))))
                halves.append(xn)
                score = jnp.broadcast_to(_rb(jnp.sum(xn * wr, axis=-1, keepdims=True)), (16, 128))
                for i in range(2):
                    sc, tok = score[8 * i:8 * i + 8], row + (r0 + 8 * i)
                    better = (sc > top[0]) | ((sc == top[0]) & (tok < top[1]))
                    top[:] = jnp.where(better, sc, top[0]), jnp.where(better, tok, top[1])
                chain.append(top[1])
            a, b = halves
            b11, b21, b12, b22 = a[:, :512], a[:, 512:], b[:, :512], b[:, 512:]
            for i, term in enumerate(_rhs_terms(b11, b12, b21, b22) + [b21, b12]):
                xs_v[t, g, i, pl.ds(r, 16), :] = term.astype(bf16)

    def xn_block(t, g, hf, kh, rows, cols):
        return xs_v[t, g, 7 - 3 * hf if kh else 1 + 7 * hf, rows, cols]

    def feature_map():
        row = lax.broadcasted_iota(jnp.int32, (128, DH), 0)
        col = lax.broadcasted_iota(jnp.int32, (128, DH), 1)
        expand = jnp.where((((row & 63) >> 4) << 3 | (row & 7)) == col, 1.0, 0.0).astype(bf16)
        full = _dot(expand, wphi_v[...], _NT)
        row = lax.broadcasted_iota(jnp.int32, (128, D), 0)
        col = lax.broadcasted_iota(jnp.int32, (128, D), 1)
        same = (((row >> 6) << 1) | ((row >> 3) & 1)) == ((col >> 5) & 3)
        return jnp.where(same, full, 0.0).astype(bf16)

    def prepare_w(j):
        blocks = []
        for c in (2 * j, 2 * j + 1):
            w = wqkv_v[:, pl.ds(128 * c, 128)]
            if j < 8:
                blocks.append(_dot(bd[:, 128 * (c % 8):128 * (c % 8 + 1)], w, _NT) * LOG2E)
            else:
                blocks.append(w.astype(f32).T)
        a, b = blocks
        for i, term in enumerate(_lhs_terms(a[:, :512], a[:, 512:], b[:, :512], b[:, 512:])):
            ws_v[j // 2, i, pl.ds(64 * (j % 2), 64), :] = _pack(term)

    def prepare_wo(n):
        for c in range(4):
            w = wo_v[pl.ds(256 * c, 256), pl.ds(256 * n, 256)].astype(f32)
            terms = _rhs_terms(w[:128, :128], w[:128, 128:], w[128:, :128], w[128:, 128:])
            for i, term in enumerate(terms):
                wos_v[n, i, pl.ds(64 * c, 64), :] = _pack(term)

    def proj_group(j0, nj, t, g):
        rows = pl.ds(64 * (j0 % 2), 64 * nj)
        return _strassen(lambda i: matmul(_unpack(ws_v[j0 // 2, i, rows, :]), xs_v[t, g, i], _NT))

    def pairs(groups):
        return [jnp.concatenate([c[2 * b + hf][r:r + 64] for c in groups for hf in range(2)], axis=1)
                for j in range(groups[0][0].shape[0] // 128) for b in range(2)
                for r in (128 * j, 128 * j + 64)]

    def proj(j0, t):
        return pairs([proj_group(j0, 2, t, g) for g in range(2)])

    kv = [None] * 16
    phi_k = [None] * 16

    def key_features(j, p):
        phi = _features(p)
        phi_k[j] = phi.reshape(128, T).astype(bf16)
        return functools.reduce(jnp.bitwise_or, [_bits(phi[i][:, n:n + 128]) for i in (7, 15)
                                                 for n in range(0, T, 128)])

    def key_tasks(blocks, j0):
        return [None] * 5 + [functools.partial(key_features, j0 + q, p) for q, p in enumerate(blocks)]

    def kv_update(v_blocks, j0):
        for j, v in enumerate(v_blocks, j0):
            v1 = jnp.concatenate([v, jnp.ones((16, T), f32)], axis=0).astype(bf16)
            upd = _dot(v1, phi_k[j], _NT)
            kv[j] = upd if kv[j] is None else kv[j] + upd

    wait_loads()
    layernorm(0, 0, 0)
    pace["zero"] = top[1] >> 31
    wait_loads()
    prepare_w(8)
    wait_loads()
    layernorm(0, 1, 0)
    first = proj_group(8, 1, 0, 0)
    wait_loads()
    v0 = pairs([first, proj_group(8, 1, 0, 1)])
    prepare_w(9)
    first = proj_group(9, 1, 0, 0)
    wait_loads()
    v0 += pairs([first, proj_group(9, 1, 0, 1)])
    for j in (10, 11):
        prepare_w(j)
    if "0" == "0":
        v0 += pairs([proj_group(10, 1, 0, g) for g in range(2)])
        first = proj_group(11, 1, 0, 0)
        wait_loads()
        v0 += pairs([first, proj_group(11, 1, 0, 1)])
    else:
        first = proj_group(10, 2, 0, 0)
        wait_loads()
        v0 += pairs([first, proj_group(10, 2, 0, 1)])
    bd = feature_map()
    for j in (4, 5):
        prepare_w(j)
    first = proj_group(4, 2, 0, 0)
    wait_loads()
    k = pairs([first, proj_group(4, 2, 0, 1)])
    for j in (6, 7):
        prepare_w(j)
    tasks += key_tasks(k, 0)
    k = proj(6, 0)
    for g in range(2):
        layernorm(1, g, 3)
    wait_loads()
    pending = [(v0[:8], 0), (v0[8:], 8)]
    j0 = 8
    for t in range(1, NT_):
        if t == NT_ - 1:
            wait_loads()
        for c in range(2):
            tasks += key_tasks(k, j0)
            v = proj(8 + 2 * c, t)
            if len(pending) > 1:
                kv_update(*pending.pop(0))
            k, j0 = proj(4 + 2 * c, t), 8 * c
            kv_update(*pending.pop(0))
            pending.append((v, j0))
            if t == NT_ - 1:
                prepare_w(2 * c)
                prepare_w(2 * c + 1)
        for g in range(2 if t + 1 < NT_ else 0):
            layernorm(t + 1, g, 1)
    tasks += key_tasks(k, j0)

    r_max = jnp.max(top[0])
    idx = jnp.clip(jnp.min(jnp.where(top[0] == r_max, top[1], S)), 0, S - 1)
    t_sel = idx // T
    grp = pl.ds(pl.multiple_of(idx % 128 // 16 * 16, 16), 16)
    x_sel = jnp.concatenate(
        [xn_block(t_sel, idx % T // 256, idx // 128 % 2, kh, grp, slice(None)) for kh in range(2)],
        axis=1).astype(f32)
    x_sel = jnp.where(lax.broadcasted_iota(jnp.int32, (16, D), 0) == idx % 16, x_sel, 0.0)
    x_sel = jnp.broadcast_to(jnp.sum(x_sel, axis=0, keepdims=True), (16, D)).astype(bf16)
    gate = jax.nn.sigmoid(jnp.full((8, D), r_max, f32))

    def ffn_program():
        def down(h, n):
            for hf in range(2):
                dep = yield
                part = _dot(after(h, dep), wd_v[pl.ds(n * 128, 128), pl.ds(hf * 512, 512)], _NN)[:8]
                ffn["y"][hf] = part if ffn["y"][hf] is None else ffn["y"][hf] + part
                ffn["done"].append(_bits(part[:, 384:]))
        h = None
        for n in range(F // 128):
            acc = []
            for w in (wg_v, wu_v):
                parts = []
                for kh in range(2):
                    dep = yield
                    parts.append(_dot(after(x_sel[:, 512 * kh:512 * (kh + 1)], dep),
                                      w[pl.ds(512 * kh, 512), pl.ds(n * 128, 128)], _NN))
                    ffn["done"].append(_bits(parts[-1][:8]))
                acc.append(parts[0] + parts[1])
            if h is not None:
                yield from down(h, n - 1)
            h = (_silu(acc[0]) * acc[1]).astype(bf16)
        yield
        ffn["done"].append(None)
        yield from down(h, F // 128 - 1)

    def attend(blocks, j0):
        terms, out = [], []
        for j, p in enumerate(blocks, j0):
            num = _dot(kv[j], _features(p).reshape(128, T).astype(bf16), _NN)
            for hd in range(2):
                inv = _rcp(num[64 + 8 * hd:72 + 8 * hd] + 1e-6)
                out.append((num[32 * hd:32 * hd + 32].reshape(4, 8, T) * inv[None]).reshape(32, T))
            if j % 4 == 3:
                ot, out = jnp.concatenate(out, axis=0), []
                terms.append([a.T for a in _lhs_terms(
                    ot[:128, :256], ot[128:, :256], ot[:128, 256:], ot[128:, 256:])])
        return terms

    stores = []

    def out_proj(i, t, o_terms, n):
        last = i == NT_ - 1
        c = _strassen(lambda k: matmul(
            jnp.concatenate([a[k] for a in o_terms], axis=1).astype(bf16), _unpack(wos_v[n, k]), _NN))
        for g in range(2):
            for nn in range(2):
                col0 = 256 * n + 128 * nn
                cols, tok = pl.ds(col0, 128), pl.ds(pl.multiple_of(T * t + 256 * g, 256), 256)
                a = jnp.concatenate(
                    [xn_block(t, g, hf, col0 // 512, slice(None), pl.ds(col0 % 512, 128))
                     for hf in range(2)], axis=0).astype(f32)
                if last:
                    hit = (lax.broadcasted_iota(jnp.int32, (32, 8, 128), 0) * 8
                           + lax.broadcasted_iota(jnp.int32, (32, 8, 128), 1)) == idx % T - 256 * g
                    a3 = a.reshape(32, 8, 128)
                    a = jnp.where(hit, a3 + ffn["y"][:, col0:col0 + 128][None], a3).reshape(256, 128)
                rows = pl.ds(T * i + 256 * g, 256)
                out_v[rows, cols] = (x_v[tok, cols].astype(f32) + c[2 * g + nn] * _silu(a)).astype(bf16)
                if last and n == 3:
                    stores.extend(group(10, (out_v.at[rows, cols], out_hbm.at[tok, cols])))
                    stores[-1].start()
        if last != (n == 3):
            cols = pl.ds(256 * n, 256) if last else slice(None)
            stores.extend(group(10, (out_v.at[pl.ds(T * i, T), cols],
                                    out_hbm.at[pl.ds(pl.multiple_of(T * t, T), T), cols])))
            stores[-1].start()

    tiles = [lax.rem(t_sel + 1 + i, NT_) for i in range(NT_)]
    o_terms = [[] for _ in range(NT_)]
    halves = [(i, c) for i in range(NT_) for c in range(2)]

    def out_half(h):
        i, c = halves[h]
        for n in (2 * c, 2 * c + 1):
            out_proj(i, tiles[i], o_terms[i], n)

    for h, (i, c) in enumerate(halves):
        q = proj(2 * c, tiles[i])
        if h == 0:
            kv_update(*pending.pop(0))
            row = lax.broadcasted_iota(jnp.int32, (80, 128), 0)
            col = lax.broadcasted_iota(jnp.int32, (80, 128), 1)
            own = jnp.where(row < 64, row >> 5, (row >> 3) & 1) == (col & 1)
            kv[:] = [jnp.where(own, a, 0.0).astype(bf16) for a in kv]
            wait_loads()
            for n in range(4):
                prepare_wo(n)
            ffn["steps"], ffn["done"] = ffn_program(), [None, None]
            next(ffn["steps"])
        else:
            o_terms[halves[h - 1][0]] += attend(prev_q, 8 * halves[h - 1][1])
        prev_q = q
        if h >= 3:
            out_half(h - 3)
    o_terms[-1] += attend(prev_q, 8)
    out_half(len(halves) - 3)
    while ffn["steps"] is not None:
        ffn_step()
    ffn["y"] = _rb(jnp.concatenate(ffn["y"], axis=1) * gate)
    out_half(len(halves) - 2)
    out_half(len(halves) - 1)
    for c in stores:
        c.wait()


@jax.jit
def pallas_recurrent_scan__linear_kernel_hedgehog__moe_arch_mod__prompt_kernel(
    A_x: jax.Array,
    A_wqkv: jax.Array,
    A_w_phi: jax.Array,
    A_wo: jax.Array,
    B_x: jax.Array,
    B_w_r: jax.Array,
    B_w_gate: jax.Array,
    B_w_up: jax.Array,
    B_w_down: jax.Array,
):
    del B_x
    hbm = pl.BlockSpec(memory_space=pl.ANY)
    out = pl.pallas_call(
        _kernel,
        out_shape=jax.ShapeDtypeStruct((S, D), bf16),
        in_specs=[hbm] * 8,
        out_specs=hbm,
        scratch_shapes=[
            pltpu.VMEM((S, D), bf16),
            pltpu.VMEM((NT_, 2, 9, 128, 512), bf16),
            pltpu.VMEM((D, 3 * D), bf16),
            pltpu.VMEM((6, 7, 128, 512), jnp.uint32),
            pltpu.VMEM((D, D), bf16),
            pltpu.VMEM((4, 7, 256, 128), jnp.uint32),
            pltpu.VMEM((D, F), bf16),
            pltpu.VMEM((D, F), bf16),
            pltpu.VMEM((F, D), bf16),
            pltpu.VMEM((S, D), bf16),
            pltpu.VMEM((H * DH, DH), bf16),
            pltpu.VMEM((D,), bf16),
            pltpu.SemaphoreType.DMA((11,)),
        ],
        compiler_params=pltpu.CompilerParams(vmem_limit_bytes=110 * 1024 * 1024),
        name="hedgehog_mod",
    )(
        A_x.reshape(S, D), A_wqkv, A_w_phi.reshape(H * DH, DH), A_wo,
        B_w_r, B_w_gate, B_w_up, B_w_down,
    )
    return out.reshape(1, S, D)
```

```python
import functools
import math

import jax
import jax.numpy as jnp
from jax import lax
import jax.experimental.pallas as pl
import jax.experimental.pallas.tpu as pltpu

S, D, H, DH, F = 2048, 1024, 32, 32, 3584
T = 512
NT_ = S // T
LOG2E = math.log2(math.e)
_NT = (((1,), (1,)), ((), ()))
_NN = (((1,), (0,)), ((), ()))
f32, bf16 = jnp.float32, jnp.bfloat16


def _dot(a, b, dn):
    return lax.dot_general(a, b, dn, preferred_element_type=f32)


def _rb(v):
    return v.astype(bf16).astype(f32)


def _rcp(v):
    r = pl.reciprocal(v, approx=True)
    return r * (2.0 - v * r)


def _silu(a):
    return a * pl.reciprocal(1.0 + jnp.exp2(a * -LOG2E), approx=True)


def _bits(v):
    return pltpu.bitcast(v, jnp.int32)


def _pack(v):
    m, n = v.shape
    v = v.reshape(m // 16, 2, 8, n)
    return pltpu.pack_elementwise([v[:, 0], v[:, 1]], packed_dtype=bf16).reshape(m // 2, n)


def _unpack(words):
    return pltpu.bitcast(words, bf16)


def _lhs_terms(a11, a12, a21, a22):
    return [a11 + a22, a21 + a22, a11, a22, a11 + a12, a21 - a11, a12 - a22]


def _rhs_terms(b11, b12, b21, b22):
    return [b11 + b22, b11, b12 - b22, b21 - b11, b22, b11 + b12, b21 + b22]


def _strassen(product):
    m = product(0)
    c11, c22 = m, m
    c21 = product(3)
    c11 = c11 + c21
    c12 = product(4)
    c11 = c11 - c12
    c11 = c11 + product(6)
    m = product(2)
    c12, c22 = c12 + m, c22 + m
    m = product(1)
    c21, c22 = c21 + m, c22 - m
    c22 = c22 + product(5)
    return c11, c12, c21, c22


_HK_TERMS = (
    ((1,), (1, -2)), ((1, 2), (2,)), ((3, 4), (3,)), ((-4,), (3, -4)),
    ((1, 4), (2, 3)), ((-1, 3), (1, 3)), ((2, -4), (2, 4)),
    ((6,), (6,)), ((5,), (5,)),
    ((-3, -4, 5), (3, -4, -6)), ((-3, -4, 5, 6), (4, 6)), ((3, -5), (3, -4, 5, -6)),
    ((1, 2, -6), (1, -2, 5)), ((-2, 6), (1, -2, 5, -6)), ((-1, -2, 5, 6), (1, 5)),
    ((7,), (7, -8)), ((7, 8), (8,)),
    ((4, 7), (3, 8)), ((3, -7), (3, 7)), ((-4, 8), (4, 8)),
    ((-6, 7, 8), (5, 7, -8)), ((6, -8), (5, -6, 7, -8)), ((5, 6, -7, -8), (5, 7)),
    ((2, -6, 7), (1, 5, 8)), ((1, -5, -7), (1, 5, 7)), ((-2, 6, 8), (2, 6, 8)),
)
_HK_SUMS = (
    ((0, 0), (2, 1)), ((1, 1), (4, 3)), ((1, 0), (6, 5, 1, -3)), ((0, 1), (7, 5, 4, -2)),
    ((2, 2), (9, 8)), ((2, 1), (11, 10, 3, -8)), ((1, 2), (12, 10, 9, -4)),
    ((0, 2), (14, 13, 8, -1)), ((2, 0), (15, 13, 2, -9)), ((3, 3), (17, 16)),
    ((1, 3), (19, 18, 16, -3)), ((3, 1), (20, 18, 4, -17)),
    ((3, 2), (22, 21, 8, -16)), ((2, 3), (23, 21, 17, -9)),
    ((0, 3), (25, 24, 16, 15), (2, 3), 1), ((3, 0), (26, 24, 14, -17), (3, 2), -1),
)


def _signed_sums(wanted, blocks):
    known = {(i + 1,): b for i, b in enumerate(blocks)}

    def value(key):
        if key not in known:
            for part in sorted(known, key=len, reverse=True):
                for sign in (1, -1):
                    signed = [sign * p for p in part]
                    if key not in known and len(part) < len(key) and all(p in key for p in signed):
                        rest = tuple(k for k in key if k not in signed)
                        if sign > 0 and rest[0] < 0:
                            known[key] = known[part] - value(tuple(-k for k in rest))
                        else:
                            known[key] = value(rest) + known[part] if sign > 0 else value(rest) - known[part]
            if key not in known:
                known[key] = -known[(-key[0],)]
        return known[key]

    for key in sorted(wanted, key=len):
        value(key)
    return [known[key] for key in wanted]


def _hopcroft_kerr(product):
    m = [product(r) for r in range(len(_HK_TERMS))]
    y = {}
    for ij, parts, *earlier in _HK_SUMS:
        total = m[parts[0] - 1]
        for p in parts[1:]:
            total = total + m[p - 1] if p > 0 else total - m[-p - 1]
        if earlier:
            total = total + y[earlier[0]] if earlier[1] > 0 else total - y[earlier[0]]
        y[ij] = total
    return y


def _allreduce(v, op):
    r = v[0]
    for i in range(1, 8):
        r = op(r, v[i])
    r = op(r, pltpu.roll(r, 4, 0))
    return op(r, pltpu.roll(r, 2, 0))


def _features(p):
    p3 = p.reshape(8, 8, p.shape[1])
    mx = _allreduce(p3, jnp.maximum)
    mn = _allreduce(p3, jnp.minimum)
    ep = jnp.exp2(p3 - mx[None])
    en = jnp.exp2(mn[None] - p3)
    ip = _rcp(_allreduce(ep, jnp.add))
    im = _rcp(_allreduce(en, jnp.add))
    return jnp.concatenate([ep * ip[None], en * im[None]], axis=0)


def _kernel(x_hbm, wqkv_hbm, wphi_hbm, wo_hbm, wr_hbm, wg_hbm, wu_hbm, wd_hbm, out_hbm,
            x_v, xs_v, wqkv_v, ws_v, wo_v, woh_v, wg_v, wu_v, wd_v, out_v, wphi_v, wr_v, sems):
    def group(k, *pairs):
        return [pltpu.make_async_copy(src, dst, sems.at[k]) for src, dst in pairs]

    def x_rows(r0, n):
        return x_hbm.at[pl.ds(r0, n)], x_v.at[pl.ds(r0, n)]

    def w_cols(j0, nj):
        cols = pl.ds(256 * j0, 256 * nj)
        return wqkv_hbm.at[:, cols], wqkv_v.at[:, cols]

    loads = [
        group(0, x_rows(0, 256), (wr_hbm, wr_v)),
        group(1, w_cols(8, 1)),
        group(2, x_rows(256, 256)),
        group(3, w_cols(9, 1)),
        group(4, w_cols(10, 2)),
        group(5, (wphi_hbm, wphi_v), w_cols(4, 2)),
        group(6, w_cols(6, 2), x_rows(T, T)),
        group(7, x_rows(2 * T, S - 2 * T)),
        group(8, w_cols(0, 4)),
        group(9, (wo_hbm, wo_v), (wg_hbm, wg_v), (wu_hbm, wu_v), (wd_hbm, wd_v)),
    ]
    for copies in loads:
        for c in copies:
            c.start()

    def wait_loads():
        for c in loads.pop(0):
            c.wait()

    tasks = []
    pace = {}

    def after(lhs, dep):
        ok = (dep & pace["zero"]) == 0
        first = jnp.where(jnp.concatenate([ok, ok], axis=0), lhs[:16, :128], jnp.zeros((16, 128), bf16))
        if lhs.shape[1] > 128:
            first = jnp.concatenate([first, lhs[:16, 128:]], axis=1)
        return first if lhs.shape[0] == 16 else jnp.concatenate([first, lhs[16:]], axis=0)

    ffn = {"steps": None, "done": [], "y": [None, None]}

    def ffn_step():
        try:
            ffn["steps"].send(ffn["main"])
        except StopIteration:
            ffn["steps"] = None

    def matmul(lhs, rhs, dn):
        task = tasks.pop(0) if tasks else None
        dep = task() if task is not None else None
        if ffn["done"]:
            dep = ffn["done"].pop(0)
        m = _dot(lhs if dep is None else after(lhs, dep), rhs, dn)
        if ffn["steps"] is not None:
            ffn_step()
        ffn["main"] = _bits(m[-8:, -128:])
        return m

    top = [jnp.full((8, 128), -jnp.inf, f32), lax.broadcasted_iota(jnp.int32, (8, 128), 0)]
    chain = []

    def layernorm(t, g, lag):
        wr = wr_v[...].astype(f32).reshape(1, D)
        row = 2 * lax.broadcasted_iota(jnp.int32, (8, 128), 0)
        for r in range(0, 128, 16):
            xn = []
            for r0 in (T * t + 256 * g + r, T * t + 256 * g + 128 + r):
                words = pltpu.bitcast(x_v[pl.ds(r0, 16), :], jnp.uint32)
                for odd in range(2):
                    x = pltpu.unpack_elementwise(words, index=odd, packed_dtype=bf16, unpacked_dtype=f32)
                    total = x[:, :128]
                    for i in range(1, D // 128):
                        total = total + x[:, 128 * i:128 * (i + 1)]
                    if lag:
                        total = jnp.where(chain[-lag] >= 0, total, 0.0)
                    xc = x - jnp.sum(total, axis=-1, keepdims=True) * (1.0 / D)
                    v = jnp.mean(xc * xc, axis=-1, keepdims=True)
                    xn.append(xc * _rcp(_rb(jnp.sqrt(_rb(_rb(v) + _rb(jnp.full_like(v, 1e-5)))))))
                    sc = jnp.broadcast_to(_rb(jnp.sum(xn[-1] * wr, axis=-1, keepdims=True)), (8, 128))
                    tok = row + (r0 + odd)
                    better = (sc > top[0]) | ((sc == top[0]) & (tok < top[1]))
                    top[:] = jnp.where(better, sc, top[0]), jnp.where(better, tok, top[1])
                chain.append(top[1])
            terms = [_rhs_terms(a[:, :512], b[:, :512], a[:, 512:], b[:, 512:]) + [a[:, 512:], b[:, :512]]
                     for a, b in ((xn[0], xn[2]), (xn[1], xn[3]))]
            for i, pair in enumerate(zip(*terms)):
                xs_v[t, g, i, pl.ds(r // 2, 8), :] = pltpu.pack_elementwise(list(pair), packed_dtype=bf16)

    def xn_block(t, g, hf, kh, rows, cols):
        return _unpack(xs_v[t, g, 7 - 3 * hf if kh else 1 + 7 * hf, rows, cols])

    def feature_map():
        row = lax.broadcasted_iota(jnp.int32, (128, DH), 0)
        col = lax.broadcasted_iota(jnp.int32, (128, DH), 1)
        expand = jnp.where((((row & 63) >> 4) << 3 | (row & 7)) == col, 1.0, 0.0).astype(bf16)
        full = _dot(expand, wphi_v[...], _NT)
        row = lax.broadcasted_iota(jnp.int32, (128, D), 0)
        col = lax.broadcasted_iota(jnp.int32, (128, D), 1)
        same = (((row >> 6) << 1) | ((row >> 3) & 1)) == ((col >> 5) & 3)
        return jnp.where(same, full, 0.0).astype(bf16)

    def prepare_w(j):
        blocks = []
        for c in (2 * j, 2 * j + 1):
            w = wqkv_v[:, pl.ds(128 * c, 128)]
            if j < 8:
                blocks.append(_dot(bd[:, 128 * (c % 8):128 * (c % 8 + 1)], w, _NT) * LOG2E)
            else:
                blocks.append(w.astype(f32).T)
        a, b = blocks
        for i, term in enumerate(_lhs_terms(a[:, :512], a[:, 512:], b[:, :512], b[:, 512:])):
            ws_v[j // 2, i, pl.ds(64 * (j % 2), 64), :] = _pack(term)

    def paced_terms(pieces, lag):
        links = []
        for blocks, dest in pieces:
            if len(links) >= lag:
                link = jnp.concatenate([links[-lag]] * (blocks[0].shape[1] // 128), axis=1)
                blocks = [pltpu.bitcast(_bits(b) ^ jnp.concatenate([link, link], axis=0), f32)
                          for b in blocks[:1]] + blocks[1:]
            words = [_pack(term) for term in _signed_sums([t[0] for t in _HK_TERMS], blocks)]
            for i, w in enumerate(words):
                dest[i] = w
            done = functools.reduce(jnp.bitwise_or, words[4:7] + words[9:15] + words[17:])
            slow = jnp.sum(pltpu.bitcast(done, f32), axis=-1, keepdims=True)
            links.append(_bits(jnp.broadcast_to(slow, (8, 128))) & pace["zero"])

    def prepare_wo(lag):
        pieces = []
        for n in range(2):
            for c in range(4):
                for r in range(0, 128, 16):
                    w = [wo_v[pl.ds(256 * c + 128 * kh + r, 16), pl.ds(512 * n, 512)].astype(f32) for kh in range(2)]
                    pieces.append(([w[kh][:, 128 * i:128 * (i + 1)] for i in range(4) for kh in range(2)],
                                   woh_v.at[n, :, pl.ds(64 * c + r // 2, 8), :]))
        paced_terms(pieces, lag)

    def proj_group(j0, nj, t, g):
        rows = pl.ds(64 * (j0 % 2), 64 * nj)
        return _strassen(lambda i: matmul(_unpack(ws_v[j0 // 2, i, rows, :]), _unpack(xs_v[t, g, i]), _NT))

    def pairs(groups):
        return [jnp.concatenate([c[2 * b + hf][r:r + 64] for c in groups for hf in range(2)], axis=1)
                for j in range(groups[0][0].shape[0] // 128) for b in range(2)
                for r in (128 * j, 128 * j + 64)]

    def proj(j0, t):
        return pairs([proj_group(j0, 2, t, g) for g in range(2)])

    kv = [None] * 16
    phi_k = [None] * 16

    def key_features(j, p):
        phi = _features(p)
        phi_k[j] = phi.reshape(128, T).astype(bf16)
        return functools.reduce(jnp.bitwise_or, [_bits(phi[i][:, n:n + 128]) for i in (7, 15)
                                                 for n in range(0, T, 128)])

    def key_tasks(blocks, j0):
        return [None] * 5 + [functools.partial(key_features, j0 + q, p) for q, p in enumerate(blocks)]

    def kv_update(v_blocks, j0):
        for j, v in enumerate(v_blocks, j0):
            v1 = jnp.concatenate([v, jnp.ones((16, T), f32)], axis=0).astype(bf16)
            upd = _dot(v1, phi_k[j], _NT)
            kv[j] = upd if kv[j] is None else kv[j] + upd

    wait_loads()
    layernorm(0, 0, 0)
    pace["zero"] = top[1] >> 31
    wait_loads()
    prepare_w(8)
    wait_loads()
    layernorm(0, 1, 0)
    first = proj_group(8, 1, 0, 0)
    wait_loads()
    v0 = pairs([first, proj_group(8, 1, 0, 1)])
    prepare_w(9)
    first = proj_group(9, 1, 0, 0)
    wait_loads()
    v0 += pairs([first, proj_group(9, 1, 0, 1)])
    for j in (10, 11):
        prepare_w(j)
    if "0" == "0":
        v0 += pairs([proj_group(10, 1, 0, g) for g in range(2)])
        first = proj_group(11, 1, 0, 0)
        wait_loads()
        v0 += pairs([first, proj_group(11, 1, 0, 1)])
    else:
        first = proj_group(10, 2, 0, 0)
        wait_loads()
        v0 += pairs([first, proj_group(10, 2, 0, 1)])
    bd = feature_map()
    for j in (4, 5):
        prepare_w(j)
    first = proj_group(4, 2, 0, 0)
    wait_loads()
    k = pairs([first, proj_group(4, 2, 0, 1)])
    for j in (6, 7):
        prepare_w(j)
    tasks += key_tasks(k, 0)
    k = proj(6, 0)
    for g in range(2):
        layernorm(1, g, 3)
    wait_loads()
    pending = [(v0[:8], 0), (v0[8:], 8)]
    j0 = 8
    for t in range(1, NT_):
        if t == NT_ - 1:
            wait_loads()
        for c in range(2):
            tasks += key_tasks(k, j0)
            v = proj(8 + 2 * c, t)
            if len(pending) > 1:
                kv_update(*pending.pop(0))
            k, j0 = proj(4 + 2 * c, t), 8 * c
            kv_update(*pending.pop(0))
            pending.append((v, j0))
            if t == NT_ - 1:
                prepare_w(2 * c)
                prepare_w(2 * c + 1)
        for g in range(2 if t + 1 < NT_ else 0):
            layernorm(t + 1, g, 1)
    tasks += key_tasks(k, j0)

    r_max = jnp.max(top[0])
    idx = jnp.clip(jnp.min(jnp.where(top[0] == r_max, top[1], S)), 0, S - 1)
    t_sel = idx // T
    grp = pl.ds(pl.multiple_of(idx % 128 // 16 * 8, 8), 8)
    x_sel = jnp.concatenate(
        [xn_block(t_sel, idx % T // 256, idx // 128 % 2, kh, grp, slice(None)) for kh in range(2)],
        axis=1).astype(f32)
    x_sel = jnp.where(lax.broadcasted_iota(jnp.int32, (16, D), 0) == idx % 16, x_sel, 0.0)
    x_sel = jnp.broadcast_to(jnp.sum(x_sel, axis=0, keepdims=True), (16, D)).astype(bf16)
    gate = jax.nn.sigmoid(jnp.full((8, 512), r_max, f32))

    def ffn_program():
        h = []
        for n in range(F // 128):
            acc = []
            for w in (wg_v, wu_v):
                parts = []
                for kh in range(2):
                    dep = yield
                    parts.append(_dot(after(x_sel[:, 512 * kh:512 * (kh + 1)], dep),
                                      w[pl.ds(512 * kh, 512), pl.ds(n * 128, 128)], _NN))
                    ffn["done"].append(_bits(parts[-1][:8]))
                acc.append(parts[0] + parts[1])
            h.append((_silu(acc[0]) * acc[1]).astype(bf16))
        for hf in range(2):
            y = None
            for n in range(F // 128):
                dep = yield
                part = _dot(after(h[n], dep), wd_v[pl.ds(n * 128, 128), pl.ds(hf * 512, 512)], _NN)[:8]
                y = part if y is None else y + part
                ffn["done"].append(_bits(part[:, 384:]))
            ffn["y"][hf] = _rb(y * gate)

    def attend(blocks, j0):
        out = []
        for j, p in enumerate(blocks, j0):
            num = _dot(kv[j], _features(p).reshape(128, T).astype(bf16), _NN)
            for hd in range(2):
                inv = _rcp(num[64 + 8 * hd:72 + 8 * hd] + 1e-6)
                out.append((num[32 * hd:32 * hd + 32].reshape(4, 8, T) * inv[None]).reshape(32, T))
        return [[[jnp.concatenate(out[8 * c + 4 * kh:8 * c + 4 * kh + 4], axis=0)[:, 256 * g:256 * (g + 1)].T
                  for kh in range(2)] for g in range(2)] for c in range(2)]

    stores = []

    def out_proj(i, o_terms, n):
        s = _hopcroft_kerr(lambda r: matmul(o_terms[r], _unpack(woh_v[n, r]), _NN))
        while i and ffn["y"][n] is None:
            ffn_step()
        for (c, q), block in s.items():
            t, g = tiles[i + q // 2], q % 2
            cols, tok = pl.ds(512 * n + 128 * c, 128), pl.ds(pl.multiple_of(T * t + 256 * g, 256), 256)
            a = jnp.concatenate([xn_block(t, g, hf, n, slice(None), pl.ds(128 * c, 128))
                                 for hf in range(2)], axis=0).astype(f32)
            if i + q // 2 == NT_ - 1:
                hit = (lax.broadcasted_iota(jnp.int32, (32, 8, 128), 0) * 8
                       + lax.broadcasted_iota(jnp.int32, (32, 8, 128), 1)) == idx % T - 256 * g
                a3 = a.reshape(32, 8, 128)
                a = jnp.where(hit, a3 + ffn["y"][n][:, 128 * c:128 * (c + 1)][None], a3).reshape(256, 128)
            rows = pl.ds(T * i + 256 * q, 256)
            out_v[rows, cols] = (x_v[tok, cols].astype(f32) + block * _silu(a)).astype(bf16)
            if i and n:
                stores.extend(group(10, (out_v.at[rows, cols], out_hbm.at[tok, cols])))
                stores[-1].start()
        if (i, n) in ((0, 1), (2, 0)):
            cols = pl.ds(0, 512) if i else slice(None)
            for q in range(2):
                stores.extend(group(10, (out_v.at[pl.ds(T * (i + q), T), cols],
                                         out_hbm.at[pl.ds(pl.multiple_of(T * tiles[i + q], T), T), cols])))
                stores[-1].start()

    def output_terms(first, second):
        per_group = [_signed_sums([t[1] for t in _HK_TERMS],
                                  [b for o in (first, second) for g in range(2) for b in o[c][g]])
                     for c in range(4)]
        return [jnp.concatenate(term, axis=1).astype(bf16) for term in zip(*per_group)]

    tiles = [lax.rem(t_sel + 1 + i, NT_) for i in range(NT_)]
    o = [[] for _ in range(NT_)]
    halves = [(i, c) for i in range(NT_) for c in range(2)]
    for h, (i, c) in enumerate(halves):
        q = proj(2 * c, tiles[i])
        if h == 0:
            kv_update(*pending.pop(0))
            row = lax.broadcasted_iota(jnp.int32, (80, 128), 0)
            col = lax.broadcasted_iota(jnp.int32, (80, 128), 1)
            own = jnp.where(row < 64, row >> 5, (row >> 3) & 1) == (col & 1)
            kv[:] = [jnp.where(own, a, 0.0).astype(bf16) for a in kv]
            wait_loads()
            prepare_wo(1)
            ffn["steps"], ffn["done"] = ffn_program(), [None, None]
            next(ffn["steps"])
        else:
            o[halves[h - 1][0]] += attend(prev, 8 * halves[h - 1][1])
        prev = q
        if h == 6:
            terms = output_terms(*o[:2])
            out_proj(0, terms, 0)
    out_proj(0, terms, 1)
    o[-1] += attend(prev, 8)
    terms = output_terms(*o[2:])
    for n in range(2):
        out_proj(2, terms, n)
    for c in stores:
        c.wait()


@jax.jit
def pallas_recurrent_scan__linear_kernel_hedgehog__moe_arch_mod__prompt_kernel(
    A_x: jax.Array,
    A_wqkv: jax.Array,
    A_w_phi: jax.Array,
    A_wo: jax.Array,
    B_x: jax.Array,
    B_w_r: jax.Array,
    B_w_gate: jax.Array,
    B_w_up: jax.Array,
    B_w_down: jax.Array,
):
    del B_x
    hbm = pl.BlockSpec(memory_space=pl.ANY)
    out = pl.pallas_call(
        _kernel,
        out_shape=jax.ShapeDtypeStruct((S, D), bf16),
        in_specs=[hbm] * 8,
        out_specs=hbm,
        scratch_shapes=[
            pltpu.VMEM((S, D), bf16),
            pltpu.VMEM((NT_, 2, 9, 64, 512), jnp.uint32),
            pltpu.VMEM((D, 3 * D), bf16),
            pltpu.VMEM((6, 7, 128, 512), jnp.uint32),
            pltpu.VMEM((D, D), bf16),
            pltpu.VMEM((2, 26, 256, 128), jnp.uint32),
            pltpu.VMEM((D, F), bf16),
            pltpu.VMEM((D, F), bf16),
            pltpu.VMEM((F, D), bf16),
            pltpu.VMEM((S, D), bf16),
            pltpu.VMEM((H * DH, DH), bf16),
            pltpu.VMEM((D,), bf16),
            pltpu.SemaphoreType.DMA((11,)),
        ],
        compiler_params=pltpu.CompilerParams(vmem_limit_bytes=110 * 1024 * 1024),
        name="hedgehog_mod",
    )(
        A_x.reshape(S, D), A_wqkv, A_w_phi.reshape(H * DH, DH), A_wo,
        B_w_r, B_w_gate, B_w_up, B_w_down,
    )
    return out.reshape(1, S, D)
```

```python
import functools
import math

import jax
import jax.numpy as jnp
from jax import lax
import jax.experimental.pallas as pl
import jax.experimental.pallas.tpu as pltpu

S, D, H, DH, F = 2048, 1024, 32, 32, 3584
T = 512
NT_ = S // T
LOG2E = math.log2(math.e)
_NT = (((1,), (1,)), ((), ()))
_NN = (((1,), (0,)), ((), ()))
f32, bf16 = jnp.float32, jnp.bfloat16


def _dot(a, b, dn):
    return lax.dot_general(a, b, dn, preferred_element_type=f32)


def _rb(v):
    return v.astype(bf16).astype(f32)


def _rcp(v):
    r = pl.reciprocal(v, approx=True)
    return r * (2.0 - v * r)


def _silu(a):
    return a * pl.reciprocal(1.0 + jnp.exp2(a * -LOG2E), approx=True)


def _bits(v):
    return pltpu.bitcast(v, jnp.int32)


def _pack(v):
    m, n = v.shape
    v = v.reshape(m // 16, 2, 8, n)
    return pltpu.pack_elementwise([v[:, 0], v[:, 1]], packed_dtype=bf16).reshape(m // 2, n)


def _unpack(words):
    return pltpu.bitcast(words, bf16)


def _lhs_terms(a11, a12, a21, a22):
    return [a11 + a22, a21 + a22, a11, a22, a11 + a12, a21 - a11, a12 - a22]


def _rhs_terms(b11, b12, b21, b22):
    return [b11 + b22, b11, b12 - b22, b21 - b11, b22, b11 + b12, b21 + b22]


def _strassen(product):
    m = product(0)
    c11, c22 = m, m
    c21 = product(3)
    c11 = c11 + c21
    c12 = product(4)
    c11 = c11 - c12
    c11 = c11 + product(6)
    m = product(2)
    c12, c22 = c12 + m, c22 + m
    m = product(1)
    c21, c22 = c21 + m, c22 - m
    c22 = c22 + product(5)
    return c11, c12, c21, c22


_HK_TERMS = (
    ((1,), (1, -2)), ((1, 2), (2,)), ((3, 4), (3,)), ((-4,), (3, -4)),
    ((1, 4), (2, 3)), ((-1, 3), (1, 3)), ((2, -4), (2, 4)),
    ((6,), (6,)), ((5,), (5,)),
    ((-3, -4, 5), (3, -4, -6)), ((-3, -4, 5, 6), (4, 6)), ((3, -5), (3, -4, 5, -6)),
    ((1, 2, -6), (1, -2, 5)), ((-2, 6), (1, -2, 5, -6)), ((-1, -2, 5, 6), (1, 5)),
    ((7,), (7, -8)), ((7, 8), (8,)),
    ((4, 7), (3, 8)), ((3, -7), (3, 7)), ((-4, 8), (4, 8)),
    ((-6, 7, 8), (5, 7, -8)), ((6, -8), (5, -6, 7, -8)), ((5, 6, -7, -8), (5, 7)),
    ((2, -6, 7), (1, 5, 8)), ((1, -5, -7), (1, 5, 7)), ((-2, 6, 8), (2, 6, 8)),
)
_HK_SUMS = (
    ((0, 0), (2, 1)), ((1, 1), (4, 3)), ((1, 0), (6, 5, 1, -3)), ((0, 1), (7, 5, 4, -2)),
    ((2, 2), (9, 8)), ((2, 1), (11, 10, 3, -8)), ((1, 2), (12, 10, 9, -4)),
    ((0, 2), (14, 13, 8, -1)), ((2, 0), (15, 13, 2, -9)), ((3, 3), (17, 16)),
    ((1, 3), (19, 18, 16, -3)), ((3, 1), (20, 18, 4, -17)),
    ((3, 2), (22, 21, 8, -16)), ((2, 3), (23, 21, 17, -9)),
    ((0, 3), (25, 24, 16, 15), (2, 3), 1), ((3, 0), (26, 24, 14, -17), (3, 2), -1),
)


def _signed_sums(wanted, blocks):
    known = {(i + 1,): b for i, b in enumerate(blocks)}

    def value(key):
        if key not in known:
            for part in sorted(known, key=len, reverse=True):
                for sign in (1, -1):
                    signed = [sign * p for p in part]
                    if key not in known and len(part) < len(key) and all(p in key for p in signed):
                        rest = tuple(k for k in key if k not in signed)
                        if sign > 0 and rest[0] < 0:
                            known[key] = known[part] - value(tuple(-k for k in rest))
                        else:
                            known[key] = value(rest) + known[part] if sign > 0 else value(rest) - known[part]
            if key not in known:
                known[key] = -known[(-key[0],)]
        return known[key]

    for key in sorted(wanted, key=len):
        value(key)
    return [known[key] for key in wanted]


def _hopcroft_kerr(product):
    m, y = [], {}
    for ij, parts, *earlier in _HK_SUMS:
        while len(m) < parts[0]:
            m.append(product(len(m)))
        total = m[parts[0] - 1]
        for p in parts[1:]:
            total = total + m[p - 1] if p > 0 else total - m[-p - 1]
        if earlier:
            total = total + y[earlier[0]] if earlier[1] > 0 else total - y[earlier[0]]
        y[ij] = total
        yield ij, total


def _allreduce(v, op):
    r = v[0]
    for i in range(1, 8):
        r = op(r, v[i])
    r = op(r, pltpu.roll(r, 4, 0))
    return op(r, pltpu.roll(r, 2, 0))


def _features(p):
    p3 = p.reshape(8, 8, p.shape[1])
    mx = _allreduce(p3, jnp.maximum)
    mn = _allreduce(p3, jnp.minimum)
    ep = jnp.exp2(p3 - mx[None])
    en = jnp.exp2(mn[None] - p3)
    ip = _rcp(_allreduce(ep, jnp.add))
    im = _rcp(_allreduce(en, jnp.add))
    return jnp.concatenate([ep * ip[None], en * im[None]], axis=0)


def _kernel(x_hbm, wqkv_hbm, wphi_hbm, wo_hbm, wr_hbm, wg_hbm, wu_hbm, wd_hbm, out_hbm,
            x_v, xs_v, wqkv_v, ws_v, wo_v, woh_v, wg_v, wu_v, wd_v, out_v, wphi_v, wr_v, sems):
    def group(k, *pairs):
        return [pltpu.make_async_copy(src, dst, sems.at[k]) for src, dst in pairs]

    def x_rows(r0, n):
        return x_hbm.at[pl.ds(r0, n)], x_v.at[pl.ds(r0, n)]

    def w_cols(j0, nj):
        cols = pl.ds(256 * j0, 256 * nj)
        return wqkv_hbm.at[:, cols], wqkv_v.at[:, cols]

    loads = [
        group(0, x_rows(0, 256), (wr_hbm, wr_v)),
        group(1, w_cols(8, 1)),
        group(2, x_rows(256, 256)),
        group(3, w_cols(9, 1)),
        group(4, w_cols(10, 2)),
        group(5, (wphi_hbm, wphi_v), w_cols(4, 2)),
        group(6, w_cols(6, 2), x_rows(T, T)),
        group(7, x_rows(2 * T, S - 2 * T)),
        group(8, w_cols(0, 4)),
        group(9, (wo_hbm, wo_v), (wg_hbm, wg_v), (wu_hbm, wu_v), (wd_hbm, wd_v)),
    ]
    for copies in loads:
        for c in copies:
            c.start()

    def wait_loads():
        for c in loads.pop(0):
            c.wait()

    tasks = []
    pace = {}

    def after(lhs, dep):
        ok = (dep & pace["zero"]) == 0
        first = jnp.where(jnp.concatenate([ok, ok], axis=0), lhs[:16, :128], jnp.zeros((16, 128), bf16))
        if lhs.shape[1] > 128:
            first = jnp.concatenate([first, lhs[:16, 128:]], axis=1)
        return first if lhs.shape[0] == 16 else jnp.concatenate([first, lhs[16:]], axis=0)

    ffn = {"steps": None, "done": [], "y": [None, None]}

    def ffn_step():
        try:
            ffn["steps"].send(ffn["main"])
        except StopIteration:
            ffn["steps"] = None

    def matmul(lhs, rhs, dn):
        task = tasks.pop(0) if tasks else None
        dep = task() if task is not None else None
        if ffn["done"]:
            dep = ffn["done"].pop(0)
        m = _dot(lhs if dep is None else after(lhs, dep), rhs, dn)
        if ffn["steps"] is not None:
            ffn_step()
        ffn["main"] = _bits(m[-8:, -128:])
        return m

    top = [jnp.full((8, 128), -jnp.inf, f32), lax.broadcasted_iota(jnp.int32, (8, 128), 0)]
    chain = []

    def layernorm(t, g, lag):
        wr = wr_v[...].astype(f32).reshape(1, D)
        row = 2 * lax.broadcasted_iota(jnp.int32, (8, 128), 0)
        for r in range(0, 128, 16):
            xn = []
            for r0 in (T * t + 256 * g + r, T * t + 256 * g + 128 + r):
                words = pltpu.bitcast(x_v[pl.ds(r0, 16), :], jnp.uint32)
                for odd in range(2):
                    x = pltpu.unpack_elementwise(words, index=odd, packed_dtype=bf16, unpacked_dtype=f32)
                    total = x[:, :128]
                    for i in range(1, D // 128):
                        total = total + x[:, 128 * i:128 * (i + 1)]
                    if lag:
                        total = jnp.where(chain[-lag] >= 0, total, 0.0)
                    xc = x - jnp.sum(total, axis=-1, keepdims=True) * (1.0 / D)
                    v = jnp.mean(xc * xc, axis=-1, keepdims=True)
                    xn.append(xc * _rcp(_rb(jnp.sqrt(_rb(_rb(v) + _rb(jnp.full_like(v, 1e-5)))))))
                    sc = jnp.broadcast_to(_rb(jnp.sum(xn[-1] * wr, axis=-1, keepdims=True)), (8, 128))
                    tok = row + (r0 + odd)
                    better = (sc > top[0]) | ((sc == top[0]) & (tok < top[1]))
                    top[:] = jnp.where(better, sc, top[0]), jnp.where(better, tok, top[1])
                chain.append(top[1])
            terms = [_rhs_terms(a[:, :512], b[:, :512], a[:, 512:], b[:, 512:]) + [a[:, 512:], b[:, :512]]
                     for a, b in ((xn[0], xn[2]), (xn[1], xn[3]))]
            for i, pair in enumerate(zip(*terms)):
                xs_v[t, g, i, pl.ds(r // 2, 8), :] = pltpu.pack_elementwise(list(pair), packed_dtype=bf16)

    def xn_block(t, g, hf, kh, rows, cols):
        return _unpack(xs_v[t, g, 7 - 3 * hf if kh else 1 + 7 * hf, rows, cols])

    def feature_map():
        row = lax.broadcasted_iota(jnp.int32, (128, DH), 0)
        col = lax.broadcasted_iota(jnp.int32, (128, DH), 1)
        expand = jnp.where((((row & 63) >> 4) << 3 | (row & 7)) == col, 1.0, 0.0).astype(bf16)
        full = _dot(expand, wphi_v[...], _NT)
        row = lax.broadcasted_iota(jnp.int32, (128, D), 0)
        col = lax.broadcasted_iota(jnp.int32, (128, D), 1)
        same = (((row >> 6) << 1) | ((row >> 3) & 1)) == ((col >> 5) & 3)
        return jnp.where(same, full, 0.0).astype(bf16)

    def prepare_w(j):
        blocks = []
        for c in (2 * j, 2 * j + 1):
            w = wqkv_v[:, pl.ds(128 * c, 128)]
            if j < 8:
                blocks.append(_dot(bd[:, 128 * (c % 8):128 * (c % 8 + 1)], w, _NT) * LOG2E)
            else:
                blocks.append(w.astype(f32).T)
        a, b = blocks
        for i, term in enumerate(_lhs_terms(a[:, :512], a[:, 512:], b[:, :512], b[:, 512:])):
            ws_v[j // 2, i, pl.ds(64 * (j % 2), 64), :] = _pack(term)

    def paced_terms(pieces, lag):
        links = []
        for blocks, dest in pieces:
            if len(links) >= lag:
                link = jnp.concatenate([links[-lag]] * (blocks[0].shape[1] // 128), axis=1)
                blocks = [pltpu.bitcast(_bits(b) ^ jnp.concatenate([link, link], axis=0), f32)
                          for b in blocks[:1]] + blocks[1:]
            words = [_pack(term) for term in _signed_sums([t[0] for t in _HK_TERMS], blocks)]
            for i, w in enumerate(words):
                dest[i] = w
            done = functools.reduce(jnp.bitwise_or, words[4:7] + words[9:15] + words[17:])
            slow = jnp.sum(pltpu.bitcast(done, f32), axis=-1, keepdims=True)
            links.append(_bits(jnp.broadcast_to(slow, (8, 128))) & pace["zero"])

    def prepare_wo(lag):
        pieces = []
        for n in range(2):
            for c in range(4):
                for r in range(0, 128, 16):
                    w = [wo_v[pl.ds(256 * c + 128 * kh + r, 16), pl.ds(512 * n, 512)].astype(f32) for kh in range(2)]
                    pieces.append(([w[kh][:, 128 * i:128 * (i + 1)] for i in range(4) for kh in range(2)],
                                   woh_v.at[n, :, pl.ds(64 * c + r // 2, 8), :]))
        paced_terms(pieces, lag)

    def proj_group(j0, nj, t, g):
        rows = pl.ds(64 * (j0 % 2), 64 * nj)
        return _strassen(lambda i: matmul(_unpack(ws_v[j0 // 2, i, rows, :]), _unpack(xs_v[t, g, i]), _NT))

    def pairs(groups):
        return [jnp.concatenate([c[2 * b + hf][r:r + 64] for c in groups for hf in range(2)], axis=1)
                for j in range(groups[0][0].shape[0] // 128) for b in range(2)
                for r in (128 * j, 128 * j + 64)]

    def proj(j0, t):
        return pairs([proj_group(j0, 2, t, g) for g in range(2)])

    kv = [None] * 16
    phi_k = [None] * 16

    def key_features(j, p):
        phi = _features(p)
        phi_k[j] = phi.reshape(128, T).astype(bf16)
        return functools.reduce(jnp.bitwise_or, [_bits(phi[i][:, n:n + 128]) for i in (7, 15)
                                                 for n in range(0, T, 128)])

    def key_tasks(blocks, j0):
        return [None] * 5 + [functools.partial(key_features, j0 + q, p) for q, p in enumerate(blocks)]

    def kv_update(v_blocks, j0):
        for j, v in enumerate(v_blocks, j0):
            v1 = jnp.concatenate([v, jnp.ones((16, T), f32)], axis=0).astype(bf16)
            upd = _dot(v1, phi_k[j], _NT)
            kv[j] = upd if kv[j] is None else kv[j] + upd

    wait_loads()
    layernorm(0, 0, 0)
    pace["zero"] = top[1] >> 31
    wait_loads()
    prepare_w(8)
    wait_loads()
    layernorm(0, 1, 0)
    first = proj_group(8, 1, 0, 0)
    wait_loads()
    v0 = pairs([first, proj_group(8, 1, 0, 1)])
    prepare_w(9)
    first = proj_group(9, 1, 0, 0)
    wait_loads()
    v0 += pairs([first, proj_group(9, 1, 0, 1)])
    for j in (10, 11):
        prepare_w(j)
    if "0" == "0":
        v0 += pairs([proj_group(10, 1, 0, g) for g in range(2)])
        first = proj_group(11, 1, 0, 0)
        wait_loads()
        v0 += pairs([first, proj_group(11, 1, 0, 1)])
    else:
        first = proj_group(10, 2, 0, 0)
        wait_loads()
        v0 += pairs([first, proj_group(10, 2, 0, 1)])
    bd = feature_map()
    for j in (4, 5):
        prepare_w(j)
    first = proj_group(4, 2, 0, 0)
    wait_loads()
    k = pairs([first, proj_group(4, 2, 0, 1)])
    for j in (6, 7):
        prepare_w(j)
    tasks += key_tasks(k[:4], 0)
    rest, k = k[4:], proj(6, 0)
    for g in range(2):
        layernorm(1, g, 3)
    wait_loads()
    for j, p in enumerate(rest, 4):
        key_features(j, p)
    pending = [(v0[:8], 0), (v0[8:], 8)]
    j0 = 8
    for t in range(1, NT_):
        if t == NT_ - 1:
            wait_loads()
        for c in range(2):
            tasks += key_tasks(k, j0)
            v = proj(8 + 2 * c, t)
            if len(pending) > 1:
                kv_update(*pending.pop(0))
            k, j0 = proj(4 + 2 * c, t), 8 * c
            kv_update(*pending.pop(0))
            pending.append((v, j0))
            if t == NT_ - 1:
                prepare_w(2 * c)
                prepare_w(2 * c + 1)
        for g in range(2 if t + 1 < NT_ else 0):
            layernorm(t + 1, g, 1)
    tasks += key_tasks(k, j0)

    r_max = jnp.max(top[0])
    idx = jnp.clip(jnp.min(jnp.where(top[0] == r_max, top[1], S)), 0, S - 1)
    t_sel = idx // T
    grp = pl.ds(pl.multiple_of(idx % 128 // 16 * 8, 8), 8)
    x_sel = jnp.concatenate(
        [xn_block(t_sel, idx % T // 256, idx // 128 % 2, kh, grp, slice(None)) for kh in range(2)],
        axis=1).astype(f32)
    x_sel = jnp.where(lax.broadcasted_iota(jnp.int32, (16, D), 0) == idx % 16, x_sel, 0.0)
    x_sel = jnp.broadcast_to(jnp.sum(x_sel, axis=0, keepdims=True), (16, D)).astype(bf16)
    gate = jax.nn.sigmoid(jnp.full((8, 512), r_max, f32))

    def ffn_program():
        h = []
        for n in range(F // 128):
            acc = []
            for w in (wg_v, wu_v):
                parts = []
                for kh in range(2):
                    dep = yield
                    parts.append(_dot(after(x_sel[:, 512 * kh:512 * (kh + 1)], dep),
                                      w[pl.ds(512 * kh, 512), pl.ds(n * 128, 128)], _NN))
                    ffn["done"].append(_bits(parts[-1][:8]))
                acc.append(parts[0] + parts[1])
            h.append((_silu(acc[0]) * acc[1]).astype(bf16))
        for hf in range(2):
            y = None
            for n in range(F // 128):
                dep = yield
                part = _dot(after(h[n], dep), wd_v[pl.ds(n * 128, 128), pl.ds(hf * 512, 512)], _NN)[:8]
                y = part if y is None else y + part
                ffn["done"].append(_bits(part[:, 384:]))
            ffn["y"][hf] = _rb(y * gate)

    def attend(blocks, j0):
        out = []
        for j, p in enumerate(blocks, j0):
            num = _dot(kv[j], p, _NN)
            for hd in range(2):
                inv = _rcp(num[64 + 8 * hd:72 + 8 * hd] + 1e-6)
                out.append((num[32 * hd:32 * hd + 32].reshape(4, 8, T) * inv[None]).reshape(32, T))
        return [[[jnp.concatenate(out[8 * c + 4 * kh:8 * c + 4 * kh + 4], axis=0)[:, 256 * g:256 * (g + 1)].T
                  for kh in range(2)] for g in range(2)] for c in range(2)]

    stores = []

    def out_proj(i, o_terms, n):
        while i and ffn["y"][n] is None:
            ffn_step()
        for (c, q), block in _hopcroft_kerr(lambda r: matmul(o_terms[r], _unpack(woh_v[n, r]), _NN)):
            t, g = tiles[i + q // 2], q % 2
            cols, tok = pl.ds(512 * n + 128 * c, 128), pl.ds(pl.multiple_of(T * t + 256 * g, 256), 256)
            a = jnp.concatenate([xn_block(t, g, hf, n, slice(None), pl.ds(128 * c, 128))
                                 for hf in range(2)], axis=0).astype(f32)
            if i + q // 2 == NT_ - 1:
                hit = (lax.broadcasted_iota(jnp.int32, (32, 8, 128), 0) * 8
                       + lax.broadcasted_iota(jnp.int32, (32, 8, 128), 1)) == idx % T - 256 * g
                a3 = a.reshape(32, 8, 128)
                a = jnp.where(hit, a3 + ffn["y"][n][:, 128 * c:128 * (c + 1)][None], a3).reshape(256, 128)
            rows = pl.ds(T * i + 256 * q, 256)
            out_v[rows, cols] = (x_v[tok, cols].astype(f32) + block * _silu(a)).astype(bf16)
            if i and n:
                stores.extend(group(10, (out_v.at[rows, cols], out_hbm.at[tok, cols])))
                stores[-1].start()
        if (i, n) in ((0, 1), (2, 0)):
            cols = pl.ds(0, 512) if i else slice(None)
            for q in range(2):
                stores.extend(group(10, (out_v.at[pl.ds(T * (i + q), T), cols],
                                         out_hbm.at[pl.ds(pl.multiple_of(T * tiles[i + q], T), T), cols])))
                stores[-1].start()

    def output_terms(first, second):
        per_group = [_signed_sums([t[1] for t in _HK_TERMS],
                                  [b for o in (first, second) for g in range(2) for b in o[c][g]])
                     for c in range(4)]
        return [jnp.concatenate(term, axis=1).astype(bf16) for term in zip(*per_group)]

    def last_loads():
        wait_loads()
        prepare_wo(1)
        ffn["steps"], ffn["done"] = ffn_program(), [None, None]
        next(ffn["steps"])

    tiles = [lax.rem(t_sel + 1 + i, NT_) for i in range(NT_)]
    o = [[] for _ in range(NT_)]
    halves = [(i, c) for i in range(NT_) for c in range(2)]
    for h, (i, c) in enumerate(halves):
        q = proj(2 * c, tiles[i])
        if h == 0:
            kv_update(*pending.pop(0))
            row = lax.broadcasted_iota(jnp.int32, (80, 128), 0)
            col = lax.broadcasted_iota(jnp.int32, (80, 128), 1)
            own = jnp.where(row < 64, row >> 5, (row >> 3) & 1) == (col & 1)
            kv[:] = [jnp.where(own, a, 0.0).astype(bf16) for a in kv]
            tasks.extend([None] * 3 + [last_loads])
        else:
            o[halves[h - 1][0]] += attend(prev, 8 * halves[h - 1][1])
        prev = [_features(p).reshape(128, T).astype(bf16) for p in q]
        if h == 7:
            terms = output_terms(*o[:2])
            out_proj(0, terms, 0)
    out_proj(0, terms, 1)
    o[-1] += attend(prev, 8)
    terms = output_terms(*o[2:])
    for n in range(2):
        out_proj(2, terms, n)
    for c in stores:
        c.wait()


@jax.jit
def pallas_recurrent_scan__linear_kernel_hedgehog__moe_arch_mod__prompt_kernel(
    A_x: jax.Array,
    A_wqkv: jax.Array,
    A_w_phi: jax.Array,
    A_wo: jax.Array,
    B_x: jax.Array,
    B_w_r: jax.Array,
    B_w_gate: jax.Array,
    B_w_up: jax.Array,
    B_w_down: jax.Array,
):
    del B_x
    hbm = pl.BlockSpec(memory_space=pl.ANY)
    out = pl.pallas_call(
        _kernel,
        out_shape=jax.ShapeDtypeStruct((S, D), bf16),
        in_specs=[hbm] * 8,
        out_specs=hbm,
        scratch_shapes=[
            pltpu.VMEM((S, D), bf16),
            pltpu.VMEM((NT_, 2, 9, 64, 512), jnp.uint32),
            pltpu.VMEM((D, 3 * D), bf16),
            pltpu.VMEM((6, 7, 128, 512), jnp.uint32),
            pltpu.VMEM((D, D), bf16),
            pltpu.VMEM((2, 26, 256, 128), jnp.uint32),
            pltpu.VMEM((D, F), bf16),
            pltpu.VMEM((D, F), bf16),
            pltpu.VMEM((F, D), bf16),
            pltpu.VMEM((S, D), bf16),
            pltpu.VMEM((H * DH, DH), bf16),
            pltpu.VMEM((D,), bf16),
            pltpu.SemaphoreType.DMA((11,)),
        ],
        compiler_params=pltpu.CompilerParams(vmem_limit_bytes=110 * 1024 * 1024),
        name="hedgehog_mod",
    )(
        A_x.reshape(S, D), A_wqkv, A_w_phi.reshape(H * DH, DH), A_wo,
        B_w_r, B_w_gate, B_w_up, B_w_down,
    )
    return out.reshape(1, S, D)
```

```python
import functools
import math

import jax
import jax.numpy as jnp
from jax import lax
import jax.experimental.pallas as pl
import jax.experimental.pallas.tpu as pltpu

S, D, H, DH, F = 2048, 1024, 32, 32, 3584
T = 512
NT_ = S // T
LOG2E = math.log2(math.e)
_NT = (((1,), (1,)), ((), ()))
_NN = (((1,), (0,)), ((), ()))
f32, bf16 = jnp.float32, jnp.bfloat16


def _dot(a, b, dn):
    return lax.dot_general(a, b, dn, preferred_element_type=f32)


def _rb(v):
    return v.astype(bf16).astype(f32)


def _rcp(v):
    r = pl.reciprocal(v, approx=True)
    return r * (2.0 - v * r)


def _silu(a):
    return a * pl.reciprocal(1.0 + jnp.exp2(a * -LOG2E), approx=True)


def _bits(v):
    return pltpu.bitcast(v, jnp.int32)


def _pack(v):
    m, n = v.shape
    v = v.reshape(m // 16, 2, 8, n)
    return pltpu.pack_elementwise([v[:, 0], v[:, 1]], packed_dtype=bf16).reshape(m // 2, n)


def _unpack(words):
    return pltpu.bitcast(words, bf16)


def _lhs_terms(a11, a12, a21, a22):
    return [a11 + a22, a21 + a22, a11, a22, a11 + a12, a21 - a11, a12 - a22]


def _rhs_terms(b11, b12, b21, b22):
    return [b11 + b22, b11, b12 - b22, b21 - b11, b22, b11 + b12, b21 + b22]


def _strassen(product):
    m = product(0)
    c11, c22 = m, m
    c21 = product(3)
    c11 = c11 + c21
    c12 = product(4)
    c11 = c11 - c12
    c11 = c11 + product(6)
    m = product(2)
    c12, c22 = c12 + m, c22 + m
    m = product(1)
    c21, c22 = c21 + m, c22 - m
    c22 = c22 + product(5)
    return c11, c12, c21, c22


_HK_TERMS = (
    ((1,), (1, -2)), ((1, 2), (2,)), ((3, 4), (3,)), ((-4,), (3, -4)),
    ((1, 4), (2, 3)), ((-1, 3), (1, 3)), ((2, -4), (2, 4)),
    ((6,), (6,)), ((5,), (5,)),
    ((-3, -4, 5), (3, -4, -6)), ((-3, -4, 5, 6), (4, 6)), ((3, -5), (3, -4, 5, -6)),
    ((1, 2, -6), (1, -2, 5)), ((-2, 6), (1, -2, 5, -6)), ((-1, -2, 5, 6), (1, 5)),
    ((7,), (7, -8)), ((7, 8), (8,)),
    ((4, 7), (3, 8)), ((3, -7), (3, 7)), ((-4, 8), (4, 8)),
    ((-6, 7, 8), (5, 7, -8)), ((6, -8), (5, -6, 7, -8)), ((5, 6, -7, -8), (5, 7)),
    ((2, -6, 7), (1, 5, 8)), ((1, -5, -7), (1, 5, 7)), ((-2, 6, 8), (2, 6, 8)),
)
_HK_SUMS = (
    ((0, 0), (2, 1)), ((1, 1), (4, 3)), ((1, 0), (6, 5, 1, -3)), ((0, 1), (7, 5, 4, -2)),
    ((2, 2), (9, 8)), ((2, 1), (11, 10, 3, -8)), ((1, 2), (12, 10, 9, -4)),
    ((0, 2), (14, 13, 8, -1)), ((2, 0), (15, 13, 2, -9)), ((3, 3), (17, 16)),
    ((1, 3), (19, 18, 16, -3)), ((3, 1), (20, 18, 4, -17)),
    ((3, 2), (22, 21, 8, -16)), ((2, 3), (23, 21, 17, -9)),
    ((0, 3), (25, 24, 16, 15), (2, 3), 1), ((3, 0), (26, 24, 14, -17), (3, 2), -1),
)


def _signed_sums(wanted, blocks):
    known = {(i + 1,): b for i, b in enumerate(blocks)}

    def value(key):
        if key not in known:
            for part in sorted(known, key=len, reverse=True):
                for sign in (1, -1):
                    signed = [sign * p for p in part]
                    if key not in known and len(part) < len(key) and all(p in key for p in signed):
                        rest = tuple(k for k in key if k not in signed)
                        if sign > 0 and rest[0] < 0:
                            known[key] = known[part] - value(tuple(-k for k in rest))
                        else:
                            known[key] = value(rest) + known[part] if sign > 0 else value(rest) - known[part]
            if key not in known:
                known[key] = -known[(-key[0],)]
        return known[key]

    for key in sorted(wanted, key=len):
        value(key)
    return [known[key] for key in wanted]


def _hopcroft_kerr(product):
    m, y = [], {}
    for ij, parts, *earlier in _HK_SUMS:
        while len(m) < parts[0]:
            m.append(product(len(m)))
        total = m[parts[0] - 1]
        for p in parts[1:]:
            total = total + m[p - 1] if p > 0 else total - m[-p - 1]
        if earlier:
            total = total + y[earlier[0]] if earlier[1] > 0 else total - y[earlier[0]]
        y[ij] = total
        yield ij, total


def _allreduce(v, op):
    r = v[0]
    for i in range(1, 8):
        r = op(r, v[i])
    r = op(r, pltpu.roll(r, 4, 0))
    return op(r, pltpu.roll(r, 2, 0))


def _features(p):
    p3 = p.reshape(8, 8, p.shape[1])
    mx = _allreduce(p3, jnp.maximum)
    mn = _allreduce(p3, jnp.minimum)
    ep = jnp.exp2(p3 - mx[None])
    en = jnp.exp2(mn[None] - p3)
    ip = _rcp(_allreduce(ep, jnp.add))
    im = _rcp(_allreduce(en, jnp.add))
    return jnp.concatenate([ep * ip[None], en * im[None]], axis=0)


def _kernel(x_hbm, wqkv_hbm, wphi_hbm, wo_hbm, wr_hbm, wg_hbm, wu_hbm, wd_hbm, out_hbm,
            x_v, xs_v, wqkv_v, ws_v, wo_v, woh_v, wg_v, wu_v, wd_v, out_v, wphi_v, wr_v, sems):
    def group(k, *pairs):
        return [pltpu.make_async_copy(src, dst, sems.at[k]) for src, dst in pairs]

    def x_rows(r0, n):
        return x_hbm.at[pl.ds(r0, n)], x_v.at[pl.ds(r0, n)]

    def w_cols(j0, nj):
        cols = pl.ds(256 * j0, 256 * nj)
        return wqkv_hbm.at[:, cols], wqkv_v.at[:, cols]

    loads = [
        group(0, x_rows(0, 256), (wr_hbm, wr_v)),
        group(1, w_cols(8, 1)),
        group(2, x_rows(256, 256)),
        group(3, w_cols(9, 1)),
        group(4, w_cols(10, 2)),
        group(5, (wphi_hbm, wphi_v), w_cols(4, 2)),
        group(6, w_cols(6, 2), x_rows(T, T)),
        group(7, x_rows(2 * T, S - 2 * T), w_cols(0, 4)),
        group(9, (wo_hbm, wo_v), (wg_hbm, wg_v), (wu_hbm, wu_v), (wd_hbm, wd_v)),
    ]
    for copies in loads:
        for c in copies:
            c.start()

    def wait_loads():
        for c in loads.pop(0):
            c.wait()

    tasks = []
    pace = {}

    def after(lhs, dep):
        ok = (dep & pace["zero"]) == 0
        first = jnp.where(jnp.concatenate([ok, ok], axis=0), lhs[:16, :128], jnp.zeros((16, 128), bf16))
        if lhs.shape[1] > 128:
            first = jnp.concatenate([first, lhs[:16, 128:]], axis=1)
        return first if lhs.shape[0] == 16 else jnp.concatenate([first, lhs[16:]], axis=0)

    ffn = {"steps": None, "done": [], "y": [None, None]}

    def ffn_step():
        try:
            ffn["steps"].send(ffn["main"])
        except StopIteration:
            ffn["steps"] = None

    def matmul(lhs, rhs, dn):
        task = tasks.pop(0) if tasks else None
        dep = task() if task is not None else None
        if ffn["done"]:
            dep = ffn["done"].pop(0)
        m = _dot(lhs if dep is None else after(lhs, dep), rhs, dn)
        if ffn["steps"] is not None:
            ffn_step()
        ffn["main"] = _bits(m[-8:, -128:])
        return m

    top = [jnp.full((8, 128), -jnp.inf, f32), lax.broadcasted_iota(jnp.int32, (8, 128), 0)]
    chain = []

    def layernorm(t, g, lag):
        wr = wr_v[...].astype(f32).reshape(1, D)
        row = 2 * lax.broadcasted_iota(jnp.int32, (8, 128), 0)
        for r in range(0, 128, 16):
            xn = []
            for r0 in (T * t + 256 * g + r, T * t + 256 * g + 128 + r):
                words = pltpu.bitcast(x_v[pl.ds(r0, 16), :], jnp.uint32)
                for odd in range(2):
                    x = pltpu.unpack_elementwise(words, index=odd, packed_dtype=bf16, unpacked_dtype=f32)
                    total = x[:, :128]
                    for i in range(1, D // 128):
                        total = total + x[:, 128 * i:128 * (i + 1)]
                    if lag:
                        total = jnp.where(chain[-lag] >= 0, total, 0.0)
                    xc = x - jnp.sum(total, axis=-1, keepdims=True) * (1.0 / D)
                    v = jnp.mean(xc * xc, axis=-1, keepdims=True)
                    xn.append(xc * (1.0 / _rb(jnp.sqrt(_rb(_rb(v) + _rb(jnp.full_like(v, 1e-5)))))))
                    sc = jnp.broadcast_to(_rb(jnp.sum(xn[-1] * wr, axis=-1, keepdims=True)), (8, 128))
                    tok = row + (r0 + odd)
                    better = (sc > top[0]) | ((sc == top[0]) & (tok < top[1]))
                    top[:] = jnp.where(better, sc, top[0]), jnp.where(better, tok, top[1])
                chain.append(top[1])
            terms = [_rhs_terms(a[:, :512], b[:, :512], a[:, 512:], b[:, 512:]) + [a[:, 512:], b[:, :512]]
                     for a, b in ((xn[0], xn[2]), (xn[1], xn[3]))]
            for i, pair in enumerate(zip(*terms)):
                xs_v[t, g, i, pl.ds(r // 2, 8), :] = pltpu.pack_elementwise(list(pair), packed_dtype=bf16)

    def xn_block(t, g, hf, kh, rows, cols):
        return _unpack(xs_v[t, g, 7 - 3 * hf if kh else 1 + 7 * hf, rows, cols])

    def feature_map():
        row = lax.broadcasted_iota(jnp.int32, (128, DH), 0)
        col = lax.broadcasted_iota(jnp.int32, (128, DH), 1)
        expand = jnp.where((((row & 63) >> 4) << 3 | (row & 7)) == col, 1.0, 0.0).astype(bf16)
        full = _dot(expand, wphi_v[...], _NT)
        row = lax.broadcasted_iota(jnp.int32, (128, D), 0)
        col = lax.broadcasted_iota(jnp.int32, (128, D), 1)
        same = (((row >> 6) << 1) | ((row >> 3) & 1)) == ((col >> 5) & 3)
        return jnp.where(same, full, 0.0).astype(bf16)

    def prepare_w(j):
        blocks = []
        for c in (2 * j, 2 * j + 1):
            w = wqkv_v[:, pl.ds(128 * c, 128)]
            if j < 8:
                blocks.append(_dot(bd[:, 128 * (c % 8):128 * (c % 8 + 1)], w, _NT) * LOG2E)
            else:
                blocks.append(w.astype(f32).T)
        a, b = blocks
        for i, term in enumerate(_lhs_terms(a[:, :512], a[:, 512:], b[:, :512], b[:, 512:])):
            ws_v[j // 2, i, pl.ds(64 * (j % 2), 64), :] = _pack(term)

    def paced_terms(pieces, lag):
        links = []
        for blocks, dest in pieces:
            if len(links) >= lag:
                link = jnp.concatenate([links[-lag]] * (blocks[0].shape[1] // 128), axis=1)
                blocks = [pltpu.bitcast(_bits(b) ^ jnp.concatenate([link, link], axis=0), f32)
                          for b in blocks[:1]] + blocks[1:]
            words = [_pack(term) for term in _signed_sums([t[0] for t in _HK_TERMS], blocks)]
            for i, w in enumerate(words):
                dest[i] = w
            done = functools.reduce(jnp.bitwise_or, words[4:7] + words[9:15] + words[17:])
            slow = jnp.sum(pltpu.bitcast(done, f32), axis=-1, keepdims=True)
            links.append(_bits(jnp.broadcast_to(slow, (8, 128))) & pace["zero"])

    def prepare_wo(lag):
        pieces = []
        for n in range(2):
            for c in range(4):
                for r in range(0, 128, 16):
                    w = [wo_v[pl.ds(256 * c + 128 * kh + r, 16), pl.ds(512 * n, 512)].astype(f32) for kh in range(2)]
                    pieces.append(([w[kh][:, 128 * i:128 * (i + 1)] for i in range(4) for kh in range(2)],
                                   woh_v.at[n, :, pl.ds(64 * c + r // 2, 8), :]))
        paced_terms(pieces, lag)

    def proj_group(j0, nj, t, g):
        rows = pl.ds(64 * (j0 % 2), 64 * nj)
        return _strassen(lambda i: matmul(_unpack(ws_v[j0 // 2, i, rows, :]), _unpack(xs_v[t, g, i]), _NT))

    def pairs(groups):
        return [jnp.concatenate([c[2 * b + hf][r:r + 64] for c in groups for hf in range(2)], axis=1)
                for j in range(groups[0][0].shape[0] // 128) for b in range(2)
                for r in (128 * j, 128 * j + 64)]

    def proj(j0, t):
        return pairs([proj_group(j0, 2, t, g) for g in range(2)])

    kv = [None] * 16
    phi_k = [None] * 16

    def key_features(j, p):
        phi = _features(p)
        phi_k[j] = phi.reshape(128, T).astype(bf16)
        return functools.reduce(jnp.bitwise_or, [_bits(phi[i][:, n:n + 128]) for i in (7, 15)
                                                 for n in range(0, T, 128)])

    def key_tasks(blocks, j0):
        return [None] * 5 + [functools.partial(key_features, j0 + q, p) for q, p in enumerate(blocks)]

    def kv_update(v_blocks, j0):
        for j, v in enumerate(v_blocks, j0):
            v1 = jnp.concatenate([v, jnp.ones((16, T), f32)], axis=0).astype(bf16)
            upd = _dot(v1, phi_k[j], _NT)
            kv[j] = upd if kv[j] is None else kv[j] + upd

    wait_loads()
    layernorm(0, 0, 0)
    pace["zero"] = top[1] >> 31
    wait_loads()
    prepare_w(8)
    wait_loads()
    layernorm(0, 1, 0)
    first = proj_group(8, 1, 0, 0)
    wait_loads()
    v0 = pairs([first, proj_group(8, 1, 0, 1)])
    prepare_w(9)
    first = proj_group(9, 1, 0, 0)
    wait_loads()
    v0 += pairs([first, proj_group(9, 1, 0, 1)])
    for j in (10, 11):
        prepare_w(j)
    if "0" == "0":
        v0 += pairs([proj_group(10, 1, 0, g) for g in range(2)])
        first = proj_group(11, 1, 0, 0)
        wait_loads()
        v0 += pairs([first, proj_group(11, 1, 0, 1)])
    else:
        first = proj_group(10, 2, 0, 0)
        wait_loads()
        v0 += pairs([first, proj_group(10, 2, 0, 1)])
    bd = feature_map()
    for j in (4, 5):
        prepare_w(j)
    first = proj_group(4, 2, 0, 0)
    wait_loads()
    k = pairs([first, proj_group(4, 2, 0, 1)])
    for j in (6, 7):
        prepare_w(j)
    tasks += key_tasks(k[:4], 0)
    rest, k = k[4:], proj(6, 0)
    for g in range(2):
        layernorm(1, g, 3)
    wait_loads()
    for j, p in enumerate(rest, 4):
        key_features(j, p)
    pending = [(v0[:8], 0), (v0[8:], 8)]
    j0 = 8
    for t in range(1, NT_):
        for c in range(2):
            tasks += key_tasks(k, j0)
            v = proj(8 + 2 * c, t)
            if len(pending) > 1:
                kv_update(*pending.pop(0))
            k, j0 = proj(4 + 2 * c, t), 8 * c
            kv_update(*pending.pop(0))
            pending.append((v, j0))
            if t == NT_ - 1:
                prepare_w(2 * c)
                prepare_w(2 * c + 1)
        for g in range(2 if t + 1 < NT_ else 0):
            layernorm(t + 1, g, 1)
    tasks += key_tasks(k, j0)

    r_max = jnp.max(top[0])
    idx = jnp.clip(jnp.min(jnp.where(top[0] == r_max, top[1], S)), 0, S - 1)
    t_sel = idx // T
    grp = pl.ds(pl.multiple_of(idx % 128 // 16 * 8, 8), 8)
    x_sel = jnp.concatenate(
        [xn_block(t_sel, idx % T // 256, idx // 128 % 2, kh, grp, slice(None)) for kh in range(2)],
        axis=1).astype(f32)
    x_sel = jnp.where(lax.broadcasted_iota(jnp.int32, (16, D), 0) == idx % 16, x_sel, 0.0)
    x_sel = jnp.broadcast_to(jnp.sum(x_sel, axis=0, keepdims=True), (16, D)).astype(bf16)
    gate = jax.nn.sigmoid(jnp.full((8, 512), r_max, f32))

    def ffn_program():
        h = []
        for n in range(F // 128):
            acc = []
            for w in (wg_v, wu_v):
                parts = []
                for kh in range(2):
                    dep = yield
                    parts.append(_dot(after(x_sel[:, 512 * kh:512 * (kh + 1)], dep),
                                      w[pl.ds(512 * kh, 512), pl.ds(n * 128, 128)], _NN))
                    ffn["done"].append(_bits(parts[-1][:8]))
                acc.append(parts[0] + parts[1])
            h.append((_silu(acc[0]) * acc[1]).astype(bf16))
        for hf in range(2):
            y = None
            for n in range(F // 128):
                dep = yield
                part = _dot(after(h[n], dep), wd_v[pl.ds(n * 128, 128), pl.ds(hf * 512, 512)], _NN)[:8]
                y = part if y is None else y + part
                ffn["done"].append(_bits(part[:, 384:]))
            ffn["y"][hf] = _rb(y * gate)

    def attend(blocks, j0):
        out = []
        for j, p in enumerate(blocks, j0):
            num = _dot(kv[j], p, _NN)
            for hd in range(2):
                inv = _rcp(num[64 + 8 * hd:72 + 8 * hd] + 1e-6)
                out.append((num[32 * hd:32 * hd + 32].reshape(4, 8, T) * inv[None]).reshape(32, T))
        return [[[jnp.concatenate(out[8 * c + 4 * kh:8 * c + 4 * kh + 4], axis=0)[:, 256 * g:256 * (g + 1)].T
                  for kh in range(2)] for g in range(2)] for c in range(2)]

    stores = []

    def out_proj(i, o_terms, n):
        while i and ffn["y"][n] is None:
            ffn_step()
        for (c, q), block in _hopcroft_kerr(lambda r: matmul(o_terms[r], _unpack(woh_v[n, r]), _NN)):
            t, g = tiles[i + q // 2], q % 2
            cols, tok = pl.ds(512 * n + 128 * c, 128), pl.ds(pl.multiple_of(T * t + 256 * g, 256), 256)
            a = jnp.concatenate([xn_block(t, g, hf, n, slice(None), pl.ds(128 * c, 128))
                                 for hf in range(2)], axis=0).astype(f32)
            if i + q // 2 == NT_ - 1:
                hit = (lax.broadcasted_iota(jnp.int32, (32, 8, 128), 0) * 8
                       + lax.broadcasted_iota(jnp.int32, (32, 8, 128), 1)) == idx % T - 256 * g
                a3 = a.reshape(32, 8, 128)
                a = jnp.where(hit, a3 + ffn["y"][n][:, 128 * c:128 * (c + 1)][None], a3).reshape(256, 128)
            rows = pl.ds(T * i + 256 * q, 256)
            out_v[rows, cols] = (x_v[tok, cols].astype(f32) + block * _silu(a)).astype(bf16)
            if i and n:
                stores.extend(group(10, (out_v.at[rows, cols], out_hbm.at[tok, cols])))
                stores[-1].start()
        if (i, n) in ((0, 1), (2, 0)):
            cols = pl.ds(0, 512) if i else slice(None)
            for q in range(2):
                stores.extend(group(10, (out_v.at[pl.ds(T * (i + q), T), cols],
                                         out_hbm.at[pl.ds(pl.multiple_of(T * tiles[i + q], T), T), cols])))
                stores[-1].start()

    def output_terms(first, second):
        per_group = [_signed_sums([t[1] for t in _HK_TERMS],
                                  [b for o in (first, second) for g in range(2) for b in o[c][g]])
                     for c in range(4)]
        return [jnp.concatenate(term, axis=1).astype(bf16) for term in zip(*per_group)]

    def last_loads():
        wait_loads()
        prepare_wo(1)
        ffn["steps"], ffn["done"] = ffn_program(), [None, None]
        next(ffn["steps"])

    tiles = [lax.rem(t_sel + 1 + i, NT_) for i in range(NT_)]
    o = [[] for _ in range(NT_)]
    halves = [(i, c) for i in range(NT_) for c in range(2)]
    for h, (i, c) in enumerate(halves):
        q = proj(2 * c, tiles[i])
        if h == 0:
            kv_update(*pending.pop(0))
            row = lax.broadcasted_iota(jnp.int32, (80, 128), 0)
            col = lax.broadcasted_iota(jnp.int32, (80, 128), 1)
            own = jnp.where(row < 64, row >> 5, (row >> 3) & 1) == (col & 1)
            kv[:] = [jnp.where(own, a, 0.0).astype(bf16) for a in kv]
            tasks.extend([None] * 3 + [last_loads])
        else:
            o[halves[h - 1][0]] += attend(prev, 8 * halves[h - 1][1])
        prev = [_features(p).reshape(128, T).astype(bf16) for p in q]
        if h == 7:
            terms = output_terms(*o[:2])
            out_proj(0, terms, 0)
    out_proj(0, terms, 1)
    o[-1] += attend(prev, 8)
    terms = output_terms(*o[2:])
    for n in range(2):
        out_proj(2, terms, n)
    for c in stores:
        c.wait()


@jax.jit
def pallas_recurrent_scan__linear_kernel_hedgehog__moe_arch_mod__prompt_kernel(
    A_x: jax.Array,
    A_wqkv: jax.Array,
    A_w_phi: jax.Array,
    A_wo: jax.Array,
    B_x: jax.Array,
    B_w_r: jax.Array,
    B_w_gate: jax.Array,
    B_w_up: jax.Array,
    B_w_down: jax.Array,
):
    del B_x
    hbm = pl.BlockSpec(memory_space=pl.ANY)
    out = pl.pallas_call(
        _kernel,
        out_shape=jax.ShapeDtypeStruct((S, D), bf16),
        in_specs=[hbm] * 8,
        out_specs=hbm,
        scratch_shapes=[
            pltpu.VMEM((S, D), bf16),
            pltpu.VMEM((NT_, 2, 9, 64, 512), jnp.uint32),
            pltpu.VMEM((D, 3 * D), bf16),
            pltpu.VMEM((6, 7, 128, 512), jnp.uint32),
            pltpu.VMEM((D, D), bf16),
            pltpu.VMEM((2, 26, 256, 128), jnp.uint32),
            pltpu.VMEM((D, F), bf16),
            pltpu.VMEM((D, F), bf16),
            pltpu.VMEM((F, D), bf16),
            pltpu.VMEM((S, D), bf16),
            pltpu.VMEM((H * DH, DH), bf16),
            pltpu.VMEM((D,), bf16),
            pltpu.SemaphoreType.DMA((11,)),
        ],
        compiler_params=pltpu.CompilerParams(vmem_limit_bytes=110 * 1024 * 1024),
        name="hedgehog_mod",
    )(
        A_x.reshape(S, D), A_wqkv, A_w_phi.reshape(H * DH, DH), A_wo,
        B_w_r, B_w_gate, B_w_up, B_w_down,
    )
    return out.reshape(1, S, D)
```

```python
import functools
import math

import jax
import jax.numpy as jnp
from jax import lax
import jax.experimental.pallas as pl
import jax.experimental.pallas.tpu as pltpu

S, D, H, DH, F = 2048, 1024, 32, 32, 3584
T = 512
NT_ = S // T
LOG2E = math.log2(math.e)
_NT = (((1,), (1,)), ((), ()))
_NN = (((1,), (0,)), ((), ()))
f32, bf16 = jnp.float32, jnp.bfloat16


def _dot(a, b, dn):
    return lax.dot_general(a, b, dn, preferred_element_type=f32)


def _rb(v):
    return v.astype(bf16).astype(f32)


def _rcp(v):
    r = pl.reciprocal(v, approx=True)
    return r * (2.0 - v * r)


def _silu(a):
    return a * pl.reciprocal(1.0 + jnp.exp2(a * -LOG2E), approx=True)


def _bits(v):
    return pltpu.bitcast(v, jnp.int32)


def _pack(v):
    m, n = v.shape
    v = v.reshape(m // 16, 2, 8, n)
    return pltpu.pack_elementwise([v[:, 0], v[:, 1]], packed_dtype=bf16).reshape(m // 2, n)


def _unpack(words):
    return pltpu.bitcast(words, bf16)


_HK_TERMS = (
    ((1,), (1, -2)), ((1, 2), (2,)), ((3, 4), (3,)), ((-4,), (3, -4)),
    ((1, 4), (2, 3)), ((-1, 3), (1, 3)), ((2, -4), (2, 4)),
    ((6,), (6,)), ((5,), (5,)),
    ((-3, -4, 5), (3, -4, -6)), ((-3, -4, 5, 6), (4, 6)), ((3, -5), (3, -4, 5, -6)),
    ((1, 2, -6), (1, -2, 5)), ((-2, 6), (1, -2, 5, -6)), ((-1, -2, 5, 6), (1, 5)),
    ((7,), (7, -8)), ((7, 8), (8,)),
    ((4, 7), (3, 8)), ((3, -7), (3, 7)), ((-4, 8), (4, 8)),
    ((-6, 7, 8), (5, 7, -8)), ((6, -8), (5, -6, 7, -8)), ((5, 6, -7, -8), (5, 7)),
    ((2, -6, 7), (1, 5, 8)), ((1, -5, -7), (1, 5, 7)), ((-2, 6, 8), (2, 6, 8)),
)
_HK_SUMS = (
    ((0, 0), (2, 1)), ((1, 1), (4, 3)), ((1, 0), (6, 5, 1, -3)), ((0, 1), (7, 5, 4, -2)),
    ((2, 2), (9, 8)), ((2, 1), (11, 10, 3, -8)), ((1, 2), (12, 10, 9, -4)),
    ((0, 2), (14, 13, 8, -1)), ((2, 0), (15, 13, 2, -9)), ((3, 3), (17, 16)),
    ((1, 3), (19, 18, 16, -3)), ((3, 1), (20, 18, 4, -17)),
    ((3, 2), (22, 21, 8, -16)), ((2, 3), (23, 21, 17, -9)),
    ((0, 3), (25, 24, 16, 15), (2, 3), 1), ((3, 0), (26, 24, 14, -17), (3, 2), -1),
)


def _signed_sums(wanted, blocks):
    known = {(i + 1,): b for i, b in enumerate(blocks)}

    def value(key):
        if key not in known:
            for part in sorted(known, key=len, reverse=True):
                for sign in (1, -1):
                    signed = [sign * p for p in part]
                    if key not in known and len(part) < len(key) and all(p in key for p in signed):
                        rest = tuple(k for k in key if k not in signed)
                        if sign > 0 and rest[0] < 0:
                            known[key] = known[part] - value(tuple(-k for k in rest))
                        else:
                            known[key] = value(rest) + known[part] if sign > 0 else value(rest) - known[part]
            if key not in known:
                known[key] = -known[(-key[0],)]
        return known[key]

    for key in sorted(wanted, key=len):
        value(key)
    return [known[key] for key in wanted]


def _block_product(product, size):
    m, y = [], {}
    for ij, parts, *earlier in _HK_SUMS[:size * size]:
        while len(m) < parts[0]:
            m.append(product(len(m)))
        total = m[parts[0] - 1]
        for p in parts[1:]:
            total = total + m[p - 1] if p > 0 else total - m[-p - 1]
        if earlier:
            total = total + y[earlier[0]] if earlier[1] > 0 else total - y[earlier[0]]
        y[ij] = total
        yield ij, total


def _allreduce(v, op):
    r = v[0]
    for i in range(1, 8):
        r = op(r, v[i])
    r = op(r, pltpu.roll(r, 4, 0))
    return op(r, pltpu.roll(r, 2, 0))


def _features(p):
    p3 = p.reshape(8, 8, p.shape[1])
    mx = _allreduce(p3, jnp.maximum)
    mn = _allreduce(p3, jnp.minimum)
    ep = jnp.exp2(p3 - mx[None])
    en = jnp.exp2(mn[None] - p3)
    ip = _rcp(_allreduce(ep, jnp.add))
    im = _rcp(_allreduce(en, jnp.add))
    return jnp.concatenate([ep * ip[None], en * im[None]], axis=0)


def _kernel(x_hbm, wqkv_hbm, wphi_hbm, wo_hbm, wr_hbm, wg_hbm, wu_hbm, wd_hbm, out_hbm,
            x_v, xs_v, wqkv_v, ws_v, wo_v, woh_v, wg_v, wu_v, wd_v, out_v, wphi_v, wr_v, sems):
    def group(k, *pairs):
        return [pltpu.make_async_copy(src, dst, sems.at[k]) for src, dst in pairs]

    def x_rows(r0, n):
        return x_hbm.at[pl.ds(r0, n)], x_v.at[pl.ds(r0, n)]

    def w_cols(j0, nj):
        cols = pl.ds(256 * j0, 256 * nj)
        return wqkv_hbm.at[:, cols], wqkv_v.at[:, cols]

    loads = [
        group(0, x_rows(0, 256), (wr_hbm, wr_v)),
        group(1, w_cols(8, 1)),
        group(2, x_rows(256, 256)),
        group(3, w_cols(9, 1)),
        group(4, w_cols(10, 2)),
        group(5, (wphi_hbm, wphi_v), w_cols(4, 2)),
        group(6, w_cols(6, 2), x_rows(T, T)),
        group(7, x_rows(2 * T, S - 2 * T), w_cols(0, 4)),
        group(9, (wo_hbm, wo_v), (wg_hbm, wg_v), (wu_hbm, wu_v), (wd_hbm, wd_v)),
    ]
    for copies in loads:
        for c in copies:
            c.start()

    def wait_loads():
        for c in loads.pop(0):
            c.wait()

    tasks = []
    pace = {}

    def after(lhs, dep):
        ok = (dep & pace["zero"]) == 0
        first = jnp.where(jnp.concatenate([ok, ok], axis=0), lhs[:16, :128], jnp.zeros((16, 128), bf16))
        if lhs.shape[1] > 128:
            first = jnp.concatenate([first, lhs[:16, 128:]], axis=1)
        return first if lhs.shape[0] == 16 else jnp.concatenate([first, lhs[16:]], axis=0)

    ffn = {"steps": None, "done": [], "y": [None, None]}

    def ffn_step():
        try:
            ffn["steps"].send(ffn["main"])
        except StopIteration:
            ffn["steps"] = None

    def matmul(lhs, rhs, dn):
        task = tasks.pop(0) if tasks else None
        dep = task() if task is not None else None
        if ffn["done"]:
            dep = ffn["done"].pop(0)
        m = _dot(lhs if dep is None else after(lhs, dep), rhs, dn)
        if ffn["steps"] is not None:
            ffn_step()
        ffn["main"] = _bits(m[-8:, -128:])
        return m

    top = [jnp.full((8, 128), -jnp.inf, f32), lax.broadcasted_iota(jnp.int32, (8, 128), 0)]
    chain = []
    x_keys = [term[1] for term in _HK_TERMS[:7]] + [(1,), (4,)]
    x_block = [x_keys.index((i + 1,)) for i in range(4)]

    def layernorm(t, g, lag):
        wr = wr_v[...].astype(f32).reshape(1, D)
        row = 2 * lax.broadcasted_iota(jnp.int32, (8, 128), 0)
        for r in range(0, 128, 16):
            xn = []
            for r0 in (T * t + 256 * g + r, T * t + 256 * g + 128 + r):
                words = pltpu.bitcast(x_v[pl.ds(r0, 16), :], jnp.uint32)
                for odd in range(2):
                    x = pltpu.unpack_elementwise(words, index=odd, packed_dtype=bf16, unpacked_dtype=f32)
                    total = x[:, :128]
                    for i in range(1, D // 128):
                        total = total + x[:, 128 * i:128 * (i + 1)]
                    if lag:
                        total = jnp.where(chain[-lag] >= 0, total, 0.0)
                    xc = x - jnp.sum(total, axis=-1, keepdims=True) * (1.0 / D)
                    v = jnp.mean(xc * xc, axis=-1, keepdims=True)
                    xn.append(xc * (1.0 / _rb(jnp.sqrt(_rb(_rb(v) + _rb(jnp.full_like(v, 1e-5)))))))
                    sc = jnp.broadcast_to(_rb(jnp.sum(xn[-1] * wr, axis=-1, keepdims=True)), (8, 128))
                    tok = row + (r0 + odd)
                    better = (sc > top[0]) | ((sc == top[0]) & (tok < top[1]))
                    top[:] = jnp.where(better, sc, top[0]), jnp.where(better, tok, top[1])
                chain.append(top[1])
            terms = [_signed_sums(x_keys, [a[:, :512], a[:, 512:], b[:, :512], b[:, 512:]])
                     for a, b in ((xn[0], xn[2]), (xn[1], xn[3]))]
            for i, pair in enumerate(zip(*terms)):
                xs_v[t, g, i, pl.ds(r // 2, 8), :] = pltpu.pack_elementwise(list(pair), packed_dtype=bf16)

    def feature_map():
        row = lax.broadcasted_iota(jnp.int32, (128, DH), 0)
        col = lax.broadcasted_iota(jnp.int32, (128, DH), 1)
        expand = jnp.where((((row & 63) >> 4) << 3 | (row & 7)) == col, 1.0, 0.0).astype(bf16)
        full = _dot(expand, wphi_v[...], _NT)
        row = lax.broadcasted_iota(jnp.int32, (128, D), 0)
        col = lax.broadcasted_iota(jnp.int32, (128, D), 1)
        same = (((row >> 6) << 1) | ((row >> 3) & 1)) == ((col >> 5) & 3)
        return jnp.where(same, full, 0.0).astype(bf16)

    def prepare_w(j):
        blocks = []
        for c in (2 * j, 2 * j + 1):
            w = wqkv_v[:, pl.ds(128 * c, 128)]
            if j < 8:
                blocks.append(_dot(bd[:, 128 * (c % 8):128 * (c % 8 + 1)], w, _NT) * LOG2E)
            else:
                blocks.append(w.astype(f32).T)
        blocks = [a[:, 512 * kh:512 * (kh + 1)] for a in blocks for kh in range(2)]
        for i, term in enumerate(_signed_sums([term[0] for term in _HK_TERMS[:7]], blocks)):
            ws_v[j // 2, i, pl.ds(64 * (j % 2), 64), :] = _pack(term)

    def paced_terms(pieces, lag):
        links = []
        for blocks, dest in pieces:
            if len(links) >= lag:
                link = jnp.concatenate([links[-lag]] * (blocks[0].shape[1] // 128), axis=1)
                blocks = [pltpu.bitcast(_bits(b) ^ jnp.concatenate([link, link], axis=0), f32)
                          for b in blocks[:1]] + blocks[1:]
            words = [_pack(term) for term in _signed_sums([t[0] for t in _HK_TERMS], blocks)]
            for i, w in enumerate(words):
                dest[i] = w
            done = functools.reduce(jnp.bitwise_or, words[4:7] + words[9:15] + words[17:])
            slow = jnp.sum(pltpu.bitcast(done, f32), axis=-1, keepdims=True)
            links.append(_bits(jnp.broadcast_to(slow, (8, 128))) & pace["zero"])

    def prepare_wo(lag):
        pieces = []
        for n in range(2):
            for c in range(4):
                for r in range(0, 128, 16):
                    w = [wo_v[pl.ds(256 * c + 128 * kh + r, 16), pl.ds(512 * n, 512)].astype(f32) for kh in range(2)]
                    pieces.append(([w[kh][:, 128 * i:128 * (i + 1)] for i in range(4) for kh in range(2)],
                                   woh_v.at[n, :, pl.ds(64 * c + r // 2, 8), :]))
        paced_terms(pieces, lag)

    def proj_group(j0, nj, t, g):
        rows = pl.ds(64 * (j0 % 2), 64 * nj)
        return dict(_block_product(
            lambda r: matmul(_unpack(ws_v[j0 // 2, r, rows, :]), _unpack(xs_v[t, g, r]), _NT), 2))

    def pairs(groups):
        return [jnp.concatenate([y[b, hf][r:r + 64] for y in groups for hf in range(2)], axis=1)
                for j in range(groups[0][0, 0].shape[0] // 128) for b in range(2)
                for r in (128 * j, 128 * j + 64)]

    def proj(j0, t):
        return pairs([proj_group(j0, 2, t, g) for g in range(2)])

    kv = [None] * 16
    phi_k = [None] * 16

    def key_features(j, p):
        phi = _features(p)
        phi_k[j] = phi.reshape(128, T).astype(bf16)
        return functools.reduce(jnp.bitwise_or, [_bits(phi[i][:, n:n + 128]) for i in (7, 15)
                                                 for n in range(0, T, 128)])

    def key_tasks(blocks, j0):
        return [None] * 5 + [functools.partial(key_features, j0 + q, p) for q, p in enumerate(blocks)]

    def kv_update(v_blocks, j0):
        for j, v in enumerate(v_blocks, j0):
            v1 = jnp.concatenate([v, jnp.ones((16, T), f32)], axis=0).astype(bf16)
            upd = _dot(v1, phi_k[j], _NT)
            kv[j] = upd if kv[j] is None else kv[j] + upd

    wait_loads()
    layernorm(0, 0, 0)
    pace["zero"] = top[1] >> 31
    wait_loads()
    prepare_w(8)
    wait_loads()
    layernorm(0, 1, 0)
    first = proj_group(8, 1, 0, 0)
    wait_loads()
    v0 = pairs([first, proj_group(8, 1, 0, 1)])
    prepare_w(9)
    first = proj_group(9, 1, 0, 0)
    wait_loads()
    v0 += pairs([first, proj_group(9, 1, 0, 1)])
    for j in (10, 11):
        prepare_w(j)
    if "0" == "0":
        v0 += pairs([proj_group(10, 1, 0, g) for g in range(2)])
        first = proj_group(11, 1, 0, 0)
        wait_loads()
        v0 += pairs([first, proj_group(11, 1, 0, 1)])
    else:
        first = proj_group(10, 2, 0, 0)
        wait_loads()
        v0 += pairs([first, proj_group(10, 2, 0, 1)])
    bd = feature_map()
    for j in (4, 5):
        prepare_w(j)
    first = proj_group(4, 2, 0, 0)
    wait_loads()
    k = pairs([first, proj_group(4, 2, 0, 1)])
    for j in (6, 7):
        prepare_w(j)
    tasks += key_tasks(k[:4], 0)
    rest, k = k[4:], proj(6, 0)
    for g in range(2):
        layernorm(1, g, 3)
    wait_loads()
    for j, p in enumerate(rest, 4):
        key_features(j, p)
    pending = [(v0[:8], 0), (v0[8:], 8)]
    j0 = 8
    for t in range(1, NT_):
        for c in range(2):
            tasks += key_tasks(k, j0)
            v = proj(8 + 2 * c, t)
            if len(pending) > 1:
                kv_update(*pending.pop(0))
            kv_update(*pending.pop(0))
            k, j0 = proj(4 + 2 * c, t), 8 * c
            pending.append((v, j0))
            if t >= 2:
                prepare_w(2 * (t - 2) + c)
        for g in range(2 if t + 1 < NT_ else 0):
            layernorm(t + 1, g, 1)
    tasks += key_tasks(k, j0)

    r_max = jnp.max(top[0])
    idx = jnp.clip(jnp.min(jnp.where(top[0] == r_max, top[1], S)), 0, S - 1)
    t_sel = idx // T
    grp = pl.ds(pl.multiple_of(idx % 128 // 16 * 8, 8), 8)
    x_sel = jnp.concatenate(
        [_unpack(xs_v[t_sel, idx % T // 256, jnp.where(idx % 256 < 128, x_block[kh], x_block[2 + kh]), grp, :])
         for kh in range(2)],
        axis=1).astype(f32)
    x_sel = jnp.where(lax.broadcasted_iota(jnp.int32, (16, D), 0) == idx % 16, x_sel, 0.0)
    x_sel = jnp.broadcast_to(jnp.sum(x_sel, axis=0, keepdims=True), (16, D)).astype(bf16)
    gate = jax.nn.sigmoid(jnp.full((8, 512), r_max, f32))

    def ffn_program():
        h = []
        for n in range(F // 128):
            acc = []
            for w in (wg_v, wu_v):
                parts = []
                for kh in range(2):
                    dep = yield
                    parts.append(_dot(after(x_sel[:, 512 * kh:512 * (kh + 1)], dep),
                                      w[pl.ds(512 * kh, 512), pl.ds(n * 128, 128)], _NN))
                    ffn["done"].append(_bits(parts[-1][:8]))
                acc.append(parts[0] + parts[1])
            h.append((_silu(acc[0]) * acc[1]).astype(bf16))
        for hf in range(2):
            y = None
            for n in range(F // 128):
                dep = yield
                part = _dot(after(h[n], dep), wd_v[pl.ds(n * 128, 128), pl.ds(hf * 512, 512)], _NN)[:8]
                y = part if y is None else y + part
                ffn["done"].append(_bits(part[:, 384:]))
            ffn["y"][hf] = _rb(y * gate)

    def attend(blocks, j0):
        out = []
        for j, p in enumerate(blocks, j0):
            num = _dot(kv[j], p, _NN)
            for hd in range(2):
                inv = _rcp(num[64 + 8 * hd:72 + 8 * hd] + 1e-6)
                out.append((num[32 * hd:32 * hd + 32].reshape(4, 8, T) * inv[None]).reshape(32, T))
        return [[[jnp.concatenate(out[8 * c + 4 * kh:8 * c + 4 * kh + 4], axis=0)[:, 256 * g:256 * (g + 1)].T
                  for kh in range(2)] for g in range(2)] for c in range(2)]

    stores = []

    def out_proj(i, o_terms, n):
        while i and ffn["y"][n] is None:
            ffn_step()
        for (c, q), block in _block_product(lambda r: matmul(o_terms[r], _unpack(woh_v[n, r]), _NN), 4):
            t, g = tiles[i + q // 2], q % 2
            cols, tok = pl.ds(512 * n + 128 * c, 128), pl.ds(pl.multiple_of(T * t + 256 * g, 256), 256)
            a = jnp.concatenate([_unpack(xs_v[t, g, x_block[2 * hf + n], :, pl.ds(128 * c, 128)])
                                 for hf in range(2)], axis=0).astype(f32)
            if i + q // 2 == NT_ - 1:
                hit = (lax.broadcasted_iota(jnp.int32, (32, 8, 128), 0) * 8
                       + lax.broadcasted_iota(jnp.int32, (32, 8, 128), 1)) == idx % T - 256 * g
                a3 = a.reshape(32, 8, 128)
                a = jnp.where(hit, a3 + ffn["y"][n][:, 128 * c:128 * (c + 1)][None], a3).reshape(256, 128)
            rows = pl.ds(T * i + 256 * q, 256)
            out_v[rows, cols] = (x_v[tok, cols].astype(f32) + block * _silu(a)).astype(bf16)
            if i and n:
                stores.extend(group(10, (out_v.at[rows, cols], out_hbm.at[tok, cols])))
                stores[-1].start()
        if (i, n) in ((0, 1), (2, 0)):
            cols = pl.ds(0, 512) if i else slice(None)
            for q in range(2):
                stores.extend(group(10, (out_v.at[pl.ds(T * (i + q), T), cols],
                                         out_hbm.at[pl.ds(pl.multiple_of(T * tiles[i + q], T), T), cols])))
                stores[-1].start()

    def output_terms(first, second):
        per_group = [_signed_sums([t[1] for t in _HK_TERMS],
                                  [b for o in (first, second) for g in range(2) for b in o[c][g]])
                     for c in range(4)]
        return [jnp.concatenate(term, axis=1).astype(bf16) for term in zip(*per_group)]

    def last_loads():
        wait_loads()
        prepare_wo(1)
        ffn["steps"], ffn["done"] = ffn_program(), [None, None]
        next(ffn["steps"])

    tiles = [lax.rem(t_sel + 1 + i, NT_) for i in range(NT_)]
    o = [[] for _ in range(NT_)]
    halves = [(i, c) for i in range(NT_) for c in range(2)]
    for h, (i, c) in enumerate(halves):
        q = proj(2 * c, tiles[i])
        if h == 0:
            kv_update(*pending.pop(0))
            row = lax.broadcasted_iota(jnp.int32, (80, 128), 0)
            col = lax.broadcasted_iota(jnp.int32, (80, 128), 1)
            own = jnp.where(row < 64, row >> 5, (row >> 3) & 1) == (col & 1)
            kv[:] = [jnp.where(own, a, 0.0).astype(bf16) for a in kv]
            tasks.extend([None] * 0 + [last_loads])
        else:
            o[halves[h - 1][0]] += attend(prev, 8 * halves[h - 1][1])
        prev = [_features(p).reshape(128, T).astype(bf16) for p in q]
        if h == 7:
            terms = output_terms(*o[:2])
            out_proj(0, terms, 0)
    out_proj(0, terms, 1)
    o[-1] += attend(prev, 8)
    terms = output_terms(*o[2:])
    for n in range(2):
        out_proj(2, terms, n)
    for c in stores:
        c.wait()


@jax.jit
def pallas_recurrent_scan__linear_kernel_hedgehog__moe_arch_mod__prompt_kernel(
    A_x: jax.Array,
    A_wqkv: jax.Array,
    A_w_phi: jax.Array,
    A_wo: jax.Array,
    B_x: jax.Array,
    B_w_r: jax.Array,
    B_w_gate: jax.Array,
    B_w_up: jax.Array,
    B_w_down: jax.Array,
):
    del B_x
    hbm = pl.BlockSpec(memory_space=pl.ANY)
    out = pl.pallas_call(
        _kernel,
        out_shape=jax.ShapeDtypeStruct((S, D), bf16),
        in_specs=[hbm] * 8,
        out_specs=hbm,
        scratch_shapes=[
            pltpu.VMEM((S, D), bf16),
            pltpu.VMEM((NT_, 2, 9, 64, 512), jnp.uint32),
            pltpu.VMEM((D, 3 * D), bf16),
            pltpu.VMEM((6, 7, 128, 512), jnp.uint32),
            pltpu.VMEM((D, D), bf16),
            pltpu.VMEM((2, 26, 256, 128), jnp.uint32),
            pltpu.VMEM((D, F), bf16),
            pltpu.VMEM((D, F), bf16),
            pltpu.VMEM((F, D), bf16),
            pltpu.VMEM((S, D), bf16),
            pltpu.VMEM((H * DH, DH), bf16),
            pltpu.VMEM((D,), bf16),
            pltpu.SemaphoreType.DMA((11,)),
        ],
        compiler_params=pltpu.CompilerParams(vmem_limit_bytes=110 * 1024 * 1024),
        name="hedgehog_mod",
    )(
        A_x.reshape(S, D), A_wqkv, A_w_phi.reshape(H * DH, DH), A_wo,
        B_w_r, B_w_gate, B_w_up, B_w_down,
    )
    return out.reshape(1, S, D)
```

```python
import functools
import math

import jax
import jax.numpy as jnp
from jax import lax
import jax.experimental.pallas as pl
import jax.experimental.pallas.tpu as pltpu

S, D, H, DH, F = 2048, 1024, 32, 32, 3584
T = 512
NT_ = S // T
LOG2E = math.log2(math.e)
_NT = (((1,), (1,)), ((), ()))
_NN = (((1,), (0,)), ((), ()))
f32, bf16 = jnp.float32, jnp.bfloat16


def _dot(a, b, dn):
    return lax.dot_general(a, b, dn, preferred_element_type=f32)


def _rb(v):
    return v.astype(bf16).astype(f32)


def _rcp(v):
    r = pl.reciprocal(v, approx=True)
    return r * (2.0 - v * r)


def _silu(a):
    return a * pl.reciprocal(1.0 + jnp.exp2(a * -LOG2E), approx=True)


def _bits(v):
    return pltpu.bitcast(v, jnp.int32)


def _pack(v):
    m, n = v.shape
    v = v.reshape(m // 16, 2, 8, n)
    return pltpu.pack_elementwise([v[:, 0], v[:, 1]], packed_dtype=bf16).reshape(m // 2, n)


def _unpack(words):
    return pltpu.bitcast(words, bf16)


_HK_TERMS = (
    ((1,), (1, -2)), ((1, 2), (2,)), ((3, 4), (3,)), ((-4,), (3, -4)),
    ((1, 4), (2, 3)), ((-1, 3), (1, 3)), ((2, -4), (2, 4)),
    ((6,), (6,)), ((5,), (5,)),
    ((-3, -4, 5), (3, -4, -6)), ((-3, -4, 5, 6), (4, 6)), ((3, -5), (3, -4, 5, -6)),
    ((1, 2, -6), (1, -2, 5)), ((-2, 6), (1, -2, 5, -6)), ((-1, -2, 5, 6), (1, 5)),
    ((7,), (7, -8)), ((7, 8), (8,)),
    ((4, 7), (3, 8)), ((3, -7), (3, 7)), ((-4, 8), (4, 8)),
    ((-6, 7, 8), (5, 7, -8)), ((6, -8), (5, -6, 7, -8)), ((5, 6, -7, -8), (5, 7)),
    ((2, -6, 7), (1, 5, 8)), ((1, -5, -7), (1, 5, 7)), ((-2, 6, 8), (2, 6, 8)),
)
_HK_SUMS = (
    ((0, 0), (2, 1)), ((1, 1), (4, 3)), ((1, 0), (6, 5, 1, -3)), ((0, 1), (7, 5, 4, -2)),
    ((2, 2), (9, 8)), ((2, 1), (11, 10, 3, -8)), ((1, 2), (12, 10, 9, -4)),
    ((0, 2), (14, 13, 8, -1)), ((2, 0), (15, 13, 2, -9)), ((3, 3), (17, 16)),
    ((1, 3), (19, 18, 16, -3)), ((3, 1), (20, 18, 4, -17)),
    ((3, 2), (22, 21, 8, -16)), ((2, 3), (23, 21, 17, -9)),
    ((0, 3), (25, 24, 16, 15), (2, 3), 1), ((3, 0), (26, 24, 14, -17), (3, 2), -1),
)
_TOKEN_GROUP = (0, 2, 3, 1)


def _signed_sums(wanted, blocks):
    known = {(i + 1,): b for i, b in enumerate(blocks)}

    def value(key):
        if key not in known:
            for part in sorted(known, key=len, reverse=True):
                for sign in (1, -1):
                    signed = [sign * p for p in part]
                    if key not in known and len(part) < len(key) and all(p in key for p in signed):
                        rest = tuple(k for k in key if k not in signed)
                        if sign > 0 and rest[0] < 0:
                            known[key] = known[part] - value(tuple(-k for k in rest))
                        else:
                            known[key] = value(rest) + known[part] if sign > 0 else value(rest) - known[part]
            if key not in known:
                known[key] = -known[(-key[0],)]
        return known[key]

    for key in sorted(wanted, key=len):
        value(key)
    return [known[key] for key in wanted]


def _block_product(product, size):
    m, y = [], {}
    for ij, parts, *earlier in _HK_SUMS[:size * size]:
        while len(m) < parts[0]:
            m.append(product(len(m)))
        total = m[parts[0] - 1]
        for p in parts[1:]:
            total = total + m[p - 1] if p > 0 else total - m[-p - 1]
        if earlier:
            total = total + y[earlier[0]] if earlier[1] > 0 else total - y[earlier[0]]
        y[ij] = total
        yield ij, total


def _allreduce(v, op):
    r = v[0]
    for i in range(1, 8):
        r = op(r, v[i])
    r = op(r, pltpu.roll(r, 4, 0))
    return op(r, pltpu.roll(r, 2, 0))


def _features(p):
    p3 = p.reshape(8, 8, p.shape[1])
    mx = _allreduce(p3, jnp.maximum)
    mn = _allreduce(p3, jnp.minimum)
    ep = jnp.exp2(p3 - mx[None])
    en = jnp.exp2(mn[None] - p3)
    ip = _rcp(_allreduce(ep, jnp.add))
    im = _rcp(_allreduce(en, jnp.add))
    return jnp.concatenate([ep * ip[None], en * im[None]], axis=0)


def _kernel(x_hbm, wqkv_hbm, wphi_hbm, wo_hbm, wr_hbm, wg_hbm, wu_hbm, wd_hbm, out_hbm,
            x_v, xs_v, wqkv_v, ws_v, wo_v, woh_v, wg_v, wu_v, wd_v, out_v, wphi_v, wr_v, sems):
    def group(k, *pairs):
        return [pltpu.make_async_copy(src, dst, sems.at[k]) for src, dst in pairs]

    def x_rows(r0, n):
        return x_hbm.at[pl.ds(r0, n)], x_v.at[pl.ds(r0, n)]

    def w_cols(j0, nj):
        cols = pl.ds(256 * j0, 256 * nj)
        return wqkv_hbm.at[:, cols], wqkv_v.at[:, cols]

    loads = [
        group(0, x_rows(0, 256), (wr_hbm, wr_v)),
        group(1, w_cols(8, 1)),
        group(2, x_rows(256, 256)),
        group(3, w_cols(9, 1)),
        group(4, w_cols(10, 2)),
        group(5, (wphi_hbm, wphi_v), w_cols(4, 2)),
        group(6, w_cols(6, 2), x_rows(T, T)),
        group(7, x_rows(2 * T, S - 2 * T), w_cols(0, 4)),
        group(9, (wo_hbm, wo_v), (wg_hbm, wg_v), (wu_hbm, wu_v), (wd_hbm, wd_v)),
    ]
    for copies in loads:
        for c in copies:
            c.start()

    def wait_loads():
        for c in loads.pop(0):
            c.wait()

    tasks = []
    pace = {}

    def after(lhs, dep):
        ok = (dep & pace["zero"]) == 0
        first = jnp.where(jnp.concatenate([ok, ok], axis=0), lhs[:16, :128], jnp.zeros((16, 128), bf16))
        if lhs.shape[1] > 128:
            first = jnp.concatenate([first, lhs[:16, 128:]], axis=1)
        return first if lhs.shape[0] == 16 else jnp.concatenate([first, lhs[16:]], axis=0)

    ffn = {"steps": None, "done": [], "y": [None, None]}

    def ffn_step():
        try:
            ffn["steps"].send(ffn["main"])
        except StopIteration:
            ffn["steps"] = None

    def matmul(lhs, rhs, dn):
        task = tasks.pop(0) if tasks else None
        dep = task() if task is not None else None
        if ffn["done"]:
            dep = ffn["done"].pop(0)
        m = _dot(lhs if dep is None else after(lhs, dep), rhs, dn)
        if ffn["steps"] is not None:
            ffn_step()
        ffn["main"] = _bits(m[-8:, -128:])
        return m

    top = [jnp.full((8, 128), -jnp.inf, f32), lax.broadcasted_iota(jnp.int32, (8, 128), 0)]
    chain = []
    x_keys = [term[1] for term in _HK_TERMS[:7]] + [(1,), (4,)]
    x_block = [x_keys.index((i + 1,)) for i in range(4)]

    def layernorm(t, g, lag):
        wr = wr_v[...].astype(f32).reshape(1, D)
        row = 2 * lax.broadcasted_iota(jnp.int32, (8, 128), 0)
        for r in range(0, 128, 16):
            xn = []
            for r0 in (T * t + 256 * g + r, T * t + 256 * g + 128 + r):
                words = pltpu.bitcast(x_v[pl.ds(r0, 16), :], jnp.uint32)
                for odd in range(2):
                    x = pltpu.unpack_elementwise(words, index=odd, packed_dtype=bf16, unpacked_dtype=f32)
                    total = x[:, :128]
                    for i in range(1, D // 128):
                        total = total + x[:, 128 * i:128 * (i + 1)]
                    if lag:
                        total = jnp.where(chain[-lag] >= 0, total, 0.0)
                    xc = x - jnp.sum(total, axis=-1, keepdims=True) * (1.0 / D)
                    v = jnp.mean(xc * xc, axis=-1, keepdims=True)
                    xn.append(xc * (1.0 / _rb(jnp.sqrt(_rb(_rb(v) + _rb(jnp.full_like(v, 1e-5)))))))
                    sc = jnp.broadcast_to(_rb(jnp.sum(xn[-1] * wr, axis=-1, keepdims=True)), (8, 128))
                    tok = row + (r0 + odd)
                    better = (sc > top[0]) | ((sc == top[0]) & (tok < top[1]))
                    top[:] = jnp.where(better, sc, top[0]), jnp.where(better, tok, top[1])
                chain.append(top[1])
            terms = [_signed_sums(x_keys, [a[:, :512], a[:, 512:], b[:, :512], b[:, 512:]])
                     for a, b in ((xn[0], xn[2]), (xn[1], xn[3]))]
            for i, pair in enumerate(zip(*terms)):
                xs_v[t, g, i, pl.ds(r // 2, 8), :] = pltpu.pack_elementwise(list(pair), packed_dtype=bf16)

    def feature_map():
        wt = wphi_v[...].astype(f32).T
        full = jnp.concatenate([wt[8 * (g % 4):8 * (g % 4) + 8] for g in range(8) for _ in range(2)], axis=0)
        row = lax.broadcasted_iota(jnp.int32, (128, D), 0)
        col = lax.broadcasted_iota(jnp.int32, (128, D), 1)
        same = (((row >> 6) << 1) | ((row >> 3) & 1)) == ((col >> 5) & 3)
        return jnp.where(same, full, 0.0).astype(bf16)

    def prepare_w(j):
        blocks = []
        for c in (2 * j, 2 * j + 1):
            w = wqkv_v[:, pl.ds(128 * c, 128)]
            if j < 8:
                blocks.append(_dot(bd[:, 128 * (c % 8):128 * (c % 8 + 1)], w, _NT) * LOG2E)
            else:
                blocks.append(w.astype(f32).T)
        blocks = [a[:, 512 * kh:512 * (kh + 1)] for a in blocks for kh in range(2)]
        for i, term in enumerate(_signed_sums([term[0] for term in _HK_TERMS[:7]], blocks)):
            ws_v[j // 2, i, pl.ds(64 * (j % 2), 64), :] = _pack(term)

    def paced_terms(pieces, lag):
        links = []
        for blocks, dest in pieces:
            if len(links) >= lag:
                link = jnp.concatenate([links[-lag]] * (blocks[0].shape[1] // 128), axis=1)
                blocks = [pltpu.bitcast(_bits(b) ^ jnp.concatenate([link, link], axis=0), f32)
                          for b in blocks[:1]] + blocks[1:]
            words = [_pack(term) for term in _signed_sums([t[0] for t in _HK_TERMS], blocks)]
            for i, w in enumerate(words):
                dest[i] = w
            done = functools.reduce(jnp.bitwise_or, words[4:7] + words[9:15] + words[17:])
            slow = jnp.sum(pltpu.bitcast(done, f32), axis=-1, keepdims=True)
            links.append(_bits(jnp.broadcast_to(slow, (8, 128))) & pace["zero"])

    def prepare_wo(lag):
        pieces = []
        for n in range(2):
            for c in range(4):
                for r in range(0, 128, 16):
                    w = [wo_v[pl.ds(256 * c + 128 * kh + r, 16), pl.ds(512 * n, 512)].astype(f32) for kh in range(2)]
                    pieces.append(([w[kh][:, 128 * i:128 * (i + 1)] for i in range(4) for kh in range(2)],
                                   woh_v.at[n, :, pl.ds(64 * c + r // 2, 8), :]))
        paced_terms(pieces, lag)

    def proj_group(j0, nj, t, g):
        rows = pl.ds(64 * (j0 % 2), 64 * nj)
        return dict(_block_product(
            lambda r: matmul(_unpack(ws_v[j0 // 2, r, rows, :]), _unpack(xs_v[t, g, r]), _NT), 2))

    def pairs(groups):
        return [jnp.concatenate([y[b, hf][r:r + 64] for y in groups for hf in range(2)], axis=1)
                for j in range(groups[0][0, 0].shape[0] // 128) for b in range(2)
                for r in (128 * j, 128 * j + 64)]

    def proj(j0, t):
        return pairs([proj_group(j0, 2, t, g) for g in range(2)])

    kv = [None] * 16
    phi_k = [None] * 16

    def key_features(j, p):
        phi = _features(p)
        phi_k[j] = phi.reshape(128, T).astype(bf16)
        return functools.reduce(jnp.bitwise_or, [_bits(phi[i][:, n:n + 128]) for i in (7, 15)
                                                 for n in range(0, T, 128)])

    def key_tasks(blocks, j0):
        return [None] * 5 + [functools.partial(key_features, j0 + q, p) for q, p in enumerate(blocks)]

    def kv_update(v_blocks, j0):
        for j, v in enumerate(v_blocks, j0):
            v1 = jnp.concatenate([v, jnp.ones((16, T), f32)], axis=0).astype(bf16)
            upd = _dot(v1, phi_k[j], _NT)
            kv[j] = upd if kv[j] is None else kv[j] + upd

    wait_loads()
    layernorm(0, 0, 0)
    pace["zero"] = top[1] >> 31
    wait_loads()
    prepare_w(8)
    wait_loads()
    layernorm(0, 1, 0)
    first = proj_group(8, 1, 0, 0)
    wait_loads()
    v0 = pairs([first, proj_group(8, 1, 0, 1)])
    prepare_w(9)
    first = proj_group(9, 1, 0, 0)
    wait_loads()
    v0 += pairs([first, proj_group(9, 1, 0, 1)])
    for j in (10, 11):
        prepare_w(j)
    if "0" == "0":
        v0 += pairs([proj_group(10, 1, 0, g) for g in range(2)])
        first = proj_group(11, 1, 0, 0)
        wait_loads()
        v0 += pairs([first, proj_group(11, 1, 0, 1)])
    else:
        first = proj_group(10, 2, 0, 0)
        wait_loads()
        v0 += pairs([first, proj_group(10, 2, 0, 1)])
    bd = feature_map()
    for j in (4, 5):
        prepare_w(j)
    first = proj_group(4, 2, 0, 0)
    wait_loads()
    k = pairs([first, proj_group(4, 2, 0, 1)])
    for j in (6, 7):
        prepare_w(j)
    tasks += key_tasks(k[:4], 0)
    rest, k = k[4:], proj(6, 0)
    for g in range(2):
        layernorm(1, g, 3)
    wait_loads()
    for j, p in enumerate(rest, 4):
        key_features(j, p)
    pending = [(v0[:8], 0), (v0[8:], 8)]
    j0 = 8
    for t in range(1, NT_):
        for c in range(2):
            tasks += key_tasks(k, j0)
            v = proj(8 + 2 * c, t)
            if len(pending) > 1:
                kv_update(*pending.pop(0))
            kv_update(*pending.pop(0))
            k, j0 = proj(4 + 2 * c, t), 8 * c
            pending.append((v, j0))
            if t >= 2:
                prepare_w(2 * (t - 2) + c)
        for g in range(2 if t + 1 < NT_ else 0):
            layernorm(t + 1, g, 1)
    tasks += key_tasks(k, j0)

    r_max = jnp.max(top[0])
    idx = jnp.clip(jnp.min(jnp.where(top[0] == r_max, top[1], S)), 0, S - 1)
    t_sel = idx // T
    grp = pl.ds(pl.multiple_of(idx % 128 // 16 * 8, 8), 8)
    x_sel = jnp.concatenate(
        [_unpack(xs_v[t_sel, idx % T // 256, jnp.where(idx % 256 < 128, x_block[kh], x_block[2 + kh]), grp, :])
         for kh in range(2)],
        axis=1).astype(f32)
    x_sel = jnp.where(lax.broadcasted_iota(jnp.int32, (16, D), 0) == idx % 16, x_sel, 0.0)
    x_sel = jnp.broadcast_to(jnp.sum(x_sel, axis=0, keepdims=True), (16, D)).astype(bf16)
    gate = jax.nn.sigmoid(jnp.full((8, 512), r_max, f32))

    def ffn_program():
        h = []
        for n in range(F // 128):
            acc = []
            for w in (wg_v, wu_v):
                parts = []
                for kh in range(2):
                    dep = yield
                    parts.append(_dot(after(x_sel[:, 512 * kh:512 * (kh + 1)], dep),
                                      w[pl.ds(512 * kh, 512), pl.ds(n * 128, 128)], _NN))
                    ffn["done"].append(_bits(parts[-1][:8]))
                acc.append(parts[0] + parts[1])
            h.append((_silu(acc[0]) * acc[1]).astype(bf16))
        for hf in range(2):
            y = None
            for n in range(F // 128):
                dep = yield
                part = _dot(after(h[n], dep), wd_v[pl.ds(n * 128, 128), pl.ds(hf * 512, 512)], _NN)[:8]
                y = part if y is None else y + part
                ffn["done"].append(_bits(part[:, 384:]))
            ffn["y"][hf] = _rb(y * gate)

    def attend(blocks, j0):
        out = []
        for j, p in enumerate(blocks, j0):
            num = _dot(kv[j], p, _NN)
            for hd in range(2):
                inv = _rcp(num[64 + 8 * hd:72 + 8 * hd] + 1e-6)
                out.append((num[32 * hd:32 * hd + 32].reshape(4, 8, T) * inv[None]).reshape(32, T))
        return [[[jnp.concatenate(out[8 * c + 4 * kh:8 * c + 4 * kh + 4], axis=0)[:, 256 * g:256 * (g + 1)].T
                  for kh in range(2)] for g in range(2)] for c in range(2)]

    stores = []

    def out_proj(i, o_terms, n):
        while i and ffn["y"][n] is None:
            ffn_step()
        for (c, j), block in _block_product(lambda r: matmul(o_terms[r], _unpack(woh_v[n, r]), _NN), 4):
            q = _TOKEN_GROUP[j]
            t, g = tiles[i + q // 2], q % 2
            cols, tok = pl.ds(512 * n + 128 * c, 128), pl.ds(pl.multiple_of(T * t + 256 * g, 256), 256)
            a = jnp.concatenate([_unpack(xs_v[t, g, x_block[2 * hf + n], :, pl.ds(128 * c, 128)])
                                 for hf in range(2)], axis=0).astype(f32)
            if i + q // 2 == NT_ - 1:
                hit = (lax.broadcasted_iota(jnp.int32, (32, 8, 128), 0) * 8
                       + lax.broadcasted_iota(jnp.int32, (32, 8, 128), 1)) == idx % T - 256 * g
                a3 = a.reshape(32, 8, 128)
                a = jnp.where(hit, a3 + ffn["y"][n][:, 128 * c:128 * (c + 1)][None], a3).reshape(256, 128)
            rows = pl.ds(T * i + 256 * q, 256)
            out_v[rows, cols] = (x_v[tok, cols].astype(f32) + block * _silu(a)).astype(bf16)
            if i and n:
                stores.extend(group(10, (out_v.at[rows, cols], out_hbm.at[tok, cols])))
                stores[-1].start()
        if (i, n) in ((0, 1), (2, 0)):
            cols = pl.ds(0, 512) if i else slice(None)
            for q in range(2):
                stores.extend(group(10, (out_v.at[pl.ds(T * (i + q), T), cols],
                                         out_hbm.at[pl.ds(pl.multiple_of(T * tiles[i + q], T), T), cols])))
                stores[-1].start()

    def output_terms(first, second):
        per_group = [_signed_sums([t[1] for t in _HK_TERMS],
                                  [b for q in _TOKEN_GROUP for b in (first, second)[q // 2][c][q % 2]])
                     for c in range(4)]
        return [jnp.concatenate(term, axis=1).astype(bf16) for term in zip(*per_group)]

    def last_loads():
        wait_loads()
        prepare_wo(1)
        ffn["steps"], ffn["done"] = ffn_program(), [None, None]
        next(ffn["steps"])

    tiles = [lax.rem(t_sel + 1 + i, NT_) for i in range(NT_)]
    o = [[] for _ in range(NT_)]
    halves = [(i, c) for i in range(NT_) for c in range(2)]
    for h, (i, c) in enumerate(halves):
        q = proj(2 * c, tiles[i])
        if h == 0:
            kv_update(*pending.pop(0))
            row = lax.broadcasted_iota(jnp.int32, (80, 128), 0)
            col = lax.broadcasted_iota(jnp.int32, (80, 128), 1)
            own = jnp.where(row < 64, row >> 5, (row >> 3) & 1) == (col & 1)
            kv[:] = [jnp.where(own, a, 0.0).astype(bf16) for a in kv]
            tasks.extend([None] * 0 + [last_loads])
        else:
            o[halves[h - 1][0]] += attend(prev, 8 * halves[h - 1][1])
        prev = [_features(p).reshape(128, T).astype(bf16) for p in q]
        if h == 7:
            terms = output_terms(*o[:2])
            out_proj(0, terms, 0)
    out_proj(0, terms, 1)
    o[-1] += attend(prev, 8)
    terms = output_terms(*o[2:])
    for n in range(2):
        out_proj(2, terms, n)
    for c in stores:
        c.wait()


@jax.jit
def pallas_recurrent_scan__linear_kernel_hedgehog__moe_arch_mod__prompt_kernel(
    A_x: jax.Array,
    A_wqkv: jax.Array,
    A_w_phi: jax.Array,
    A_wo: jax.Array,
    B_x: jax.Array,
    B_w_r: jax.Array,
    B_w_gate: jax.Array,
    B_w_up: jax.Array,
    B_w_down: jax.Array,
):
    del B_x
    hbm = pl.BlockSpec(memory_space=pl.ANY)
    out = pl.pallas_call(
        _kernel,
        out_shape=jax.ShapeDtypeStruct((S, D), bf16),
        in_specs=[hbm] * 8,
        out_specs=hbm,
        scratch_shapes=[
            pltpu.VMEM((S, D), bf16),
            pltpu.VMEM((NT_, 2, 9, 64, 512), jnp.uint32),
            pltpu.VMEM((D, 3 * D), bf16),
            pltpu.VMEM((6, 7, 128, 512), jnp.uint32),
            pltpu.VMEM((D, D), bf16),
            pltpu.VMEM((2, 26, 256, 128), jnp.uint32),
            pltpu.VMEM((D, F), bf16),
            pltpu.VMEM((D, F), bf16),
            pltpu.VMEM((F, D), bf16),
            pltpu.VMEM((S, D), bf16),
            pltpu.VMEM((H * DH, DH), bf16),
            pltpu.VMEM((D,), bf16),
            pltpu.SemaphoreType.DMA((11,)),
        ],
        compiler_params=pltpu.CompilerParams(vmem_limit_bytes=110 * 1024 * 1024),
        name="hedgehog_mod",
    )(
        A_x.reshape(S, D), A_wqkv, A_w_phi.reshape(H * DH, DH), A_wo,
        B_w_r, B_w_gate, B_w_up, B_w_down,
    )
    return out.reshape(1, S, D)
```

```python
import functools
import math

import jax
import jax.numpy as jnp
from jax import lax
import jax.experimental.pallas as pl
import jax.experimental.pallas.tpu as pltpu

S, D, H, DH, F = 2048, 1024, 32, 32, 3584
T = 512
NT_ = S // T
LOG2E = math.log2(math.e)
_NT = (((1,), (1,)), ((), ()))
_NN = (((1,), (0,)), ((), ()))
f32, bf16 = jnp.float32, jnp.bfloat16


def _dot(a, b, dn):
    return lax.dot_general(a, b, dn, preferred_element_type=f32)


def _rb(v):
    return v.astype(bf16).astype(f32)


def _rcp(v):
    r = pl.reciprocal(v, approx=True)
    return r * (2.0 - v * r)


def _silu(a):
    return a * pl.reciprocal(1.0 + jnp.exp2(a * -LOG2E), approx=True)


def _bits(v):
    return pltpu.bitcast(v, jnp.int32)


def _pack(v):
    m, n = v.shape
    v = v.reshape(m // 16, 2, 8, n)
    return pltpu.pack_elementwise([v[:, 0], v[:, 1]], packed_dtype=bf16).reshape(m // 2, n)


def _unpack(words):
    return pltpu.bitcast(words, bf16)


_HK_TERMS = (
    ((1,), (1, -2)), ((1, 2), (2,)), ((3, 4), (3,)), ((-4,), (3, -4)),
    ((1, 4), (2, 3)), ((-1, 3), (1, 3)), ((2, -4), (2, 4)),
    ((6,), (6,)), ((5,), (5,)),
    ((-3, -4, 5), (3, -4, -6)), ((-3, -4, 5, 6), (4, 6)), ((3, -5), (3, -4, 5, -6)),
    ((1, 2, -6), (1, -2, 5)), ((-2, 6), (1, -2, 5, -6)), ((-1, -2, 5, 6), (1, 5)),
    ((7,), (7, -8)), ((7, 8), (8,)),
    ((4, 7), (3, 8)), ((3, -7), (3, 7)), ((-4, 8), (4, 8)),
    ((-6, 7, 8), (5, 7, -8)), ((6, -8), (5, -6, 7, -8)), ((5, 6, -7, -8), (5, 7)),
    ((2, -6, 7), (1, 5, 8)), ((1, -5, -7), (1, 5, 7)), ((-2, 6, 8), (2, 6, 8)),
)
_HK_SUMS = (
    ((0, 0), (2, 1)), ((1, 1), (4, 3)), ((1, 0), (6, 5, 1, -3)), ((0, 1), (7, 5, 4, -2)),
    ((2, 2), (9, 8)), ((2, 1), (11, 10, 3, -8)), ((1, 2), (12, 10, 9, -4)),
    ((0, 2), (14, 13, 8, -1)), ((2, 0), (15, 13, 2, -9)), ((3, 3), (17, 16)),
    ((1, 3), (19, 18, 16, -3)), ((3, 1), (20, 18, 4, -17)),
    ((3, 2), (22, 21, 8, -16)), ((2, 3), (23, 21, 17, -9)),
    ((0, 3), (25, 24, 16, 15), (2, 3), 1), ((3, 0), (26, 24, 14, -17), (3, 2), -1),
)
_TOKEN_GROUP = (0, 2, 3, 1)


def _signed_sums(wanted, blocks):
    known = {(i + 1,): b for i, b in enumerate(blocks)}

    def value(key):
        if key not in known:
            for part in sorted(known, key=len, reverse=True):
                for sign in (1, -1):
                    signed = [sign * p for p in part]
                    if key not in known and len(part) < len(key) and all(p in key for p in signed):
                        rest = tuple(k for k in key if k not in signed)
                        if sign > 0 and rest[0] < 0:
                            known[key] = known[part] - value(tuple(-k for k in rest))
                        else:
                            known[key] = value(rest) + known[part] if sign > 0 else value(rest) - known[part]
            if key not in known:
                known[key] = -known[(-key[0],)]
        return known[key]

    for key in sorted(wanted, key=len):
        value(key)
    return [known[key] for key in wanted]


def _block_product(product, size):
    m, y = [], {}
    for ij, parts, *earlier in _HK_SUMS[:size * size]:
        while len(m) < parts[0]:
            m.append(product(len(m)))
        total = m[parts[0] - 1]
        for p in parts[1:]:
            total = total + m[p - 1] if p > 0 else total - m[-p - 1]
        if earlier:
            total = total + y[earlier[0]] if earlier[1] > 0 else total - y[earlier[0]]
        y[ij] = total
        yield ij, total


def _allreduce(v, op):
    r = v[0]
    for i in range(1, 8):
        r = op(r, v[i])
    r = op(r, pltpu.roll(r, 4, 0))
    return op(r, pltpu.roll(r, 2, 0))


def _features(p):
    p3 = p.reshape(8, 8, p.shape[1])
    mx = _allreduce(p3, jnp.maximum)
    mn = _allreduce(p3, jnp.minimum)
    ep = jnp.exp2(p3 - mx[None])
    en = jnp.exp2(mn[None] - p3)
    ip = _rcp(_allreduce(ep, jnp.add))
    im = _rcp(_allreduce(en, jnp.add))
    return jnp.concatenate([ep * ip[None], en * im[None]], axis=0)


def _kernel(x_hbm, wqkv_hbm, wphi_hbm, wo_hbm, wr_hbm, wg_hbm, wu_hbm, wd_hbm, out_hbm,
            x_v, xs_v, wqkv_v, ws_v, wo_v, woh_v, wg_v, wu_v, wd_v, out_v, wphi_v, wr_v, sems):
    def group(k, *pairs):
        return [pltpu.make_async_copy(src, dst, sems.at[k]) for src, dst in pairs]

    def x_rows(r0, n):
        return x_hbm.at[pl.ds(r0, n)], x_v.at[pl.ds(r0, n)]

    def w_cols(j0, nj):
        cols = pl.ds(256 * j0, 256 * nj)
        return wqkv_hbm.at[:, cols], wqkv_v.at[:, cols]

    loads = [
        group(0, x_rows(0, 256), (wr_hbm, wr_v)),
        group(1, w_cols(8, 1)),
        group(2, x_rows(256, 256)),
        group(3, w_cols(9, 1)),
        group(4, w_cols(10, 2)),
        group(5, (wphi_hbm, wphi_v), w_cols(4, 2)),
        group(6, w_cols(6, 2), x_rows(T, T)),
        group(7, x_rows(2 * T, S - 2 * T), w_cols(0, 4)),
        group(9, (wo_hbm, wo_v), (wg_hbm, wg_v), (wu_hbm, wu_v), (wd_hbm, wd_v)),
    ]
    for copies in loads:
        for c in copies:
            c.start()

    def wait_loads():
        for c in loads.pop(0):
            c.wait()

    tasks = []
    pace = {}

    def after(v, dep):
        first = pltpu.bitcast(_bits(v[:8, :128]) ^ (dep & pace["zero"]), v.dtype)
        if v.shape[1] > 128:
            first = jnp.concatenate([first, v[:8, 128:]], axis=1)
        return jnp.concatenate([first, v[8:]], axis=0)

    ffn = {"steps": None, "done": [], "y": [None, None]}

    def ffn_step():
        try:
            ffn["steps"].send(ffn["main"])
        except StopIteration:
            ffn["steps"] = None

    def matmul(lhs, rhs, dn):
        task = tasks.pop(0) if tasks else None
        dep = task() if task is not None else None
        if ffn["done"]:
            dep = ffn["done"].pop(0)
        if dep is not None:
            lhs = after(lhs, dep)
        m = _dot(lhs.astype(bf16) if lhs.dtype == f32 else _unpack(lhs), _unpack(rhs), dn)
        if ffn["steps"] is not None:
            ffn_step()
        ffn["main"] = _bits(m[-8:, -128:])
        return m

    top = [jnp.full((8, 128), -jnp.inf, f32), lax.broadcasted_iota(jnp.int32, (8, 128), 0)]
    chain = []
    x_keys = [term[1] for term in _HK_TERMS[:7]] + [(1,), (4,)]
    x_block = [x_keys.index((i + 1,)) for i in range(4)]

    def layernorm(t, g, lag):
        wr = wr_v[...].astype(f32).reshape(1, D)
        row = 2 * lax.broadcasted_iota(jnp.int32, (8, 128), 0)
        for r in range(0, 128, 16):
            xn = []
            for r0 in (T * t + 256 * g + r, T * t + 256 * g + 128 + r):
                words = pltpu.bitcast(x_v[pl.ds(r0, 16), :], jnp.uint32)
                for odd in range(2):
                    x = pltpu.unpack_elementwise(words, index=odd, packed_dtype=bf16, unpacked_dtype=f32)
                    total = x[:, :128]
                    for i in range(1, D // 128):
                        total = total + x[:, 128 * i:128 * (i + 1)]
                    if lag:
                        total = jnp.where(chain[-lag] >= 0, total, 0.0)
                    xc = x - jnp.sum(total, axis=-1, keepdims=True) * (1.0 / D)
                    v = jnp.mean(xc * xc, axis=-1, keepdims=True)
                    xn.append(xc * (1.0 / _rb(jnp.sqrt(_rb(_rb(v) + _rb(jnp.full_like(v, 1e-5)))))))
                    sc = jnp.broadcast_to(_rb(jnp.sum(xn[-1] * wr, axis=-1, keepdims=True)), (8, 128))
                    tok = row + (r0 + odd)
                    better = (sc > top[0]) | ((sc == top[0]) & (tok < top[1]))
                    top[:] = jnp.where(better, sc, top[0]), jnp.where(better, tok, top[1])
                chain.append(top[1])
            terms = [_signed_sums(x_keys, [a[:, :512], a[:, 512:], b[:, :512], b[:, 512:]])
                     for a, b in ((xn[0], xn[2]), (xn[1], xn[3]))]
            for i, pair in enumerate(zip(*terms)):
                xs_v[t, g, i, pl.ds(r // 2, 8), :] = pltpu.pack_elementwise(list(pair), packed_dtype=bf16)

    def feature_map():
        wt = wphi_v[...].astype(f32).T
        full = jnp.concatenate([wt[8 * (g % 4):8 * (g % 4) + 8] for g in range(8) for _ in range(2)], axis=0)
        row = lax.broadcasted_iota(jnp.int32, (128, D), 0)
        col = lax.broadcasted_iota(jnp.int32, (128, D), 1)
        same = (((row >> 6) << 1) | ((row >> 3) & 1)) == ((col >> 5) & 3)
        return jnp.where(same, full, 0.0).astype(bf16)

    def prepare_w(j):
        blocks = []
        for c in (2 * j, 2 * j + 1):
            w = wqkv_v[:, pl.ds(128 * c, 128)]
            if j < 8:
                blocks.append(_dot(bd[:, 128 * (c % 8):128 * (c % 8 + 1)], w, _NT) * LOG2E)
            else:
                blocks.append(w.astype(f32).T)
        blocks = [a[:, 512 * kh:512 * (kh + 1)] for a in blocks for kh in range(2)]
        for i, term in enumerate(_signed_sums([term[0] for term in _HK_TERMS[:7]], blocks)):
            ws_v[j // 2, i, pl.ds(64 * (j % 2), 64), :] = _pack(term)

    def paced_terms(pieces, lag):
        links = []
        for blocks, dest in pieces:
            if len(links) >= lag:
                first = blocks[0]
                blocks = [pltpu.bitcast(_bits(first) ^ jnp.concatenate([links[-lag]] * 2, axis=0), f32)] + blocks[1:]
            words = [_pack(term) for term in _signed_sums([t[0] for t in _HK_TERMS], blocks)]
            for i, w in enumerate(words):
                dest[i] = w
            done = functools.reduce(jnp.bitwise_or, words[4:7] + words[9:15] + words[17:])
            slow = jnp.sum(pltpu.bitcast(done, f32), axis=-1, keepdims=True)
            links.append(_bits(jnp.broadcast_to(slow, (8, 128))) & pace["zero"])

    def prepare_wo(lag):
        pieces = []
        for n in range(2):
            for c in range(4):
                for r in range(0, 128, 16):
                    w = [wo_v[pl.ds(256 * c + 128 * kh + r, 16), pl.ds(512 * n, 512)].astype(f32) for kh in range(2)]
                    pieces.append(([w[kh][:, 128 * i:128 * (i + 1)] for i in range(4) for kh in range(2)],
                                   woh_v.at[n, :, pl.ds(64 * c + r // 2, 8), :]))
        paced_terms(pieces, lag)

    def proj_group(j0, nj, t, g):
        rows = pl.ds(64 * (j0 % 2), 64 * nj)
        return dict(_block_product(
            lambda r: matmul(ws_v[j0 // 2, r, rows, :], xs_v[t, g, r], _NT), 2))

    def pairs(groups):
        return [jnp.concatenate([y[b, hf][r:r + 64] for y in groups for hf in range(2)], axis=1)
                for j in range(groups[0][0, 0].shape[0] // 128) for b in range(2)
                for r in (128 * j, 128 * j + 64)]

    def proj(j0, t):
        return pairs([proj_group(j0, 2, t, g) for g in range(2)])

    kv = [None] * 16
    phi_k = [None] * 16

    def key_features(j, p):
        phi = _features(p)
        phi_k[j] = phi.reshape(128, T).astype(bf16)
        return functools.reduce(jnp.bitwise_or, [_bits(phi[i][:, n:n + 128]) for i in (7, 15)
                                                 for n in range(0, T, 128)])

    def key_tasks(blocks, j0):
        return [None] * 5 + [functools.partial(key_features, j0 + q, p) for q, p in enumerate(blocks)]

    def kv_update(v_blocks, j0):
        for j, v in enumerate(v_blocks, j0):
            v1 = jnp.concatenate([v, jnp.ones((16, T), f32)], axis=0).astype(bf16)
            upd = _dot(v1, phi_k[j], _NT)
            kv[j] = upd if kv[j] is None else kv[j] + upd

    wait_loads()
    layernorm(0, 0, 0)
    pace["zero"] = top[1] >> 31
    wait_loads()
    prepare_w(8)
    wait_loads()
    layernorm(0, 1, 0)
    first = proj_group(8, 1, 0, 0)
    wait_loads()
    v0 = pairs([first, proj_group(8, 1, 0, 1)])
    prepare_w(9)
    first = proj_group(9, 1, 0, 0)
    wait_loads()
    v0 += pairs([first, proj_group(9, 1, 0, 1)])
    for j in (10, 11):
        prepare_w(j)
    if "0" == "0":
        v0 += pairs([proj_group(10, 1, 0, g) for g in range(2)])
        first = proj_group(11, 1, 0, 0)
        wait_loads()
        v0 += pairs([first, proj_group(11, 1, 0, 1)])
    else:
        first = proj_group(10, 2, 0, 0)
        wait_loads()
        v0 += pairs([first, proj_group(10, 2, 0, 1)])
    bd = feature_map()
    for j in (4, 5):
        prepare_w(j)
    first = proj_group(4, 2, 0, 0)
    wait_loads()
    k = pairs([first, proj_group(4, 2, 0, 1)])
    for j in (6, 7):
        prepare_w(j)
    tasks += key_tasks(k[:4], 0)
    rest, k = k[4:], proj(6, 0)
    for g in range(2):
        layernorm(1, g, 3)
    wait_loads()
    for j, p in enumerate(rest, 4):
        key_features(j, p)
    pending = [(v0[:8], 0), (v0[8:], 8)]
    j0 = 8
    for t in range(1, NT_):
        for c in range(2):
            tasks += key_tasks(k, j0)
            v = proj(8 + 2 * c, t)
            if len(pending) > 1:
                kv_update(*pending.pop(0))
            kv_update(*pending.pop(0))
            k, j0 = proj(4 + 2 * c, t), 8 * c
            pending.append((v, j0))
            if t >= 2:
                prepare_w(2 * (t - 2) + c)
        for g in range(2 if t + 1 < NT_ else 0):
            layernorm(t + 1, g, 1)
    tasks += key_tasks(k, j0)

    r_max = jnp.max(top[0])
    idx = jnp.clip(jnp.min(jnp.where(top[0] == r_max, top[1], S)), 0, S - 1)
    t_sel = idx // T
    grp = pl.ds(pl.multiple_of(idx % 128 // 16 * 8, 8), 8)
    x_sel = jnp.concatenate(
        [_unpack(xs_v[t_sel, idx % T // 256, jnp.where(idx % 256 < 128, x_block[kh], x_block[2 + kh]), grp, :])
         for kh in range(2)],
        axis=1).astype(f32)
    x_sel = jnp.where(lax.broadcasted_iota(jnp.int32, (16, D), 0) == idx % 16, x_sel, 0.0)
    x_sel = jnp.broadcast_to(jnp.sum(x_sel, axis=0, keepdims=True), (16, D))
    gate = jax.nn.sigmoid(jnp.full((8, 512), r_max, f32))

    def ffn_program():
        h = []
        for n in range(F // 128):
            acc = []
            for w in (wg_v, wu_v):
                parts = []
                for kh in range(2):
                    dep = yield
                    parts.append(_dot(after(x_sel[:, 512 * kh:512 * (kh + 1)], dep).astype(bf16),
                                      w[pl.ds(512 * kh, 512), pl.ds(n * 128, 128)], _NN))
                    ffn["done"].append(_bits(parts[-1][:8]))
                acc.append(parts[0] + parts[1])
            h.append(_silu(acc[0]) * acc[1])
        for hf in range(2):
            y = None
            for n in range(F // 128):
                dep = yield
                part = _dot(after(h[n], dep).astype(bf16), wd_v[pl.ds(n * 128, 128), pl.ds(hf * 512, 512)], _NN)[:8]
                y = part if y is None else y + part
                ffn["done"].append(_bits(part[:, 384:]))
            ffn["y"][hf] = _rb(y * gate)

    def attend(blocks, j0):
        out = []
        for j, p in enumerate(blocks, j0):
            num = _dot(kv[j], p, _NN)
            for hd in range(2):
                inv = _rcp(num[64 + 8 * hd:72 + 8 * hd] + 1e-6)
                out.append((num[32 * hd:32 * hd + 32].reshape(4, 8, T) * inv[None]).reshape(32, T))
        return [[[jnp.concatenate(out[8 * c + 4 * kh:8 * c + 4 * kh + 4], axis=0)[:, 256 * g:256 * (g + 1)].T
                  for kh in range(2)] for g in range(2)] for c in range(2)]

    stores = []

    def out_proj(i, o_terms, n):
        while i and ffn["y"][n] is None:
            ffn_step()
        for (c, j), block in _block_product(lambda r: matmul(o_terms[r], woh_v[n, r], _NN), 4):
            q = _TOKEN_GROUP[j]
            t, g = tiles[i + q // 2], q % 2
            cols, tok = pl.ds(512 * n + 128 * c, 128), pl.ds(pl.multiple_of(T * t + 256 * g, 256), 256)
            a = jnp.concatenate([_unpack(xs_v[t, g, x_block[2 * hf + n], :, pl.ds(128 * c, 128)])
                                 for hf in range(2)], axis=0).astype(f32)
            if i + q // 2 == NT_ - 1:
                hit = (lax.broadcasted_iota(jnp.int32, (32, 8, 128), 0) * 8
                       + lax.broadcasted_iota(jnp.int32, (32, 8, 128), 1)) == idx % T - 256 * g
                a3 = a.reshape(32, 8, 128)
                a = jnp.where(hit, a3 + ffn["y"][n][:, 128 * c:128 * (c + 1)][None], a3).reshape(256, 128)
            rows = pl.ds(T * i + 256 * q, 256)
            out_v[rows, cols] = (x_v[tok, cols].astype(f32) + block * _silu(a)).astype(bf16)
            if i and n:
                stores.extend(group(10, (out_v.at[rows, cols], out_hbm.at[tok, cols])))
                stores[-1].start()
        if (i, n) in ((0, 1), (2, 0)):
            cols = pl.ds(0, 512) if i else slice(None)
            for q in range(2):
                stores.extend(group(10, (out_v.at[pl.ds(T * (i + q), T), cols],
                                         out_hbm.at[pl.ds(pl.multiple_of(T * tiles[i + q], T), T), cols])))
                stores[-1].start()

    def output_terms(first, second):
        per_group = [_signed_sums([t[1] for t in _HK_TERMS],
                                  [b for q in _TOKEN_GROUP for b in (first, second)[q // 2][c][q % 2]])
                     for c in range(4)]
        return [jnp.concatenate(term, axis=1) for term in zip(*per_group)]

    def last_loads():
        wait_loads()
        prepare_wo(1)
        ffn["steps"], ffn["done"] = ffn_program(), [None, None]
        next(ffn["steps"])

    tiles = [lax.rem(t_sel + 1 + i, NT_) for i in range(NT_)]
    o = [[] for _ in range(NT_)]
    halves = [(i, c) for i in range(NT_) for c in range(2)]
    for h, (i, c) in enumerate(halves):
        q = proj(2 * c, tiles[i])
        if h == 0:
            kv_update(*pending.pop(0))
            row = lax.broadcasted_iota(jnp.int32, (80, 128), 0)
            col = lax.broadcasted_iota(jnp.int32, (80, 128), 1)
            own = jnp.where(row < 64, row >> 5, (row >> 3) & 1) == (col & 1)
            kv[:] = [jnp.where(own, a, 0.0).astype(bf16) for a in kv]
            tasks.extend([None] * 0 + [last_loads])
        else:
            o[halves[h - 1][0]] += attend(prev, 8 * halves[h - 1][1])
        prev = [_features(p).reshape(128, T).astype(bf16) for p in q]
        if h == 6:
            terms = output_terms(*o[:2])
            out_proj(0, terms, 0)
    out_proj(0, terms, 1)
    o[-1] += attend(prev, 8)
    terms = output_terms(*o[2:])
    for n in range(2):
        out_proj(2, terms, n)
    for c in stores:
        c.wait()


@jax.jit
def pallas_recurrent_scan__linear_kernel_hedgehog__moe_arch_mod__prompt_kernel(
    A_x: jax.Array,
    A_wqkv: jax.Array,
    A_w_phi: jax.Array,
    A_wo: jax.Array,
    B_x: jax.Array,
    B_w_r: jax.Array,
    B_w_gate: jax.Array,
    B_w_up: jax.Array,
    B_w_down: jax.Array,
):
    del B_x
    hbm = pl.BlockSpec(memory_space=pl.ANY)
    out = pl.pallas_call(
        _kernel,
        out_shape=jax.ShapeDtypeStruct((S, D), bf16),
        in_specs=[hbm] * 8,
        out_specs=hbm,
        scratch_shapes=[
            pltpu.VMEM((S, D), bf16),
            pltpu.VMEM((NT_, 2, 9, 64, 512), jnp.uint32),
            pltpu.VMEM((D, 3 * D), bf16),
            pltpu.VMEM((6, 7, 128, 512), jnp.uint32),
            pltpu.VMEM((D, D), bf16),
            pltpu.VMEM((2, 26, 256, 128), jnp.uint32),
            pltpu.VMEM((D, F), bf16),
            pltpu.VMEM((D, F), bf16),
            pltpu.VMEM((F, D), bf16),
            pltpu.VMEM((S, D), bf16),
            pltpu.VMEM((H * DH, DH), bf16),
            pltpu.VMEM((D,), bf16),
            pltpu.SemaphoreType.DMA((11,)),
        ],
        compiler_params=pltpu.CompilerParams(vmem_limit_bytes=110 * 1024 * 1024),
        name="hedgehog_mod",
    )(
        A_x.reshape(S, D), A_wqkv, A_w_phi.reshape(H * DH, DH), A_wo,
        B_w_r, B_w_gate, B_w_up, B_w_down,
    )
    return out.reshape(1, S, D)
```

```python
import functools
import math

import jax
import jax.numpy as jnp
from jax import lax
import jax.experimental.pallas as pl
import jax.experimental.pallas.tpu as pltpu

S, D, H, DH, F = 2048, 1024, 32, 32, 3584
T = 512
NT_ = S // T
LOG2E = math.log2(math.e)
_NT = (((1,), (1,)), ((), ()))
_NN = (((1,), (0,)), ((), ()))
f32, bf16 = jnp.float32, jnp.bfloat16


def _dot(a, b, dn):
    return lax.dot_general(a, b, dn, preferred_element_type=f32)


def _rb(v):
    return v.astype(bf16).astype(f32)


def _rcp(v):
    r = pl.reciprocal(v, approx=True)
    return r * (2.0 - v * r)


def _silu(a):
    return a * pl.reciprocal(1.0 + jnp.exp2(a * -LOG2E), approx=True)


def _bits(v):
    return pltpu.bitcast(v, jnp.int32)


def _pack(v):
    m, n = v.shape
    v = v.reshape(m // 16, 2, 8, n)
    return pltpu.pack_elementwise([v[:, 0], v[:, 1]], packed_dtype=bf16).reshape(m // 2, n)


def _unpack(words):
    return pltpu.bitcast(words, bf16)


_HK_TERMS = (
    ((1,), (1, -2)), ((1, 2), (2,)), ((3, 4), (3,)), ((-4,), (3, -4)),
    ((1, 4), (2, 3)), ((-1, 3), (1, 3)), ((2, -4), (2, 4)),
    ((6,), (6,)), ((5,), (5,)),
    ((-3, -4, 5), (3, -4, -6)), ((-3, -4, 5, 6), (4, 6)), ((3, -5), (3, -4, 5, -6)),
    ((1, 2, -6), (1, -2, 5)), ((-2, 6), (1, -2, 5, -6)), ((-1, -2, 5, 6), (1, 5)),
    ((7,), (7, -8)), ((7, 8), (8,)),
    ((4, 7), (3, 8)), ((3, -7), (3, 7)), ((-4, 8), (4, 8)),
    ((-6, 7, 8), (5, 7, -8)), ((6, -8), (5, -6, 7, -8)), ((5, 6, -7, -8), (5, 7)),
    ((2, -6, 7), (1, 5, 8)), ((1, -5, -7), (1, 5, 7)), ((-2, 6, 8), (2, 6, 8)),
)
_HK_SUMS = (
    ((0, 0), (2, 1)), ((1, 1), (4, 3)), ((1, 0), (6, 5, 1, -3)), ((0, 1), (7, 5, 4, -2)),
    ((2, 2), (9, 8)), ((2, 1), (11, 10, 3, -8)), ((1, 2), (12, 10, 9, -4)),
    ((0, 2), (14, 13, 8, -1)), ((2, 0), (15, 13, 2, -9)), ((3, 3), (17, 16)),
    ((1, 3), (19, 18, 16, -3)), ((3, 1), (20, 18, 4, -17)),
    ((3, 2), (22, 21, 8, -16)), ((2, 3), (23, 21, 17, -9)),
    ((0, 3), (25, 24, 16, 15), (2, 3), 1), ((3, 0), (26, 24, 14, -17), (3, 2), -1),
)
_TOKEN_GROUP = (0, 2, 3, 1)


def _signed_sums(wanted, blocks):
    known = {(i + 1,): b for i, b in enumerate(blocks)}

    def value(key):
        if key not in known:
            for part in sorted(known, key=len, reverse=True):
                for sign in (1, -1):
                    signed = [sign * p for p in part]
                    if key not in known and len(part) < len(key) and all(p in key for p in signed):
                        rest = tuple(k for k in key if k not in signed)
                        if sign > 0 and rest[0] < 0:
                            known[key] = known[part] - value(tuple(-k for k in rest))
                        else:
                            known[key] = value(rest) + known[part] if sign > 0 else value(rest) - known[part]
            if key not in known:
                known[key] = -known[(-key[0],)]
        return known[key]

    for key in sorted(wanted, key=len):
        value(key)
    return [known[key] for key in wanted]


def _block_product(product, size):
    m, y = [], {}
    for ij, parts, *earlier in _HK_SUMS[:size * size]:
        while len(m) < parts[0]:
            m.append(product(len(m)))
        total = m[parts[0] - 1]
        for p in parts[1:]:
            total = total + m[p - 1] if p > 0 else total - m[-p - 1]
        if earlier:
            total = total + y[earlier[0]] if earlier[1] > 0 else total - y[earlier[0]]
        y[ij] = total
        yield ij, total


def _allreduce(v, op):
    r = v[0]
    for i in range(1, 8):
        r = op(r, v[i])
    r = op(r, pltpu.roll(r, 4, 0))
    return op(r, pltpu.roll(r, 2, 0))


def _features(p):
    p3 = p.reshape(8, 8, p.shape[1])
    mx = _allreduce(p3, jnp.maximum)
    mn = _allreduce(p3, jnp.minimum)
    ep = jnp.exp2(p3 - mx[None])
    en = jnp.exp2(mn[None] - p3)
    ip = _rcp(_allreduce(ep, jnp.add))
    im = _rcp(_allreduce(en, jnp.add))
    return jnp.concatenate([ep * ip[None], en * im[None]], axis=0)


def _kernel(x_hbm, wqkv_hbm, wphi_hbm, wo_hbm, wr_hbm, wg_hbm, wu_hbm, wd_hbm, out_hbm,
            x_v, xs_v, wqkv_v, ws_v, wo_v, woh_v, wg_v, wu_v, wd_v, out_v, wphi_v, wr_v, sems):
    def group(k, *pairs):
        return [pltpu.make_async_copy(src, dst, sems.at[k]) for src, dst in pairs]

    def x_rows(r0, n):
        return x_hbm.at[pl.ds(r0, n)], x_v.at[pl.ds(r0, n)]

    def w_cols(j0, nj):
        cols = pl.ds(256 * j0, 256 * nj)
        return wqkv_hbm.at[:, cols], wqkv_v.at[:, cols]

    loads = [
        group(0, x_rows(0, 256), (wr_hbm, wr_v)),
        group(1, w_cols(8, 1)),
        group(2, x_rows(256, 256)),
        group(3, w_cols(9, 1)),
        group(4, w_cols(10, 2)),
        group(5, (wphi_hbm, wphi_v), w_cols(4, 2), x_rows(T, 256)),
        group(6, w_cols(6, 2), x_rows(T + 256, 256)),
        group(7, x_rows(2 * T, S - 2 * T), w_cols(0, 4)),
        group(9, (wo_hbm, wo_v), (wg_hbm, wg_v), (wu_hbm, wu_v), (wd_hbm, wd_v)),
    ]
    for copies in loads:
        for c in copies:
            c.start()

    def wait_loads():
        for c in loads.pop(0):
            c.wait()

    tasks = []
    pace = {}

    def after(v, dep):
        first = pltpu.bitcast(_bits(v[:8, :128]) ^ (dep & pace["zero"]), v.dtype)
        if v.shape[1] > 128:
            first = jnp.concatenate([first, v[:8, 128:]], axis=1)
        return jnp.concatenate([first, v[8:]], axis=0)

    ffn = {"steps": None, "done": [], "y": [None, None]}

    def ffn_step():
        try:
            ffn["steps"].send(ffn["main"])
        except StopIteration:
            ffn["steps"] = None

    def matmul(lhs, rhs, dn):
        task = tasks.pop(0) if tasks else None
        dep = task() if task is not None else None
        if ffn["done"]:
            dep = ffn["done"].pop(0)
        if dep is not None:
            lhs = after(lhs, dep)
        m = _dot(lhs.astype(bf16) if lhs.dtype == f32 else _unpack(lhs), _unpack(rhs), dn)
        if ffn["steps"] is not None:
            ffn_step()
        ffn["main"] = _bits(m[-8:, -128:])
        return m

    top = [jnp.full((8, 128), -jnp.inf, f32), lax.broadcasted_iota(jnp.int32, (8, 128), 0)]
    chain = []
    x_keys = [term[1] for term in _HK_TERMS[:7]] + [(1,), (4,)]
    x_block = [x_keys.index((i + 1,)) for i in range(4)]

    def layernorm(t, g, lag):
        wr = wr_v[...].astype(f32).reshape(1, D)
        row = 2 * lax.broadcasted_iota(jnp.int32, (8, 128), 0)
        for r in range(0, 128, 16):
            xn = []
            for r0 in (T * t + 256 * g + r, T * t + 256 * g + 128 + r):
                words = pltpu.bitcast(x_v[pl.ds(r0, 16), :], jnp.uint32)
                for odd in range(2):
                    x = pltpu.unpack_elementwise(words, index=odd, packed_dtype=bf16, unpacked_dtype=f32)
                    total = x[:, :128]
                    for i in range(1, D // 128):
                        total = total + x[:, 128 * i:128 * (i + 1)]
                    if lag:
                        total = jnp.where(chain[-lag] >= 0, total, 0.0)
                    xc = x - jnp.sum(total, axis=-1, keepdims=True) * (1.0 / D)
                    v = jnp.mean(xc * xc, axis=-1, keepdims=True)
                    xn.append(xc * (1.0 / _rb(jnp.sqrt(_rb(_rb(v) + _rb(jnp.full_like(v, 1e-5)))))))
                    sc = jnp.broadcast_to(_rb(jnp.sum(xn[-1] * wr, axis=-1, keepdims=True)), (8, 128))
                    tok = row + (r0 + odd)
                    better = (sc > top[0]) | ((sc == top[0]) & (tok < top[1]))
                    top[:] = jnp.where(better, sc, top[0]), jnp.where(better, tok, top[1])
                chain.append(top[1])
            terms = [_signed_sums(x_keys, [a[:, :512], a[:, 512:], b[:, :512], b[:, 512:]])
                     for a, b in ((xn[0], xn[2]), (xn[1], xn[3]))]
            for i, pair in enumerate(zip(*terms)):
                xs_v[t, g, i, pl.ds(r // 2, 8), :] = pltpu.pack_elementwise(list(pair), packed_dtype=bf16)

    def feature_map():
        wt = wphi_v[...].astype(f32).T
        full = jnp.concatenate([wt[8 * (g % 4):8 * (g % 4) + 8] for g in range(8) for _ in range(2)], axis=0)
        row = lax.broadcasted_iota(jnp.int32, (128, D), 0)
        col = lax.broadcasted_iota(jnp.int32, (128, D), 1)
        same = (((row >> 6) << 1) | ((row >> 3) & 1)) == ((col >> 5) & 3)
        return jnp.where(same, full, 0.0).astype(bf16)

    def prepare_w(j):
        blocks = []
        for c in (2 * j, 2 * j + 1):
            w = wqkv_v[:, pl.ds(128 * c, 128)]
            if j < 8:
                blocks.append(_dot(bd[:, 128 * (c % 8):128 * (c % 8 + 1)], w, _NT) * LOG2E)
            else:
                blocks.append(w.astype(f32).T)
        blocks = [a[:, 512 * kh:512 * (kh + 1)] for a in blocks for kh in range(2)]
        for i, term in enumerate(_signed_sums([term[0] for term in _HK_TERMS[:7]], blocks)):
            ws_v[j // 2, i, pl.ds(64 * (j % 2), 64), :] = _pack(term)

    def paced_terms(pieces, lag):
        links = []
        for blocks, dest in pieces:
            if len(links) >= lag:
                first = blocks[0]
                blocks = [pltpu.bitcast(_bits(first) ^ jnp.concatenate([links[-lag]] * 2, axis=0), f32)] + blocks[1:]
            words = [_pack(term) for term in _signed_sums([t[0] for t in _HK_TERMS], blocks)]
            for i, w in enumerate(words):
                dest[i] = w
            done = functools.reduce(jnp.bitwise_or, words[4:7] + words[9:15] + words[17:])
            slow = jnp.sum(pltpu.bitcast(done, f32), axis=-1, keepdims=True)
            links.append(_bits(jnp.broadcast_to(slow, (8, 128))) & pace["zero"])

    def prepare_wo(lag):
        pieces = []
        for n in range(2):
            for c in range(4):
                for r in range(0, 128, 16):
                    w = [wo_v[pl.ds(256 * c + 128 * kh + r, 16), pl.ds(512 * n, 512)].astype(f32) for kh in range(2)]
                    pieces.append(([w[kh][:, 128 * i:128 * (i + 1)] for i in range(4) for kh in range(2)],
                                   woh_v.at[n, :, pl.ds(64 * c + r // 2, 8), :]))
        paced_terms(pieces, lag)

    def proj_group(j0, nj, t, g):
        rows = pl.ds(64 * (j0 % 2), 64 * nj)
        return dict(_block_product(
            lambda r: matmul(ws_v[j0 // 2, r, rows, :], xs_v[t, g, r], _NT), 2))

    def pairs(groups):
        return [jnp.concatenate([y[b, hf][r:r + 64] for y in groups for hf in range(2)], axis=1)
                for j in range(groups[0][0, 0].shape[0] // 128) for b in range(2)
                for r in (128 * j, 128 * j + 64)]

    def proj(j0, t):
        return pairs([proj_group(j0, 2, t, g) for g in range(2)])

    kv = [None] * 16
    phi_k = [None] * 16

    def key_features(j, p):
        phi = _features(p)
        phi_k[j] = phi.reshape(128, T).astype(bf16)
        return functools.reduce(jnp.bitwise_or, [_bits(phi[i][:, n:n + 128]) for i in (7, 15)
                                                 for n in range(0, T, 128)])

    def key_tasks(blocks, j0):
        return [None] * 5 + [functools.partial(key_features, j0 + q, p) for q, p in enumerate(blocks)]

    def kv_update(v_blocks, j0):
        for j, v in enumerate(v_blocks, j0):
            v1 = jnp.concatenate([v, jnp.ones((16, T), f32)], axis=0).astype(bf16)
            upd = _dot(v1, phi_k[j], _NT)
            kv[j] = upd if kv[j] is None else kv[j] + upd

    wait_loads()
    layernorm(0, 0, 0)
    pace["zero"] = top[1] >> 31
    wait_loads()
    prepare_w(8)
    wait_loads()
    layernorm(0, 1, 0)
    first = proj_group(8, 1, 0, 0)
    wait_loads()
    v0 = pairs([first, proj_group(8, 1, 0, 1)])
    prepare_w(9)
    first = proj_group(9, 1, 0, 0)
    wait_loads()
    v0 += pairs([first, proj_group(9, 1, 0, 1)])
    for j in (10, 11):
        prepare_w(j)
    if "0" == "0":
        v0 += pairs([proj_group(10, 1, 0, g) for g in range(2)])
        first = proj_group(11, 1, 0, 0)
        wait_loads()
        v0 += pairs([first, proj_group(11, 1, 0, 1)])
    else:
        first = proj_group(10, 2, 0, 0)
        wait_loads()
        v0 += pairs([first, proj_group(10, 2, 0, 1)])
    bd = feature_map()
    for j in (4, 5):
        prepare_w(j)
    first = proj_group(4, 2, 0, 0)
    layernorm(1, 0, 2)
    wait_loads()
    k = pairs([first, proj_group(4, 2, 0, 1)])
    for j in (6, 7):
        prepare_w(j)
    tasks += key_tasks(k[:4], 0)
    rest, k = k[4:], proj(6, 0)
    layernorm(1, 1, 2)
    wait_loads()
    for j, p in enumerate(rest, 4):
        key_features(j, p)
    pending = [(v0[:8], 0), (v0[8:], 8)]
    j0 = 8
    for t in range(1, NT_):
        for c in range(2):
            tasks += key_tasks(k, j0)
            v = proj(8 + 2 * c, t)
            if len(pending) > 1:
                kv_update(*pending.pop(0))
            kv_update(*pending.pop(0))
            k, j0 = proj(4 + 2 * c, t), 8 * c
            pending.append((v, j0))
            if t >= 2:
                prepare_w(2 * (t - 2) + c)
        for g in range(2 if t + 1 < NT_ else 0):
            layernorm(t + 1, g, 1)
    tasks += key_tasks(k, j0)

    r_max = jnp.max(top[0])
    idx = jnp.clip(jnp.min(jnp.where(top[0] == r_max, top[1], S)), 0, S - 1)
    t_sel = idx // T
    grp = pl.ds(pl.multiple_of(idx % 128 // 16 * 8, 8), 8)
    x_sel = jnp.concatenate(
        [_unpack(xs_v[t_sel, idx % T // 256, jnp.where(idx % 256 < 128, x_block[kh], x_block[2 + kh]), grp, :])
         for kh in range(2)],
        axis=1).astype(f32)
    x_sel = jnp.where(lax.broadcasted_iota(jnp.int32, (16, D), 0) == idx % 16, x_sel, 0.0)
    x_sel = jnp.broadcast_to(jnp.sum(x_sel, axis=0, keepdims=True), (16, D))
    gate = jax.nn.sigmoid(jnp.full((8, 512), r_max, f32))

    def ffn_program():
        h = []
        for n in range(F // 128):
            acc = []
            for w in (wg_v, wu_v):
                parts = []
                for kh in range(2):
                    dep = yield
                    parts.append(_dot(after(x_sel[:, 512 * kh:512 * (kh + 1)], dep).astype(bf16),
                                      w[pl.ds(512 * kh, 512), pl.ds(n * 128, 128)], _NN))
                    ffn["done"].append(_bits(parts[-1][:8]))
                acc.append(parts[0] + parts[1])
            h.append(_silu(acc[0]) * acc[1])
        for hf in range(2):
            y = None
            for n in range(F // 128):
                dep = yield
                part = _dot(after(h[n], dep).astype(bf16), wd_v[pl.ds(n * 128, 128), pl.ds(hf * 512, 512)], _NN)[:8]
                y = part if y is None else y + part
                ffn["done"].append(_bits(part[:, 384:]))
            ffn["y"][hf] = _rb(y * gate)

    def attend(blocks, j0):
        out = []
        for j, p in enumerate(blocks, j0):
            num = _dot(kv[j], p, _NN)
            for hd in range(2):
                inv = _rcp(num[64 + 8 * hd:72 + 8 * hd] + 1e-6)
                out.append((num[32 * hd:32 * hd + 32].reshape(4, 8, T) * inv[None]).reshape(32, T))
        return [[[jnp.concatenate(out[8 * c + 4 * kh:8 * c + 4 * kh + 4], axis=0)[:, 256 * g:256 * (g + 1)].T
                  for kh in range(2)] for g in range(2)] for c in range(2)]

    stores = []

    def out_proj(i, o_terms, n):
        while i and ffn["y"][n] is None:
            ffn_step()
        for (c, j), block in _block_product(lambda r: matmul(o_terms[r], woh_v[n, r], _NN), 4):
            q = _TOKEN_GROUP[j]
            t, g = tiles[i + q // 2], q % 2
            cols, tok = pl.ds(512 * n + 128 * c, 128), pl.ds(pl.multiple_of(T * t + 256 * g, 256), 256)
            a = jnp.concatenate([_unpack(xs_v[t, g, x_block[2 * hf + n], :, pl.ds(128 * c, 128)])
                                 for hf in range(2)], axis=0).astype(f32)
            if i + q // 2 == NT_ - 1:
                hit = (lax.broadcasted_iota(jnp.int32, (32, 8, 128), 0) * 8
                       + lax.broadcasted_iota(jnp.int32, (32, 8, 128), 1)) == idx % T - 256 * g
                a3 = a.reshape(32, 8, 128)
                a = jnp.where(hit, a3 + ffn["y"][n][:, 128 * c:128 * (c + 1)][None], a3).reshape(256, 128)
            rows = pl.ds(T * i + 256 * q, 256)
            out_v[rows, cols] = (x_v[tok, cols].astype(f32) + block * _silu(a)).astype(bf16)
            if i and n:
                stores.extend(group(10, (out_v.at[rows, cols], out_hbm.at[tok, cols])))
                stores[-1].start()
        if (i, n) in ((0, 1), (2, 0)):
            cols = pl.ds(0, 512) if i else slice(None)
            for q in range(2):
                stores.extend(group(10, (out_v.at[pl.ds(T * (i + q), T), cols],
                                         out_hbm.at[pl.ds(pl.multiple_of(T * tiles[i + q], T), T), cols])))
                stores[-1].start()

    def output_terms(first, second):
        per_group = [_signed_sums([t[1] for t in _HK_TERMS],
                                  [b for q in _TOKEN_GROUP for b in (first, second)[q // 2][c][q % 2]])
                     for c in range(4)]
        return [jnp.concatenate(term, axis=1) for term in zip(*per_group)]

    def last_loads():
        wait_loads()
        prepare_wo(1)
        ffn["steps"], ffn["done"] = ffn_program(), [None, None]
        next(ffn["steps"])

    tiles = [lax.rem(t_sel + 1 + i, NT_) for i in range(NT_)]
    o = [[] for _ in range(NT_)]
    halves = [(i, c) for i in range(NT_) for c in range(2)]
    for h, (i, c) in enumerate(halves):
        q = proj(2 * c, tiles[i])
        if h == 0:
            kv_update(*pending.pop(0))
            row = lax.broadcasted_iota(jnp.int32, (80, 128), 0)
            col = lax.broadcasted_iota(jnp.int32, (80, 128), 1)
            own = jnp.where(row < 64, row >> 5, (row >> 3) & 1) == (col & 1)
            kv[:] = [jnp.where(own, a, 0.0).astype(bf16) for a in kv]
            tasks.extend([None] * 0 + [last_loads])
        else:
            o[halves[h - 1][0]] += attend(prev, 8 * halves[h - 1][1])
        prev = [_features(p).reshape(128, T).astype(bf16) for p in q]
        if h == 6:
            terms = output_terms(*o[:2])
            out_proj(0, terms, 0)
    out_proj(0, terms, 1)
    o[-1] += attend(prev, 8)
    terms = output_terms(*o[2:])
    for n in range(2):
        out_proj(2, terms, n)
    for c in stores:
        c.wait()


@jax.jit
def pallas_recurrent_scan__linear_kernel_hedgehog__moe_arch_mod__prompt_kernel(
    A_x: jax.Array,
    A_wqkv: jax.Array,
    A_w_phi: jax.Array,
    A_wo: jax.Array,
    B_x: jax.Array,
    B_w_r: jax.Array,
    B_w_gate: jax.Array,
    B_w_up: jax.Array,
    B_w_down: jax.Array,
):
    del B_x
    hbm = pl.BlockSpec(memory_space=pl.ANY)
    out = pl.pallas_call(
        _kernel,
        out_shape=jax.ShapeDtypeStruct((S, D), bf16),
        in_specs=[hbm] * 8,
        out_specs=hbm,
        scratch_shapes=[
            pltpu.VMEM((S, D), bf16),
            pltpu.VMEM((NT_, 2, 9, 64, 512), jnp.uint32),
            pltpu.VMEM((D, 3 * D), bf16),
            pltpu.VMEM((6, 7, 128, 512), jnp.uint32),
            pltpu.VMEM((D, D), bf16),
            pltpu.VMEM((2, 26, 256, 128), jnp.uint32),
            pltpu.VMEM((D, F), bf16),
            pltpu.VMEM((D, F), bf16),
            pltpu.VMEM((F, D), bf16),
            pltpu.VMEM((S, D), bf16),
            pltpu.VMEM((H * DH, DH), bf16),
            pltpu.VMEM((D,), bf16),
            pltpu.SemaphoreType.DMA((11,)),
        ],
        compiler_params=pltpu.CompilerParams(vmem_limit_bytes=110 * 1024 * 1024),
        name="hedgehog_mod",
    )(
        A_x.reshape(S, D), A_wqkv, A_w_phi.reshape(H * DH, DH), A_wo,
        B_w_r, B_w_gate, B_w_up, B_w_down,
    )
    return out.reshape(1, S, D)
```

```python
import functools
import math

import jax
import jax.numpy as jnp
from jax import lax
import jax.experimental.pallas as pl
import jax.experimental.pallas.tpu as pltpu

S, D, H, DH, F = 2048, 1024, 32, 32, 3584
T = 512
NT_ = S // T
LOG2E = math.log2(math.e)
_NT = (((1,), (1,)), ((), ()))
_NN = (((1,), (0,)), ((), ()))
f32, bf16 = jnp.float32, jnp.bfloat16


def _dot(a, b, dn):
    return lax.dot_general(a, b, dn, preferred_element_type=f32)


def _rb(v):
    return v.astype(bf16).astype(f32)


def _rcp(v):
    r = pl.reciprocal(v, approx=True)
    return r * (2.0 - v * r)


def _silu(a):
    return a * pl.reciprocal(1.0 + jnp.exp2(a * -LOG2E), approx=True)


def _bits(v):
    return pltpu.bitcast(v, jnp.int32)


def _pack(v):
    m, n = v.shape
    v = v.reshape(m // 16, 2, 8, n)
    return pltpu.pack_elementwise([v[:, 0], v[:, 1]], packed_dtype=bf16).reshape(m // 2, n)


def _unpack(words):
    return pltpu.bitcast(words, bf16)


_HK_TERMS = (
    ((1,), (1, -2)), ((1, 2), (2,)), ((3, 4), (3,)), ((-4,), (3, -4)),
    ((1, 4), (2, 3)), ((-1, 3), (1, 3)), ((2, -4), (2, 4)),
    ((6,), (6,)), ((5,), (5,)),
    ((-3, -4, 5), (3, -4, -6)), ((-3, -4, 5, 6), (4, 6)), ((3, -5), (3, -4, 5, -6)),
    ((1, 2, -6), (1, -2, 5)), ((-2, 6), (1, -2, 5, -6)), ((-1, -2, 5, 6), (1, 5)),
    ((7,), (7, -8)), ((7, 8), (8,)),
    ((4, 7), (3, 8)), ((3, -7), (3, 7)), ((-4, 8), (4, 8)),
    ((-6, 7, 8), (5, 7, -8)), ((6, -8), (5, -6, 7, -8)), ((5, 6, -7, -8), (5, 7)),
    ((2, -6, 7), (1, 5, 8)), ((1, -5, -7), (1, 5, 7)), ((-2, 6, 8), (2, 6, 8)),
)
_HK_SUMS = (
    ((0, 0), (2, 1)), ((1, 1), (4, 3)), ((1, 0), (6, 5, 1, -3)), ((0, 1), (7, 5, 4, -2)),
    ((2, 2), (9, 8)), ((2, 1), (11, 10, 3, -8)), ((1, 2), (12, 10, 9, -4)),
    ((0, 2), (14, 13, 8, -1)), ((2, 0), (15, 13, 2, -9)), ((3, 3), (17, 16)),
    ((1, 3), (19, 18, 16, -3)), ((3, 1), (20, 18, 4, -17)),
    ((3, 2), (22, 21, 8, -16)), ((2, 3), (23, 21, 17, -9)),
    ((0, 3), (25, 24, 16, 15), (2, 3), 1), ((3, 0), (26, 24, 14, -17), (3, 2), -1),
)
_TOKEN_GROUP = (0, 2, 3, 1)


def _signed_sums(wanted, blocks):
    known = {(i + 1,): b for i, b in enumerate(blocks)}

    def value(key):
        if key not in known:
            for part in sorted(known, key=len, reverse=True):
                for sign in (1, -1):
                    signed = [sign * p for p in part]
                    if key not in known and len(part) < len(key) and all(p in key for p in signed):
                        rest = tuple(k for k in key if k not in signed)
                        if sign > 0 and rest[0] < 0:
                            known[key] = known[part] - value(tuple(-k for k in rest))
                        else:
                            known[key] = value(rest) + known[part] if sign > 0 else value(rest) - known[part]
            if key not in known:
                known[key] = -known[(-key[0],)]
        return known[key]

    for key in sorted(wanted, key=len):
        value(key)
    return [known[key] for key in wanted]


def _block_product(product, size):
    m, y = [], {}
    for ij, parts, *earlier in _HK_SUMS[:size * size]:
        while len(m) < parts[0]:
            m.append(product(len(m)))
        total = m[parts[0] - 1]
        for p in parts[1:]:
            total = total + m[p - 1] if p > 0 else total - m[-p - 1]
        if earlier:
            total = total + y[earlier[0]] if earlier[1] > 0 else total - y[earlier[0]]
        y[ij] = total
        yield ij, total


def _allreduce(v, op):
    r = v[0]
    for i in range(1, 8):
        r = op(r, v[i])
    r = op(r, pltpu.roll(r, 4, 0))
    return op(r, pltpu.roll(r, 2, 0))


def _features(p):
    p3 = p.reshape(8, 8, p.shape[1])
    mx = _allreduce(p3, jnp.maximum)
    mn = _allreduce(p3, jnp.minimum)
    ep = jnp.exp2(p3 - mx[None])
    en = jnp.exp2(mn[None] - p3)
    ip = _rcp(_allreduce(ep, jnp.add))
    im = _rcp(_allreduce(en, jnp.add))
    return jnp.concatenate([ep * ip[None], en * im[None]], axis=0)


def _kernel(x_hbm, wqkv_hbm, wphi_hbm, wo_hbm, wr_hbm, wg_hbm, wu_hbm, wd_hbm, out_hbm,
            x_v, xs_v, wqkv_v, ws_v, wo_v, woh_v, wg_v, wu_v, wd_v, out_v, wphi_v, wr_v, sems):
    def group(k, *pairs):
        return [pltpu.make_async_copy(src, dst, sems.at[k]) for src, dst in pairs]

    def x_rows(r0, n):
        return x_hbm.at[pl.ds(r0, n)], x_v.at[pl.ds(r0, n)]

    def w_cols(j0, nj):
        cols = pl.ds(256 * j0, 256 * nj)
        return wqkv_hbm.at[:, cols], wqkv_v.at[:, cols]

    loads = [
        group(0, x_rows(0, 256), (wr_hbm, wr_v)),
        group(1, w_cols(8, 1)),
        group(2, x_rows(256, 256)),
        group(3, w_cols(9, 1)),
        group(4, w_cols(10, 2)),
        group(5, (wphi_hbm, wphi_v), w_cols(4, 2), x_rows(T, 256)),
        group(6, w_cols(6, 2), x_rows(T + 256, 256)),
        group(7, x_rows(2 * T, S - 2 * T), w_cols(0, 4)),
        group(8, (wo_hbm, wo_v), (wg_hbm, wg_v), (wu_hbm, wu_v), (wd_hbm, wd_v)),
    ]
    for copies in loads:
        for c in copies:
            c.start()

    def wait_loads():
        for c in loads.pop(0):
            c.wait()

    tasks = []
    pace = {}

    def after(v, dep):
        first = pltpu.bitcast(_bits(v[:8, :128]) ^ (dep & pace["zero"]), v.dtype)
        if v.shape[1] > 128:
            first = jnp.concatenate([first, v[:8, 128:]], axis=1)
        return jnp.concatenate([first, v[8:]], axis=0)

    ffn = {"steps": None, "done": [], "y": [None, None]}

    def ffn_step():
        try:
            ffn["steps"].send(ffn["main"])
        except StopIteration:
            ffn["steps"] = None

    def matmul(lhs, rhs, dn):
        task = tasks.pop(0) if tasks else None
        dep = task() if task is not None else None
        if ffn["done"]:
            dep = ffn["done"].pop(0)
        if dep is not None:
            lhs = after(lhs, dep)
        m = _dot(lhs.astype(bf16) if lhs.dtype == f32 else _unpack(lhs), _unpack(rhs), dn)
        if ffn["steps"] is not None:
            ffn_step()
        ffn["main"] = _bits(m[-8:, -128:])
        return m

    top = [jnp.full((8, 128), -jnp.inf, f32), lax.broadcasted_iota(jnp.int32, (8, 128), 0)]
    chain = []
    x_keys = [term[1] for term in _HK_TERMS[:7]] + [(1,), (4,)]
    x_block = [x_keys.index((i + 1,)) for i in range(4)]

    def layernorm(t, g, lag):
        wr = wr_v[...].astype(f32).reshape(1, D)
        row = 2 * lax.broadcasted_iota(jnp.int32, (8, 128), 0)
        for r in range(0, 128, 16):
            xn = []
            for r0 in (T * t + 256 * g + r, T * t + 256 * g + 128 + r):
                words = pltpu.bitcast(x_v[pl.ds(r0, 16), :], jnp.uint32)
                for odd in range(2):
                    x = pltpu.unpack_elementwise(words, index=odd, packed_dtype=bf16, unpacked_dtype=f32)
                    total = x[:, :128]
                    for i in range(1, D // 128):
                        total = total + x[:, 128 * i:128 * (i + 1)]
                    if lag:
                        total = jnp.where(chain[-lag] >= 0, total, 0.0)
                    xc = x - jnp.sum(total, axis=-1, keepdims=True) * (1.0 / D)
                    v = jnp.mean(xc * xc, axis=-1, keepdims=True)
                    xn.append(xc * (1.0 / _rb(jnp.sqrt(_rb(_rb(v) + _rb(jnp.full_like(v, 1e-5)))))))
                    sc = jnp.broadcast_to(_rb(jnp.sum(xn[-1] * wr, axis=-1, keepdims=True)), (8, 128))
                    tok = row + (r0 + odd)
                    better = (sc > top[0]) | ((sc == top[0]) & (tok < top[1]))
                    top[:] = jnp.where(better, sc, top[0]), jnp.where(better, tok, top[1])
                chain.append(top[1])
            terms = [_signed_sums(x_keys, [a[:, :512], a[:, 512:], b[:, :512], b[:, 512:]])
                     for a, b in ((xn[0], xn[2]), (xn[1], xn[3]))]
            for i, pair in enumerate(zip(*terms)):
                xs_v[t, g, i, pl.ds(r // 2, 8), :] = pltpu.pack_elementwise(list(pair), packed_dtype=bf16)

    def feature_map():
        wt = wphi_v[...].astype(f32).T
        full = jnp.concatenate([wt[8 * (g % 4):8 * (g % 4) + 8] for g in range(8) for _ in range(2)], axis=0)
        row = lax.broadcasted_iota(jnp.int32, (128, D), 0)
        col = lax.broadcasted_iota(jnp.int32, (128, D), 1)
        same = (((row >> 6) << 1) | ((row >> 3) & 1)) == ((col >> 5) & 3)
        return jnp.where(same, full, 0.0).astype(bf16)

    def prepare_w(j):
        blocks = []
        for c in (2 * j, 2 * j + 1):
            w = wqkv_v[:, pl.ds(128 * c, 128)]
            if j < 8:
                blocks.append(_dot(bd[:, 128 * (c % 8):128 * (c % 8 + 1)], w, _NT) * LOG2E)
            else:
                blocks.append(w.astype(f32).T)
        blocks = [a[:, 512 * kh:512 * (kh + 1)] for a in blocks for kh in range(2)]
        for i, term in enumerate(_signed_sums([term[0] for term in _HK_TERMS[:7]], blocks)):
            ws_v[j // 2, i, pl.ds(64 * (j % 2), 64), :] = _pack(term)

    def paced_terms(pieces, lag):
        links = []
        for blocks, dest in pieces:
            if len(links) >= lag:
                first = blocks[0]
                blocks = [pltpu.bitcast(_bits(first) ^ jnp.concatenate([links[-lag]] * 2, axis=0), f32)] + blocks[1:]
            words = [_pack(term) for term in _signed_sums([t[0] for t in _HK_TERMS], blocks)]
            for i, w in enumerate(words):
                dest[i] = w
            done = functools.reduce(jnp.bitwise_or, words[4:7] + words[9:15] + words[17:])
            slow = jnp.sum(pltpu.bitcast(done, f32), axis=-1, keepdims=True)
            links.append(_bits(jnp.broadcast_to(slow, (8, 128))) & pace["zero"])

    def prepare_wo(lag):
        pieces = []
        for n in range(2):
            for c in range(4):
                for r in range(0, 128, 16):
                    w = [wo_v[pl.ds(256 * c + 128 * kh + r, 16), pl.ds(512 * n, 512)].astype(f32) for kh in range(2)]
                    pieces.append(([w[kh][:, 128 * i:128 * (i + 1)] for i in range(4) for kh in range(2)],
                                   woh_v.at[n, :, pl.ds(64 * c + r // 2, 8), :]))
        paced_terms(pieces, lag)

    def proj_group(j0, nj, t, g):
        rows = pl.ds(64 * (j0 % 2), 64 * nj)
        return dict(_block_product(
            lambda r: matmul(ws_v[j0 // 2, r, rows, :], xs_v[t, g, r], _NT), 2))

    def pairs(groups):
        return [jnp.concatenate([y[b, hf][r:r + 64] for y in groups for hf in range(2)], axis=1)
                for j in range(groups[0][0, 0].shape[0] // 128) for b in range(2)
                for r in (128 * j, 128 * j + 64)]

    def proj(j0, t):
        return pairs([proj_group(j0, 2, t, g) for g in range(2)])

    kv = [None] * 16
    phi_k = [None] * 16

    def key_features(j, p):
        phi = _features(p)
        phi_k[j] = phi.reshape(128, T).astype(bf16)
        return functools.reduce(jnp.bitwise_or, [_bits(phi[i][:, n:n + 128]) for i in (7, 15)
                                                 for n in range(0, T, 128)])

    def key_tasks(blocks, j0):
        return [None] * 5 + [functools.partial(key_features, j0 + q, p) for q, p in enumerate(blocks)]

    def kv_update(v_blocks, j0):
        for j, v in enumerate(v_blocks, j0):
            v1 = jnp.concatenate([v, jnp.ones((16, T), f32)], axis=0).astype(bf16)
            upd = _dot(v1, phi_k[j], _NT)
            kv[j] = upd if kv[j] is None else kv[j] + upd

    wait_loads()
    layernorm(0, 0, 0)
    pace["zero"] = top[1] >> 31
    wait_loads()
    prepare_w(8)
    wait_loads()
    layernorm(0, 1, 0)
    first = proj_group(8, 1, 0, 0)
    wait_loads()
    v0 = pairs([first, proj_group(8, 1, 0, 1)])
    prepare_w(9)
    first = proj_group(9, 1, 0, 0)
    wait_loads()
    v0 += pairs([first, proj_group(9, 1, 0, 1)])
    for j in (10, 11):
        prepare_w(j)
    if "0" == "0":
        v0 += pairs([proj_group(10, 1, 0, g) for g in range(2)])
        first = proj_group(11, 1, 0, 0)
        wait_loads()
        v0 += pairs([first, proj_group(11, 1, 0, 1)])
    else:
        first = proj_group(10, 2, 0, 0)
        wait_loads()
        v0 += pairs([first, proj_group(10, 2, 0, 1)])
    bd = feature_map()
    for j in (4, 5):
        prepare_w(j)
    first = proj_group(4, 2, 0, 0)
    layernorm(1, 0, 2)
    wait_loads()
    k = pairs([first, proj_group(4, 2, 0, 1)])
    for j in (6, 7):
        prepare_w(j)
    tasks += key_tasks(k[:4], 0)
    rest, k = k[4:], proj(6, 0)
    layernorm(1, 1, 2)
    wait_loads()
    for j, p in enumerate(rest, 4):
        key_features(j, p)
    pending = [(v0[:8], 0), (v0[8:], 8)]
    j0 = 8
    for t in range(1, NT_):
        for c in range(2):
            tasks += key_tasks(k, j0)
            v = proj(8 + 2 * c, t)
            if len(pending) > 1:
                kv_update(*pending.pop(0))
            kv_update(*pending.pop(0))
            k, j0 = proj(4 + 2 * c, t), 8 * c
            pending.append((v, j0))
            if t >= 2:
                prepare_w(2 * (t - 2) + c)
        for g in range(2 if t + 1 < NT_ else 0):
            layernorm(t + 1, g, 1)
    tasks += key_tasks(k, j0)

    r_max = jnp.max(top[0])
    idx = jnp.clip(jnp.min(jnp.where(top[0] == r_max, top[1], S)), 0, S - 1)
    t_sel = idx // T
    grp = pl.ds(pl.multiple_of(idx % 128 // 16 * 8, 8), 8)
    x_sel = jnp.concatenate(
        [_unpack(xs_v[t_sel, idx % T // 256, jnp.where(idx % 256 < 128, x_block[kh], x_block[2 + kh]), grp, :])
         for kh in range(2)],
        axis=1).astype(f32)
    x_sel = jnp.where(lax.broadcasted_iota(jnp.int32, (16, D), 0) == idx % 16, x_sel, 0.0)
    x_sel = jnp.broadcast_to(jnp.sum(x_sel, axis=0, keepdims=True), (16, D))
    gate = jax.nn.sigmoid(jnp.full((8, 512), r_max, f32))

    def ffn_program():
        h = []
        for n in range(F // 128):
            acc = []
            for w in (wg_v, wu_v):
                parts = []
                for kh in range(2):
                    dep = yield
                    parts.append(_dot(after(x_sel[:, 512 * kh:512 * (kh + 1)], dep).astype(bf16),
                                      w[pl.ds(512 * kh, 512), pl.ds(n * 128, 128)], _NN))
                    ffn["done"].append(_bits(parts[-1][:8]))
                acc.append(parts[0] + parts[1])
            h.append(_silu(acc[0]) * acc[1])
        for hf in range(2):
            y = None
            for n in range(F // 128):
                dep = yield
                part = _dot(after(h[n], dep).astype(bf16), wd_v[pl.ds(n * 128, 128), pl.ds(hf * 512, 512)], _NN)[:8]
                y = part if y is None else y + part
                ffn["done"].append(_bits(part[:, 384:]))
            ffn["y"][hf] = _rb(y * gate)

    def attend(blocks, j0):
        out = []
        for j, p in enumerate(blocks, j0):
            num = _dot(kv[j], p, _NN)
            for hd in range(2):
                inv = _rcp(num[64 + 8 * hd:72 + 8 * hd] + 1e-6)
                out.append((num[32 * hd:32 * hd + 32].reshape(4, 8, T) * inv[None]).reshape(32, T))
        return [[[jnp.concatenate(out[8 * c + 4 * kh:8 * c + 4 * kh + 4], axis=0)[:, 256 * g:256 * (g + 1)].T
                  for kh in range(2)] for g in range(2)] for c in range(2)]

    stores = []

    def out_proj(i, o_terms, n):
        while i and ffn["y"][n] is None:
            ffn_step()
        for (c, j), block in _block_product(lambda r: matmul(o_terms[r], woh_v[n, r], _NN), 4):
            q = _TOKEN_GROUP[j]
            t, g = tiles[i + q // 2], q % 2
            cols, tok = pl.ds(512 * n + 128 * c, 128), pl.ds(pl.multiple_of(T * t + 256 * g, 256), 256)
            a = jnp.concatenate([_unpack(xs_v[t, g, x_block[2 * hf + n], :, pl.ds(128 * c, 128)])
                                 for hf in range(2)], axis=0).astype(f32)
            if i + q // 2 == NT_ - 1:
                hit = (lax.broadcasted_iota(jnp.int32, (32, 8, 128), 0) * 8
                       + lax.broadcasted_iota(jnp.int32, (32, 8, 128), 1)) == idx % T - 256 * g
                a3 = a.reshape(32, 8, 128)
                a = jnp.where(hit, a3 + ffn["y"][n][:, 128 * c:128 * (c + 1)][None], a3).reshape(256, 128)
            rows = pl.ds(T * i + 256 * q, 256)
            out_v[rows, cols] = (x_v[tok, cols].astype(f32) + block * _silu(a)).astype(bf16)
            if i and n:
                stores.extend(group(9, (out_v.at[rows, cols], out_hbm.at[tok, cols])))
                stores[-1].start()
        if (i, n) in ((0, 1), (2, 0)):
            cols = pl.ds(0, 512) if i else slice(None)
            for q in range(2):
                stores.extend(group(9, (out_v.at[pl.ds(T * (i + q), T), cols],
                                         out_hbm.at[pl.ds(pl.multiple_of(T * tiles[i + q], T), T), cols])))
                stores[-1].start()

    def output_terms(first, second):
        per_group = [_signed_sums([t[1] for t in _HK_TERMS],
                                  [b for q in _TOKEN_GROUP for b in (first, second)[q // 2][c][q % 2]])
                     for c in range(4)]
        return [jnp.concatenate(term, axis=1) for term in zip(*per_group)]

    def last_loads():
        wait_loads()
        prepare_wo(1)
        ffn["steps"], ffn["done"] = ffn_program(), [None, None]
        next(ffn["steps"])

    tiles = [lax.rem(t_sel + 1 + i, NT_) for i in range(NT_)]
    o = [[] for _ in range(NT_)]
    halves = [(i, c) for i in range(NT_) for c in range(2)]
    for h, (i, c) in enumerate(halves):
        q = proj(2 * c, tiles[i])
        if h == 0:
            kv_update(*pending.pop(0))
            row = lax.broadcasted_iota(jnp.int32, (80, 128), 0)
            col = lax.broadcasted_iota(jnp.int32, (80, 128), 1)
            own = jnp.where(row < 64, row >> 5, (row >> 3) & 1) == (col & 1)
            kv[:] = [jnp.where(own, a, 0.0).astype(bf16) for a in kv]
            tasks.extend([None] * 0 + [last_loads])
        else:
            o[halves[h - 1][0]] += attend(prev, 8 * halves[h - 1][1])
        prev = [_features(p).reshape(128, T).astype(bf16) for p in q]
        if h == 6:
            terms = output_terms(*o[:2])
            out_proj(0, terms, 0)
    out_proj(0, terms, 1)
    o[-1] += attend(prev, 8)
    terms = output_terms(*o[2:])
    for n in range(2):
        out_proj(2, terms, n)
    for c in stores:
        c.wait()


@jax.jit
def pallas_recurrent_scan__linear_kernel_hedgehog__moe_arch_mod__prompt_kernel(
    A_x: jax.Array,
    A_wqkv: jax.Array,
    A_w_phi: jax.Array,
    A_wo: jax.Array,
    B_x: jax.Array,
    B_w_r: jax.Array,
    B_w_gate: jax.Array,
    B_w_up: jax.Array,
    B_w_down: jax.Array,
):
    del B_x
    hbm = pl.BlockSpec(memory_space=pl.ANY)
    out = pl.pallas_call(
        _kernel,
        out_shape=jax.ShapeDtypeStruct((S, D), bf16),
        in_specs=[hbm] * 8,
        out_specs=hbm,
        scratch_shapes=[
            pltpu.VMEM((S, D), bf16),
            pltpu.VMEM((NT_, 2, 9, 64, 512), jnp.uint32),
            pltpu.VMEM((D, 3 * D), bf16),
            pltpu.VMEM((6, 7, 128, 512), jnp.uint32),
            pltpu.VMEM((D, D), bf16),
            pltpu.VMEM((2, 26, 256, 128), jnp.uint32),
            pltpu.VMEM((D, F), bf16),
            pltpu.VMEM((D, F), bf16),
            pltpu.VMEM((F, D), bf16),
            pltpu.VMEM((S, D), bf16),
            pltpu.VMEM((H * DH, DH), bf16),
            pltpu.VMEM((D,), bf16),
            pltpu.SemaphoreType.DMA((10,)),
        ],
        compiler_params=pltpu.CompilerParams(vmem_limit_bytes=110 * 1024 * 1024),
        name="hedgehog_mod",
    )(
        A_x.reshape(S, D), A_wqkv, A_w_phi.reshape(H * DH, DH), A_wo,
        B_w_r, B_w_gate, B_w_up, B_w_down,
    )
    return out.reshape(1, S, D)
```

```python
import functools
import math

import jax
import jax.numpy as jnp
from jax import lax
import jax.experimental.pallas as pl
import jax.experimental.pallas.tpu as pltpu

S, D, H, DH, F = 2048, 1024, 32, 32, 3584
T = 512
NT_ = S // T
LOG2E = math.log2(math.e)
_NT = (((1,), (1,)), ((), ()))
_NN = (((1,), (0,)), ((), ()))
f32, bf16 = jnp.float32, jnp.bfloat16


def _dot(a, b, dn):
    return lax.dot_general(a, b, dn, preferred_element_type=f32)


def _rb(v):
    return v.astype(bf16).astype(f32)


def _rcp(v):
    r = pl.reciprocal(v, approx=True)
    return r * (2.0 - v * r)


def _silu(a):
    return a * pl.reciprocal(1.0 + jnp.exp2(a * -LOG2E), approx=True)


def _bits(v):
    return pltpu.bitcast(v, jnp.int32)


def _pack(v):
    m, n = v.shape
    v = v.reshape(m // 16, 2, 8, n)
    return pltpu.pack_elementwise([v[:, 0], v[:, 1]], packed_dtype=bf16).reshape(m // 2, n)


def _unpack(words):
    return pltpu.bitcast(words, bf16)


_HK_TERMS = (
    ((1,), (1, -2)), ((1, 2), (2,)), ((3, 4), (3,)), ((-4,), (3, -4)),
    ((1, 4), (2, 3)), ((-1, 3), (1, 3)), ((2, -4), (2, 4)),
    ((6,), (6,)), ((5,), (5,)),
    ((-3, -4, 5), (3, -4, -6)), ((-3, -4, 5, 6), (4, 6)), ((3, -5), (3, -4, 5, -6)),
    ((1, 2, -6), (1, -2, 5)), ((-2, 6), (1, -2, 5, -6)), ((-1, -2, 5, 6), (1, 5)),
    ((7,), (7, -8)), ((7, 8), (8,)),
    ((4, 7), (3, 8)), ((3, -7), (3, 7)), ((-4, 8), (4, 8)),
    ((-6, 7, 8), (5, 7, -8)), ((6, -8), (5, -6, 7, -8)), ((5, 6, -7, -8), (5, 7)),
    ((2, -6, 7), (1, 5, 8)), ((1, -5, -7), (1, 5, 7)), ((-2, 6, 8), (2, 6, 8)),
)
_HK_SUMS = (
    ((0, 0), (2, 1)), ((1, 1), (4, 3)), ((1, 0), (6, 5, 1, -3)), ((0, 1), (7, 5, 4, -2)),
    ((2, 2), (9, 8)), ((2, 1), (11, 10, 3, -8)), ((1, 2), (12, 10, 9, -4)),
    ((0, 2), (14, 13, 8, -1)), ((2, 0), (15, 13, 2, -9)), ((3, 3), (17, 16)),
    ((1, 3), (19, 18, 16, -3)), ((3, 1), (20, 18, 4, -17)),
    ((3, 2), (22, 21, 8, -16)), ((2, 3), (23, 21, 17, -9)),
    ((0, 3), (25, 24, 16, 15), (2, 3), 1), ((3, 0), (26, 24, 14, -17), (3, 2), -1),
)
_TOKEN_GROUP = (0, 2, 3, 1)


def _signed_sums(wanted, blocks):
    known = {(i + 1,): b for i, b in enumerate(blocks)}

    def value(key):
        if key not in known:
            for part in sorted(known, key=len, reverse=True):
                for sign in (1, -1):
                    signed = [sign * p for p in part]
                    if key not in known and len(part) < len(key) and all(p in key for p in signed):
                        rest = tuple(k for k in key if k not in signed)
                        if sign > 0 and rest[0] < 0:
                            known[key] = known[part] - value(tuple(-k for k in rest))
                        else:
                            known[key] = value(rest) + known[part] if sign > 0 else value(rest) - known[part]
            if key not in known:
                known[key] = -known[(-key[0],)]
        return known[key]

    for key in sorted(wanted, key=len):
        value(key)
    return [known[key] for key in wanted]


def _block_product(product, size):
    m, y = [], {}
    for ij, parts, *earlier in _HK_SUMS[:size * size]:
        while len(m) < parts[0]:
            m.append(product(len(m)))
        total = m[parts[0] - 1]
        for p in parts[1:]:
            total = total + m[p - 1] if p > 0 else total - m[-p - 1]
        if earlier:
            total = total + y[earlier[0]] if earlier[1] > 0 else total - y[earlier[0]]
        y[ij] = total
        yield ij, total


def _allreduce(v, op):
    r = v[0]
    for i in range(1, 8):
        r = op(r, v[i])
    r = op(r, pltpu.roll(r, 4, 0))
    return op(r, pltpu.roll(r, 2, 0))


def _features(p):
    p3 = p.reshape(8, 8, p.shape[1])
    mx = _allreduce(p3, jnp.maximum)
    mn = _allreduce(p3, jnp.minimum)
    ep = jnp.exp2(p3 - mx[None])
    en = jnp.exp2(mn[None] - p3)
    ip = _rcp(_allreduce(ep, jnp.add))
    im = _rcp(_allreduce(en, jnp.add))
    return jnp.concatenate([ep * ip[None], en * im[None]], axis=0)


def _kernel(x_hbm, wqkv_hbm, wphi_hbm, wo_hbm, wr_hbm, wg_hbm, wu_hbm, wd_hbm, out_hbm,
            x_v, xs_v, wqkv_v, ws_v, wo_v, woh_v, wg_v, wu_v, wd_v, out_v, wphi_v, wr_v, sems):
    def group(k, *pairs):
        return [pltpu.make_async_copy(src, dst, sems.at[k]) for src, dst in pairs]

    def x_rows(r0, n):
        return x_hbm.at[pl.ds(r0, n)], x_v.at[pl.ds(r0, n)]

    def w_cols(j0, nj):
        cols = pl.ds(256 * j0, 256 * nj)
        return wqkv_hbm.at[:, cols], wqkv_v.at[:, cols]

    loads = [
        group(0, x_rows(0, 256), (wr_hbm, wr_v)),
        group(1, w_cols(8, 1)),
        group(2, x_rows(256, 256)),
        group(3, w_cols(9, 1)),
        group(4, w_cols(10, 2)),
        group(5, (wphi_hbm, wphi_v), w_cols(4, 2), x_rows(T, 256)),
        group(6, w_cols(6, 2), x_rows(T + 256, 256)),
        group(7, x_rows(2 * T, S - 2 * T), w_cols(0, 4)),
        group(8, (wo_hbm, wo_v), (wg_hbm, wg_v), (wu_hbm, wu_v), (wd_hbm, wd_v)),
    ]
    for copies in loads:
        for c in copies:
            c.start()

    def wait_loads():
        for c in loads.pop(0):
            c.wait()

    tasks = []
    pace = {}

    def after(v, dep):
        first = pltpu.bitcast(_bits(v[:8, :128]) ^ (dep & pace["zero"]), v.dtype)
        if v.shape[1] > 128:
            first = jnp.concatenate([first, v[:8, 128:]], axis=1)
        return jnp.concatenate([first, v[8:]], axis=0)

    ffn = {"steps": None, "done": [], "y": [None, None]}

    def ffn_step():
        try:
            ffn["steps"].send(ffn["main"])
        except StopIteration:
            ffn["steps"] = None

    def matmul(lhs, rhs, dn):
        task = tasks.pop(0) if tasks else None
        dep = task() if task is not None else None
        if ffn["done"]:
            dep = ffn["done"].pop(0)
        if dep is not None:
            lhs = after(lhs, dep)
        m = _dot(lhs.astype(bf16) if lhs.dtype == f32 else _unpack(lhs), _unpack(rhs), dn)
        if ffn["steps"] is not None:
            ffn_step()
        ffn["main"] = _bits(m[-8:, -128:])
        return m

    top = [jnp.full((8, 128), -jnp.inf, f32), lax.broadcasted_iota(jnp.int32, (8, 128), 0)]
    chain = []
    x_keys = [term[1] for term in _HK_TERMS[:7]] + [(1,), (4,)]
    x_block = [x_keys.index((i + 1,)) for i in range(4)]

    def layernorm(t, g, lag):
        wr = wr_v[...].astype(f32).reshape(1, D)
        row = 2 * lax.broadcasted_iota(jnp.int32, (8, 128), 0)
        for r in range(0, 128, 16):
            xn = []
            for r0 in (T * t + 256 * g + r, T * t + 256 * g + 128 + r):
                words = pltpu.bitcast(x_v[pl.ds(r0, 16), :], jnp.uint32)
                for odd in range(2):
                    x = pltpu.unpack_elementwise(words, index=odd, packed_dtype=bf16, unpacked_dtype=f32)
                    total = x[:, :128]
                    for i in range(1, D // 128):
                        total = total + x[:, 128 * i:128 * (i + 1)]
                    if lag:
                        total = jnp.where(chain[-lag] >= 0, total, 0.0)
                    xc = x - jnp.sum(total, axis=-1, keepdims=True) * (1.0 / D)
                    v = jnp.mean(xc * xc, axis=-1, keepdims=True)
                    xn.append(xc * (1.0 / _rb(jnp.sqrt(_rb(_rb(v) + _rb(jnp.full_like(v, 1e-5)))))))
                    sc = jnp.broadcast_to(_rb(jnp.sum(xn[-1] * wr, axis=-1, keepdims=True)), (8, 128))
                    tok = row + (r0 + odd)
                    better = (sc > top[0]) | ((sc == top[0]) & (tok < top[1]))
                    top[:] = jnp.where(better, sc, top[0]), jnp.where(better, tok, top[1])
                chain.append(top[1])
            terms = [_signed_sums(x_keys, [a[:, :512], a[:, 512:], b[:, :512], b[:, 512:]])
                     for a, b in ((xn[0], xn[2]), (xn[1], xn[3]))]
            for i, pair in enumerate(zip(*terms)):
                xs_v[t, g, i, pl.ds(r // 2, 8), :] = pltpu.pack_elementwise(list(pair), packed_dtype=bf16)

    def feature_map():
        wt = wphi_v[...].astype(f32).T
        full = jnp.concatenate([wt[8 * (g % 4):8 * (g % 4) + 8] for g in range(8) for _ in range(2)], axis=0)
        row = lax.broadcasted_iota(jnp.int32, (128, D), 0)
        col = lax.broadcasted_iota(jnp.int32, (128, D), 1)
        same = (((row >> 6) << 1) | ((row >> 3) & 1)) == ((col >> 5) & 3)
        return jnp.where(same, full, 0.0).astype(bf16)

    def prepare_w(j):
        blocks = []
        for c in (2 * j, 2 * j + 1):
            w = wqkv_v[:, pl.ds(128 * c, 128)]
            if j < 8:
                blocks.append(_dot(bd[:, 128 * (c % 8):128 * (c % 8 + 1)], w, _NT) * LOG2E)
            else:
                blocks.append(w.astype(f32).T)
        blocks = [a[:, 512 * kh:512 * (kh + 1)] for a in blocks for kh in range(2)]
        for i, term in enumerate(_signed_sums([term[0] for term in _HK_TERMS[:7]], blocks)):
            ws_v[j // 2, i, pl.ds(64 * (j % 2), 64), :] = _pack(term)

    def paced_terms(pieces, lag):
        links = []
        for blocks, dest in pieces:
            if len(links) >= lag:
                first = blocks[0]
                blocks = [pltpu.bitcast(_bits(first) ^ jnp.concatenate([links[-lag]] * 2, axis=0), f32)] + blocks[1:]
            words = [_pack(term) for term in _signed_sums([t[0] for t in _HK_TERMS], blocks)]
            for i, w in enumerate(words):
                dest[i] = w
            done = functools.reduce(jnp.bitwise_or, words[4:7] + words[9:15] + words[17:])
            slow = jnp.sum(pltpu.bitcast(done, f32), axis=-1, keepdims=True)
            links.append(_bits(jnp.broadcast_to(slow, (8, 128))) & pace["zero"])

    def prepare_wo(lag):
        pieces = []
        for n in range(2):
            for c in range(4):
                for r in range(0, 128, 16):
                    w = [wo_v[pl.ds(256 * c + 128 * kh + r, 16), pl.ds(512 * n, 512)].astype(f32) for kh in range(2)]
                    pieces.append(([w[kh][:, 128 * i:128 * (i + 1)] for i in range(4) for kh in range(2)],
                                   woh_v.at[n, :, pl.ds(64 * c + r // 2, 8), :]))
        paced_terms(pieces, lag)

    def proj_group(j0, nj, t, g):
        rows = pl.ds(64 * (j0 % 2), 64 * nj)
        return dict(_block_product(
            lambda r: matmul(ws_v[j0 // 2, r, rows, :], xs_v[t, g, r], _NT), 2))

    def pairs(groups):
        return [jnp.concatenate([y[b, hf][r:r + 64] for y in groups for hf in range(2)], axis=1)
                for j in range(groups[0][0, 0].shape[0] // 128) for b in range(2)
                for r in (128 * j, 128 * j + 64)]

    def proj(j0, t):
        return pairs([proj_group(j0, 2, t, g) for g in range(2)])

    kv = [None] * 16
    phi_k = [None] * 16

    def key_features(j, p):
        phi = _features(p)
        phi_k[j] = phi.reshape(128, T).astype(bf16)
        return functools.reduce(jnp.bitwise_or, [_bits(phi[i][:, n:n + 128]) for i in (7, 15)
                                                 for n in range(0, T, 128)])

    def key_tasks(blocks, j0):
        return [None] * 4 + [functools.partial(key_features, j0 + q, p) for q, p in enumerate(blocks)]

    def kv_update(v_blocks, j0):
        for j, v in enumerate(v_blocks, j0):
            v1 = jnp.concatenate([v, jnp.ones((16, T), f32)], axis=0).astype(bf16)
            upd = _dot(v1, phi_k[j], _NT)
            kv[j] = upd if kv[j] is None else kv[j] + upd

    wait_loads()
    layernorm(0, 0, 0)
    pace["zero"] = top[1] >> 31
    wait_loads()
    prepare_w(8)
    wait_loads()
    layernorm(0, 1, 0)
    first = proj_group(8, 1, 0, 0)
    wait_loads()
    v0 = pairs([first, proj_group(8, 1, 0, 1)])
    prepare_w(9)
    first = proj_group(9, 1, 0, 0)
    wait_loads()
    v0 += pairs([first, proj_group(9, 1, 0, 1)])
    for j in (10, 11):
        prepare_w(j)
    if "0" == "0":
        v0 += pairs([proj_group(10, 1, 0, g) for g in range(2)])
        first = proj_group(11, 1, 0, 0)
        wait_loads()
        v0 += pairs([first, proj_group(11, 1, 0, 1)])
    else:
        first = proj_group(10, 2, 0, 0)
        wait_loads()
        v0 += pairs([first, proj_group(10, 2, 0, 1)])
    bd = feature_map()
    for j in (4, 5):
        prepare_w(j)
    first = proj_group(4, 2, 0, 0)
    layernorm(1, 0, 2)
    wait_loads()
    k = pairs([first, proj_group(4, 2, 0, 1)])
    for j in (6, 7):
        prepare_w(j)
    tasks += key_tasks(k[:4], 0)
    rest, k = k[4:], proj(6, 0)
    layernorm(1, 1, 2)
    wait_loads()
    for j, p in enumerate(rest, 4):
        key_features(j, p)
    pending = [(v0[:8], 0), (v0[8:], 8)]
    j0 = 8
    for t in range(1, NT_):
        for c in range(2):
            tasks += key_tasks(k, j0)
            v = proj(8 + 2 * c, t)
            if len(pending) > 1:
                kv_update(*pending.pop(0))
            kv_update(*pending.pop(0))
            if t == NT_ - 1:
                prepare_w(1 + 2 * c)
            k, j0 = proj(4 + 2 * c, t), 8 * c
            pending.append((v, j0))
            if (t, c) in ((NT_ - 2, 1), (NT_ - 1, 0)):
                prepare_w(2 - 2 * c)
        for g in range(2 if t + 1 < NT_ else 0):
            layernorm(t + 1, g, 1)
    tasks += key_tasks(k, j0)

    r_max = jnp.max(top[0])
    idx = jnp.clip(jnp.min(jnp.where(top[0] == r_max, top[1], S)), 0, S - 1)
    t_sel = idx // T
    grp = pl.ds(pl.multiple_of(idx % 128 // 16 * 8, 8), 8)
    x_sel = jnp.concatenate(
        [_unpack(xs_v[t_sel, idx % T // 256, jnp.where(idx % 256 < 128, x_block[kh], x_block[2 + kh]), grp, :])
         for kh in range(2)],
        axis=1).astype(f32)
    x_sel = jnp.where(lax.broadcasted_iota(jnp.int32, (16, D), 0) == idx % 16, x_sel, 0.0)
    x_sel = jnp.broadcast_to(jnp.sum(x_sel, axis=0, keepdims=True), (16, D))
    gate = jax.nn.sigmoid(jnp.full((8, 512), r_max, f32))

    def ffn_program():
        h = []
        for n in range(F // 128):
            acc = []
            for w in (wg_v, wu_v):
                parts = []
                for kh in range(2):
                    dep = yield
                    parts.append(_dot(after(x_sel[:, 512 * kh:512 * (kh + 1)], dep).astype(bf16),
                                      w[pl.ds(512 * kh, 512), pl.ds(n * 128, 128)], _NN))
                    ffn["done"].append(_bits(parts[-1][:8]))
                acc.append(parts[0] + parts[1])
            h.append(_silu(acc[0]) * acc[1])
        for hf in range(2):
            y = None
            for n in range(F // 128):
                dep = yield
                part = _dot(after(h[n], dep).astype(bf16), wd_v[pl.ds(n * 128, 128), pl.ds(hf * 512, 512)], _NN)[:8]
                y = part if y is None else y + part
                ffn["done"].append(_bits(part[:, 384:]))
            ffn["y"][hf] = _rb(y * gate)

    def attend(blocks, j0):
        out = []
        for j, p in enumerate(blocks, j0):
            num = _dot(kv[j], p, _NN)
            for hd in range(2):
                inv = _rcp(num[64 + 8 * hd:72 + 8 * hd] + 1e-6)
                out.append((num[32 * hd:32 * hd + 32].reshape(4, 8, T) * inv[None]).reshape(32, T))
        return [[[jnp.concatenate(out[8 * c + 4 * kh:8 * c + 4 * kh + 4], axis=0)[:, 256 * g:256 * (g + 1)].T
                  for kh in range(2)] for g in range(2)] for c in range(2)]

    stores = []

    def out_proj(i, o_terms, n):
        while i and ffn["y"][n] is None:
            ffn_step()
        for (c, j), block in _block_product(lambda r: matmul(o_terms[r], woh_v[n, r], _NN), 4):
            q = _TOKEN_GROUP[j]
            t, g = tiles[i + q // 2], q % 2
            cols, tok = pl.ds(512 * n + 128 * c, 128), pl.ds(pl.multiple_of(T * t + 256 * g, 256), 256)
            a = jnp.concatenate([_unpack(xs_v[t, g, x_block[2 * hf + n], :, pl.ds(128 * c, 128)])
                                 for hf in range(2)], axis=0).astype(f32)
            if i + q // 2 == NT_ - 1:
                hit = (lax.broadcasted_iota(jnp.int32, (32, 8, 128), 0) * 8
                       + lax.broadcasted_iota(jnp.int32, (32, 8, 128), 1)) == idx % T - 256 * g
                a3 = a.reshape(32, 8, 128)
                a = jnp.where(hit, a3 + ffn["y"][n][:, 128 * c:128 * (c + 1)][None], a3).reshape(256, 128)
            rows = pl.ds(T * i + 256 * q, 256)
            out_v[rows, cols] = (x_v[tok, cols].astype(f32) + block * _silu(a)).astype(bf16)
            if i and n:
                stores.extend(group(9, (out_v.at[rows, cols], out_hbm.at[tok, cols])))
                stores[-1].start()
        if (i, n) in ((0, 1), (2, 0)):
            cols = pl.ds(0, 512) if i else slice(None)
            for q in range(2):
                stores.extend(group(9, (out_v.at[pl.ds(T * (i + q), T), cols],
                                         out_hbm.at[pl.ds(pl.multiple_of(T * tiles[i + q], T), T), cols])))
                stores[-1].start()

    def output_terms(first, second):
        per_group = [_signed_sums([t[1] for t in _HK_TERMS],
                                  [b for q in _TOKEN_GROUP for b in (first, second)[q // 2][c][q % 2]])
                     for c in range(4)]
        return [jnp.concatenate(term, axis=1) for term in zip(*per_group)]

    def last_loads():
        wait_loads()
        prepare_wo(1)
        ffn["steps"], ffn["done"] = ffn_program(), [None, None]
        next(ffn["steps"])

    tiles = [lax.rem(t_sel + 1 + i, NT_) for i in range(NT_)]
    o = [[] for _ in range(NT_)]
    halves = [(i, c) for i in range(NT_) for c in range(2)]
    for h, (i, c) in enumerate(halves):
        q = proj(2 * c, tiles[i])
        if h == 0:
            kv_update(*pending.pop(0))
            row = lax.broadcasted_iota(jnp.int32, (80, 128), 0)
            col = lax.broadcasted_iota(jnp.int32, (80, 128), 1)
            own = jnp.where(row < 64, row >> 5, (row >> 3) & 1) == (col & 1)
            kv[:] = [jnp.where(own, a, 0.0).astype(bf16) for a in kv]
            tasks.extend([None] * 0 + [last_loads])
        else:
            o[halves[h - 1][0]] += attend(prev, 8 * halves[h - 1][1])
        prev = [_features(p).reshape(128, T).astype(bf16) for p in q]
        if h == 6:
            terms = output_terms(*o[:2])
            out_proj(0, terms, 0)
    out_proj(0, terms, 1)
    o[-1] += attend(prev, 8)
    terms = output_terms(*o[2:])
    for n in range(2):
        out_proj(2, terms, n)
    for c in stores:
        c.wait()


@jax.jit
def pallas_recurrent_scan__linear_kernel_hedgehog__moe_arch_mod__prompt_kernel(
    A_x: jax.Array,
    A_wqkv: jax.Array,
    A_w_phi: jax.Array,
    A_wo: jax.Array,
    B_x: jax.Array,
    B_w_r: jax.Array,
    B_w_gate: jax.Array,
    B_w_up: jax.Array,
    B_w_down: jax.Array,
):
    del B_x
    hbm = pl.BlockSpec(memory_space=pl.ANY)
    out = pl.pallas_call(
        _kernel,
        out_shape=jax.ShapeDtypeStruct((S, D), bf16),
        in_specs=[hbm] * 8,
        out_specs=hbm,
        scratch_shapes=[
            pltpu.VMEM((S, D), bf16),
            pltpu.VMEM((NT_, 2, 9, 64, 512), jnp.uint32),
            pltpu.VMEM((D, 3 * D), bf16),
            pltpu.VMEM((6, 7, 128, 512), jnp.uint32),
            pltpu.VMEM((D, D), bf16),
            pltpu.VMEM((2, 26, 256, 128), jnp.uint32),
            pltpu.VMEM((D, F), bf16),
            pltpu.VMEM((D, F), bf16),
            pltpu.VMEM((F, D), bf16),
            pltpu.VMEM((S, D), bf16),
            pltpu.VMEM((H * DH, DH), bf16),
            pltpu.VMEM((D,), bf16),
            pltpu.SemaphoreType.DMA((10,)),
        ],
        compiler_params=pltpu.CompilerParams(vmem_limit_bytes=110 * 1024 * 1024),
        name="hedgehog_mod",
    )(
        A_x.reshape(S, D), A_wqkv, A_w_phi.reshape(H * DH, DH), A_wo,
        B_w_r, B_w_gate, B_w_up, B_w_down,
    )
    return out.reshape(1, S, D)
```

```python
import functools
import math

import jax
import jax.numpy as jnp
from jax import lax
import jax.experimental.pallas as pl
import jax.experimental.pallas.tpu as pltpu

S, D, H, DH, F = 2048, 1024, 32, 32, 3584
T = 512
NT_ = S // T
LOG2E = math.log2(math.e)
_NT = (((1,), (1,)), ((), ()))
_NN = (((1,), (0,)), ((), ()))
f32, bf16 = jnp.float32, jnp.bfloat16


def _dot(a, b, dn):
    return lax.dot_general(a, b, dn, preferred_element_type=f32)


def _rb(v):
    return v.astype(bf16).astype(f32)


def _rcp(v):
    r = pl.reciprocal(v, approx=True)
    return r * (2.0 - v * r)


def _silu(a):
    return a * pl.reciprocal(1.0 + jnp.exp2(a * -LOG2E), approx=True)


def _bits(v):
    return pltpu.bitcast(v, jnp.int32)


def _pack(v):
    return pltpu.bitcast(v.astype(bf16), jnp.uint32)


def _unpack(words):
    return pltpu.bitcast(words, bf16)


_HK_TERMS = (
    ((1,), (1, -2)), ((1, 2), (2,)), ((3, 4), (3,)), ((-4,), (3, -4)),
    ((1, 4), (2, 3)), ((-1, 3), (1, 3)), ((2, -4), (2, 4)),
    ((6,), (6,)), ((5,), (5,)),
    ((-3, -4, 5), (3, -4, -6)), ((-3, -4, 5, 6), (4, 6)), ((3, -5), (3, -4, 5, -6)),
    ((1, 2, -6), (1, -2, 5)), ((-2, 6), (1, -2, 5, -6)), ((-1, -2, 5, 6), (1, 5)),
    ((7,), (7, -8)), ((7, 8), (8,)),
    ((4, 7), (3, 8)), ((3, -7), (3, 7)), ((-4, 8), (4, 8)),
    ((-6, 7, 8), (5, 7, -8)), ((6, -8), (5, -6, 7, -8)), ((5, 6, -7, -8), (5, 7)),
    ((2, -6, 7), (1, 5, 8)), ((1, -5, -7), (1, 5, 7)), ((-2, 6, 8), (2, 6, 8)),
)
_HK_SUMS = (
    ((0, 0), (2, 1)), ((1, 1), (4, 3)), ((1, 0), (6, 5, 1, -3)), ((0, 1), (7, 5, 4, -2)),
    ((2, 2), (9, 8)), ((2, 1), (11, 10, 3, -8)), ((1, 2), (12, 10, 9, -4)),
    ((0, 2), (14, 13, 8, -1)), ((2, 0), (15, 13, 2, -9)), ((3, 3), (17, 16)),
    ((1, 3), (19, 18, 16, -3)), ((3, 1), (20, 18, 4, -17)),
    ((3, 2), (22, 21, 8, -16)), ((2, 3), (23, 21, 17, -9)),
    ((0, 3), (25, 24, 16, 15), (2, 3), 1), ((3, 0), (26, 24, 14, -17), (3, 2), -1),
)
_TOKEN_GROUP = (0, 2, 3, 1)


def _signed_sums(wanted, blocks):
    known = {(i + 1,): b for i, b in enumerate(blocks)}

    def value(key):
        if key not in known:
            for part in sorted(known, key=len, reverse=True):
                for sign in (1, -1):
                    signed = [sign * p for p in part]
                    if key not in known and len(part) < len(key) and all(p in key for p in signed):
                        rest = tuple(k for k in key if k not in signed)
                        if sign > 0 and rest[0] < 0:
                            known[key] = known[part] - value(tuple(-k for k in rest))
                        else:
                            known[key] = value(rest) + known[part] if sign > 0 else value(rest) - known[part]
            if key not in known:
                known[key] = -known[(-key[0],)]
        return known[key]

    for key in sorted(wanted, key=len):
        value(key)
    return [known[key] for key in wanted]


def _block_product(product, size):
    m, y = [], {}
    for ij, parts, *earlier in _HK_SUMS[:size * size]:
        while len(m) < parts[0]:
            m.append(product(len(m)))
        total = m[parts[0] - 1]
        for p in parts[1:]:
            total = total + m[p - 1] if p > 0 else total - m[-p - 1]
        if earlier:
            total = total + y[earlier[0]] if earlier[1] > 0 else total - y[earlier[0]]
        y[ij] = total
        yield ij, total


def _allreduce(v, op):
    r = v[0]
    for i in range(1, 8):
        r = op(r, v[i])
    r = op(r, pltpu.roll(r, 4, 0))
    return op(r, pltpu.roll(r, 2, 0))


def _features(p):
    p3 = p.reshape(8, 8, p.shape[1])
    mx = _allreduce(p3, jnp.maximum)
    mn = _allreduce(p3, jnp.minimum)
    ep = jnp.exp2(p3 - mx[None])
    en = jnp.exp2(mn[None] - p3)
    ip = _rcp(_allreduce(ep, jnp.add))
    im = _rcp(_allreduce(en, jnp.add))
    return jnp.concatenate([ep * ip[None], en * im[None]], axis=0)


def _kernel(x_hbm, wqkv_hbm, wphi_hbm, wo_hbm, wr_hbm, wg_hbm, wu_hbm, wd_hbm, out_hbm,
            x_v, xs_v, wqkv_v, ws_v, wo_v, woh_v, wg_v, wu_v, wd_v, out_v, wphi_v, wr_v, sems):
    def group(k, *pairs):
        return [pltpu.make_async_copy(src, dst, sems.at[k]) for src, dst in pairs]

    def x_rows(r0, n):
        return x_hbm.at[pl.ds(r0, n)], x_v.at[pl.ds(r0, n)]

    def w_cols(j0, nj):
        cols = pl.ds(256 * j0, 256 * nj)
        return wqkv_hbm.at[:, cols], wqkv_v.at[:, cols]

    loads = [
        group(0, x_rows(0, 256), (wr_hbm, wr_v)),
        group(1, w_cols(8, 1)),
        group(2, x_rows(256, 256)),
        group(3, w_cols(9, 1)),
        group(4, w_cols(10, 2)),
        group(5, (wphi_hbm, wphi_v), w_cols(4, 2), x_rows(T, 256)),
        group(6, w_cols(6, 2), x_rows(T + 256, 256)),
        group(7, x_rows(2 * T, S - 2 * T), w_cols(0, 4)),
        group(8, (wo_hbm, wo_v), (wg_hbm, wg_v), (wu_hbm, wu_v), (wd_hbm, wd_v)),
    ]
    for copies in loads:
        for c in copies:
            c.start()

    def wait_loads():
        for c in loads.pop(0):
            c.wait()

    tasks = []
    pace = {}

    def after(v, dep):
        first = pltpu.bitcast(_bits(v[:8, :128]) ^ (dep & pace["zero"]), v.dtype)
        if v.shape[1] > 128:
            first = jnp.concatenate([first, v[:8, 128:]], axis=1)
        return jnp.concatenate([first, v[8:]], axis=0)

    ffn = {"steps": None, "done": [], "y": [None, None]}

    def ffn_step():
        try:
            ffn["steps"].send(ffn["main"])
        except StopIteration:
            ffn["steps"] = None

    def matmul(lhs, rhs, dn):
        task = tasks.pop(0) if tasks else None
        dep = task() if task is not None else None
        if ffn["done"]:
            dep = ffn["done"].pop(0)
        if dep is not None:
            lhs = after(lhs, dep)
        m = _dot(lhs.astype(bf16) if lhs.dtype == f32 else _unpack(lhs), _unpack(rhs), dn)
        if ffn["steps"] is not None:
            ffn_step()
        ffn["main"] = _bits(m[-8:, -128:])
        return m

    top = [jnp.full((8, 128), -jnp.inf, f32), lax.broadcasted_iota(jnp.int32, (8, 128), 0)]
    chain = []
    x_keys = [term[1] for term in _HK_TERMS[:7]] + [(1,), (4,)]
    x_block = [x_keys.index((i + 1,)) for i in range(4)]

    def layernorm(t, g, lag):
        wr = wr_v[...].astype(f32).reshape(1, D)
        row = lax.broadcasted_iota(jnp.int32, (8, 128), 0)
        for r in range(0, 128, 16):
            blocks = []
            for r0 in (T * t + 256 * g + r, T * t + 256 * g + 128 + r):
                x = x_v[pl.ds(r0, 16), :].astype(f32)
                total = x[:, :128]
                for i in range(1, D // 128):
                    total = total + x[:, 128 * i:128 * (i + 1)]
                if lag:
                    total = jnp.where(jnp.concatenate([chain[-lag]] * 2, axis=0) >= 0, total, 0.0)
                xc = x - jnp.sum(total, axis=-1, keepdims=True) * (1.0 / D)
                v = jnp.mean(xc * xc, axis=-1, keepdims=True)
                xn = xc * (1.0 / _rb(jnp.sqrt(_rb(_rb(v) + _rb(jnp.full_like(v, 1e-5))))))
                blocks += [xn[:, :512], xn[:, 512:]]
                score = jnp.broadcast_to(_rb(jnp.sum(xn * wr, axis=-1, keepdims=True)), (16, 128))
                for i in (0, 8):
                    sc, tok = score[i:i + 8], row + (r0 + i)
                    better = (sc > top[0]) | ((sc == top[0]) & (tok < top[1]))
                    top[:] = jnp.where(better, sc, top[0]), jnp.where(better, tok, top[1])
                chain.append(top[1])
            for i, term in enumerate(_signed_sums(x_keys, blocks)):
                xs_v.at[t, g, i][pl.ds(r // 2, 8), :] = _pack(term)

    def feature_map():
        high = pltpu.bitcast(wphi_v[...].astype(f32).T, jnp.uint32)
        head = (lax.broadcasted_iota(jnp.int32, (DH, D), 1) >> 5) & 3
        none = jnp.zeros_like(high)
        return _unpack(jnp.concatenate(
            [jnp.where(head == 2 * p, high >> 16, none) | jnp.where(head == 2 * p + 1, high, none)
             for p in range(2)], axis=0))

    def prepare_w(j):
        blocks = []
        for c in (2 * j, 2 * j + 1):
            w = wqkv_v[:, pl.ds(128 * c, 128)]
            if j < 8:
                blocks.append(_dot(bd[:, 128 * (c % 8):128 * (c % 8 + 1)], w, _NT) * LOG2E)
            else:
                blocks.append(w.astype(f32).T)
        blocks = [a[:, 512 * kh:512 * (kh + 1)] for a in blocks for kh in range(2)]
        for i, term in enumerate(_signed_sums([term[0] for term in _HK_TERMS[:7]], blocks)):
            ws_v.at[j // 2, i][pl.ds(64 * (j % 2), 64), :] = _pack(term)

    def prepare_wo():
        link = pace["zero"]
        for n in range(2):
            for r in range(0, D // 2, 16):
                w = [wo_v[pl.ds(r // 128 * 256 + 128 * kh + r % 128, 16), pl.ds(512 * n, 512)].astype(f32)
                     for kh in range(2)]
                blocks = [w[kh][:, 128 * i:128 * (i + 1)] for i in range(4) for kh in range(2)]
                blocks[0] = pltpu.bitcast(_bits(blocks[0]) ^ jnp.concatenate([link] * 2, axis=0), f32)
                terms = _signed_sums([term[0] for term in _HK_TERMS], blocks)
                woh_v.at[n][pl.ds(r // 2, 8), :] = _pack(jnp.concatenate(terms, axis=1))
                done = functools.reduce(jnp.bitwise_or, [
                    _bits(term[h:h + 8]) for term in terms[4:7] + terms[9:15] + terms[17:] for h in (0, 8)])
                slow = jnp.sum(pltpu.bitcast(done, f32), axis=-1, keepdims=True)
                link = _bits(jnp.broadcast_to(slow, (8, 128))) & pace["zero"]

    def proj_group(j0, nj, t, g):
        rows = pl.ds(64 * (j0 % 2), 64 * nj)
        return dict(_block_product(
            lambda r: matmul(ws_v[j0 // 2, r, rows, :], xs_v[t, g, r], _NT), 2))

    def pairs(groups):
        return [jnp.concatenate([y[b, hf][r:r + 64] for y in groups for hf in range(2)], axis=1)
                for j in range(groups[0][0, 0].shape[0] // 128) for b in range(2)
                for r in (128 * j, 128 * j + 64)]

    def proj(j0, t):
        return pairs([proj_group(j0, 2, t, g) for g in range(2)])

    kv = [None] * 16
    phi_k = [None] * 16

    def key_features(j, p):
        phi = _features(p)
        phi_k[j] = phi.reshape(128, T).astype(bf16)
        return functools.reduce(jnp.bitwise_or, [_bits(phi[i][:, n:n + 128]) for i in (7, 15)
                                                 for n in range(0, T, 128)])

    def key_tasks(blocks, j0):
        return [None] * 4 + [functools.partial(key_features, j0 + q, p) for q, p in enumerate(blocks)]

    def kv_update(v_blocks, j0):
        for j, v in enumerate(v_blocks, j0):
            v1 = jnp.concatenate([v, jnp.ones((16, T), f32)], axis=0).astype(bf16)
            upd = _dot(v1, phi_k[j], _NT)
            kv[j] = upd if kv[j] is None else kv[j] + upd

    wait_loads()
    layernorm(0, 0, 0)
    pace["zero"] = top[1] >> 31
    wait_loads()
    prepare_w(8)
    wait_loads()
    layernorm(0, 1, 0)
    first = proj_group(8, 1, 0, 0)
    wait_loads()
    v0 = pairs([first, proj_group(8, 1, 0, 1)])
    prepare_w(9)
    first = proj_group(9, 1, 0, 0)
    wait_loads()
    v0 += pairs([first, proj_group(9, 1, 0, 1)])
    for j in (10, 11):
        prepare_w(j)
    if "0" == "0":
        v0 += pairs([proj_group(10, 1, 0, g) for g in range(2)])
        first = proj_group(11, 1, 0, 0)
        wait_loads()
        v0 += pairs([first, proj_group(11, 1, 0, 1)])
    else:
        first = proj_group(10, 2, 0, 0)
        wait_loads()
        v0 += pairs([first, proj_group(10, 2, 0, 1)])
    bd = feature_map()
    for j in (4, 5):
        prepare_w(j)
    first = proj_group(4, 2, 0, 0)
    layernorm(1, 0, 2)
    wait_loads()
    k = pairs([first, proj_group(4, 2, 0, 1)])
    for j in (6, 7):
        prepare_w(j)
    tasks += key_tasks(k[:4], 0)
    rest, k = k[4:], proj(6, 0)
    layernorm(1, 1, 2)
    wait_loads()
    for j, p in enumerate(rest, 4):
        key_features(j, p)
    pending = [(v0[:8], 0), (v0[8:], 8)]
    j0 = 8
    for t in range(1, NT_):
        for c in range(2):
            tasks += key_tasks(k, j0)
            v = proj(8 + 2 * c, t)
            if len(pending) > 1:
                kv_update(*pending.pop(0))
            kv_update(*pending.pop(0))
            if t == NT_ - 1:
                prepare_w(1 + 2 * c)
            k, j0 = proj(4 + 2 * c, t), 8 * c
            pending.append((v, j0))
            if (t, c) in ((NT_ - 2, 1), (NT_ - 1, 0)):
                prepare_w(2 - 2 * c)
        for g in range(2 if t + 1 < NT_ else 0):
            layernorm(t + 1, g, 1)
    tasks += key_tasks(k, j0)

    r_max = jnp.max(top[0])
    idx = jnp.clip(jnp.min(jnp.where(top[0] == r_max, top[1], S)), 0, S - 1)
    t_sel = idx // T
    grp = pl.ds(pl.multiple_of(idx % 128 // 16 * 8, 8), 8)
    x_sel = jnp.concatenate(
        [_unpack(xs_v[t_sel, idx % T // 256, jnp.where(idx % 256 < 128, x_block[kh], x_block[2 + kh]), grp, :])
         for kh in range(2)],
        axis=1).astype(f32)
    x_sel = jnp.where(lax.broadcasted_iota(jnp.int32, (16, D), 0) == idx % 16, x_sel, 0.0)
    x_sel = jnp.broadcast_to(jnp.sum(x_sel, axis=0, keepdims=True), (16, D))
    gate = jax.nn.sigmoid(jnp.full((8, 512), r_max, f32))

    def ffn_program():
        h = []
        for n in range(F // 128):
            acc = []
            for w in (wg_v, wu_v):
                parts = []
                for kh in range(2):
                    dep = yield
                    parts.append(_dot(after(x_sel[:, 512 * kh:512 * (kh + 1)], dep).astype(bf16),
                                      w[pl.ds(512 * kh, 512), pl.ds(n * 128, 128)], _NN))
                    ffn["done"].append(_bits(parts[-1][:8]))
                acc.append(parts[0] + parts[1])
            h.append(_silu(acc[0]) * acc[1])
        for hf in range(2):
            y = None
            for n in range(F // 128):
                dep = yield
                part = _dot(after(h[n], dep).astype(bf16), wd_v[pl.ds(n * 128, 128), pl.ds(hf * 512, 512)], _NN)[:8]
                y = part if y is None else y + part
                ffn["done"].append(_bits(part[:, 384:]))
            ffn["y"][hf] = _rb(y * gate)

    def attend(blocks, j0):
        out = []
        for j, p in enumerate(blocks, j0):
            num = _dot(kv[j], p, _NN)
            for hd in range(2):
                inv = _rcp(num[64 + 8 * hd:72 + 8 * hd] + 1e-6)
                out.append((num[32 * hd:32 * hd + 32].reshape(4, 8, T) * inv[None]).reshape(32, T))
        return [[[jnp.concatenate(out[8 * c + 4 * kh:8 * c + 4 * kh + 4], axis=0)[:, 256 * g:256 * (g + 1)].T
                  for kh in range(2)] for g in range(2)] for c in range(2)]

    stores = []

    def out_proj(i, o_terms, n):
        while i and ffn["y"][n] is None:
            ffn_step()
        for (c, j), block in _block_product(lambda r: matmul(o_terms[r], woh_v[n, :, pl.ds(128 * r, 128)], _NN), 4):
            q = _TOKEN_GROUP[j]
            t, g = tiles[i + q // 2], q % 2
            cols, tok = pl.ds(512 * n + 128 * c, 128), pl.ds(pl.multiple_of(T * t + 256 * g, 256), 256)
            a = jnp.concatenate([_unpack(xs_v[t, g, x_block[2 * hf + n], :, pl.ds(128 * c, 128)])
                                 for hf in range(2)], axis=0).astype(f32)
            if i + q // 2 == NT_ - 1:
                hit = (lax.broadcasted_iota(jnp.int32, (32, 8, 128), 0) * 8
                       + lax.broadcasted_iota(jnp.int32, (32, 8, 128), 1)) == idx % T - 256 * g
                a3 = a.reshape(32, 8, 128)
                a = jnp.where(hit, a3 + ffn["y"][n][:, 128 * c:128 * (c + 1)][None], a3).reshape(256, 128)
            rows = pl.ds(T * i + 256 * q, 256)
            out_v[rows, cols] = (x_v[tok, cols].astype(f32) + block * _silu(a)).astype(bf16)
            if i and n:
                stores.extend(group(9, (out_v.at[rows, cols], out_hbm.at[tok, cols])))
                stores[-1].start()
        if (i, n) in ((0, 1), (2, 0)):
            cols = pl.ds(0, 512) if i else slice(None)
            for q in range(2):
                stores.extend(group(9, (out_v.at[pl.ds(T * (i + q), T), cols],
                                         out_hbm.at[pl.ds(pl.multiple_of(T * tiles[i + q], T), T), cols])))
                stores[-1].start()

    def output_terms(first, second):
        per_group = [_signed_sums([t[1] for t in _HK_TERMS],
                                  [b for q in _TOKEN_GROUP for b in (first, second)[q // 2][c][q % 2]])
                     for c in range(4)]
        return [jnp.concatenate(term, axis=1) for term in zip(*per_group)]

    def last_loads():
        wait_loads()
        prepare_wo()
        ffn["steps"], ffn["done"] = ffn_program(), [None, None]
        next(ffn["steps"])

    tiles = [lax.rem(t_sel + 1 + i, NT_) for i in range(NT_)]
    o = [[] for _ in range(NT_)]
    halves = [(i, c) for i in range(NT_) for c in range(2)]
    for h, (i, c) in enumerate(halves):
        q = proj(2 * c, tiles[i])
        if h == 0:
            kv_update(*pending.pop(0))
            row = lax.broadcasted_iota(jnp.int32, (80, 128), 0)
            col = lax.broadcasted_iota(jnp.int32, (80, 128), 1)
            own = jnp.where(row < 64, row >> 5, (row >> 3) & 1) == (col & 1)
            kv[:] = [jnp.where(own, a, 0.0).astype(bf16) for a in kv]
            tasks.extend([None] * 0 + [last_loads])
        else:
            o[halves[h - 1][0]] += attend(prev, 8 * halves[h - 1][1])
        prev = [_features(p).reshape(128, T).astype(bf16) for p in q]
        if h == 7:
            terms = output_terms(*o[:2])
            out_proj(0, terms, 0)
    out_proj(0, terms, 1)
    o[-1] += attend(prev, 8)
    terms = output_terms(*o[2:])
    for n in range(2):
        out_proj(2, terms, n)
    for c in stores:
        c.wait()


@jax.jit
def pallas_recurrent_scan__linear_kernel_hedgehog__moe_arch_mod__prompt_kernel(
    A_x: jax.Array,
    A_wqkv: jax.Array,
    A_w_phi: jax.Array,
    A_wo: jax.Array,
    B_x: jax.Array,
    B_w_r: jax.Array,
    B_w_gate: jax.Array,
    B_w_up: jax.Array,
    B_w_down: jax.Array,
):
    del B_x
    hbm = pl.BlockSpec(memory_space=pl.ANY)
    out = pl.pallas_call(
        _kernel,
        out_shape=jax.ShapeDtypeStruct((S, D), bf16),
        in_specs=[hbm] * 8,
        out_specs=hbm,
        scratch_shapes=[
            pltpu.VMEM((S, D), bf16),
            pltpu.VMEM((NT_, 2, 9, 64, 512), jnp.uint32),
            pltpu.VMEM((D, 3 * D), bf16),
            pltpu.VMEM((6, 7, 128, 512), jnp.uint32),
            pltpu.VMEM((D, D), bf16),
            pltpu.VMEM((2, 256, 26 * 128), jnp.uint32),
            pltpu.VMEM((D, F), bf16),
            pltpu.VMEM((D, F), bf16),
            pltpu.VMEM((F, D), bf16),
            pltpu.VMEM((S, D), bf16),
            pltpu.VMEM((H * DH, DH), bf16),
            pltpu.VMEM((D,), bf16),
            pltpu.SemaphoreType.DMA((10,)),
        ],
        compiler_params=pltpu.CompilerParams(vmem_limit_bytes=110 * 1024 * 1024),
        name="hedgehog_mod",
    )(
        A_x.reshape(S, D), A_wqkv, A_w_phi.reshape(H * DH, DH), A_wo,
        B_w_r, B_w_gate, B_w_up, B_w_down,
    )
    return out.reshape(1, S, D)
```

```python
import functools
import math

import jax
import jax.numpy as jnp
from jax import lax
import jax.experimental.pallas as pl
import jax.experimental.pallas.tpu as pltpu

S, D, H, DH, F = 2048, 1024, 32, 32, 3584
T = 512
NT_ = S // T
LOG2E = math.log2(math.e)
_NT = (((1,), (1,)), ((), ()))
_NN = (((1,), (0,)), ((), ()))
f32, bf16 = jnp.float32, jnp.bfloat16


def _dot(a, b, dn):
    return lax.dot_general(a, b, dn, preferred_element_type=f32)


def _rb(v):
    return v.astype(bf16).astype(f32)


def _rcp(v):
    r = pl.reciprocal(v, approx=True)
    return r * (2.0 - v * r)


def _silu(a):
    return a * pl.reciprocal(1.0 + jnp.exp2(a * -LOG2E), approx=True)


def _bits(v):
    return pltpu.bitcast(v, jnp.int32)


def _pack(v):
    return pltpu.bitcast(v.astype(bf16), jnp.uint32)


def _unpack(words):
    return pltpu.bitcast(words, bf16)


_HK_TERMS = (
    ((1,), (1, -2)), ((1, 2), (2,)), ((3, 4), (3,)), ((-4,), (3, -4)),
    ((1, 4), (2, 3)), ((-1, 3), (1, 3)), ((2, -4), (2, 4)),
    ((6,), (6,)), ((5,), (5,)),
    ((-3, -4, 5), (3, -4, -6)), ((-3, -4, 5, 6), (4, 6)), ((3, -5), (3, -4, 5, -6)),
    ((1, 2, -6), (1, -2, 5)), ((-2, 6), (1, -2, 5, -6)), ((-1, -2, 5, 6), (1, 5)),
    ((7,), (7, -8)), ((7, 8), (8,)),
    ((4, 7), (3, 8)), ((3, -7), (3, 7)), ((-4, 8), (4, 8)),
    ((-6, 7, 8), (5, 7, -8)), ((6, -8), (5, -6, 7, -8)), ((5, 6, -7, -8), (5, 7)),
    ((2, -6, 7), (1, 5, 8)), ((1, -5, -7), (1, 5, 7)), ((-2, 6, 8), (2, 6, 8)),
)
_HK_SUMS = (
    ((0, 0), (2, 1)), ((1, 1), (4, 3)), ((1, 0), (6, 5, 1, -3)), ((0, 1), (7, 5, 4, -2)),
    ((2, 2), (9, 8)), ((2, 1), (11, 10, 3, -8)), ((1, 2), (12, 10, 9, -4)),
    ((0, 2), (14, 13, 8, -1)), ((2, 0), (15, 13, 2, -9)), ((3, 3), (17, 16)),
    ((1, 3), (19, 18, 16, -3)), ((3, 1), (20, 18, 4, -17)),
    ((3, 2), (22, 21, 8, -16)), ((2, 3), (23, 21, 17, -9)),
    ((0, 3), (25, 24, 16, 15), (2, 3), 1), ((3, 0), (26, 24, 14, -17), (3, 2), -1),
)
_TOKEN_GROUP = (0, 2, 3, 1)


def _signed_sums(wanted, blocks):
    known = {(i + 1,): b for i, b in enumerate(blocks)}

    def value(key):
        if key not in known:
            for part in sorted(known, key=len, reverse=True):
                for sign in (1, -1):
                    signed = [sign * p for p in part]
                    if key not in known and len(part) < len(key) and all(p in key for p in signed):
                        rest = tuple(k for k in key if k not in signed)
                        if sign > 0 and rest[0] < 0:
                            known[key] = known[part] - value(tuple(-k for k in rest))
                        else:
                            known[key] = value(rest) + known[part] if sign > 0 else value(rest) - known[part]
            if key not in known:
                known[key] = -known[(-key[0],)]
        return known[key]

    for key in sorted(wanted, key=len):
        value(key)
    return [known[key] for key in wanted]


def _block_product(product, size):
    m, y = [], {}
    for ij, parts, *earlier in _HK_SUMS[:size * size]:
        while len(m) < parts[0]:
            m.append(product(len(m)))
        total = m[parts[0] - 1]
        for p in parts[1:]:
            total = total + m[p - 1] if p > 0 else total - m[-p - 1]
        if earlier:
            total = total + y[earlier[0]] if earlier[1] > 0 else total - y[earlier[0]]
        y[ij] = total
        yield ij, total


def _allreduce(v, op):
    r = v[0]
    for i in range(1, 8):
        r = op(r, v[i])
    r = op(r, pltpu.roll(r, 4, 0))
    return op(r, pltpu.roll(r, 2, 0))


def _features(p):
    p3 = p.reshape(8, 8, p.shape[1])
    mx = _allreduce(p3, jnp.maximum)
    mn = _allreduce(p3, jnp.minimum)
    ep = jnp.exp2(p3 - mx[None])
    en = jnp.exp2(mn[None] - p3)
    ip = _rcp(_allreduce(ep, jnp.add))
    im = _rcp(_allreduce(en, jnp.add))
    return jnp.concatenate([ep * ip[None], en * im[None]], axis=0)


def _kernel(x_hbm, wqkv_hbm, wphi_hbm, wo_hbm, wr_hbm, wg_hbm, wu_hbm, wd_hbm, out_hbm,
            x_v, xs_v, wqkv_v, ws_v, wo_v, woh_v, wg_v, wu_v, wd_v, out_v, wphi_v, wr_v, sems):
    def group(k, *pairs):
        return [pltpu.make_async_copy(src, dst, sems.at[k]) for src, dst in pairs]

    def x_rows(r0, n):
        return x_hbm.at[pl.ds(r0, n)], x_v.at[pl.ds(r0, n)]

    def w_cols(j0, nj):
        cols = pl.ds(256 * j0, 256 * nj)
        return wqkv_hbm.at[:, cols], wqkv_v.at[:, cols]

    loads = [
        group(0, x_rows(0, 256), (wr_hbm, wr_v)),
        group(1, w_cols(8, 1)),
        group(2, x_rows(256, 256)),
        group(3, w_cols(9, 1)),
        group(4, w_cols(10, 2)),
        group(5, (wphi_hbm, wphi_v), w_cols(4, 2), x_rows(T, 256)),
        group(6, w_cols(6, 2), x_rows(T + 256, 256)),
        group(7, x_rows(2 * T, S - 2 * T), w_cols(0, 4)),
        group(8, (wo_hbm, wo_v), (wg_hbm, wg_v), (wu_hbm, wu_v), (wd_hbm, wd_v)),
    ]
    for copies in loads:
        for c in copies:
            c.start()

    def wait_loads():
        for c in loads.pop(0):
            c.wait()

    tasks = []
    pace = {}

    def after(v, dep):
        first = pltpu.bitcast(_bits(v[:8, :128]) ^ (dep & pace["zero"]), v.dtype)
        if v.shape[1] > 128:
            first = jnp.concatenate([first, v[:8, 128:]], axis=1)
        return jnp.concatenate([first, v[8:]], axis=0)

    ffn = {"steps": None, "done": [], "y": [None, None]}

    def ffn_step():
        try:
            ffn["steps"].send(ffn["main"])
        except StopIteration:
            ffn["steps"] = None

    def matmul(lhs, rhs, dn):
        task = tasks.pop(0) if tasks else None
        dep = task() if task is not None else None
        if ffn["done"]:
            dep = ffn["done"].pop(0)
        if dep is not None:
            lhs = after(lhs, dep)
        m = _dot(lhs.astype(bf16) if lhs.dtype == f32 else _unpack(lhs), _unpack(rhs), dn)
        if ffn["steps"] is not None:
            ffn_step()
        ffn["main"] = _bits(m[:8, :128])
        return m

    top = [jnp.full((8, 128), -jnp.inf, f32), lax.broadcasted_iota(jnp.int32, (8, 128), 0)]
    chain = []
    x_keys = [term[1] for term in _HK_TERMS[:7]] + [(1,), (4,)]
    x_block = [x_keys.index((i + 1,)) for i in range(4)]

    def layernorm(t, g, lag):
        wr = wr_v[...].astype(f32).reshape(1, D)
        row = lax.broadcasted_iota(jnp.int32, (8, 128), 0)
        for r in range(0, 128, 16):
            blocks = []
            for r0 in (T * t + 256 * g + r, T * t + 256 * g + 128 + r):
                x = x_v[pl.ds(r0, 16), :].astype(f32)
                total = x[:, :128]
                for i in range(1, D // 128):
                    total = total + x[:, 128 * i:128 * (i + 1)]
                if lag:
                    total = jnp.where(jnp.concatenate([chain[-lag]] * 2, axis=0) >= 0, total, 0.0)
                xc = x - jnp.sum(total, axis=-1, keepdims=True) * (1.0 / D)
                v = jnp.mean(xc * xc, axis=-1, keepdims=True)
                xn = xc * (1.0 / _rb(jnp.sqrt(_rb(_rb(v) + _rb(jnp.full_like(v, 1e-5))))))
                blocks += [xn[:, :512], xn[:, 512:]]
                score = jnp.broadcast_to(_rb(jnp.sum(xn * wr, axis=-1, keepdims=True)), (16, 128))
                for i in (0, 8):
                    sc, tok = score[i:i + 8], row + (r0 + i)
                    better = (sc > top[0]) | ((sc == top[0]) & (tok < top[1]))
                    top[:] = jnp.where(better, sc, top[0]), jnp.where(better, tok, top[1])
                chain.append(top[1])
            for i, term in enumerate(_signed_sums(x_keys, blocks)):
                xs_v.at[t, g, i][pl.ds(r // 2, 8), :] = _pack(term)

    def feature_map():
        high = pltpu.bitcast(wphi_v[...].astype(f32).T, jnp.uint32)
        head = (lax.broadcasted_iota(jnp.int32, (DH, D), 1) >> 5) & 3
        none = jnp.zeros_like(high)
        return _unpack(jnp.concatenate(
            [jnp.where(head == 2 * p, high >> 16, none) | jnp.where(head == 2 * p + 1, high, none)
             for p in range(2)], axis=0))

    def prepare_w(j):
        blocks = []
        for c in (2 * j, 2 * j + 1):
            w = wqkv_v[:, pl.ds(128 * c, 128)]
            if j < 8:
                blocks.append(_dot(bd[:, 128 * (c % 8):128 * (c % 8 + 1)], w, _NT) * LOG2E)
            else:
                blocks.append(w.astype(f32).T)
        blocks = [a[:, 512 * kh:512 * (kh + 1)] for a in blocks for kh in range(2)]
        for i, term in enumerate(_signed_sums([term[0] for term in _HK_TERMS[:7]], blocks)):
            ws_v.at[j // 2, i][pl.ds(64 * (j % 2), 64), :] = _pack(term)

    def prepare_wo():
        link = pace["zero"]
        for n in range(2):
            for r in range(0, D // 2, 16):
                w = [wo_v[pl.ds(r // 128 * 256 + 128 * kh + r % 128, 16), pl.ds(512 * n, 512)].astype(f32)
                     for kh in range(2)]
                blocks = [w[kh][:, 128 * i:128 * (i + 1)] for i in range(4) for kh in range(2)]
                blocks[0] = pltpu.bitcast(_bits(blocks[0]) ^ jnp.concatenate([link] * 2, axis=0), f32)
                terms = _signed_sums([term[0] for term in _HK_TERMS], blocks)
                woh_v.at[n][pl.ds(r // 2, 8), :] = _pack(jnp.concatenate(terms, axis=1))
                done = functools.reduce(jnp.bitwise_or, [
                    _bits(term[h:h + 8]) for term in terms[4:7] + terms[9:15] + terms[17:] for h in (0, 8)])
                for _ in range(2):
                    slow = jnp.sum(pltpu.bitcast(done, f32), axis=-1, keepdims=True)
                    done = link = _bits(jnp.broadcast_to(slow, (8, 128))) & pace["zero"]

    def proj_group(j0, nj, t, g):
        rows = pl.ds(64 * (j0 % 2), 64 * nj)
        return dict(_block_product(
            lambda r: matmul(ws_v[j0 // 2, r, rows, :], xs_v[t, g, r], _NT), 2))

    def pairs(groups):
        return [jnp.concatenate([y[b, hf][r:r + 64] for y in groups for hf in range(2)], axis=1)
                for j in range(groups[0][0, 0].shape[0] // 128) for b in range(2)
                for r in (128 * j, 128 * j + 64)]

    def proj(j0, t):
        return pairs([proj_group(j0, 2, t, g) for g in range(2)])

    kv = [None] * 16
    phi_k = [None] * 16

    def key_features(j, p):
        phi = _features(p)
        phi_k[j] = phi.reshape(128, T).astype(bf16)
        return functools.reduce(jnp.bitwise_or, [_bits(phi[7][:, n:n + 128]) for n in range(0, T, 128)])

    def key_tasks(blocks, j0):
        return [None] * 4 + [functools.partial(key_features, j0 + q, p) for q, p in enumerate(blocks)]

    def kv_update(v_blocks, j0):
        for j, v in enumerate(v_blocks, j0):
            v1 = jnp.concatenate([v, jnp.ones((16, T), f32)], axis=0).astype(bf16)
            upd = _dot(v1, phi_k[j], _NT)
            kv[j] = upd if kv[j] is None else kv[j] + upd

    wait_loads()
    layernorm(0, 0, 0)
    pace["zero"] = top[1] >> 31
    wait_loads()
    prepare_w(8)
    wait_loads()
    layernorm(0, 1, 0)
    first = proj_group(8, 1, 0, 0)
    wait_loads()
    v0 = pairs([first, proj_group(8, 1, 0, 1)])
    prepare_w(9)
    first = proj_group(9, 1, 0, 0)
    wait_loads()
    v0 += pairs([first, proj_group(9, 1, 0, 1)])
    for j in (10, 11):
        prepare_w(j)
    if "0" == "0":
        v0 += pairs([proj_group(10, 1, 0, g) for g in range(2)])
        first = proj_group(11, 1, 0, 0)
        wait_loads()
        v0 += pairs([first, proj_group(11, 1, 0, 1)])
    else:
        first = proj_group(10, 2, 0, 0)
        wait_loads()
        v0 += pairs([first, proj_group(10, 2, 0, 1)])
    bd = feature_map()
    for j in (4, 5):
        prepare_w(j)
    first = proj_group(4, 2, 0, 0)
    layernorm(1, 0, 2)
    wait_loads()
    k = pairs([first, proj_group(4, 2, 0, 1)])
    for j in (6, 7):
        prepare_w(j)
    tasks += key_tasks(k, 0)
    k = proj(6, 0)
    layernorm(1, 1, 2)
    wait_loads()
    pending = [(v0[:8], 0), (v0[8:], 8)]
    j0 = 8
    for t in range(1, NT_):
        for c in range(2):
            tasks += key_tasks(k, j0)
            v = proj(8 + 2 * c, t)
            if len(pending) > 1:
                kv_update(*pending.pop(0))
            kv_update(*pending.pop(0))
            if t == NT_ - 1:
                prepare_w(1 + 2 * c)
            k, j0 = proj(4 + 2 * c, t), 8 * c
            pending.append((v, j0))
            if (t, c) in ((NT_ - 2, 1), (NT_ - 1, 0)):
                prepare_w(2 - 2 * c)
        for g in range(2 if t + 1 < NT_ else 0):
            layernorm(t + 1, g, 1)
    tasks += key_tasks(k, j0)

    r_max = jnp.max(top[0])
    idx = jnp.clip(jnp.min(jnp.where(top[0] == r_max, top[1], S)), 0, S - 1)
    t_sel = idx // T
    grp = pl.ds(pl.multiple_of(idx % 128 // 16 * 8, 8), 8)
    x_sel = jnp.concatenate(
        [_unpack(xs_v[t_sel, idx % T // 256, jnp.where(idx % 256 < 128, x_block[kh], x_block[2 + kh]), grp, :])
         for kh in range(2)],
        axis=1).astype(f32)
    x_sel = jnp.where(lax.broadcasted_iota(jnp.int32, (16, D), 0) == idx % 16, x_sel, 0.0)
    x_sel = jnp.broadcast_to(jnp.sum(x_sel, axis=0, keepdims=True), (16, D))
    gate = jax.nn.sigmoid(jnp.full((8, 512), r_max, f32))

    def ffn_program():
        h = []
        for n in range(F // 128):
            acc = []
            for w in (wg_v, wu_v):
                parts = []
                for kh in range(2):
                    dep = yield
                    parts.append(_dot(after(x_sel[:, 512 * kh:512 * (kh + 1)], dep).astype(bf16),
                                      w[pl.ds(512 * kh, 512), pl.ds(n * 128, 128)], _NN))
                    ffn["done"].append(_bits(parts[-1][:8]))
                acc.append(parts[0] + parts[1])
            h.append(_silu(acc[0]) * acc[1])
        for hf in range(2):
            y = None
            for n in range(F // 128):
                dep = yield
                part = _dot(after(h[n], dep).astype(bf16), wd_v[pl.ds(n * 128, 128), pl.ds(hf * 512, 512)], _NN)[:8]
                y = part if y is None else y + part
                ffn["done"].append(_bits(part[:, 384:]))
            ffn["y"][hf] = _rb(y * gate)

    def attend(blocks, j0):
        out = []
        for j, p in enumerate(blocks, j0):
            num = _dot(kv[j], p, _NN)
            for hd in range(2):
                inv = _rcp(num[64 + 8 * hd:72 + 8 * hd] + 1e-6)
                out.append((num[32 * hd:32 * hd + 32].reshape(4, 8, T) * inv[None]).reshape(32, T))
        return [[[jnp.concatenate(out[8 * c + 4 * kh:8 * c + 4 * kh + 4], axis=0)[:, 256 * g:256 * (g + 1)].T
                  for kh in range(2)] for g in range(2)] for c in range(2)]

    stores = []

    def out_proj(i, o_terms, n):
        while i and ffn["y"][n] is None:
            ffn_step()
        for (c, j), block in _block_product(lambda r: matmul(o_terms[r], woh_v[n, :, pl.ds(128 * r, 128)], _NN), 4):
            q = _TOKEN_GROUP[j]
            t, g = tiles[i + q // 2], q % 2
            cols, tok = pl.ds(512 * n + 128 * c, 128), pl.ds(pl.multiple_of(T * t + 256 * g, 256), 256)
            a = jnp.concatenate([_unpack(xs_v[t, g, x_block[2 * hf + n], :, pl.ds(128 * c, 128)])
                                 for hf in range(2)], axis=0).astype(f32)
            if i + q // 2 == NT_ - 1:
                hit = (lax.broadcasted_iota(jnp.int32, (32, 8, 128), 0) * 8
                       + lax.broadcasted_iota(jnp.int32, (32, 8, 128), 1)) == idx % T - 256 * g
                a3 = a.reshape(32, 8, 128)
                a = jnp.where(hit, a3 + ffn["y"][n][:, 128 * c:128 * (c + 1)][None], a3).reshape(256, 128)
            rows = pl.ds(T * i + 256 * q, 256)
            out_v[rows, cols] = (x_v[tok, cols].astype(f32) + block * _silu(a)).astype(bf16)
            if i and n:
                stores.extend(group(9, (out_v.at[rows, cols], out_hbm.at[tok, cols])))
                stores[-1].start()
        if (i, n) in ((0, 1), (2, 0)):
            cols = pl.ds(0, 512) if i else slice(None)
            for q in range(2):
                stores.extend(group(9, (out_v.at[pl.ds(T * (i + q), T), cols],
                                         out_hbm.at[pl.ds(pl.multiple_of(T * tiles[i + q], T), T), cols])))
                stores[-1].start()

    def output_terms(first, second):
        per_group = [_signed_sums([t[1] for t in _HK_TERMS],
                                  [b for q in _TOKEN_GROUP for b in (first, second)[q // 2][c][q % 2]])
                     for c in range(4)]
        return [jnp.concatenate(term, axis=1) for term in zip(*per_group)]

    def last_loads():
        wait_loads()
        prepare_wo()
        ffn["steps"], ffn["done"] = ffn_program(), [None, None]
        next(ffn["steps"])

    tiles = [lax.rem(t_sel + 1 + i, NT_) for i in range(NT_)]
    o = [[] for _ in range(NT_)]
    halves = [(i, c) for i in range(NT_) for c in range(2)]
    for h, (i, c) in enumerate(halves):
        q = proj(2 * c, tiles[i])
        if h == 0:
            kv_update(*pending.pop(0))
            row = lax.broadcasted_iota(jnp.int32, (80, 128), 0)
            col = lax.broadcasted_iota(jnp.int32, (80, 128), 1)
            own = jnp.where(row < 64, row >> 5, (row >> 3) & 1) == (col & 1)
            kv[:] = [jnp.where(own, a, 0.0).astype(bf16) for a in kv]
            tasks.extend([None] * 0 + [last_loads])
        else:
            o[halves[h - 1][0]] += attend(prev, 8 * halves[h - 1][1])
        prev = [_features(p).reshape(128, T).astype(bf16) for p in q]
        if h == 7:
            terms = output_terms(*o[:2])
            out_proj(0, terms, 0)
    out_proj(0, terms, 1)
    o[-1] += attend(prev, 8)
    terms = output_terms(*o[2:])
    for n in range(2):
        out_proj(2, terms, n)
    for c in stores:
        c.wait()


@jax.jit
def pallas_recurrent_scan__linear_kernel_hedgehog__moe_arch_mod__prompt_kernel(
    A_x: jax.Array,
    A_wqkv: jax.Array,
    A_w_phi: jax.Array,
    A_wo: jax.Array,
    B_x: jax.Array,
    B_w_r: jax.Array,
    B_w_gate: jax.Array,
    B_w_up: jax.Array,
    B_w_down: jax.Array,
):
    del B_x
    hbm = pl.BlockSpec(memory_space=pl.ANY)
    out = pl.pallas_call(
        _kernel,
        out_shape=jax.ShapeDtypeStruct((S, D), bf16),
        in_specs=[hbm] * 8,
        out_specs=hbm,
        scratch_shapes=[
            pltpu.VMEM((S, D), bf16),
            pltpu.VMEM((NT_, 2, 9, 64, 512), jnp.uint32),
            pltpu.VMEM((D, 3 * D), bf16),
            pltpu.VMEM((6, 7, 128, 512), jnp.uint32),
            pltpu.VMEM((D, D), bf16),
            pltpu.VMEM((2, 256, 26 * 128), jnp.uint32),
            pltpu.VMEM((D, F), bf16),
            pltpu.VMEM((D, F), bf16),
            pltpu.VMEM((F, D), bf16),
            pltpu.VMEM((S, D), bf16),
            pltpu.VMEM((H * DH, DH), bf16),
            pltpu.VMEM((D,), bf16),
            pltpu.SemaphoreType.DMA((10,)),
        ],
        compiler_params=pltpu.CompilerParams(vmem_limit_bytes=110 * 1024 * 1024),
        name="hedgehog_mod",
    )(
        A_x.reshape(S, D), A_wqkv, A_w_phi.reshape(H * DH, DH), A_wo,
        B_w_r, B_w_gate, B_w_up, B_w_down,
    )
    return out.reshape(1, S, D)
```

```python
import functools
import math

import jax
import jax.numpy as jnp
from jax import lax
import jax.experimental.pallas as pl
import jax.experimental.pallas.tpu as pltpu

S, D, H, DH, F = 2048, 1024, 32, 32, 3584
T = 512
NT_ = S // T
LOG2E = math.log2(math.e)
_NT = (((1,), (1,)), ((), ()))
_NN = (((1,), (0,)), ((), ()))
f32, bf16 = jnp.float32, jnp.bfloat16


def _dot(a, b, dn):
    return lax.dot_general(a, b, dn, preferred_element_type=f32)


def _rb(v):
    return v.astype(bf16).astype(f32)


def _rcp(v):
    r = pl.reciprocal(v, approx=True)
    return r * (2.0 - v * r)


def _silu(a):
    return a * pl.reciprocal(1.0 + jnp.exp2(a * -LOG2E), approx=True)


def _bits(v):
    return pltpu.bitcast(v, jnp.int32)


def _pack(v):
    return pltpu.bitcast(v.astype(bf16), jnp.uint32)


def _unpack(words):
    return pltpu.bitcast(words, bf16)


_HK_TERMS = (
    ((1,), (1, -2)), ((1, 2), (2,)), ((3, 4), (3,)), ((-4,), (3, -4)),
    ((1, 4), (2, 3)), ((-1, 3), (1, 3)), ((2, -4), (2, 4)),
    ((6,), (6,)), ((5,), (5,)),
    ((-3, -4, 5), (3, -4, -6)), ((-3, -4, 5, 6), (4, 6)), ((3, -5), (3, -4, 5, -6)),
    ((1, 2, -6), (1, -2, 5)), ((-2, 6), (1, -2, 5, -6)), ((-1, -2, 5, 6), (1, 5)),
    ((7,), (7, -8)), ((7, 8), (8,)),
    ((4, 7), (3, 8)), ((3, -7), (3, 7)), ((-4, 8), (4, 8)),
    ((-6, 7, 8), (5, 7, -8)), ((6, -8), (5, -6, 7, -8)), ((5, 6, -7, -8), (5, 7)),
    ((2, -6, 7), (1, 5, 8)), ((1, -5, -7), (1, 5, 7)), ((-2, 6, 8), (2, 6, 8)),
)
_HK_SUMS = (
    ((0, 0), (2, 1)), ((1, 1), (4, 3)), ((1, 0), (6, 5, 1, -3)), ((0, 1), (7, 5, 4, -2)),
    ((2, 2), (9, 8)), ((2, 1), (11, 10, 3, -8)), ((1, 2), (12, 10, 9, -4)),
    ((0, 2), (14, 13, 8, -1)), ((2, 0), (15, 13, 2, -9)), ((3, 3), (17, 16)),
    ((1, 3), (19, 18, 16, -3)), ((3, 1), (20, 18, 4, -17)),
    ((3, 2), (22, 21, 8, -16)), ((2, 3), (23, 21, 17, -9)),
    ((0, 3), (25, 24, 16, 15), (2, 3), 1), ((3, 0), (26, 24, 14, -17), (3, 2), -1),
)
_TOKEN_GROUP = (0, 2, 3, 1)


def _signed_sums(wanted, blocks):
    known = {(i + 1,): b for i, b in enumerate(blocks)}

    def value(key):
        if key not in known:
            for part in sorted(known, key=len, reverse=True):
                for sign in (1, -1):
                    signed = [sign * p for p in part]
                    if key not in known and len(part) < len(key) and all(p in key for p in signed):
                        rest = tuple(k for k in key if k not in signed)
                        if sign > 0 and rest[0] < 0:
                            known[key] = known[part] - value(tuple(-k for k in rest))
                        else:
                            known[key] = value(rest) + known[part] if sign > 0 else value(rest) - known[part]
            if key not in known:
                known[key] = -known[(-key[0],)]
        return known[key]

    for key in sorted(wanted, key=len):
        value(key)
    return [known[key] for key in wanted]


def _block_product(product, size):
    m, y = [], {}
    for ij, parts, *earlier in _HK_SUMS[:size * size]:
        while len(m) < parts[0]:
            m.append(product(len(m)))
        total = m[parts[0] - 1]
        for p in parts[1:]:
            total = total + m[p - 1] if p > 0 else total - m[-p - 1]
        if earlier:
            total = total + y[earlier[0]] if earlier[1] > 0 else total - y[earlier[0]]
        y[ij] = total
        yield ij, total


def _allreduce(v, op):
    r = v[0]
    for i in range(1, 8):
        r = op(r, v[i])
    r = op(r, pltpu.roll(r, 4, 0))
    return op(r, pltpu.roll(r, 2, 0))


def _features(p):
    p3 = p.reshape(8, 8, p.shape[1])
    mx = _allreduce(p3, jnp.maximum)
    mn = _allreduce(p3, jnp.minimum)
    ep = jnp.exp2(p3 - mx[None])
    en = jnp.exp2(mn[None] - p3)
    ip = _rcp(_allreduce(ep, jnp.add))
    im = _rcp(_allreduce(en, jnp.add))
    return jnp.concatenate([ep * ip[None], en * im[None]], axis=0)


def _kernel(x_hbm, wqkv_hbm, wphi_hbm, wo_hbm, wr_hbm, wg_hbm, wu_hbm, wd_hbm, out_hbm,
            x_v, xs_v, wqkv_v, ws_v, wo_v, woh_v, wg_v, wu_v, wd_v, out_v, wphi_v, wr_v, sems):
    def group(k, *pairs):
        return [pltpu.make_async_copy(src, dst, sems.at[k]) for src, dst in pairs]

    def x_rows(r0, n):
        return x_hbm.at[pl.ds(r0, n)], x_v.at[pl.ds(r0, n)]

    def w_cols(j0, nj):
        cols = pl.ds(256 * j0, 256 * nj)
        return wqkv_hbm.at[:, cols], wqkv_v.at[:, cols]

    loads = [
        group(0, x_rows(0, 256), (wr_hbm, wr_v)),
        group(1, w_cols(8, 1)),
        group(2, x_rows(256, 256)),
        group(3, w_cols(9, 1)),
        group(4, w_cols(10, 2)),
        group(5, (wphi_hbm, wphi_v), w_cols(4, 2), x_rows(T, 256)),
        group(6, w_cols(6, 2), x_rows(T + 256, 256)),
        group(7, x_rows(2 * T, S - 2 * T), w_cols(0, 4)),
        group(8, (wo_hbm, wo_v), (wg_hbm, wg_v), (wu_hbm, wu_v), (wd_hbm, wd_v)),
    ]
    for copies in loads:
        for c in copies:
            c.start()

    def wait_loads():
        for c in loads.pop(0):
            c.wait()

    tasks = []
    pace = {}

    def after(v, dep):
        first = pltpu.bitcast(_bits(v[:8, :128]) ^ (dep & pace["zero"]), v.dtype)
        if v.shape[1] > 128:
            first = jnp.concatenate([first, v[:8, 128:]], axis=1)
        return jnp.concatenate([first, v[8:]], axis=0)

    ffn = {"steps": None, "done": [], "y": [None, None]}

    def ffn_step():
        try:
            ffn["steps"].send(ffn["main"])
        except StopIteration:
            ffn["steps"] = None

    def matmul(lhs, rhs, dn):
        task = tasks.pop(0) if tasks else None
        dep = task() if task is not None else None
        if ffn["done"]:
            dep = ffn["done"].pop(0)
        if dep is not None:
            lhs = after(lhs, dep)
        m = _dot(lhs.astype(bf16) if lhs.dtype == f32 else _unpack(lhs), _unpack(rhs), dn)
        if ffn["steps"] is not None:
            ffn_step()
        ffn["main"] = _bits(m[:8, :128])
        return m

    top = [jnp.full((8, 128), -jnp.inf, f32), lax.broadcasted_iota(jnp.int32, (8, 128), 0)]
    chain = []
    x_keys = [term[1] for term in _HK_TERMS[:7]] + [(1,), (4,)]
    x_block = [x_keys.index((i + 1,)) for i in range(4)]

    def layernorm(t, g, lag):
        wr = wr_v[...].astype(f32).reshape(1, D)
        row = lax.broadcasted_iota(jnp.int32, (8, 128), 0)
        for r in range(0, 128, 16):
            blocks = []
            for r0 in (T * t + 256 * g + r, T * t + 256 * g + 128 + r):
                x = x_v[pl.ds(r0, 16), :].astype(f32)
                total = x[:, :128]
                for i in range(1, D // 128):
                    total = total + x[:, 128 * i:128 * (i + 1)]
                if lag:
                    total = jnp.where(jnp.concatenate([chain[-lag]] * 2, axis=0) >= 0, total, 0.0)
                xc = x - jnp.sum(total, axis=-1, keepdims=True) * (1.0 / D)
                v = jnp.mean(xc * xc, axis=-1, keepdims=True)
                xn = xc * (1.0 / _rb(jnp.sqrt(_rb(_rb(v) + _rb(jnp.full_like(v, 1e-5))))))
                blocks += [xn[:, :512], xn[:, 512:]]
                score = jnp.broadcast_to(_rb(jnp.sum(xn * wr, axis=-1, keepdims=True)), (16, 128))
                for i in (0, 8):
                    sc, tok = score[i:i + 8], row + (r0 + i)
                    better = (sc > top[0]) | ((sc == top[0]) & (tok < top[1]))
                    top[:] = jnp.where(better, sc, top[0]), jnp.where(better, tok, top[1])
                chain.append(top[1])
            for i, term in enumerate(_signed_sums(x_keys, blocks)):
                xs_v.at[t, g, i][pl.ds(r // 2, 8), :] = _pack(term)

    def feature_map():
        high = pltpu.bitcast(wphi_v[...].astype(f32).T, jnp.uint32)
        head = (lax.broadcasted_iota(jnp.int32, (DH, D), 1) >> 5) & 3
        none = jnp.zeros_like(high)
        return _unpack(jnp.concatenate(
            [jnp.where(head == 2 * p, high >> 16, none) | jnp.where(head == 2 * p + 1, high, none)
             for p in range(2)], axis=0))

    def prepare_w(j):
        blocks = []
        for c in (2 * j, 2 * j + 1):
            w = wqkv_v[:, pl.ds(128 * c, 128)]
            if j < 8:
                blocks.append(_dot(bd[:, 128 * (c % 8):128 * (c % 8 + 1)], w, _NT) * LOG2E)
            else:
                blocks.append(w.astype(f32).T)
        blocks = [a[:, 512 * kh:512 * (kh + 1)] for a in blocks for kh in range(2)]
        for i, term in enumerate(_signed_sums([term[0] for term in _HK_TERMS[:7]], blocks)):
            ws_v.at[j // 2, i][pl.ds(64 * (j % 2), 64), :] = _pack(term)

    def prepare_wo():
        link = pace["zero"]
        for n in range(2):
            for r in range(0, D // 2, 16):
                w = [wo_v[pl.ds(r // 128 * 256 + 128 * kh + r % 128, 16), pl.ds(512 * n, 512)].astype(f32)
                     for kh in range(2)]
                blocks = [w[kh][:, 128 * i:128 * (i + 1)] for i in range(4) for kh in range(2)]
                blocks[0] = pltpu.bitcast(_bits(blocks[0]) ^ jnp.concatenate([link] * 2, axis=0), f32)
                terms = _signed_sums([term[0] for term in _HK_TERMS], blocks)
                woh_v.at[n][pl.ds(r // 2, 8), :] = _pack(jnp.concatenate(terms, axis=1))
                done = functools.reduce(jnp.bitwise_or, [
                    _bits(term[h:h + 8]) for term in terms[4:7] + terms[9:15] + terms[17:] for h in (0, 8)])
                for _ in range(2):
                    slow = jnp.sum(pltpu.bitcast(done, f32), axis=-1, keepdims=True)
                    done = link = _bits(jnp.broadcast_to(slow, (8, 128))) & pace["zero"]

    def proj_group(j0, nj, t, g):
        rows = pl.ds(64 * (j0 % 2), 64 * nj)
        return dict(_block_product(
            lambda r: matmul(ws_v[j0 // 2, r, rows, :], xs_v[t, g, r], _NT), 2))

    def pairs(groups):
        return [jnp.concatenate([y[b, hf][r:r + 64] for y in groups for hf in range(2)], axis=1)
                for j in range(groups[0][0, 0].shape[0] // 128) for b in range(2)
                for r in (128 * j, 128 * j + 64)]

    def proj(j0, t):
        return pairs([proj_group(j0, 2, t, g) for g in range(2)])

    kv = [None] * 16
    phi_k = [None] * 16

    def key_features(j, p):
        phi = _features(p)
        phi_k[j] = phi.reshape(128, T).astype(bf16)
        return functools.reduce(jnp.bitwise_or, [_bits(phi[7][:, n:n + 128]) for n in range(0, T, 128)])

    def key_tasks(blocks, j0):
        return [None] * 4 + [functools.partial(key_features, j0 + q, p) for q, p in enumerate(blocks)]

    def kv_update(v_blocks, j0):
        for j, v in enumerate(v_blocks, j0):
            v1 = jnp.concatenate([v, jnp.ones((16, T), f32)], axis=0).astype(bf16)
            upd = _dot(v1, phi_k[j], _NT)
            kv[j] = upd if kv[j] is None else kv[j] + upd

    wait_loads()
    layernorm(0, 0, 0)
    pace["zero"] = top[1] >> 31
    wait_loads()
    prepare_w(8)
    wait_loads()
    layernorm(0, 1, 0)
    first = proj_group(8, 1, 0, 0)
    wait_loads()
    v0 = pairs([first, proj_group(8, 1, 0, 1)])
    prepare_w(9)
    first = proj_group(9, 1, 0, 0)
    wait_loads()
    v0 += pairs([first, proj_group(9, 1, 0, 1)])
    for j in (10, 11):
        prepare_w(j)
    v0 += pairs([proj_group(10, 1, 0, g) for g in range(2)])
    first = proj_group(11, 1, 0, 0)
    wait_loads()
    v0 += pairs([first, proj_group(11, 1, 0, 1)])
    bd = feature_map()
    for j in (4, 5):
        prepare_w(j)
    first = proj_group(4, 2, 0, 0)
    layernorm(1, 0, 2)
    wait_loads()
    k = pairs([first, proj_group(4, 2, 0, 1)])
    for j in (6, 7):
        prepare_w(j)
    tasks += key_tasks(k, 0)
    k = proj(6, 0)
    layernorm(1, 1, 2)
    wait_loads()
    pending = [(v0[:8], 0), (v0[8:], 8)]
    j0 = 8
    for t in range(1, NT_):
        for c in range(2):
            tasks += key_tasks(k, j0)
            v = proj(8 + 2 * c, t)
            while pending:
                kv_update(*pending.pop(0))
            if t == NT_ - 1:
                prepare_w(1 + 2 * c)
            k, j0 = proj(4 + 2 * c, t), 8 * c
            pending.append((v, j0))
            if (t, c) in ((NT_ - 2, 1), (NT_ - 1, 0)):
                prepare_w(2 - 2 * c)
        for g in range(2 if t + 1 < NT_ else 0):
            layernorm(t + 1, g, 1)
    tasks += key_tasks(k, j0)

    r_max = jnp.max(top[0])
    idx = jnp.clip(jnp.min(jnp.where(top[0] == r_max, top[1], S)), 0, S - 1)
    t_sel = idx // T
    grp = pl.ds(pl.multiple_of(idx % 128 // 16 * 8, 8), 8)
    x_sel = jnp.concatenate(
        [_unpack(xs_v[t_sel, idx % T // 256, jnp.where(idx % 256 < 128, x_block[kh], x_block[2 + kh]), grp, :])
         for kh in range(2)],
        axis=1).astype(f32)
    x_sel = jnp.where(lax.broadcasted_iota(jnp.int32, (16, D), 0) == idx % 16, x_sel, 0.0)
    x_sel = jnp.broadcast_to(jnp.sum(x_sel, axis=0, keepdims=True), (16, D))
    gate = jax.nn.sigmoid(jnp.full((8, 512), r_max, f32))

    def ffn_program():
        h = []
        for n in range(F // 128):
            acc = []
            for w in (wg_v, wu_v):
                parts = []
                for kh in range(2):
                    dep = yield
                    parts.append(_dot(after(x_sel[:, 512 * kh:512 * (kh + 1)], dep).astype(bf16),
                                      w[pl.ds(512 * kh, 512), pl.ds(n * 128, 128)], _NN))
                    ffn["done"].append(_bits(parts[-1][:8]))
                acc.append(parts[0] + parts[1])
            h.append(_silu(acc[0]) * acc[1])
        for hf in range(2):
            y = None
            for n in range(F // 128):
                dep = yield
                part = _dot(after(h[n], dep).astype(bf16), wd_v[pl.ds(n * 128, 128), pl.ds(hf * 512, 512)], _NN)[:8]
                y = part if y is None else y + part
                ffn["done"].append(_bits(part[:, 384:]))
            ffn["y"][hf] = _rb(y * gate)

    def attend(blocks, j0):
        out = []
        for j, p in enumerate(blocks, j0):
            num = _dot(kv[j], p, _NN)
            for hd in range(2):
                inv = _rcp(num[64 + 8 * hd:72 + 8 * hd] + 1e-6)
                out.append((num[32 * hd:32 * hd + 32].reshape(4, 8, T) * inv[None]).reshape(32, T))
        return [[[jnp.concatenate(out[8 * c + 4 * kh:8 * c + 4 * kh + 4], axis=0)[:, 256 * g:256 * (g + 1)].T
                  for kh in range(2)] for g in range(2)] for c in range(2)]

    stores = []

    def out_proj(i, o_terms, n):
        while i and ffn["y"][n] is None:
            ffn_step()
        for (c, j), block in _block_product(lambda r: matmul(o_terms[r], woh_v[n, :, pl.ds(128 * r, 128)], _NN), 4):
            q = _TOKEN_GROUP[j]
            t, g = tiles[i + q // 2], q % 2
            cols, tok = pl.ds(512 * n + 128 * c, 128), pl.ds(pl.multiple_of(T * t + 256 * g, 256), 256)
            a = jnp.concatenate([_unpack(xs_v[t, g, x_block[2 * hf + n], :, pl.ds(128 * c, 128)])
                                 for hf in range(2)], axis=0).astype(f32)
            if i + q // 2 == NT_ - 1:
                hit = (lax.broadcasted_iota(jnp.int32, (32, 8, 128), 0) * 8
                       + lax.broadcasted_iota(jnp.int32, (32, 8, 128), 1)) == idx % T - 256 * g
                a3 = a.reshape(32, 8, 128)
                a = jnp.where(hit, a3 + ffn["y"][n][:, 128 * c:128 * (c + 1)][None], a3).reshape(256, 128)
            rows = pl.ds(T * i + 256 * q, 256)
            out_v[rows, cols] = (x_v[tok, cols].astype(f32) + block * _silu(a)).astype(bf16)
            if i and n:
                stores.extend(group(9, (out_v.at[rows, cols], out_hbm.at[tok, cols])))
                stores[-1].start()
        if (i, n) in ((0, 1), (2, 0)):
            cols = pl.ds(0, 512) if i else slice(None)
            for q in range(2):
                stores.extend(group(9, (out_v.at[pl.ds(T * (i + q), T), cols],
                                         out_hbm.at[pl.ds(pl.multiple_of(T * tiles[i + q], T), T), cols])))
                stores[-1].start()

    def output_terms(first, second):
        per_group = [_signed_sums([t[1] for t in _HK_TERMS],
                                  [b for q in _TOKEN_GROUP for b in (first, second)[q // 2][c][q % 2]])
                     for c in range(4)]
        return [jnp.concatenate(term, axis=1) for term in zip(*per_group)]

    def last_loads():
        wait_loads()
        prepare_wo()
        ffn["steps"], ffn["done"] = ffn_program(), [None, None]
        next(ffn["steps"])

    tiles = [lax.rem(t_sel + 1 + i, NT_) for i in range(NT_)]
    o = [[] for _ in range(NT_)]
    halves = [(i, c) for i in range(NT_) for c in range(2)]
    for h, (i, c) in enumerate(halves):
        q = proj(2 * c, tiles[i])
        if h == 0:
            kv_update(*pending.pop(0))
            row = lax.broadcasted_iota(jnp.int32, (80, 128), 0)
            col = lax.broadcasted_iota(jnp.int32, (80, 128), 1)
            own = jnp.where(row < 64, row >> 5, (row >> 3) & 1) == (col & 1)
            kv[:] = [jnp.where(own, a, 0.0).astype(bf16) for a in kv]
            tasks.append(last_loads)
        else:
            o[halves[h - 1][0]] += attend(prev, 8 * halves[h - 1][1])
        prev = [_features(p).reshape(128, T).astype(bf16) for p in q]
    terms = output_terms(*o[:2])
    for n in range(2):
        out_proj(0, terms, n)
    o[-1] += attend(prev, 8)
    terms = output_terms(*o[2:])
    for n in range(2):
        out_proj(2, terms, n)
    for c in stores:
        c.wait()


@jax.jit
def pallas_recurrent_scan__linear_kernel_hedgehog__moe_arch_mod__prompt_kernel(
    A_x: jax.Array,
    A_wqkv: jax.Array,
    A_w_phi: jax.Array,
    A_wo: jax.Array,
    B_x: jax.Array,
    B_w_r: jax.Array,
    B_w_gate: jax.Array,
    B_w_up: jax.Array,
    B_w_down: jax.Array,
):
    del B_x
    hbm = pl.BlockSpec(memory_space=pl.ANY)
    out = pl.pallas_call(
        _kernel,
        out_shape=jax.ShapeDtypeStruct((S, D), bf16),
        in_specs=[hbm] * 8,
        out_specs=hbm,
        scratch_shapes=[
            pltpu.VMEM((S, D), bf16),
            pltpu.VMEM((NT_, 2, 9, 64, 512), jnp.uint32),
            pltpu.VMEM((D, 3 * D), bf16),
            pltpu.VMEM((6, 7, 128, 512), jnp.uint32),
            pltpu.VMEM((D, D), bf16),
            pltpu.VMEM((2, 256, 26 * 128), jnp.uint32),
            pltpu.VMEM((D, F), bf16),
            pltpu.VMEM((D, F), bf16),
            pltpu.VMEM((F, D), bf16),
            pltpu.VMEM((S, D), bf16),
            pltpu.VMEM((H * DH, DH), bf16),
            pltpu.VMEM((D,), bf16),
            pltpu.SemaphoreType.DMA((10,)),
        ],
        compiler_params=pltpu.CompilerParams(vmem_limit_bytes=110 * 1024 * 1024),
        name="hedgehog_mod",
    )(
        A_x.reshape(S, D), A_wqkv, A_w_phi.reshape(H * DH, DH), A_wo,
        B_w_r, B_w_gate, B_w_up, B_w_down,
    )
    return out.reshape(1, S, D)
```

```python
import functools
import math

import jax
import jax.numpy as jnp
from jax import lax
import jax.experimental.pallas as pl
import jax.experimental.pallas.tpu as pltpu

S, D, H, DH, F = 2048, 1024, 32, 32, 3584
T = 512
NT_ = S // T
LOG2E = math.log2(math.e)
_NT = (((1,), (1,)), ((), ()))
_NN = (((1,), (0,)), ((), ()))
f32, bf16 = jnp.float32, jnp.bfloat16


def _dot(a, b, dn):
    return lax.dot_general(a, b, dn, preferred_element_type=f32)


def _rb(v):
    return v.astype(bf16).astype(f32)


def _rcp(v):
    r = pl.reciprocal(v, approx=True)
    return r * (2.0 - v * r)


def _silu(a):
    return a * pl.reciprocal(1.0 + jnp.exp2(a * -LOG2E), approx=True)


def _bits(v):
    return pltpu.bitcast(v, jnp.int32)


def _pack(v):
    return pltpu.bitcast(v.astype(bf16), jnp.uint32)


def _unpack(words):
    return pltpu.bitcast(words, bf16)


_HK_TERMS = (
    ((1,), (1, -2)), ((1, 2), (2,)), ((3, 4), (3,)), ((-4,), (3, -4)),
    ((1, 4), (2, 3)), ((-1, 3), (1, 3)), ((2, -4), (2, 4)),
    ((6,), (6,)), ((5,), (5,)),
    ((-3, -4, 5), (3, -4, -6)), ((-3, -4, 5, 6), (4, 6)), ((3, -5), (3, -4, 5, -6)),
    ((1, 2, -6), (1, -2, 5)), ((-2, 6), (1, -2, 5, -6)), ((-1, -2, 5, 6), (1, 5)),
    ((7,), (7, -8)), ((7, 8), (8,)),
    ((4, 7), (3, 8)), ((3, -7), (3, 7)), ((-4, 8), (4, 8)),
    ((-6, 7, 8), (5, 7, -8)), ((6, -8), (5, -6, 7, -8)), ((5, 6, -7, -8), (5, 7)),
    ((2, -6, 7), (1, 5, 8)), ((1, -5, -7), (1, 5, 7)), ((-2, 6, 8), (2, 6, 8)),
)
_HK_SUMS = (
    ((0, 0), (2, 1)), ((1, 1), (4, 3)), ((1, 0), (6, 5, 1, -3)), ((0, 1), (7, 5, 4, -2)),
    ((2, 2), (9, 8)), ((2, 1), (11, 10, 3, -8)), ((1, 2), (12, 10, 9, -4)),
    ((0, 2), (14, 13, 8, -1)), ((2, 0), (15, 13, 2, -9)), ((3, 3), (17, 16)),
    ((1, 3), (19, 18, 16, -3)), ((3, 1), (20, 18, 4, -17)),
    ((3, 2), (22, 21, 8, -16)), ((2, 3), (23, 21, 17, -9)),
    ((0, 3), (25, 24, 16, 15), (2, 3), 1), ((3, 0), (26, 24, 14, -17), (3, 2), -1),
)
_TOKEN_GROUP = (0, 2, 3, 1)


def _signed_sums(wanted, blocks):
    known = {(i + 1,): b for i, b in enumerate(blocks)}

    def value(key):
        if key not in known:
            for part in sorted(known, key=len, reverse=True):
                for sign in (1, -1):
                    signed = [sign * p for p in part]
                    if key not in known and len(part) < len(key) and all(p in key for p in signed):
                        rest = tuple(k for k in key if k not in signed)
                        if sign > 0 and rest[0] < 0:
                            known[key] = known[part] - value(tuple(-k for k in rest))
                        else:
                            known[key] = value(rest) + known[part] if sign > 0 else value(rest) - known[part]
            if key not in known:
                known[key] = -known[(-key[0],)]
        return known[key]

    for key in sorted(wanted, key=len):
        value(key)
    return [known[key] for key in wanted]


def _block_product(product, size):
    m, y = [], {}
    for ij, parts, *earlier in _HK_SUMS[:size * size]:
        while len(m) < parts[0]:
            m.append(product(len(m)))
        total = m[parts[0] - 1]
        for p in parts[1:]:
            total = total + m[p - 1] if p > 0 else total - m[-p - 1]
        if earlier:
            total = total + y[earlier[0]] if earlier[1] > 0 else total - y[earlier[0]]
        y[ij] = total
        yield ij, total


def _allreduce(v, op):
    r = v[0]
    for i in range(1, 8):
        r = op(r, v[i])
    r = op(r, pltpu.roll(r, 4, 0))
    return op(r, pltpu.roll(r, 2, 0))


def _features(p):
    p3 = p.reshape(8, 8, p.shape[1])
    mx = _allreduce(p3, jnp.maximum)
    mn = _allreduce(p3, jnp.minimum)
    ep = jnp.exp2(p3 - mx[None])
    en = jnp.exp2(mn[None] - p3)
    ip = _rcp(_allreduce(ep, jnp.add))
    im = _rcp(_allreduce(en, jnp.add))
    return jnp.concatenate([ep * ip[None], en * im[None]], axis=0)


def _kernel(x_hbm, wqkv_hbm, wphi_hbm, wo_hbm, wr_hbm, wg_hbm, wu_hbm, wd_hbm, out_hbm,
            x_v, xs_v, wqkv_v, ws_v, wo_v, woh_v, wg_v, wu_v, wd_v, out_v, wphi_v, wr_v, sems):
    def group(k, *pairs):
        return [pltpu.make_async_copy(src, dst, sems.at[k]) for src, dst in pairs]

    def x_rows(r0, n):
        return x_hbm.at[pl.ds(r0, n)], x_v.at[pl.ds(r0, n)]

    def w_cols(j0, nj):
        cols = pl.ds(256 * j0, 256 * nj)
        return wqkv_hbm.at[:, cols], wqkv_v.at[:, cols]

    loads = [
        group(0, x_rows(0, 256), (wr_hbm, wr_v)),
        group(1, w_cols(8, 1)),
        group(2, x_rows(256, 256)),
        group(3, w_cols(9, 1)),
        group(4, w_cols(10, 2)),
        group(5, (wphi_hbm, wphi_v), w_cols(4, 2), x_rows(T, 256)),
        group(6, w_cols(6, 2), x_rows(T + 256, 256)),
        group(7, x_rows(2 * T, S - 2 * T), w_cols(0, 4)),
        group(8, (wo_hbm, wo_v), (wg_hbm, wg_v), (wu_hbm, wu_v), (wd_hbm, wd_v)),
    ]
    for copies in loads:
        for c in copies:
            c.start()

    def wait_loads():
        for c in loads.pop(0):
            c.wait()

    tasks = []
    pace = {}

    def after(v, dep):
        first = pltpu.bitcast(_bits(v[:8, :128]) ^ (dep & pace["zero"]), v.dtype)
        if v.shape[1] > 128:
            first = jnp.concatenate([first, v[:8, 128:]], axis=1)
        return jnp.concatenate([first, v[8:]], axis=0)

    ffn = {"steps": None, "done": [], "y": [None, None]}

    def ffn_step():
        try:
            ffn["steps"].send(ffn["main"])
        except StopIteration:
            ffn["steps"] = None

    def matmul(lhs, rhs, dn):
        task = tasks.pop(0) if tasks else None
        dep = task() if task is not None else None
        if ffn["done"]:
            dep = ffn["done"].pop(0)
        if dep is not None:
            lhs = after(lhs, dep)
        m = _dot(lhs.astype(bf16) if lhs.dtype == f32 else _unpack(lhs), _unpack(rhs), dn)
        if ffn["steps"] is not None:
            ffn_step()
        ffn["main"] = _bits(m[:8, :128])
        return m

    top = [jnp.full((8, 128), -jnp.inf, f32), lax.broadcasted_iota(jnp.int32, (8, 128), 0)]
    chain = []
    x_keys = [term[1] for term in _HK_TERMS[:7]] + [(1,), (4,)]
    x_block = [x_keys.index((i + 1,)) for i in range(4)]

    def layernorm(t, g, lag):
        wr = wr_v[...].astype(f32).reshape(1, D)
        row = lax.broadcasted_iota(jnp.int32, (8, 128), 0)
        for r in range(0, 128, 16):
            blocks = []
            for r0 in (T * t + 256 * g + r, T * t + 256 * g + 128 + r):
                x = x_v[pl.ds(r0, 16), :].astype(f32)
                if lag:
                    x = after(x, chain[-lag])
                xc = x - jnp.mean(x, axis=-1, keepdims=True)
                v = jnp.mean(xc * xc, axis=-1, keepdims=True)
                xn = xc * (1.0 / _rb(jnp.sqrt(_rb(_rb(v) + _rb(jnp.full_like(v, 1e-5))))))
                blocks += [xn[:, :512], xn[:, 512:]]
                score = jnp.broadcast_to(_rb(jnp.sum(xn * wr, axis=-1, keepdims=True)), (16, 128))
                for i in (0, 8):
                    sc, tok = score[i:i + 8], row + (r0 + i)
                    better = (sc > top[0]) | ((sc == top[0]) & (tok < top[1]))
                    top[:] = jnp.where(better, sc, top[0]), jnp.where(better, tok, top[1])
                chain.append(top[1])
            for i, term in enumerate(_signed_sums(x_keys, blocks)):
                xs_v.at[t, g, i][pl.ds(r // 2, 8), :] = _pack(term)

    def feature_map():
        high = pltpu.bitcast(wphi_v[...].astype(f32).T, jnp.uint32)
        head = (lax.broadcasted_iota(jnp.int32, (DH, D), 1) >> 5) & 3
        none = jnp.zeros_like(high)
        return _unpack(jnp.concatenate(
            [jnp.where(head == 2 * p, high >> 16, none) | jnp.where(head == 2 * p + 1, high, none)
             for p in range(2)], axis=0))

    def prepare_w(j):
        blocks = []
        for c in (2 * j, 2 * j + 1):
            w = wqkv_v[:, pl.ds(128 * c, 128)]
            if j < 8:
                blocks.append(_dot(bd[:, 128 * (c % 8):128 * (c % 8 + 1)], w, _NT) * LOG2E)
            else:
                blocks.append(w.astype(f32).T)
        blocks = [a[:, 512 * kh:512 * (kh + 1)] for a in blocks for kh in range(2)]
        for i, term in enumerate(_signed_sums([term[0] for term in _HK_TERMS[:7]], blocks)):
            ws_v.at[j // 2, i][pl.ds(64 * (j % 2), 64), :] = _pack(term)

    def prepare_wo():
        link = pace["zero"]
        for n in range(2):
            for r in range(0, D // 2, 16):
                w = [wo_v[pl.ds(r // 128 * 256 + 128 * kh + r % 128, 16), pl.ds(512 * n, 512)].astype(f32)
                     for kh in range(2)]
                blocks = [w[kh][:, 128 * i:128 * (i + 1)] for i in range(4) for kh in range(2)]
                blocks[0] = after(blocks[0], link)
                terms = _signed_sums([term[0] for term in _HK_TERMS], blocks)
                woh_v.at[n][pl.ds(r // 2, 8), :] = _pack(jnp.concatenate(terms, axis=1))
                done = functools.reduce(jnp.bitwise_or, [
                    _bits(term[h:h + 8]) for term in terms[4:7] + terms[9:15] + terms[17:] for h in (0, 8)])
                for _ in range(2):
                    slow = jnp.sum(pltpu.bitcast(done, f32), axis=-1, keepdims=True)
                    done = link = _bits(jnp.broadcast_to(slow, (8, 128))) & pace["zero"]

    def proj_group(j0, nj, t, g):
        rows = pl.ds(64 * (j0 % 2), 64 * nj)
        return dict(_block_product(
            lambda r: matmul(ws_v[j0 // 2, r, rows, :], xs_v[t, g, r], _NT), 2))

    def pairs(groups):
        return [jnp.concatenate([y[b, hf][r:r + 64] for y in groups for hf in range(2)], axis=1)
                for j in range(groups[0][0, 0].shape[0] // 128) for b in range(2)
                for r in (128 * j, 128 * j + 64)]

    def proj(j0, t):
        return pairs([proj_group(j0, 2, t, g) for g in range(2)])

    kv = [None] * 16
    phi_k = [None] * 16

    def key_features(j, p):
        phi = _features(p)
        phi_k[j] = phi.reshape(128, T).astype(bf16)
        return functools.reduce(jnp.bitwise_or, [_bits(phi[7][:, n:n + 128]) for n in range(0, T, 128)])

    def key_tasks(blocks, j0):
        return [None] * 5 + [functools.partial(key_features, j0 + q, p) for q, p in enumerate(blocks)]

    def kv_update(v_blocks, j0):
        for j, v in enumerate(v_blocks, j0):
            v1 = jnp.concatenate([v, jnp.ones((16, T), f32)], axis=0).astype(bf16)
            upd = _dot(v1, phi_k[j], _NT)
            kv[j] = upd if kv[j] is None else kv[j] + upd

    wait_loads()
    layernorm(0, 0, 0)
    pace["zero"] = top[1] >> 31
    wait_loads()
    prepare_w(8)
    wait_loads()
    layernorm(0, 1, 8)
    first = proj_group(8, 1, 0, 0)
    wait_loads()
    v0 = pairs([first, proj_group(8, 1, 0, 1)])
    prepare_w(9)
    first = proj_group(9, 1, 0, 0)
    wait_loads()
    v0 += pairs([first, proj_group(9, 1, 0, 1)])
    for j in (10, 11):
        prepare_w(j)
    v0 += pairs([proj_group(10, 1, 0, g) for g in range(2)])
    first = proj_group(11, 1, 0, 0)
    wait_loads()
    v0 += pairs([first, proj_group(11, 1, 0, 1)])
    bd = feature_map()
    for j in (4, 5):
        prepare_w(j)
    first = proj_group(4, 2, 0, 0)
    layernorm(1, 0, 2)
    wait_loads()
    k = pairs([first, proj_group(4, 2, 0, 1)])
    for j in (6, 7):
        prepare_w(j)
    tasks += key_tasks(k, 0)
    k = proj(6, 0)
    layernorm(1, 1, 2)
    wait_loads()
    pending = [(v0[:8], 0), (v0[8:], 8)]
    j0 = 8
    for t in range(1, NT_):
        for c in range(2):
            tasks += key_tasks(k, j0)
            v = proj(8 + 2 * c, t)
            while pending:
                kv_update(*pending.pop(0))
            if t == NT_ - 1:
                prepare_w(1 + 2 * c)
            k, j0 = proj(4 + 2 * c, t), 8 * c
            pending.append((v, j0))
            if (t, c) in ((NT_ - 2, 1), (NT_ - 1, 0)):
                prepare_w(2 - 2 * c)
        for g in range(2 if t + 1 < NT_ else 0):
            layernorm(t + 1, g, 1)
    tasks += key_tasks(k, j0)

    r_max = jnp.max(top[0])
    idx = jnp.clip(jnp.min(jnp.where(top[0] == r_max, top[1], S)), 0, S - 1)
    t_sel = idx // T
    grp = pl.ds(pl.multiple_of(idx % 128 // 16 * 8, 8), 8)
    x_sel = jnp.concatenate(
        [_unpack(xs_v[t_sel, idx % T // 256, jnp.where(idx % 256 < 128, x_block[kh], x_block[2 + kh]), grp, :])
         for kh in range(2)],
        axis=1).astype(f32)
    x_sel = jnp.where(lax.broadcasted_iota(jnp.int32, (16, D), 0) == idx % 16, x_sel, 0.0)
    x_sel = jnp.broadcast_to(jnp.sum(x_sel, axis=0, keepdims=True), (16, D))
    gate = jax.nn.sigmoid(jnp.full((8, 512), r_max, f32))

    def ffn_program():
        h = []
        for n in range(F // 128):
            acc = []
            for w in (wg_v, wu_v):
                parts = []
                for kh in range(2):
                    dep = yield
                    parts.append(_dot(after(x_sel[:, 512 * kh:512 * (kh + 1)], dep).astype(bf16),
                                      w[pl.ds(512 * kh, 512), pl.ds(n * 128, 128)], _NN))
                    ffn["done"].append(_bits(parts[-1][:8]))
                acc.append(parts[0] + parts[1])
            h.append(_silu(acc[0]) * acc[1])
        for hf in range(2):
            y = None
            for n in range(F // 128):
                dep = yield
                part = _dot(after(h[n], dep).astype(bf16), wd_v[pl.ds(n * 128, 128), pl.ds(hf * 512, 512)], _NN)[:8]
                y = part if y is None else y + part
                ffn["done"].append(_bits(part[:, 384:]))
            ffn["y"][hf] = _rb(y * gate)

    def attend(blocks, j0):
        out = []
        for j, p in enumerate(blocks, j0):
            num = _dot(kv[j], p, _NN)
            for hd in range(2):
                inv = _rcp(num[64 + 8 * hd:72 + 8 * hd] + 1e-6)
                out.append((num[32 * hd:32 * hd + 32].reshape(4, 8, T) * inv[None]).reshape(32, T))
        return [[[jnp.concatenate(out[8 * c + 4 * kh:8 * c + 4 * kh + 4], axis=0)[:, 256 * g:256 * (g + 1)].T
                  for kh in range(2)] for g in range(2)] for c in range(2)]

    stores = []

    def out_proj(i, o_terms, n):
        while i and ffn["y"][n] is None:
            ffn_step()
        for (c, j), block in _block_product(lambda r: matmul(o_terms[r], woh_v[n, :, pl.ds(128 * r, 128)], _NN), 4):
            q = _TOKEN_GROUP[j]
            t, g = tiles[i + q // 2], q % 2
            cols, tok = pl.ds(512 * n + 128 * c, 128), pl.ds(pl.multiple_of(T * t + 256 * g, 256), 256)
            a = jnp.concatenate([_unpack(xs_v[t, g, x_block[2 * hf + n], :, pl.ds(128 * c, 128)])
                                 for hf in range(2)], axis=0).astype(f32)
            if i + q // 2 == NT_ - 1:
                hit = (lax.broadcasted_iota(jnp.int32, (32, 8, 128), 0) * 8
                       + lax.broadcasted_iota(jnp.int32, (32, 8, 128), 1)) == idx % T - 256 * g
                a3 = a.reshape(32, 8, 128)
                a = jnp.where(hit, a3 + ffn["y"][n][:, 128 * c:128 * (c + 1)][None], a3).reshape(256, 128)
            rows = pl.ds(T * i + 256 * q, 256)
            out_v[rows, cols] = (x_v[tok, cols].astype(f32) + block * _silu(a)).astype(bf16)
            if i and n:
                stores.extend(group(9, (out_v.at[rows, cols], out_hbm.at[tok, cols])))
                stores[-1].start()
        if (i, n) in ((0, 1), (2, 0)):
            cols = pl.ds(0, 512) if i else slice(None)
            for q in range(2):
                stores.extend(group(9, (out_v.at[pl.ds(T * (i + q), T), cols],
                                         out_hbm.at[pl.ds(pl.multiple_of(T * tiles[i + q], T), T), cols])))
                stores[-1].start()

    def output_terms(first, second):
        per_group = [_signed_sums([t[1] for t in _HK_TERMS],
                                  [b for q in _TOKEN_GROUP for b in (first, second)[q // 2][c][q % 2]])
                     for c in range(4)]
        return [jnp.concatenate(term, axis=1) for term in zip(*per_group)]

    def last_loads():
        wait_loads()
        prepare_wo()
        ffn["steps"], ffn["done"] = ffn_program(), [None, None]
        next(ffn["steps"])

    tiles = [lax.rem(t_sel + 1 + i, NT_) for i in range(NT_)]
    o = [[] for _ in range(NT_)]
    halves = [(i, c) for i in range(NT_) for c in range(2)]
    for h, (i, c) in enumerate(halves):
        q = proj(2 * c, tiles[i])
        if h == 0:
            kv_update(*pending.pop(0))
            row = lax.broadcasted_iota(jnp.int32, (80, 128), 0)
            col = lax.broadcasted_iota(jnp.int32, (80, 128), 1)
            own = jnp.where(row < 64, row >> 5, (row >> 3) & 1) == (col & 1)
            kv[:] = [jnp.where(own, a, 0.0).astype(bf16) for a in kv]
            tasks.append(last_loads)
        else:
            o[halves[h - 1][0]] += attend(prev, 8 * halves[h - 1][1])
        prev = [_features(p).reshape(128, T).astype(bf16) for p in q]
    terms = output_terms(*o[:2])
    for n in range(2):
        out_proj(0, terms, n)
    o[-1] += attend(prev, 8)
    terms = output_terms(*o[2:])
    for n in range(2):
        out_proj(2, terms, n)
    for c in stores:
        c.wait()


@jax.jit
def pallas_recurrent_scan__linear_kernel_hedgehog__moe_arch_mod__prompt_kernel(
    A_x: jax.Array,
    A_wqkv: jax.Array,
    A_w_phi: jax.Array,
    A_wo: jax.Array,
    B_x: jax.Array,
    B_w_r: jax.Array,
    B_w_gate: jax.Array,
    B_w_up: jax.Array,
    B_w_down: jax.Array,
):
    del B_x
    hbm = pl.BlockSpec(memory_space=pl.ANY)
    out = pl.pallas_call(
        _kernel,
        out_shape=jax.ShapeDtypeStruct((S, D), bf16),
        in_specs=[hbm] * 8,
        out_specs=hbm,
        scratch_shapes=[
            pltpu.VMEM((S, D), bf16),
            pltpu.VMEM((NT_, 2, 9, 64, 512), jnp.uint32),
            pltpu.VMEM((D, 3 * D), bf16),
            pltpu.VMEM((6, 7, 128, 512), jnp.uint32),
            pltpu.VMEM((D, D), bf16),
            pltpu.VMEM((2, 256, 26 * 128), jnp.uint32),
            pltpu.VMEM((D, F), bf16),
            pltpu.VMEM((D, F), bf16),
            pltpu.VMEM((F, D), bf16),
            pltpu.VMEM((S, D), bf16),
            pltpu.VMEM((H * DH, DH), bf16),
            pltpu.VMEM((D,), bf16),
            pltpu.SemaphoreType.DMA((10,)),
        ],
        compiler_params=pltpu.CompilerParams(vmem_limit_bytes=110 * 1024 * 1024),
        name="hedgehog_mod",
    )(
        A_x.reshape(S, D), A_wqkv, A_w_phi.reshape(H * DH, DH), A_wo,
        B_w_r, B_w_gate, B_w_up, B_w_down,
    )
    return out.reshape(1, S, D)
```
